```python
import jax
import jax.numpy as jnp

def _softmax(x, axis=-1):
    return jax.nn.softmax(x, axis=axis)

def _gelu(x):
    return jax.nn.gelu(x, approximate=True)

def _silu(x):
    return jax.nn.silu(x)

def _sigmoid(x):
    return jax.nn.sigmoid(x)

def _layernorm(x, axis=-1, eps=1e-05):
    m = jnp.mean(x, axis=axis, keepdims=True)
    v = jnp.var(x, axis=axis, keepdims=True)
    return (x - m) / jnp.sqrt(v + eps)

def _scatter_add(tgt, idx, src, axis=0):
    return tgt.at[idx].add(src)

def _segment_sum(src, seg, n):
    return jax.ops.segment_sum(src, seg, n)

class _Rng:

    def __init__(self, key):
        self._k = key

    def _next(self):
        self._k, sub = jax.random.split(self._k)
        return sub

    def normal(self, shape):
        return jax.random.normal(self._next(), shape, dtype=jnp.bfloat16)

    def randint(self, lo, hi, shape):
        return jax.random.randint(self._next(), shape, lo, hi, dtype=jnp.int32)

    def uniform(self, shape, lo=0.0, hi=1.0):
        return jax.random.uniform(self._next(), shape, jnp.bfloat16, lo, hi)

    def permutation(self, n):
        return jax.random.permutation(self._next(), n)
kernel_name = 'adaLN_cond__sliding_local_dilated__mixer_s_mlp__prompt'

def setup_inputs():
    _rng = _Rng(jax.random.key(int.from_bytes(__import__("os").urandom(4), "little")))
    _w = lambda a: (lambda t: t.astype(jnp.bfloat16) if jnp.issubdtype(t.dtype, jnp.floating) else t)(jnp.asarray(a))

    def _A_setup():
        B, S, D = (1, 2048, 1024)
        return {'x': _w((lambda *s: _rng.normal(s) * 0.05)(B, S, D)), 'wqkv': _w((lambda *s: _rng.normal(s) * 0.05)(D, 3 * D)), 'wo': _w((lambda *s: _rng.normal(s) * 0.05)(D, D))}
    _A_in = _A_setup()

    def _B_setup():
        B, S, D, F = (1, 2048, 1024, 3584)
        return {'x': _w((lambda *s: _rng.normal(s) * 0.05)(B, S, D)), 'w1': _w((lambda *s: _rng.normal(s) * 0.05)(D, D) * D ** (-0.5)), 'w2': _w((lambda *s: _rng.normal(s) * 0.05)(D, D) * D ** (-0.5)), 'w3': _w((lambda *s: _rng.normal(s) * 0.05)(D, F) * D ** (-0.5)), 'w4': _w((lambda *s: _rng.normal(s) * 0.05)(F, D) * F ** (-0.5))}
    _B_in = _B_setup()
    return {'A_x': _A_in['x'], 'A_wqkv': _A_in['wqkv'], 'A_wo': _A_in['wo'], 'B_x': _B_in['x'], 'B_w1': _B_in['w1'], 'B_w2': _B_in['w2'], 'B_w3': _B_in['w3'], 'B_w4': _B_in['w4'], 'c': _w((lambda *s: _rng.normal(s) * 0.05)(1, 1024)), 'w_mod': _w((lambda *s: _rng.normal(s) * 0.05)(1024, 6 * 1024) * 1024 ** (-0.5))}

def reference(A_x, A_wqkv, A_wo, B_x, B_w1, B_w2, B_w3, B_w4, c, w_mod):

    def _A_ref(x, wqkv, wo):
        B, S, D = x.shape
        H = 32
        Dh = D // H
        W, dil = (8, 2)
        qkv = (lambda x, *d: x.transpose(*d))((x @ wqkv).reshape(B, S, 3, H, Dh), 2, 0, 3, 1, 4)
        q, k, v = (qkv[0], qkv[1], qkv[2])
        scale = Dh ** (-0.5)
        pos = jnp.arange(S)
        off = jnp.arange(W) * dil
        idx = pos[:, None] - off[None, :]
        mask = idx >= 0
        idx_c = jnp.where(mask, idx, 0).reshape(-1)
        kg = k[:, :, idx_c, :].reshape(B, H, S, W, Dh)
        vg = v[:, :, idx_c, :].reshape(B, H, S, W, Dh)
        logits = jnp.einsum('bhsd,bhswd->bhsw', q, kg) * scale
        logits = jnp.where(mask[None, None, :, :], logits, -1000000000.0)
        attn = _softmax(logits, axis=-1)
        o = jnp.einsum('bhsw,bhswd->bhsd', attn, vg)
        return (lambda x, *d: x.transpose(*d))(o, 0, 2, 1, 3).reshape(B, S, D) @ wo

    def _B_ref(x, w1, w2, w3, w4):
        B, S, D = x.shape
        h = _gelu(_layernorm(x, axis=-1) @ w1)
        c = D // 4
        g0 = jnp.pad(h[:, :, 0 * c:1 * c], ((0, 0), (1, 0), (0, 0)))[:, :S, :]
        g1 = jnp.pad(h[:, :, 1 * c:2 * c], ((0, 0), (0, 1), (0, 0)))[:, 1:, :]
        g2 = jnp.pad(h[:, :, 2 * c:3 * c], ((0, 0), (2, 0), (0, 0)))[:, :S, :]
        g3 = jnp.pad(h[:, :, 3 * c:], ((0, 0), (0, 2), (0, 0)))[:, 2:, :]
        hs = jnp.concatenate([g0, g1, g2, g3], axis=-1) @ w2
        x1 = x + hs
        h2 = _gelu(_layernorm(x1, axis=-1) @ w3) @ w4
        return x1 + h2
    x = A_x
    mod = (_silu(c) @ w_mod).reshape(c.shape[0], 6, 1, -1)
    sa, ca, ga, sb, cb, gb = (mod[:, 0].copy(), mod[:, 1].copy(), mod[:, 2].copy(), mod[:, 3].copy(), mod[:, 4].copy(), mod[:, 5].copy())
    h = _layernorm(x, axis=-1) * (1 + ca) + sa
    x = x + ga * _A_ref(h, A_wqkv, A_wo)
    h = _layernorm(x, axis=-1) * (1 + cb) + sb
    x = x + gb * _B_ref(h, B_w1, B_w2, B_w3, B_w4)
    return x
```

```python
import functools
import jax
import jax.numpy as jnp
from jax import lax
import jax.experimental.pallas as pl
import jax.experimental.pallas.tpu as pltpu

S, D, F = 2048, 1024, 3584
H, DH, W, DIL = 32, 32, 8, 2
NCH = D // 128
EPS = 1e-5
SCALE = DH ** -0.5
f32, bf16 = jnp.float32, jnp.bfloat16


def _ln(x):
    m = jnp.mean(x, axis=-1, keepdims=True)
    xc = x - m
    v = jnp.mean(xc * xc, axis=-1, keepdims=True)
    return xc * lax.rsqrt(v + EPS)


def _gelu(x):
    c0 = 0.7978845608028654
    c1 = c0 * 0.044715
    t = jnp.tanh(x * (c0 + c1 * (x * x)))
    hx = 0.5 * x
    return hx + hx * t


def _dot(a, b):
    return jnp.dot(a, b, preferred_element_type=f32)


def make(T=256, RB=8):
    NT = S // T
    HALO = 16

    def kernel(x_ref, wqkv_ref, wo_ref, w1_ref, w2_ref, w3_ref, w4_ref, c_ref, wmod_ref,
               o_ref, mod_ref, kbuf, vbuf, qbuf, xmid, hb, h1buf):
        i = pl.program_id(0)

        def stage1(first):
            M = T + HALO if first else T
            off = 0 if first else HALO
            sa = mod_ref[0:1, 0 * D:1 * D]
            ca = mod_ref[0:1, 1 * D:2 * D]
            ga = mod_ref[0:1, 2 * D:3 * D]
            sb = mod_ref[0:1, 3 * D:4 * D]
            cb = mod_ref[0:1, 4 * D:5 * D]
            if first:
                x = x_ref[0:M, :].astype(f32)
            else:
                a = pl.multiple_of(i * T + HALO, 16)
                b = pl.multiple_of(jnp.minimum(i * T + T, S - HALO), 16)
                x = jnp.concatenate([x_ref[pl.ds(a, T - HALO), :], x_ref[pl.ds(b, HALO), :]], axis=0).astype(f32)
            h = (_ln(x) * (1.0 + ca) + sa).astype(bf16)
            qkv = _dot(h, wqkv_ref[...])
            if first:
                for j in range(NCH):
                    kbuf[j, 0:HALO, :] = jnp.zeros((HALO, 128), f32)
                    vbuf[j, 0:HALO, :] = jnp.zeros((HALO, 128), f32)
            else:
                for j in range(NCH):
                    kbuf[j, HALO:2 * HALO, :] = kbuf[j, HALO + T:2 * HALO + T, :]
                    vbuf[j, HALO:2 * HALO, :] = vbuf[j, HALO + T:2 * HALO + T, :]
            base = HALO + off
            for j in range(NCH):
                qbuf[j, 0:M, :] = qkv[:, j * 128:(j + 1) * 128]
                kbuf[j, base:base + M, :] = qkv[:, D + j * 128:D + (j + 1) * 128]
                vbuf[j, base:base + M, :] = qkv[:, 2 * D + j * 128:2 * D + (j + 1) * 128]
            o_rows = []
            for r in range(0, M, RB):
                q = [qbuf[j, r:r + RB, :] for j in range(NCH)]
                s = []
                for w in range(W):
                    acc = None
                    for j in range(NCH):
                        p = q[j] * kbuf[j, base + r - DIL * w:base + r - DIL * w + RB, :]
                        acc = p if acc is None else acc + p
                    acc = acc + pltpu.roll(acc, 64, 1)
                    acc = acc + pltpu.roll(acc, 32, 1)
                    if first and r < DIL * (W - 1):
                        rows = r + lax.broadcasted_iota(jnp.int32, (RB, 128), 0)
                        acc = jnp.where(rows >= DIL * w, acc, -1e30)
                    s.append(acc)
                m = functools.reduce(jnp.maximum, s)
                e = [jnp.exp((sw - m) * SCALE) for sw in s]
                den = functools.reduce(lambda a, b: a + b, e)
                rinv = 1.0 / den
                oc = []
                for j in range(NCH):
                    acc = None
                    for w in range(W):
                        p = e[w] * vbuf[j, base + r - DIL * w:base + r - DIL * w + RB, :]
                        acc = p if acc is None else acc + p
                    oc.append(acc * rinv)
                o_rows.append(jnp.concatenate(oc, axis=1))
            o = jnp.concatenate(o_rows, axis=0).astype(bf16)
            A = _dot(o, wo_ref[...])
            xm = x + ga * A
            hB = _ln(xm) * (1.0 + cb) + sb
            n3 = _ln(hB).astype(bf16)
            h1 = _gelu(_dot(n3, w1_ref[...]))
            if not first:
                rows = lax.broadcasted_iota(jnp.int32, (M, 1), 0) + (i * T + HALO)
                h1 = jnp.where(rows < S, h1, 0.0)
                xmid[0:HALO, :] = xmid[T:T + HALO, :]
                hb[0:HALO, :] = hb[T:T + HALO, :]
                for j in range(NCH):
                    h1buf[j, 0:2 * HALO, :] = h1buf[j, T:T + 2 * HALO, :]
            else:
                for j in range(NCH):
                    h1buf[j, 0:HALO, :] = jnp.zeros((HALO, 128), f32)
            xmid[off:off + M, :] = xm
            hb[off:off + M, :] = hB
            for j in range(NCH):
                h1buf[j, HALO + off:HALO + off + M, :] = h1[:, j * 128:(j + 1) * 128]

        def stage2():
            gb = mod_ref[0:1, 5 * D:6 * D]
            shifts = [-1, -1, 1, 1, -2, -2, 2, 2]
            g = jnp.concatenate(
                [h1buf[j, HALO + shifts[j]:HALO + shifts[j] + T, :] for j in range(NCH)], axis=1).astype(bf16)
            hs = _dot(g, w2_ref[...])
            x1 = hb[0:T, :] + hs
            base = xmid[0:T, :] + gb * x1
            n4 = _ln(x1).astype(bf16)
            u = _gelu(_dot(n4, w3_ref[...])).astype(bf16)
            h2 = _dot(u, w4_ref[...])
            o_ref[...] = (base + gb * h2).astype(o_ref.dtype)

        @pl.when(i == 0)
        def _():
            c = c_ref[...].astype(f32)
            sc = (c * jax.nn.sigmoid(c)).astype(bf16)
            sc = jnp.broadcast_to(sc, (16, D))
            mod_ref[...] = _dot(sc, wmod_ref[...])
            stage1(True)

        @pl.when(jnp.logical_and(i > 0, i < NT))
        def _():
            stage2()
            stage1(False)

        @pl.when(i == NT)
        def _():
            stage2()

    def full(shape):
        return pl.BlockSpec(shape, lambda i: (0,) * len(shape), pipeline_mode=pl.Buffered(1))

    @jax.jit
    def fn(A_x, A_wqkv, A_wo, B_x, B_w1, B_w2, B_w3, B_w4, c, w_mod):
        x = A_x.reshape(S, D)
        wqkv = A_wqkv.reshape(D, 3, H, DH).transpose(0, 1, 3, 2).reshape(D, 3 * D)
        wo = A_wo.reshape(H, DH, D).transpose(1, 0, 2).reshape(D, D)
        out = pl.pallas_call(
            kernel,
            grid=(NT + 1,),
            in_specs=[full((S, D)), full((D, 3 * D)), full((D, D)), full((D, D)), full((D, D)),
                      full((D, F)), full((F, D)), full((1, D)), full((D, 6 * D))],
            out_specs=pl.BlockSpec((T, D), lambda i: (jnp.maximum(i - 1, 0), 0)),
            out_shape=jax.ShapeDtypeStruct((S, D), bf16),
            scratch_shapes=[
                pltpu.VMEM((16, 6 * D), f32),
                pltpu.VMEM((NCH, T + 2 * HALO, 128), f32),
                pltpu.VMEM((NCH, T + 2 * HALO, 128), f32),
                pltpu.VMEM((NCH, T + HALO, 128), f32),
                pltpu.VMEM((T + HALO, D), f32),
                pltpu.VMEM((T + HALO, D), f32),
                pltpu.VMEM((NCH, T + 2 * HALO, 128), f32),
            ],
            compiler_params=pltpu.CompilerParams(
                dimension_semantics=("arbitrary",), vmem_limit_bytes=110 * 1024 * 1024),
        )(x, wqkv, wo, B_w1, B_w2, B_w3, B_w4, c, w_mod)
        return out.reshape(1, S, D)
    return fn


_fn = make()


def pallas_adaLN_cond__sliding_local_dilated__mixer_s_mlp__prompt_kernel(A_x, A_wqkv, A_wo, B_x, B_w1, B_w2, B_w3, B_w4, c, w_mod):
    return _fn(A_x, A_wqkv, A_wo, B_x, B_w1, B_w2, B_w3, B_w4, c, w_mod)
```

```python
import functools
import jax
import jax.numpy as jnp
from jax import lax
import jax.experimental.pallas as pl
import jax.experimental.pallas.tpu as pltpu

S, D, F = 2048, 1024, 3584
H, DH, W, DIL = 32, 32, 8, 2
NCH = D // 128
EPS = 1e-5
SCALE = DH ** -0.5
f32, bf16, u32 = jnp.float32, jnp.bfloat16, jnp.uint32
HALO = 16


def _ln(x):
    m = jnp.mean(x, axis=-1, keepdims=True)
    xc = x - m
    v = jnp.mean(xc * xc, axis=-1, keepdims=True)
    return xc * lax.rsqrt(v + EPS)


def _gelu(x):
    c0 = 0.7978845608028654
    c1 = c0 * 0.044715
    t = jnp.tanh(x * (c0 + c1 * (x * x)))
    hx = 0.5 * x
    return hx + hx * t


def _dot(a, b):
    return jnp.dot(a, b, preferred_element_type=f32)


def _bf(w):
    return pltpu.bitcast(w, bf16)


def _lane_xor(x, s):
    lane = lax.broadcasted_iota(jnp.int32, x.shape, 1)
    return jnp.take_along_axis(x, lane ^ s, axis=1)


def _exchange8(X):
    X = list(X)
    lane = lax.broadcasted_iota(jnp.int32, X[0].shape, 1)
    for t in range(3):
        s = 1 << (t + 2)
        m = (lane & s) != 0
        for p in range(8):
            if p & (1 << t):
                continue
            p2 = p | (1 << t)
            tmp = _lane_xor(jnp.where(m, X[p], X[p2]), s)
            X[p], X[p2] = jnp.where(m, tmp, X[p]), jnp.where(m, X[p2], tmp)
    return X


def make(T=128, TA=128, RB=8, PG=4):
    NT = S // T
    NTA = S // TA

    def kernel(x_hbm, wqkv_hbm, wo_hbm, w1_hbm, w2_hbm, w3_hbm, w4_hbm, c_hbm, wmod_hbm,
               o_hbm,
               x_v, wqkv_raw, wqkv_v, wo_raw, wo_v, w1_v, w2_v, w3_v, w4_v, c_v, wmod_v,
               mod_ref, qbuf, kbuf, vbuf, xmid, hb, h1buf, obuf, sems, osems):
        def cp(src, dst, k):
            return pltpu.make_async_copy(src, dst, sems.at[k])

        xu = x_hbm.bitcast(u32)
        wqkvu = wqkv_hbm.bitcast(u32)
        wou = wo_hbm.bitcast(u32)
        wmodu = wmod_hbm.bitcast(u32)
        X0 = 2 * TA // 2
        c_c = cp(c_hbm, c_v, 0)
        c_x0 = cp(xu.at[0:X0], x_v.at[0:X0], 1)
        c_ma = cp(wmodu.at[:, 0:2 * D], wmod_v.at[:, 0:2 * D], 2)
        c_q = [cp(wqkvu.at[:, b * D:(b + 1) * D], wqkv_raw.at[:, b * D:(b + 1) * D], 3 + b) for b in range(3)]
        c_x1 = cp(xu.at[X0:S // 2], x_v.at[X0:S // 2], 6)
        c_wo = [cp(wou.at[:, n * 128:(n + 1) * 128], wo_raw.at[n, 8:8 + D // 2], 7 + n) for n in range(NCH)]
        c_mb = cp(wmodu.at[:, 2 * D:6 * D], wmod_v.at[:, 2 * D:6 * D], 15)
        c_w1 = cp(w1_hbm.bitcast(u32), w1_v, 16)
        c_w2 = cp(w2_hbm.bitcast(u32), w2_v, 17)
        c_w3 = cp(w3_hbm.bitcast(u32), w3_v, 18)
        c_w4 = cp(w4_hbm.bitcast(u32), w4_v, 19)
        for c in [c_c, c_x0, c_ma] + c_q + [c_x1] + c_wo + [c_mb, c_w1, c_w2, c_w3, c_w4]:
            c.start()

        x_v[S // 2:S // 2 + HALO // 2, :] = jnp.zeros((HALO // 2, D), u32)
        for j in range(NCH):
            z = jnp.zeros((HALO, 128), f32)
            qbuf[j, S:S + HALO, :] = z
            kbuf[j, 0:HALO, :] = z
            vbuf[j, 0:HALO, :] = z
            kbuf[j, HALO + S:2 * HALO + S, :] = z
            vbuf[j, HALO + S:2 * HALO + S, :] = z

        c_c.wait()
        c = c_v[...].astype(f32)
        sc = jnp.broadcast_to((c * jax.nn.sigmoid(c)).astype(bf16), (16, D))
        c_ma.wait()
        mod_ref[:, 0:2 * D] = _dot(sc, _bf(wmod_v[:, 0:2 * D]))

        for b in range(3):
            c_q[b].wait()

            def pbody(g, carry):
                for gg in range(PG):
                    r0 = pl.multiple_of((g * PG + gg) * 8, 8)
                    X = [wqkv_raw[pl.ds(r0, 8), b * D + a * 128:b * D + (a + 1) * 128] for a in range(NCH)]
                    X = _exchange8(X)
                    for a in range(NCH):
                        wqkv_v[pl.ds(r0, 8), b * D + a * 128:b * D + (a + 1) * 128] = X[a]
                return carry
            lax.fori_loop(0, D // 2 // 8 // PG, pbody, 0)

        c_x0.wait()

        def abody(i, carry):
            @pl.when(i == 2)
            def _():
                c_x1.wait()
            sa = mod_ref[0:1, 0 * D:1 * D]
            ca = mod_ref[0:1, 1 * D:2 * D]
            r2 = pl.multiple_of(i * (TA // 2), 8)
            x = _bf(x_v[pl.ds(r2, TA // 2), :]).astype(f32)
            h = (_ln(x) * (1.0 + ca) + sa).astype(bf16)
            qkv = _dot(h, _bf(wqkv_v[...]))
            r = pl.multiple_of(i * TA, 8)
            for j in range(NCH):
                qbuf[j, pl.ds(r, TA), :] = qkv[:, j * 128:(j + 1) * 128]
                kbuf[j, pl.ds(r + HALO, TA), :] = qkv[:, D + j * 128:D + (j + 1) * 128]
                vbuf[j, pl.ds(r + HALO, TA), :] = qkv[:, 2 * D + j * 128:2 * D + (j + 1) * 128]
            return carry
        lax.fori_loop(0, NTA, abody, 0)

        c_mb.wait()
        mod_ref[:, 2 * D:6 * D] = _dot(sc, _bf(wmod_v[:, 2 * D:6 * D]))
        sub = lax.broadcasted_iota(jnp.int32, (8, 128), 0)
        for n in range(NCH):
            c_wo[n].wait()
        for n in range(NCH):
            for tv in range(D // 2 // 8):
                j = tv >> 3
                hh = (tv >> 1) & 3
                a2 = tv & 1
                parts = []
                for al in range(4):
                    a = a2 * 4 + al
                    src = a * 64 + hh * 16 + j * 2
                    st = src - 2 * al + 8
                    parts.append(wo_raw[n, st:st + 8, :])
                v = jnp.where(sub < 2, parts[0], parts[1])
                v2 = jnp.where(sub < 6, parts[2], parts[3])
                wo_v[n, 8 * tv:8 * tv + 8, :] = jnp.where(sub < 4, v, v2)
        c_w1.wait(); c_w2.wait(); c_w3.wait(); c_w4.wait()

        def stage1b(row0, first):
            M = T + HALO if first else T
            off = 0 if first else HALO
            ga = mod_ref[0:1, 2 * D:3 * D]
            sb = mod_ref[0:1, 3 * D:4 * D]
            cb = mod_ref[0:1, 4 * D:5 * D]
            o_rows = []
            for r in range(0, M, RB):
                q = [qbuf[j, pl.ds(row0 + r, RB), :] for j in range(NCH)]
                s = []
                for w in range(W):
                    acc = None
                    for j in range(NCH):
                        p = q[j] * kbuf[j, pl.ds(row0 + HALO + r - DIL * w, RB), :]
                        acc = p if acc is None else acc + p
                    acc = acc + _lane_xor(acc, 1)
                    acc = acc + _lane_xor(acc, 2)
                    if first and r < DIL * (W - 1):
                        rows = r + lax.broadcasted_iota(jnp.int32, (RB, 128), 0)
                        acc = jnp.where(rows >= DIL * w, acc, -1e30)
                    s.append(acc)
                m = functools.reduce(jnp.maximum, s)
                e = [jnp.exp((sw - m) * SCALE) for sw in s]
                den = functools.reduce(lambda a, b: a + b, e)
                rinv = 1.0 / den
                oc = []
                for j in range(NCH):
                    acc = None
                    for w in range(W):
                        p = e[w] * vbuf[j, pl.ds(row0 + HALO + r - DIL * w, RB), :]
                        acc = p if acc is None else acc + p
                    oc.append(acc * rinv)
                o_rows.append(jnp.concatenate(oc, axis=1))
            o = jnp.concatenate(o_rows, axis=0).astype(bf16)
            A = jnp.concatenate([_dot(o, _bf(wo_v[n])) for n in range(NCH)], axis=1)
            if first:
                x = _bf(x_v[0:M // 2, :]).astype(f32)
            else:
                x = _bf(x_v[pl.ds(pl.multiple_of(row0 // 2, 8), M // 2), :]).astype(f32)
            xm = x + ga * A
            hB = _ln(xm) * (1.0 + cb) + sb
            n3 = _ln(hB).astype(bf16)
            h1 = _gelu(_dot(n3, _bf(w1_v[...])))
            if not first:
                xmid[0:HALO, :] = xmid[T:T + HALO, :]
                hb[0:HALO, :] = hb[T:T + HALO, :]
                for j in range(NCH):
                    h1buf[j, 0:2 * HALO, :] = h1buf[j, T:T + 2 * HALO, :]
            else:
                for j in range(NCH):
                    h1buf[j, 0:HALO, :] = jnp.zeros((HALO, 128), f32)
            xmid[off:off + M, :] = xm
            hb[off:off + M, :] = hB
            for j in range(NCH):
                h1buf[j, HALO + off:HALO + off + M, :] = h1[:, j * 128:(j + 1) * 128]

        def out_copy(tile, slot):
            r0 = pl.multiple_of(tile * (T // 2), 8)
            return pltpu.make_async_copy(obuf.at[slot], o_hbm.bitcast(u32).at[pl.ds(r0, T // 2)], osems.at[slot])

        def stage2(slot):
            gb = mod_ref[0:1, 5 * D:6 * D]
            shifts = [-1, -1, 1, 1, -2, -2, 2, 2]
            g = jnp.concatenate(
                [h1buf[j, HALO + shifts[j]:HALO + shifts[j] + T, :] for j in range(NCH)], axis=1).astype(bf16)
            hs = _dot(g, _bf(w2_v[...]))
            x1 = hb[0:T, :] + hs
            base = xmid[0:T, :] + gb * x1
            n4 = _ln(x1).astype(bf16)
            u = _gelu(_dot(n4, _bf(w3_v[...]))).astype(bf16)
            h2 = _dot(u, _bf(w4_v[...]))
            obuf[slot] = pltpu.bitcast((base + gb * h2).astype(bf16), u32)

        stage1b(0, True)

        def bbody(i, carry):
            slot = (i - 1) % 2

            @pl.when(i >= 3)
            def _():
                out_copy(i - 3, slot).wait()
            stage2(slot)
            stage1b(pl.multiple_of(i * T + HALO, 16), False)
            out_copy(i - 1, slot).start()
            return carry
        lax.fori_loop(1, NT, bbody, 0)

        slot = (NT - 1) % 2
        out_copy(NT - 3, slot).wait()
        for j in range(NCH):
            h1buf[j, T + HALO:T + 2 * HALO, :] = jnp.zeros((HALO, 128), f32)
        stage2(slot)
        out_copy(NT - 1, slot).start()
        out_copy(NT - 2, 1 - slot).wait()
        out_copy(NT - 1, slot).wait()

    @jax.jit
    def fn(A_x, A_wqkv, A_wo, B_x, B_w1, B_w2, B_w3, B_w4, c, w_mod):
        x = A_x.reshape(S, D)
        any_spec = pl.BlockSpec(memory_space=pl.ANY)
        out = pl.pallas_call(
            kernel,
            in_specs=[any_spec] * 9,
            out_specs=any_spec,
            out_shape=jax.ShapeDtypeStruct((S, D), bf16),
            scratch_shapes=[
                pltpu.VMEM((S // 2 + HALO // 2, D), u32),
                pltpu.VMEM((D // 2, 3 * D), u32),
                pltpu.VMEM((D // 2, 3 * D), u32),
                pltpu.VMEM((NCH, D // 2 + 16, 128), u32),
                pltpu.VMEM((NCH, D // 2, 128), u32),
                pltpu.VMEM((D // 2, D), u32),
                pltpu.VMEM((D // 2, D), u32),
                pltpu.VMEM((D // 2, F), u32),
                pltpu.VMEM((F // 2, D), u32),
                pltpu.VMEM((1, D), bf16),
                pltpu.VMEM((D // 2, 6 * D), u32),
                pltpu.VMEM((16, 6 * D), f32),
                pltpu.VMEM((NCH, S + HALO, 128), f32),
                pltpu.VMEM((NCH, S + 2 * HALO, 128), f32),
                pltpu.VMEM((NCH, S + 2 * HALO, 128), f32),
                pltpu.VMEM((T + HALO, D), f32),
                pltpu.VMEM((T + HALO, D), f32),
                pltpu.VMEM((NCH, T + 2 * HALO, 128), f32),
                pltpu.VMEM((2, T // 2, D), u32),
                pltpu.SemaphoreType.DMA((20,)),
                pltpu.SemaphoreType.DMA((2,)),
            ],
            compiler_params=pltpu.CompilerParams(vmem_limit_bytes=120 * 1024 * 1024),
        )(x, A_wqkv, A_wo, B_w1, B_w2, B_w3, B_w4, c, w_mod)
        return out.reshape(1, S, D)
    return fn


_fn = make()


def pallas_adaLN_cond__sliding_local_dilated__mixer_s_mlp__prompt_kernel(A_x, A_wqkv, A_wo, B_x, B_w1, B_w2, B_w3, B_w4, c, w_mod):
    return _fn(A_x, A_wqkv, A_wo, B_x, B_w1, B_w2, B_w3, B_w4, c, w_mod)
```

```python
import functools
import jax
import jax.numpy as jnp
from jax import lax
import jax.experimental.pallas as pl
import jax.experimental.pallas.tpu as pltpu

S, D, F = 2048, 1024, 3584
H, DH, W, DIL = 32, 32, 8, 2
NCH = D // 128
EPS = 1e-5
SCALE = DH ** -0.5
f32, bf16, u32 = jnp.float32, jnp.bfloat16, jnp.uint32
HALO = 16


def _ln(x):
    m = jnp.mean(x, axis=-1, keepdims=True)
    xc = x - m
    v = jnp.mean(xc * xc, axis=-1, keepdims=True)
    return xc * lax.rsqrt(v + EPS)


def _gelu(x):
    c0 = 0.7978845608028654
    c1 = c0 * 0.044715
    t = jnp.tanh(x * (c0 + c1 * (x * x)))
    hx = 0.5 * x
    return hx + hx * t


def _dot(a, b):
    return jnp.dot(a, b, preferred_element_type=f32)


def _bf(w):
    return pltpu.bitcast(w, bf16)


def _lane_xor(x, s):
    lane = lax.broadcasted_iota(jnp.int32, x.shape, 1)
    return jnp.take_along_axis(x, lane ^ s, axis=1)


def _exchange8(X, use_roll):
    X = list(X)
    lane = lax.broadcasted_iota(jnp.int32, X[0].shape, 1)
    for t in range(3):
        s = 1 << (t + 2)
        m = (lane & s) != 0
        for p in range(8):
            if p & (1 << t):
                continue
            p2 = p | (1 << t)
            if use_roll:
                a = pltpu.roll(X[p2], s, 1)
                b = pltpu.roll(X[p], 128 - s, 1)
                X[p], X[p2] = jnp.where(m, a, X[p]), jnp.where(m, X[p2], b)
            else:
                tmp = _lane_xor(jnp.where(m, X[p], X[p2]), s)
                X[p], X[p2] = jnp.where(m, tmp, X[p]), jnp.where(m, X[p2], tmp)
    return X


def _group4_sum(acc):
    lane = lax.broadcasted_iota(jnp.int32, acc.shape, 1)
    acc = acc + jnp.where((lane & 1) != 0, pltpu.roll(acc, 1, 1), pltpu.roll(acc, 127, 1))
    acc = acc + jnp.where((lane & 2) != 0, pltpu.roll(acc, 2, 1), pltpu.roll(acc, 126, 1))
    return acc


def make(T=128, M0=512, TA=192, RB=8, AR=48, perm_roll=False):
    NT = S // T
    NTA = (S - M0) // TA
    assert NTA == 8 and NTA * TA + M0 == S
    XP = 32
    NXP = TA // XP
    CP0 = 256
    CPR = (M0 - CP0) // NTA
    S_C, S_X0, S_SA, S_CA, S_WQ, S_XA, S_WO, S_MB, S_W = 0, 1, 5, 13, 21, 29, 37, 45, 53

    def kernel(x_hbm, wqkv_hbm, wo_hbm, w1_hbm, w2_hbm, w3_hbm, w4_hbm, c_hbm, wmod_hbm,
               o_hbm,
               x_v, wqkv_raw, wqkv_v, wo_raw, wo_v, w1_v, w2_v, w3_v, w4_v, c_v, sc_v, wmA_v, wmB_v,
               modA, modB, st_m, st_r, xhatA, q0, k0, v0, qbuf, kbuf, vbuf, xmid, hb, h1buf, obuf, o_scr, g_scr,
               sems, osems):
        def cp(src, dst, k):
            return pltpu.make_async_copy(src, dst, sems.at[k])

        xu = x_hbm.bitcast(u32)
        wqkvu = wqkv_hbm.bitcast(u32)
        wou = wo_hbm.bitcast(u32)
        wmodu = wmod_hbm.bitcast(u32)

        def lane_ds(k, n):
            if isinstance(k, int):
                return pl.ds(k * n, n)
            return pl.ds(pl.multiple_of(k * n, 128), n)

        def row_ds(base, k, n):
            if isinstance(k, int):
                return pl.ds(base + k * n, n)
            return pl.ds(pl.multiple_of(base + k * n, 8), n)

        c_c = cp(c_hbm, c_v, S_C)

        def c_x0(b):
            return cp(xu.at[row_ds(0, b, 64)], x_v.at[row_ds(0, b, 64)], S_X0 + b)

        def c_sa(k):
            return cp(wmodu.at[:, lane_ds(k, 128)], wmA_v.at[k, :, 0:128], S_SA + k)

        def c_ca(k):
            if isinstance(k, int):
                src = wmodu.at[:, pl.ds(D + k * 128, 128)]
            else:
                src = wmodu.at[:, pl.ds(pl.multiple_of(D + k * 128, 128), 128)]
            return cp(src, wmA_v.at[k, :, 128:256], S_CA + k)

        def c_wq(k):
            return cp(wqkvu.at[row_ds(0, k, 64)], wqkv_raw.at[row_ds(0, k, 64)], S_WQ + k)

        def c_xa(p):
            return cp(xu.at[row_ds(M0 // 2, p, TA // 2)], x_v.at[row_ds(M0 // 2, p, TA // 2)], S_XA + p)

        def c_wo(p):
            return cp(wou.at[:, lane_ds(p, 128)], wo_raw.at[p, 8:8 + D // 2], S_WO + p)

        def c_mb(p):
            if isinstance(p, int):
                src = wmodu.at[:, pl.ds(2 * D + p * 512, 512)]
            else:
                src = wmodu.at[:, pl.ds(pl.multiple_of(2 * D + p * 512, 128), 512)]
            return cp(src, wmB_v.at[p], S_MB + p)

        c_w = [cp(w1_hbm.bitcast(u32), w1_v, S_W), cp(w2_hbm.bitcast(u32), w2_v, S_W + 1),
               cp(w3_hbm.bitcast(u32), w3_v, S_W + 2), cp(w4_hbm.bitcast(u32), w4_v, S_W + 3)]

        c_c.start()
        for b in range(4):
            c_x0(b).start()
        for k in range(8):
            c_sa(k).start()
            c_ca(k).start()
            c_wq(k).start()
            if k == 2:
                c_xa(0).start()
        for p in range(8):
            if p < 7:
                c_xa(p + 1).start()
            c_wo(p).start()
            c_mb(p).start()
        for c in c_w:
            c.start()

        x_v[S // 2:S // 2 + HALO // 2, :] = jnp.zeros((HALO // 2, D), u32)
        for j in range(NCH):
            z = jnp.zeros((HALO, 128), f32)
            qbuf[j, S:S + HALO, :] = z
            kbuf[j, HALO + S:2 * HALO + S, :] = z
            vbuf[j, HALO + S:2 * HALO + S, :] = z
            q0[j] = jnp.zeros((M0, 128), f32)
            k0[j] = jnp.zeros((M0 + HALO, 128), f32)
            v0[j] = jnp.zeros((M0 + HALO, 128), f32)
            wo_raw[j, 0:8, :] = jnp.zeros((8, 128), u32)
            wo_raw[j, 8 + D // 2:16 + D // 2, :] = jnp.zeros((8, 128), u32)

        c_c.wait()
        c = c_v[...].astype(f32)
        sc_v[...] = pltpu.bitcast(jnp.broadcast_to((c * jax.nn.sigmoid(c)).astype(bf16), (16, D)), u32)

        def sbody(b, carry):
            c_x0(b).wait()
            xb = _bf(x_v[row_ds(0, b, 64), :])
            m = _dot(xb, jnp.ones((D, 128), bf16)) * (1.0 / D)
            acc = None
            for j in range(NCH):
                xc = xb[:, j * 128:(j + 1) * 128].astype(f32) - m
                acc = xc * xc if acc is None else acc + xc * xc
            var = jnp.sum(acc, axis=-1, keepdims=True) * (1.0 / D)
            r = pl.multiple_of(b * 128, 128)
            st_m[pl.ds(r, 128), :] = m
            st_r[pl.ds(r, 128), :] = jnp.broadcast_to(lax.rsqrt(var + EPS), (128, 128))
            return carry
        lax.fori_loop(0, 4, sbody, 0)

        def prep(k):
            modc = _dot(_bf(sc_v[...]), _bf(wmA_v[k]))
            modA[k] = modc[0:8]
            sa_c = modc[0:1, 0:128]
            ca_c = modc[0:1, 128:256]
            xk = _bf(x_v[0:M0 // 2, lane_ds(k, 128)]).astype(f32)
            h = (((xk - st_m[...]) * st_r[...]) * (1.0 + ca_c) + sa_c).astype(bf16)
            rows = []
            for rg in range(8):
                if isinstance(k, int):
                    rs = pl.ds(k * 64 + rg * 8, 8)
                else:
                    rs = pl.ds(pl.multiple_of(k * 64 + rg * 8, 8), 8)
                parts = []
                for b in range(3):
                    X = [wqkv_raw[rs, b * D + a * 128:b * D + (a + 1) * 128] for a in range(NCH)]
                    parts += _exchange8(X, perm_roll)
                rw = jnp.concatenate(parts, axis=1)
                wqkv_v[rs, :] = rw
                rows.append(rw)
            return h, jnp.concatenate(rows, axis=0)

        c_sa(0).wait(); c_ca(0).wait(); c_wq(0).wait()
        hw0 = prep(0)

        def pbody(kc, hw):
            h, w = hw

            @pl.when(kc < 7)
            def _():
                c_sa(kc + 1).wait(); c_ca(kc + 1).wait(); c_wq(kc + 1).wait()

            @pl.when(kc == 2)
            def _():
                c_xa(0).wait()
            res = _dot(h, _bf(w))
            for j in range(NCH):
                q0[j] += res[:, j * 128:(j + 1) * 128]
                k0[j, HALO:HALO + M0, :] += res[:, D + j * 128:D + (j + 1) * 128]
                v0[j, HALO:HALO + M0, :] += res[:, 2 * D + j * 128:2 * D + (j + 1) * 128]
            nxt = prep(jnp.minimum(kc + 1, 7))
            pc = jnp.maximum(kc - 2, 0)
            src = pl.multiple_of(jnp.where(kc >= 2, M0 // 2 + pc * (XP // 2), 0), 8)
            xp = _bf(x_v[pl.ds(src, XP // 2), :]).astype(f32)
            xhatA[pl.ds(pl.multiple_of(pc * XP, 8), XP), :] = _ln(xp)
            return nxt
        lax.fori_loop(0, 8, pbody, hw0)

        def attention(qb, kb, vb, row0, M, mask_rows):
            o_rows = []
            for r in range(0, M, RB):
                q = [qb[j, pl.ds(row0 + r, RB), :] for j in range(NCH)]
                s = []
                for w in range(W):
                    acc = None
                    for j in range(NCH):
                        p = q[j] * kb[j, pl.ds(row0 + HALO + r - DIL * w, RB), :]
                        acc = p if acc is None else acc + p
                    acc = _group4_sum(acc)
                    if mask_rows and r < DIL * (W - 1) and w > 0:
                        rows = row0 + r + lax.broadcasted_iota(jnp.int32, (RB, 128), 0)
                        acc = jnp.where(rows >= DIL * w, acc, -1e30)
                    s.append(acc)
                m = functools.reduce(jnp.maximum, s)
                e = [jnp.exp((sw - m) * SCALE) for sw in s]
                den = functools.reduce(lambda a, b: a + b, e)
                rinv = 1.0 / den
                oc = []
                for j in range(NCH):
                    acc = None
                    for w in range(W):
                        p = e[w] * vb[j, pl.ds(row0 + HALO + r - DIL * w, RB), :]
                        acc = p if acc is None else acc + p
                    oc.append(acc * rinv)
                o_rows.append(jnp.concatenate(oc, axis=1))
            o = jnp.concatenate(o_rows, axis=0).astype(bf16)
            o_scr[pl.ds(pl.multiple_of(row0 // 2, 8), M // 2), :] = pltpu.bitcast(o, u32)

        sub = lax.broadcasted_iota(jnp.int32, (8, 128), 0)

        def abody(p, carry):
            @pl.when(p < 7)
            def _():
                c_xa(p + 1).wait()
            c_wo(p).wait()
            c_mb(p).wait()
            sa = jnp.concatenate([modA[j, 0:1, 0:128] for j in range(NCH)], axis=1)
            ca = jnp.concatenate([modA[j, 0:1, 128:256] for j in range(NCH)], axis=1)
            h = (xhatA[...] * (1.0 + ca) + sa).astype(bf16)
            qkv = _dot(h, _bf(wqkv_v[...]))
            r = pl.multiple_of(M0 + p * TA, 8)
            for j in range(NCH):
                qbuf[j, pl.ds(r, TA), :] = qkv[:, j * 128:(j + 1) * 128]
                kbuf[j, pl.ds(r + HALO, TA), :] = qkv[:, D + j * 128:D + (j + 1) * 128]
                vbuf[j, pl.ds(r + HALO, TA), :] = qkv[:, 2 * D + j * 128:2 * D + (j + 1) * 128]
            nr = pl.multiple_of(M0 // 2 + jnp.minimum(p + 1, NTA - 1) * (TA // 2), 8)
            xhatA[...] = _ln(_bf(x_v[pl.ds(nr, TA // 2), :]).astype(f32))
            modB[p] = _dot(_bf(sc_v[...]), _bf(wmB_v[p]))[0:8]
            for tv in range(D // 2 // 8):
                j = tv >> 3
                hh = (tv >> 1) & 3
                a2 = tv & 1
                parts = []
                for al in range(4):
                    a = a2 * 4 + al
                    src = a * 64 + hh * 16 + j * 2
                    st = src - 2 * al + 8
                    parts.append(wo_raw[p, st:st + 8, :])
                v = jnp.where(sub < 2, parts[0], parts[1])
                v2 = jnp.where(sub < 6, parts[2], parts[3])
                wo_v[p, 8 * tv:8 * tv + 8, :] = jnp.where(sub < 4, v, v2)
            attention(q0, k0, v0, pl.multiple_of(p * AR, 16), AR, True)
            cr = pl.multiple_of(CP0 + p * CPR, 8)
            for j in range(NCH):
                qbuf[j, pl.ds(cr, CPR), :] = q0[j, pl.ds(cr, CPR), :]
                kbuf[j, pl.ds(cr + HALO, CPR), :] = k0[j, pl.ds(cr + HALO, CPR), :]
                vbuf[j, pl.ds(cr + HALO, CPR), :] = v0[j, pl.ds(cr + HALO, CPR), :]
            return carry
        lax.fori_loop(0, NTA, abody, 0)

        for c in c_w:
            c.wait()

        def rows_u32(ref, row0, M):
            if isinstance(row0, int):
                return _bf(ref[row0 // 2:(row0 + M) // 2, :])
            return _bf(ref[pl.ds(pl.multiple_of(row0 // 2, 8), M // 2), :])

        def wo_dot(row0, M):
            o = rows_u32(o_scr, row0, M)
            return jnp.concatenate([_dot(o, _bf(wo_v[n])) for n in range(NCH)], axis=1)

        def row(k):
            return jnp.concatenate([modB[2 * (k - 2), 0:1, :], modB[2 * (k - 2) + 1, 0:1, :]], axis=1)

        def ln23(row0, M, A):
            ga = row(2); sb = row(3); cb = row(4)
            x = rows_u32(x_v, row0, M).astype(f32)
            xm = x + ga * A
            hB = _ln(xm) * (1.0 + cb) + sb
            n3 = _ln(hB).astype(bf16)
            return xm, hB, n3

        shifts = [-1, -1, 1, 1, -2, -2, 2, 2]

        def make_g():
            g = jnp.concatenate(
                [h1buf[j, HALO + shifts[j]:HALO + shifts[j] + T, :] for j in range(NCH)], axis=1).astype(bf16)
            g_scr[...] = pltpu.bitcast(g, u32)

        def out_copy(tile, slot):
            r0 = pl.multiple_of(tile * (T // 2), 8)
            return pltpu.make_async_copy(obuf.at[slot], o_hbm.bitcast(u32).at[pl.ds(r0, T // 2)], osems.at[slot])

        def ln4(hs):
            gb = row(5)
            x1 = hb[0:T, :] + hs
            base = xmid[0:T, :] + gb * x1
            n4 = _ln(x1).astype(bf16)
            return base, n4

        for j in range(NCH):
            h1buf[j, 0:HALO, :] = jnp.zeros((HALO, 128), f32)
        halves = [(0, 80), (80, T + HALO - 80)]
        As = [wo_dot(r0, m) for r0, m in halves]
        for (r0, m), A in zip(halves, As):
            xm, hB, n3 = ln23(r0, m, A)
            h1 = _gelu(_dot(n3, _bf(w1_v[...])))
            xmid[r0:r0 + m, :] = xm
            hb[r0:r0 + m, :] = hB
            for j in range(NCH):
                h1buf[j, HALO + r0:HALO + r0 + m, :] = h1[:, j * 128:(j + 1) * 128]
        make_g()

        def bbody(i, carry):
            slot = (i - 1) % 2
            row0 = pl.multiple_of(i * T + HALO, 16)
            nrow0 = pl.multiple_of(jnp.minimum(i + 1, NT - 1) * T + HALO, 16)

            @pl.when(i >= 3)
            def _():
                out_copy(i - 3, slot).wait()
            hs = _dot(_bf(g_scr[...]), _bf(w2_v[...]))
            A = wo_dot(row0, T)
            base, n4 = ln4(hs)
            u = _gelu(_dot(n4, _bf(w3_v[...]))).astype(bf16)
            xm, hB, n3 = ln23(row0, T, A)
            h1 = _gelu(_dot(n3, _bf(w1_v[...])))
            xmid[0:HALO, :] = xmid[T:T + HALO, :]
            hb[0:HALO, :] = hb[T:T + HALO, :]
            for j in range(NCH):
                h1buf[j, 0:2 * HALO, :] = h1buf[j, T:T + 2 * HALO, :]
            xmid[HALO:HALO + T, :] = xm
            hb[HALO:HALO + T, :] = hB
            notlast = i < NT - 1
            for j in range(NCH):
                h1j = h1[:, j * 128:(j + 1) * 128]
                h1buf[j, 2 * HALO:HALO + T, :] = h1j[0:T - HALO]
                h1buf[j, HALO + T:2 * HALO + T, :] = jnp.where(notlast, h1j[T - HALO:T], 0.0)
            make_g()
            attention(qbuf, kbuf, vbuf, nrow0, T, False)
            h2 = _dot(u, _bf(w4_v[...]))
            obuf[slot] = pltpu.bitcast((base + row(5) * h2).astype(bf16), u32)
            out_copy(i - 1, slot).start()
            return carry
        lax.fori_loop(1, NT, bbody, 0)

        slot = (NT - 1) % 2
        out_copy(NT - 3, slot).wait()
        hs = _dot(_bf(g_scr[...]), _bf(w2_v[...]))
        base, n4 = ln4(hs)
        u = _gelu(_dot(n4, _bf(w3_v[...]))).astype(bf16)
        h2 = _dot(u, _bf(w4_v[...]))
        obuf[slot] = pltpu.bitcast((base + row(5) * h2).astype(bf16), u32)
        out_copy(NT - 1, slot).start()
        out_copy(NT - 2, 1 - slot).wait()
        out_copy(NT - 1, slot).wait()

    @jax.jit
    def fn(A_x, A_wqkv, A_wo, B_x, B_w1, B_w2, B_w3, B_w4, c, w_mod):
        x = A_x.reshape(S, D)
        any_spec = pl.BlockSpec(memory_space=pl.ANY)
        out = pl.pallas_call(
            kernel,
            in_specs=[any_spec] * 9,
            out_specs=any_spec,
            out_shape=jax.ShapeDtypeStruct((S, D), bf16),
            scratch_shapes=[
                pltpu.VMEM((S // 2 + HALO // 2, D), u32),
                pltpu.VMEM((D // 2, 3 * D), u32),
                pltpu.VMEM((D // 2, 3 * D), u32),
                pltpu.VMEM((NCH, D // 2 + 16, 128), u32),
                pltpu.VMEM((NCH, D // 2, 128), u32),
                pltpu.VMEM((D // 2, D), u32),
                pltpu.VMEM((D // 2, D), u32),
                pltpu.VMEM((D // 2, F), u32),
                pltpu.VMEM((F // 2, D), u32),
                pltpu.VMEM((1, D), bf16),
                pltpu.VMEM((8, D), u32),
                pltpu.VMEM((8, D // 2, 256), u32),
                pltpu.VMEM((8, D // 2, 512), u32),
                pltpu.VMEM((8, 8, 256), f32),
                pltpu.VMEM((8, 8, 512), f32),
                pltpu.VMEM((M0, 128), f32),
                pltpu.VMEM((M0, 128), f32),
                pltpu.VMEM((TA, D), f32),
                pltpu.VMEM((NCH, M0, 128), f32),
                pltpu.VMEM((NCH, M0 + HALO, 128), f32),
                pltpu.VMEM((NCH, M0 + HALO, 128), f32),
                pltpu.VMEM((NCH, S + HALO, 128), f32),
                pltpu.VMEM((NCH, S + 2 * HALO, 128), f32),
                pltpu.VMEM((NCH, S + 2 * HALO, 128), f32),
                pltpu.VMEM((T + HALO, D), f32),
                pltpu.VMEM((T + HALO, D), f32),
                pltpu.VMEM((NCH, T + 2 * HALO, 128), f32),
                pltpu.VMEM((2, T // 2, D), u32),
                pltpu.VMEM((S // 2 + HALO // 2, D), u32),
                pltpu.VMEM((T // 2, D), u32),
                pltpu.SemaphoreType.DMA((57,)),
                pltpu.SemaphoreType.DMA((2,)),
            ],
            compiler_params=pltpu.CompilerParams(vmem_limit_bytes=120 * 1024 * 1024),
        )(x, A_wqkv, A_wo, B_w1, B_w2, B_w3, B_w4, c, w_mod)
        return out.reshape(1, S, D)
    return fn


_fn = make()


def pallas_adaLN_cond__sliding_local_dilated__mixer_s_mlp__prompt_kernel(A_x, A_wqkv, A_wo, B_x, B_w1, B_w2, B_w3, B_w4, c, w_mod):
    return _fn(A_x, A_wqkv, A_wo, B_x, B_w1, B_w2, B_w3, B_w4, c, w_mod)
```

```python
import functools
import jax
import jax.numpy as jnp
from jax import lax
import jax.experimental.pallas as pl
import jax.experimental.pallas.tpu as pltpu

S, D, F = 2048, 1024, 3584
H, DH, W, DIL = 32, 32, 8, 2
NCH = D // 128
EPS = 1e-5
SCALE = DH ** -0.5
f32, bf16, u32 = jnp.float32, jnp.bfloat16, jnp.uint32
HALO = 16


def _ln(x):
    m = jnp.mean(x, axis=-1, keepdims=True)
    xc = x - m
    v = jnp.mean(xc * xc, axis=-1, keepdims=True)
    return xc * lax.rsqrt(v + EPS)


def _gelu(x):
    c0 = 0.7978845608028654
    c1 = c0 * 0.044715
    t = jnp.tanh(x * (c0 + c1 * (x * x)))
    hx = 0.5 * x
    return hx + hx * t


def _dot(a, b):
    return jnp.dot(a, b, preferred_element_type=f32)


def _bf(w):
    return pltpu.bitcast(w, bf16)


def _lane_xor(x, s):
    lane = lax.broadcasted_iota(jnp.int32, x.shape, 1)
    return jnp.take_along_axis(x, lane ^ s, axis=1)


def _exchange8(X):
    X = list(X)
    lane = lax.broadcasted_iota(jnp.int32, X[0].shape, 1)
    for t in range(3):
        s = 1 << (t + 2)
        m = (lane & s) != 0
        for p in range(8):
            if p & (1 << t):
                continue
            p2 = p | (1 << t)
            tmp = _lane_xor(jnp.where(m, X[p], X[p2]), s)
            X[p], X[p2] = jnp.where(m, tmp, X[p]), jnp.where(m, X[p2], tmp)
    return X


def _group4_sum(acc):
    lane = lax.broadcasted_iota(jnp.int32, acc.shape, 1)
    acc = acc + jnp.where((lane & 1) != 0, pltpu.roll(acc, 1, 1), pltpu.roll(acc, 127, 1))
    acc = acc + jnp.where((lane & 2) != 0, pltpu.roll(acc, 2, 1), pltpu.roll(acc, 126, 1))
    return acc


def make(T=128, M0=512, TA=192, RB=8, AR=48):
    NT = S // T
    NTA = (S - M0) // TA
    assert NTA == 8 and NTA * TA + M0 == S
    XP = 32
    NXP = TA // XP
    CP0 = 256
    CPR = (M0 - CP0) // NTA
    S_C, S_X0, S_SA, S_CA, S_WQ, S_XA, S_WO, S_MB, S_W = 0, 1, 5, 13, 21, 29, 37, 45, 53

    def kernel(x_hbm, wqkv_hbm, wo_hbm, w1_hbm, w2_hbm, w3_hbm, w4_hbm, c_hbm, wmod_hbm,
               o_hbm,
               x_v, wqkv_raw, wqkv_v, wo_raw, wo_v, w1_v, w2_v, w3_v, w4_v, c_v, sc_v, wmA_v, wmB_v,
               modA, modB, st_m, st_r, xhatA, q0, k0, v0, qbuf, kbuf, vbuf, xmid, hb, h1buf, obuf, o_scr,
               sems, osems):
        def cp(src, dst, k):
            return pltpu.make_async_copy(src, dst, sems.at[k])

        xu = x_hbm.bitcast(u32)
        wqkvu = wqkv_hbm.bitcast(u32)
        wou = wo_hbm.bitcast(u32)
        wmodu = wmod_hbm.bitcast(u32)

        def lane_ds(k, n):
            if isinstance(k, int):
                return pl.ds(k * n, n)
            return pl.ds(pl.multiple_of(k * n, 128), n)

        def row_ds(base, k, n):
            if isinstance(k, int):
                return pl.ds(base + k * n, n)
            return pl.ds(pl.multiple_of(base + k * n, 8), n)

        c_c = cp(c_hbm, c_v, S_C)

        def c_x0(b):
            return cp(xu.at[row_ds(0, b, 64)], x_v.at[row_ds(0, b, 64)], S_X0 + b)

        def c_sa(k):
            return cp(wmodu.at[:, lane_ds(k, 128)], wmA_v.at[k, :, 0:128], S_SA + k)

        def c_ca(k):
            if isinstance(k, int):
                src = wmodu.at[:, pl.ds(D + k * 128, 128)]
            else:
                src = wmodu.at[:, pl.ds(pl.multiple_of(D + k * 128, 128), 128)]
            return cp(src, wmA_v.at[k, :, 128:256], S_CA + k)

        def c_wq(k):
            return cp(wqkvu.at[row_ds(0, k, 64)], wqkv_raw.at[row_ds(0, k, 64)], S_WQ + k)

        def c_xa(p):
            return cp(xu.at[row_ds(M0 // 2, p, TA // 2)], x_v.at[row_ds(M0 // 2, p, TA // 2)], S_XA + p)

        def c_wo(p):
            return cp(wou.at[:, lane_ds(p, 128)], wo_raw.at[p, 8:8 + D // 2], S_WO + p)

        def c_mb(p):
            if isinstance(p, int):
                src = wmodu.at[:, pl.ds(2 * D + p * 512, 512)]
            else:
                src = wmodu.at[:, pl.ds(pl.multiple_of(2 * D + p * 512, 128), 512)]
            return cp(src, wmB_v.at[p], S_MB + p)

        c_w = [cp(w1_hbm.bitcast(u32), w1_v, S_W), cp(w2_hbm.bitcast(u32), w2_v, S_W + 1),
               cp(w3_hbm.bitcast(u32), w3_v, S_W + 2), cp(w4_hbm.bitcast(u32), w4_v, S_W + 3)]

        c_c.start()
        c_wq(0).start()
        for b in range(4):
            c_x0(b).start()
        for k in range(8):
            c_sa(k).start()
            c_ca(k).start()
            if k > 0:
                c_wq(k).start()
            if k == 2:
                c_xa(0).start()
        for p in range(8):
            if p < 7:
                c_xa(p + 1).start()
            c_wo(p).start()
            c_mb(p).start()
        for c in c_w:
            c.start()

        x_v[S // 2:S // 2 + HALO // 2, :] = jnp.zeros((HALO // 2, D), u32)
        for j in range(NCH):
            z = jnp.zeros((HALO, 128), f32)
            qbuf[j, S:S + HALO, :] = z
            kbuf[j, HALO + S:2 * HALO + S, :] = z
            vbuf[j, HALO + S:2 * HALO + S, :] = z
            k0[j, 0:HALO, :] = z
            v0[j, 0:HALO, :] = z
            wo_raw[j, 0:8, :] = jnp.zeros((8, 128), u32)
            wo_raw[j, 8 + D // 2:16 + D // 2, :] = jnp.zeros((8, 128), u32)

        c_c.wait()
        c = c_v[...].astype(f32)
        sc_v[...] = pltpu.bitcast(jnp.broadcast_to((c * jax.nn.sigmoid(c)).astype(bf16), (16, D)), u32)

        def stats(b):
            c_x0(b).wait()
            xb = _bf(x_v[b * 64:(b + 1) * 64, :])
            m = _dot(xb, jnp.ones((D, 128), bf16)) * (1.0 / D)
            acc = None
            for j in range(NCH):
                xc = xb[:, j * 128:(j + 1) * 128].astype(f32) - m
                acc = xc * xc if acc is None else acc + xc * xc
            var = jnp.sum(acc, axis=-1, keepdims=True) * (1.0 / D)
            st_m[b * 128:(b + 1) * 128, :] = m
            st_r[b * 128:(b + 1) * 128, :] = jnp.broadcast_to(lax.rsqrt(var + EPS), (128, 128))

        def exch(k, b):
            for rg in range(8):
                rs = pl.ds(k * 64 + rg * 8, 8)
                X = [wqkv_raw[rs, b * D + a * 128:b * D + (a + 1) * 128] for a in range(NCH)]
                wqkv_v[rs, b * D:(b + 1) * D] = jnp.concatenate(_exchange8(X), axis=1)

        def modh(k):
            modc = _dot(_bf(sc_v[...]), _bf(wmA_v[k]))
            modA[k] = modc[0:8]
            sa_c = modc[0:1, 0:128]
            ca_c = modc[0:1, 128:256]
            xk = _bf(x_v[0:M0 // 2, k * 128:(k + 1) * 128]).astype(f32)
            return (((xk - st_m[...]) * st_r[...]) * (1.0 + ca_c) + sa_c).astype(bf16)

        c_wq(0).wait()
        exch(0, 0)
        stats(0)
        exch(0, 1)
        stats(1)
        exch(0, 2)
        stats(2)
        stats(3)
        c_sa(0).wait(); c_ca(0).wait()
        h = modh(0)

        for kc in range(8):
            if kc < 7:
                c_sa(kc + 1).wait(); c_ca(kc + 1).wait(); c_wq(kc + 1).wait()
            if kc == 2:
                c_xa(0).wait()
            res = _dot(h, _bf(wqkv_v[kc * 64:(kc + 1) * 64, :]))
            for j in range(NCH):
                if kc == 0:
                    q0[j] = res[:, j * 128:(j + 1) * 128]
                    k0[j, HALO:HALO + M0, :] = res[:, D + j * 128:D + (j + 1) * 128]
                    v0[j, HALO:HALO + M0, :] = res[:, 2 * D + j * 128:2 * D + (j + 1) * 128]
                else:
                    q0[j] += res[:, j * 128:(j + 1) * 128]
                    k0[j, HALO:HALO + M0, :] += res[:, D + j * 128:D + (j + 1) * 128]
                    v0[j, HALO:HALO + M0, :] += res[:, 2 * D + j * 128:2 * D + (j + 1) * 128]
            if kc < 7:
                for b in range(3):
                    exch(kc + 1, b)
                h = modh(kc + 1)
            if kc >= 2:
                pc = kc - 2
                xp = _bf(x_v[M0 // 2 + pc * (XP // 2):M0 // 2 + (pc + 1) * (XP // 2), :]).astype(f32)
                xhatA[pc * XP:(pc + 1) * XP, :] = _ln(xp)

        def attention(qb, kb, vb, base, off, M, mask_rows):
            row0 = base + off

            def kvds(r, w):
                return pl.ds(base + (off + HALO + r - DIL * w), RB)

            o_rows = []
            for r in range(0, M, RB):
                q = [qb[j, pl.ds(base + (off + r), RB), :] for j in range(NCH)]
                s = []
                for w in range(W):
                    acc = None
                    for j in range(NCH):
                        p = q[j] * kb[j, kvds(r, w), :]
                        acc = p if acc is None else acc + p
                    acc = _group4_sum(acc)
                    if mask_rows and r < DIL * (W - 1) and w > 0:
                        rows = row0 + r + lax.broadcasted_iota(jnp.int32, (RB, 128), 0)
                        acc = jnp.where(rows >= DIL * w, acc, -1e30)
                    s.append(acc)
                m = functools.reduce(jnp.maximum, s)
                e = [jnp.exp((sw - m) * SCALE) for sw in s]
                den = functools.reduce(lambda a, b: a + b, e)
                rinv = 1.0 / den
                oc = []
                for j in range(NCH):
                    acc = None
                    for w in range(W):
                        p = e[w] * vb[j, kvds(r, w), :]
                        acc = p if acc is None else acc + p
                    oc.append(acc * rinv)
                o_rows.append(jnp.concatenate(oc, axis=1))
            o = jnp.concatenate(o_rows, axis=0).astype(bf16)
            if isinstance(row0, int):
                o_scr[row0 // 2:(row0 + M) // 2, :] = pltpu.bitcast(o, u32)
            else:
                o_scr[pl.ds(pl.multiple_of(row0 // 2, 8), M // 2), :] = pltpu.bitcast(o, u32)

        sub = lax.broadcasted_iota(jnp.int32, (8, 128), 0)

        def abody(p, carry):
            @pl.when(p < 7)
            def _():
                c_xa(p + 1).wait()
            c_wo(p).wait()
            c_mb(p).wait()
            sa = jnp.concatenate([modA[j, 0:1, 0:128] for j in range(NCH)], axis=1)
            ca = jnp.concatenate([modA[j, 0:1, 128:256] for j in range(NCH)], axis=1)
            h = (xhatA[...] * (1.0 + ca) + sa).astype(bf16)
            qkv = _dot(h, _bf(wqkv_v[...]))
            r = pl.multiple_of(M0 + p * TA, 8)
            for j in range(NCH):
                qbuf[j, pl.ds(r, TA), :] = qkv[:, j * 128:(j + 1) * 128]
                kbuf[j, pl.ds(r + HALO, TA), :] = qkv[:, D + j * 128:D + (j + 1) * 128]
                vbuf[j, pl.ds(r + HALO, TA), :] = qkv[:, 2 * D + j * 128:2 * D + (j + 1) * 128]
            nr = pl.multiple_of(M0 // 2 + jnp.minimum(p + 1, NTA - 1) * (TA // 2), 8)
            xhatA[...] = _ln(_bf(x_v[pl.ds(nr, TA // 2), :]).astype(f32))
            modB[p] = _dot(_bf(sc_v[...]), _bf(wmB_v[p]))[0:8]
            for tv in range(D // 2 // 8):
                j = tv >> 3
                hh = (tv >> 1) & 3
                a2 = tv & 1
                parts = []
                for al in range(4):
                    a = a2 * 4 + al
                    src = a * 64 + hh * 16 + j * 2
                    st = src - 2 * al + 8
                    parts.append(wo_raw[p, st:st + 8, :])
                v = jnp.where(sub < 2, parts[0], parts[1])
                v2 = jnp.where(sub < 6, parts[2], parts[3])
                wo_v[p, 8 * tv:8 * tv + 8, :] = jnp.where(sub < 4, v, v2)
            attention(q0, k0, v0, pl.multiple_of(p * AR, 16), 0, AR, True)
            cr = pl.multiple_of(CP0 + p * CPR, 8)
            for j in range(NCH):
                qbuf[j, pl.ds(cr, CPR), :] = q0[j, pl.ds(cr, CPR), :]
                kbuf[j, pl.ds(cr + HALO, CPR), :] = k0[j, pl.ds(cr + HALO, CPR), :]
                vbuf[j, pl.ds(cr + HALO, CPR), :] = v0[j, pl.ds(cr + HALO, CPR), :]
            return carry
        lax.fori_loop(0, NTA, abody, 0)

        for c in c_w:
            c.wait()

        def rows_u32(ref, row0, M):
            if isinstance(row0, int):
                return _bf(ref[row0 // 2:(row0 + M) // 2, :])
            return _bf(ref[pl.ds(pl.multiple_of(row0 // 2, 8), M // 2), :])

        def wo_dot(row0, M):
            o = rows_u32(o_scr, row0, M)
            return jnp.concatenate([_dot(o, _bf(wo_v[n])) for n in range(NCH)], axis=1)

        def row(k):
            return jnp.concatenate([modB[2 * (k - 2), 0:1, :], modB[2 * (k - 2) + 1, 0:1, :]], axis=1)

        def ln23(row0, M, A):
            ga = row(2); sb = row(3); cb = row(4)
            x = rows_u32(x_v, row0, M).astype(f32)
            xm = x + ga * A
            hB = _ln(xm) * (1.0 + cb) + sb
            n3 = _ln(hB).astype(bf16)
            return xm, hB, n3

        shifts = [-1, -1, 1, 1, -2, -2, 2, 2]

        def g_val():
            return jnp.concatenate(
                [h1buf[j, HALO + shifts[j]:HALO + shifts[j] + T, :] for j in range(NCH)], axis=1).astype(bf16)

        def out_copy(tile, slot):
            r0 = pl.multiple_of(tile * (T // 2), 8)
            return pltpu.make_async_copy(obuf.at[slot], o_hbm.bitcast(u32).at[pl.ds(r0, T // 2)], osems.at[slot])

        def ln4(hs):
            gb = row(5)
            x1 = hb[0:T, :] + hs
            base = xmid[0:T, :] + gb * x1
            n4 = _ln(x1).astype(bf16)
            return base, n4

        for j in range(NCH):
            h1buf[j, 0:HALO, :] = jnp.zeros((HALO, 128), f32)
        halves = [(0, 80), (80, T + HALO - 80)]
        As = [wo_dot(r0, m) for r0, m in halves]
        for (r0, m), A in zip(halves, As):
            xm, hB, n3 = ln23(r0, m, A)
            h1 = _gelu(_dot(n3, _bf(w1_v[...])))
            xmid[r0:r0 + m, :] = xm
            hb[r0:r0 + m, :] = hB
            for j in range(NCH):
                h1buf[j, HALO + r0:HALO + r0 + m, :] = h1[:, j * 128:(j + 1) * 128]

        def bbody(i, carry):
            slot = (i - 1) % 2
            row0 = pl.multiple_of(i * T + HALO, 16)

            @pl.when(i >= 3)
            def _():
                out_copy(i - 3, slot).wait()

            hs = _dot(g_val(), _bf(w2_v[...]))
            A = wo_dot(row0, T)
            base, n4 = ln4(hs)
            u = _gelu(_dot(n4, _bf(w3_v[...]))).astype(bf16)
            xm, hB, n3 = ln23(row0, T, A)
            h1 = _gelu(_dot(n3, _bf(w1_v[...])))
            xmid[0:HALO, :] = xmid[T:T + HALO, :]
            hb[0:HALO, :] = hb[T:T + HALO, :]
            for j in range(NCH):
                h1buf[j, 0:2 * HALO, :] = h1buf[j, T:T + 2 * HALO, :]
            xmid[HALO:HALO + T, :] = xm
            hb[HALO:HALO + T, :] = hB
            notlast = i < NT - 1
            for j in range(NCH):
                h1j = h1[:, j * 128:(j + 1) * 128]
                h1buf[j, 2 * HALO:HALO + T, :] = h1j[0:T - HALO]
                h1buf[j, HALO + T:2 * HALO + T, :] = jnp.where(notlast, h1j[T - HALO:T], 0.0)
            attention(qbuf, kbuf, vbuf, pl.multiple_of(jnp.minimum(i + 1, NT - 1) * T, T), HALO, T, False)
            h2 = _dot(u, _bf(w4_v[...]))
            obuf[slot] = pltpu.bitcast((base + row(5) * h2).astype(bf16), u32)
            out_copy(i - 1, slot).start()
            return carry
        lax.fori_loop(1, NT, bbody, 0)

        slot = (NT - 1) % 2
        out_copy(NT - 3, slot).wait()
        hs = _dot(g_val(), _bf(w2_v[...]))
        base, n4 = ln4(hs)
        u = _gelu(_dot(n4, _bf(w3_v[...]))).astype(bf16)
        h2 = _dot(u, _bf(w4_v[...]))
        obuf[slot] = pltpu.bitcast((base + row(5) * h2).astype(bf16), u32)
        out_copy(NT - 1, slot).start()
        out_copy(NT - 2, 1 - slot).wait()
        out_copy(NT - 1, slot).wait()

    @jax.jit
    def fn(A_x, A_wqkv, A_wo, B_x, B_w1, B_w2, B_w3, B_w4, c, w_mod):
        x = A_x.reshape(S, D)
        any_spec = pl.BlockSpec(memory_space=pl.ANY)
        out = pl.pallas_call(
            kernel,
            in_specs=[any_spec] * 9,
            out_specs=any_spec,
            out_shape=jax.ShapeDtypeStruct((S, D), bf16),
            scratch_shapes=[
                pltpu.VMEM((S // 2 + HALO // 2, D), u32),
                pltpu.VMEM((D // 2, 3 * D), u32),
                pltpu.VMEM((D // 2, 3 * D), u32),
                pltpu.VMEM((NCH, D // 2 + 16, 128), u32),
                pltpu.VMEM((NCH, D // 2, 128), u32),
                pltpu.VMEM((D // 2, D), u32),
                pltpu.VMEM((D // 2, D), u32),
                pltpu.VMEM((D // 2, F), u32),
                pltpu.VMEM((F // 2, D), u32),
                pltpu.VMEM((1, D), bf16),
                pltpu.VMEM((8, D), u32),
                pltpu.VMEM((8, D // 2, 256), u32),
                pltpu.VMEM((8, D // 2, 512), u32),
                pltpu.VMEM((8, 8, 256), f32),
                pltpu.VMEM((8, 8, 512), f32),
                pltpu.VMEM((M0, 128), f32),
                pltpu.VMEM((M0, 128), f32),
                pltpu.VMEM((TA, D), f32),
                pltpu.VMEM((NCH, M0, 128), f32),
                pltpu.VMEM((NCH, M0 + HALO, 128), f32),
                pltpu.VMEM((NCH, M0 + HALO, 128), f32),
                pltpu.VMEM((NCH, S + HALO, 128), f32),
                pltpu.VMEM((NCH, S + 2 * HALO, 128), f32),
                pltpu.VMEM((NCH, S + 2 * HALO, 128), f32),
                pltpu.VMEM((T + HALO, D), f32),
                pltpu.VMEM((T + HALO, D), f32),
                pltpu.VMEM((NCH, T + 2 * HALO, 128), f32),
                pltpu.VMEM((2, T // 2, D), u32),
                pltpu.VMEM((S // 2 + HALO // 2, D), u32),
                pltpu.SemaphoreType.DMA((57,)),
                pltpu.SemaphoreType.DMA((2,)),
            ],
            compiler_params=pltpu.CompilerParams(vmem_limit_bytes=120 * 1024 * 1024),
        )(x, A_wqkv, A_wo, B_w1, B_w2, B_w3, B_w4, c, w_mod)
        return out.reshape(1, S, D)
    return fn


_fn = make()


def pallas_adaLN_cond__sliding_local_dilated__mixer_s_mlp__prompt_kernel(A_x, A_wqkv, A_wo, B_x, B_w1, B_w2, B_w3, B_w4, c, w_mod):
    return _fn(A_x, A_wqkv, A_wo, B_x, B_w1, B_w2, B_w3, B_w4, c, w_mod)
```

```python
import functools
import jax
import jax.numpy as jnp
from jax import lax
import jax.experimental.pallas as pl
import jax.experimental.pallas.tpu as pltpu

S, D, F = 2048, 1024, 3584
H, DH, W, DIL = 32, 32, 8, 2
NCH = D // 128
EPS = 1e-5
SCALE = DH ** -0.5
f32, bf16, u32 = jnp.float32, jnp.bfloat16, jnp.uint32
HALO = 16


def _ln(x):
    m = jnp.mean(x, axis=-1, keepdims=True)
    xc = x - m
    v = jnp.mean(xc * xc, axis=-1, keepdims=True)
    return xc * lax.rsqrt(v + EPS)


def _gelu(x):
    c0 = 0.7978845608028654
    c1 = c0 * 0.044715
    t = jnp.tanh(x * (c0 + c1 * (x * x)))
    hx = 0.5 * x
    return hx + hx * t


def _dot(a, b):
    return jnp.dot(a, b, preferred_element_type=f32)


def _bf(w):
    return pltpu.bitcast(w, bf16)


def _lane_xor(x, s):
    lane = lax.broadcasted_iota(jnp.int32, x.shape, 1)
    return jnp.take_along_axis(x, lane ^ s, axis=1)


def _exchange8_multi(XS):
    XS = [list(X) for X in XS]
    lane = lax.broadcasted_iota(jnp.int32, XS[0][0].shape, 1)
    for t in range(3):
        s = 1 << (t + 2)
        m = (lane & s) != 0
        for X in XS:
            for p in range(8):
                if p & (1 << t):
                    continue
                p2 = p | (1 << t)
                tmp = _lane_xor(jnp.where(m, X[p], X[p2]), s)
                X[p], X[p2] = jnp.where(m, tmp, X[p]), jnp.where(m, X[p2], tmp)
    return XS


def _group4_sum(acc):
    lane = lax.broadcasted_iota(jnp.int32, acc.shape, 1)
    acc = acc + jnp.where((lane & 1) != 0, pltpu.roll(acc, 1, 1), pltpu.roll(acc, 127, 1))
    acc = acc + jnp.where((lane & 2) != 0, pltpu.roll(acc, 2, 1), pltpu.roll(acc, 126, 1))
    return acc


def make(T=128, M0=512, TA=192, RB=8, AR=48, CP0=256, EG=4, IL0=512):
    NT = S // T
    NTA = (S - M0) // TA
    assert NTA == 8 and NTA * TA + M0 == S
    XP = 32
    NXP = TA // XP
    CPR = (M0 - CP0) // NTA
    S_C, S_X0, S_SA, S_CA, S_WQ, S_XA, S_WO, S_MB, S_W = 0, 1, 5, 13, 21, 29, 37, 45, 53

    def kernel(x_hbm, wqkv_hbm, wo_hbm, w1_hbm, w2_hbm, w3_hbm, w4_hbm, c_hbm, wmod_hbm,
               o_hbm,
               x_v, wqkv_raw, wqkv_v, wo_raw, wo_v, w1_v, w2_v, w3_v, w4_v, c_v, sc_v, wmA_v, wmB_v,
               modA, modB, st_m, st_r, xhatA, q0, k0, v0, qbuf, kbuf, vbuf, xmid, hb, h1buf, obuf, o_scr,
               sems, osems):
        def cp(src, dst, k):
            return pltpu.make_async_copy(src, dst, sems.at[k])

        xu = x_hbm.bitcast(u32)
        wqkvu = wqkv_hbm.bitcast(u32)
        wou = wo_hbm.bitcast(u32)
        wmodu = wmod_hbm.bitcast(u32)

        def lane_ds(k, n):
            if isinstance(k, int):
                return pl.ds(k * n, n)
            return pl.ds(pl.multiple_of(k * n, 128), n)

        def row_ds(base, k, n):
            if isinstance(k, int):
                return pl.ds(base + k * n, n)
            return pl.ds(pl.multiple_of(base + k * n, 8), n)

        c_c = cp(c_hbm, c_v, S_C)

        def c_x0(b):
            return cp(xu.at[row_ds(0, b, 64)], x_v.at[row_ds(0, b, 64)], S_X0 + b)

        def c_sa(k):
            return cp(wmodu.at[:, lane_ds(k, 128)], wmA_v.at[k, :, 0:128], S_SA + k)

        def c_ca(k):
            if isinstance(k, int):
                src = wmodu.at[:, pl.ds(D + k * 128, 128)]
            else:
                src = wmodu.at[:, pl.ds(pl.multiple_of(D + k * 128, 128), 128)]
            return cp(src, wmA_v.at[k, :, 128:256], S_CA + k)

        def c_wq(k):
            return cp(wqkvu.at[row_ds(0, k, 64)], wqkv_raw.at[row_ds(0, k, 64)], S_WQ + k)

        def c_xa(p):
            return cp(xu.at[row_ds(M0 // 2, p, TA // 2)], x_v.at[row_ds(M0 // 2, p, TA // 2)], S_XA + p)

        def c_wo(p):
            return cp(wou.at[:, lane_ds(p, 128)], wo_raw.at[p, 8:8 + D // 2], S_WO + p)

        def c_mb(p):
            if isinstance(p, int):
                src = wmodu.at[:, pl.ds(2 * D + p * 512, 512)]
            else:
                src = wmodu.at[:, pl.ds(pl.multiple_of(2 * D + p * 512, 128), 512)]
            return cp(src, wmB_v.at[p], S_MB + p)

        c_w = [cp(w1_hbm.bitcast(u32), w1_v, S_W), cp(w2_hbm.bitcast(u32), w2_v, S_W + 1),
               cp(w3_hbm.bitcast(u32), w3_v, S_W + 2), cp(w4_hbm.bitcast(u32), w4_v, S_W + 3)]

        c_c.start()
        c_wq(0).start()
        for b in range(4):
            c_x0(b).start()
        for k in range(8):
            c_sa(k).start()
            c_ca(k).start()
            if k > 0:
                c_wq(k).start()
            if k == 2:
                c_xa(0).start()
        for p in range(8):
            if p < 7:
                c_xa(p + 1).start()
            c_wo(p).start()
            c_mb(p).start()
        for c in c_w:
            c.start()

        x_v[S // 2:S // 2 + HALO // 2, :] = jnp.zeros((HALO // 2, D), u32)
        for j in range(NCH):
            z = jnp.zeros((HALO, 128), f32)
            qbuf[j, S:S + HALO, :] = z
            kbuf[j, HALO + S:2 * HALO + S, :] = z
            vbuf[j, HALO + S:2 * HALO + S, :] = z
            k0[j, 0:HALO, :] = z
            v0[j, 0:HALO, :] = z
            wo_raw[j, 0:8, :] = jnp.zeros((8, 128), u32)
            wo_raw[j, 8 + D // 2:16 + D // 2, :] = jnp.zeros((8, 128), u32)

        c_c.wait()
        c = c_v[...].astype(f32)
        sc_v[...] = pltpu.bitcast(jnp.broadcast_to((c * jax.nn.sigmoid(c)).astype(bf16), (16, D)), u32)

        def stats(b):
            c_x0(b).wait()
            xb = _bf(x_v[b * 64:(b + 1) * 64, :])
            m = _dot(xb, jnp.ones((D, 128), bf16)) * (1.0 / D)
            acc = None
            for j in range(NCH):
                xc = xb[:, j * 128:(j + 1) * 128].astype(f32) - m
                acc = xc * xc if acc is None else acc + xc * xc
            var = jnp.sum(acc, axis=-1, keepdims=True) * (1.0 / D)
            st_m[b * 128:(b + 1) * 128, :] = m
            st_r[b * 128:(b + 1) * 128, :] = jnp.broadcast_to(lax.rsqrt(var + EPS), (128, 128))

        def exch_groups(groups):
            for g0 in range(0, len(groups), EG):
                gs = groups[g0:g0 + EG]
                XS = [[wqkv_raw[pl.ds(k * 64 + rg * 8, 8), b * D + a * 128:b * D + (a + 1) * 128] for a in range(NCH)]
                      for (k, b, rg) in gs]
                YS = _exchange8_multi(XS)
                for (k, b, rg), Y in zip(gs, YS):
                    wqkv_v[pl.ds(k * 64 + rg * 8, 8), b * D:(b + 1) * D] = jnp.concatenate(Y, axis=1)

        def exch(k, b):
            exch_groups([(k, b, rg) for rg in range(8)])

        def exch3(k):
            exch_groups([(k, b, rg) for b in range(3) for rg in range(8)])

        def modh(k):
            modc = _dot(_bf(sc_v[...]), _bf(wmA_v[k]))
            modA[k] = modc[0:8]
            sa_c = modc[0:1, 0:128]
            ca_c = modc[0:1, 128:256]
            xk = _bf(x_v[0:M0 // 2, k * 128:(k + 1) * 128]).astype(f32)
            return (((xk - st_m[...]) * st_r[...]) * (1.0 + ca_c) + sa_c).astype(bf16)

        c_wq(0).wait()
        exch(0, 0)
        stats(0)
        exch(0, 1)
        stats(1)
        exch(0, 2)
        stats(2)
        stats(3)
        c_sa(0).wait(); c_ca(0).wait()
        h = modh(0)

        for kc in range(8):
            if kc < 7:
                c_sa(kc + 1).wait(); c_ca(kc + 1).wait(); c_wq(kc + 1).wait()
            if kc == 2:
                c_xa(0).wait()

            pieces = []
            st = {}
            if kc < 7:
                k1 = kc + 1

                def p_mv():
                    modc = _dot(_bf(sc_v[...]), _bf(wmA_v[k1]))
                    modA[k1] = modc[0:8]
                    st['sa'] = modc[0:1, 0:128]
                    st['ca'] = modc[0:1, 128:256]
                    st['h'] = []

                def p_h(rb):
                    def f():
                        xk = _bf(x_v[rb * 64:(rb + 1) * 64, k1 * 128:(k1 + 1) * 128]).astype(f32)
                        hh = ((xk - st_m[rb * 128:(rb + 1) * 128, :]) * st_r[rb * 128:(rb + 1) * 128, :]) * (1.0 + st['ca']) + st['sa']
                        st['h'].append(hh.astype(bf16))
                    return f

                def p_ex(g0):
                    groups = [(k1, b, rg) for b in range(3) for rg in range(8)]
                    return lambda: exch_groups(groups[g0:g0 + EG])
                exs = [p_ex(g0) for g0 in range(0, 24, EG)]
                hs_ = [p_h(rb) for rb in range(M0 // 128)]
            else:
                exs, hs_ = [], []

            def p_ln():
                r0 = kc * (XP // 2) if kc < 2 else M0 // 2 + (kc - 2) * (XP // 2)
                pc = kc if kc < 2 else kc - 2
                xp = _bf(x_v[r0:r0 + XP // 2, :]).astype(f32)
                xhatA[pc * XP:(pc + 1) * XP, :] = _ln(xp)
            if kc < 7:
                pieces.append(p_mv)
            pieces.append(p_ln)
            a, bq = list(exs), list(hs_)
            while a or bq:
                if a:
                    pieces.append(a.pop(0))
                if bq and len(bq) >= len(a) - 1:
                    pieces.append(bq.pop(0))
            nsub = 3 * D // IL0
            slots = [[] for _ in range(nsub)]
            for i, pc_ in enumerate(pieces):
                slots[min(nsub - 2, (i * (nsub - 1)) // len(pieces))].append(pc_)
            for sd in range(nsub):
                c0 = sd * IL0
                b = c0 // D
                res = _dot(h, _bf(wqkv_v[kc * 64:(kc + 1) * 64, c0:c0 + IL0]))
                buf = (q0, k0, v0)[b]
                o = 0 if b == 0 else HALO
                for jj in range(IL0 // 128):
                    j = (c0 % D) // 128 + jj
                    if kc == 0:
                        buf[j, o:o + M0, :] = res[:, jj * 128:(jj + 1) * 128]
                    else:
                        buf[j, o:o + M0, :] += res[:, jj * 128:(jj + 1) * 128]
                for f in slots[sd]:
                    f()
            if kc < 7:
                h = jnp.concatenate(st['h'], axis=0)

        def attention(qb, kb, vb, base, off, M, mask_rows):
            row0 = base + off

            def kvds(r, w):
                return pl.ds(base + (off + HALO + r - DIL * w), RB)

            o_rows = []
            for r in range(0, M, RB):
                q = [qb[j, pl.ds(base + (off + r), RB), :] for j in range(NCH)]
                s = []
                for w in range(W):
                    acc = None
                    for j in range(NCH):
                        p = q[j] * kb[j, kvds(r, w), :]
                        acc = p if acc is None else acc + p
                    acc = _group4_sum(acc)
                    if mask_rows and r < DIL * (W - 1) and w > 0:
                        rows = row0 + r + lax.broadcasted_iota(jnp.int32, (RB, 128), 0)
                        acc = jnp.where(rows >= DIL * w, acc, -1e30)
                    s.append(acc)
                m = functools.reduce(jnp.maximum, s)
                e = [jnp.exp((sw - m) * SCALE) for sw in s]
                den = functools.reduce(lambda a, b: a + b, e)
                rinv = 1.0 / den
                oc = []
                for j in range(NCH):
                    acc = None
                    for w in range(W):
                        p = e[w] * vb[j, kvds(r, w), :]
                        acc = p if acc is None else acc + p
                    oc.append(acc * rinv)
                o_rows.append(jnp.concatenate(oc, axis=1))
            o = jnp.concatenate(o_rows, axis=0).astype(bf16)
            if isinstance(row0, int):
                o_scr[row0 // 2:(row0 + M) // 2, :] = pltpu.bitcast(o, u32)
            else:
                o_scr[pl.ds(pl.multiple_of(row0 // 2, 8), M // 2), :] = pltpu.bitcast(o, u32)

        sub = lax.broadcasted_iota(jnp.int32, (8, 128), 0)

        def abody(p, carry):
            @pl.when(p < 7)
            def _():
                c_xa(p + 1).wait()
            c_wo(p).wait()
            c_mb(p).wait()
            sa = jnp.concatenate([modA[j, 0:1, 0:128] for j in range(NCH)], axis=1)
            ca = jnp.concatenate([modA[j, 0:1, 128:256] for j in range(NCH)], axis=1)
            h = (xhatA[0:TA, :] * (1.0 + ca) + sa).astype(bf16)
            r = pl.multiple_of(M0 + p * TA, 8)
            qkv = _dot(h, _bf(wqkv_v[0:D // 2, :]))
            for j in range(NCH):
                qbuf[j, pl.ds(r, TA), :] = qkv[:, j * 128:(j + 1) * 128]
                kbuf[j, pl.ds(r + HALO, TA), :] = qkv[:, D + j * 128:D + (j + 1) * 128]
                vbuf[j, pl.ds(r + HALO, TA), :] = qkv[:, 2 * D + j * 128:2 * D + (j + 1) * 128]
            nr = pl.multiple_of(M0 // 2 + jnp.minimum(p + 1, NTA - 1) * (TA // 2), 8)
            xhatA[0:TA, :] = _ln(_bf(x_v[pl.ds(nr, TA // 2), :]).astype(f32))
            modB[p] = _dot(_bf(sc_v[...]), _bf(wmB_v[p]))[0:8]
            for tv in range(D // 2 // 8):
                j = tv >> 3
                hh = (tv >> 1) & 3
                a2 = tv & 1
                parts = []
                for al in range(4):
                    a = a2 * 4 + al
                    src = a * 64 + hh * 16 + j * 2
                    st = src - 2 * al + 8
                    parts.append(wo_raw[p, st:st + 8, :])
                v = jnp.where(sub < 2, parts[0], parts[1])
                v2 = jnp.where(sub < 6, parts[2], parts[3])
                wo_v[p, 8 * tv:8 * tv + 8, :] = jnp.where(sub < 4, v, v2)
            attention(q0, k0, v0, pl.multiple_of(p * AR, 16), 0, AR, True)
            cr = pl.multiple_of(CP0 + p * CPR, 8)
            for j in range(NCH):
                qbuf[j, pl.ds(cr, CPR), :] = q0[j, pl.ds(cr, CPR), :]
                kbuf[j, pl.ds(cr + HALO, CPR), :] = k0[j, pl.ds(cr + HALO, CPR), :]
                vbuf[j, pl.ds(cr + HALO, CPR), :] = v0[j, pl.ds(cr + HALO, CPR), :]
            return carry
        lax.fori_loop(0, NTA, abody, 0)

        for c in c_w:
            c.wait()

        def rows_u32(ref, row0, M):
            if isinstance(row0, int):
                return _bf(ref[row0 // 2:(row0 + M) // 2, :])
            return _bf(ref[pl.ds(pl.multiple_of(row0 // 2, 8), M // 2), :])

        def wo_dot(row0, M):
            o = rows_u32(o_scr, row0, M)
            return jnp.concatenate([_dot(o, _bf(wo_v[n])) for n in range(NCH)], axis=1)

        def row(k):
            return jnp.concatenate([modB[2 * (k - 2), 0:1, :], modB[2 * (k - 2) + 1, 0:1, :]], axis=1)

        def ln23(row0, M, A):
            ga = row(2); sb = row(3); cb = row(4)
            x = rows_u32(x_v, row0, M).astype(f32)
            xm = x + ga * A
            hB = _ln(xm) * (1.0 + cb) + sb
            n3 = _ln(hB).astype(bf16)
            return xm, hB, n3

        shifts = [-1, -1, 1, 1, -2, -2, 2, 2]

        def g_val():
            return jnp.concatenate(
                [h1buf[j, HALO + shifts[j]:HALO + shifts[j] + T, :] for j in range(NCH)], axis=1).astype(bf16)

        def out_copy(tile, slot):
            r0 = pl.multiple_of(tile * (T // 2), 8)
            return pltpu.make_async_copy(obuf.at[slot], o_hbm.bitcast(u32).at[pl.ds(r0, T // 2)], osems.at[slot])

        def ln4(hs):
            gb = row(5)
            x1 = hb[0:T, :] + hs
            base = xmid[0:T, :] + gb * x1
            n4 = _ln(x1).astype(bf16)
            return base, n4

        for j in range(NCH):
            h1buf[j, 0:HALO, :] = jnp.zeros((HALO, 128), f32)
        if NTA * AR < 2 * T + HALO:
            attention(qbuf, kbuf, vbuf, 0, NTA * AR, 2 * T + HALO - NTA * AR, False)
        h0 = (T + HALO) // 2 // 16 * 16 + (16 if T == 128 else 0)
        halves = [(0, h0), (h0, T + HALO - h0)]
        As = [wo_dot(r0, m) for r0, m in halves]
        for (r0, m), A in zip(halves, As):
            xm, hB, n3 = ln23(r0, m, A)
            h1 = _gelu(_dot(n3, _bf(w1_v[...])))
            xmid[r0:r0 + m, :] = xm
            hb[r0:r0 + m, :] = hB
            for j in range(NCH):
                h1buf[j, HALO + r0:HALO + r0 + m, :] = h1[:, j * 128:(j + 1) * 128]

        def bbody(i, carry):
            slot = (i - 1) % 2
            row0 = pl.multiple_of(i * T + HALO, 16)

            @pl.when(i >= 3)
            def _():
                out_copy(i - 3, slot).wait()

            hs = _dot(g_val(), _bf(w2_v[...]))
            A = wo_dot(row0, T)
            base, n4 = ln4(hs)
            u = _gelu(_dot(n4, _bf(w3_v[...]))).astype(bf16)
            xm, hB, n3 = ln23(row0, T, A)
            h1 = _gelu(_dot(n3, _bf(w1_v[...])))
            xmid[0:HALO, :] = xmid[T:T + HALO, :]
            hb[0:HALO, :] = hb[T:T + HALO, :]
            for j in range(NCH):
                h1buf[j, 0:2 * HALO, :] = h1buf[j, T:T + 2 * HALO, :]
            xmid[HALO:HALO + T, :] = xm
            hb[HALO:HALO + T, :] = hB
            notlast = i < NT - 1
            for j in range(NCH):
                h1j = h1[:, j * 128:(j + 1) * 128]
                h1buf[j, 2 * HALO:HALO + T, :] = h1j[0:T - HALO]
                h1buf[j, HALO + T:2 * HALO + T, :] = jnp.where(notlast, h1j[T - HALO:T], 0.0)
            attention(qbuf, kbuf, vbuf, pl.multiple_of(jnp.minimum(i + 1, NT - 1) * T, T), HALO, T, False)
            h2 = _dot(u, _bf(w4_v[...]))
            obuf[slot] = pltpu.bitcast((base + row(5) * h2).astype(bf16), u32)
            out_copy(i - 1, slot).start()
            return carry
        lax.fori_loop(1, NT, bbody, 0)

        slot = (NT - 1) % 2
        out_copy(NT - 3, slot).wait()
        hs = _dot(g_val(), _bf(w2_v[...]))
        base, n4 = ln4(hs)
        u = _gelu(_dot(n4, _bf(w3_v[...]))).astype(bf16)
        h2 = _dot(u, _bf(w4_v[...]))
        obuf[slot] = pltpu.bitcast((base + row(5) * h2).astype(bf16), u32)
        out_copy(NT - 1, slot).start()
        out_copy(NT - 2, 1 - slot).wait()
        out_copy(NT - 1, slot).wait()

    @jax.jit
    def fn(A_x, A_wqkv, A_wo, B_x, B_w1, B_w2, B_w3, B_w4, c, w_mod):
        x = A_x.reshape(S, D)
        any_spec = pl.BlockSpec(memory_space=pl.ANY)
        out = pl.pallas_call(
            kernel,
            in_specs=[any_spec] * 9,
            out_specs=any_spec,
            out_shape=jax.ShapeDtypeStruct((S, D), bf16),
            scratch_shapes=[
                pltpu.VMEM((S // 2 + HALO // 2, D), u32),
                pltpu.VMEM((D // 2, 3 * D), u32),
                pltpu.VMEM((D // 2, 3 * D), u32),
                pltpu.VMEM((NCH, D // 2 + 16, 128), u32),
                pltpu.VMEM((NCH, D // 2, 128), u32),
                pltpu.VMEM((D // 2, D), u32),
                pltpu.VMEM((D // 2, D), u32),
                pltpu.VMEM((D // 2, F), u32),
                pltpu.VMEM((F // 2, D), u32),
                pltpu.VMEM((1, D), bf16),
                pltpu.VMEM((8, D), u32),
                pltpu.VMEM((8, D // 2, 256), u32),
                pltpu.VMEM((8, D // 2, 512), u32),
                pltpu.VMEM((8, 8, 256), f32),
                pltpu.VMEM((8, 8, 512), f32),
                pltpu.VMEM((M0, 128), f32),
                pltpu.VMEM((M0, 128), f32),
                pltpu.VMEM((TA, D), f32),
                pltpu.VMEM((NCH, M0, 128), f32),
                pltpu.VMEM((NCH, M0 + HALO, 128), f32),
                pltpu.VMEM((NCH, M0 + HALO, 128), f32),
                pltpu.VMEM((NCH, S + HALO, 128), f32),
                pltpu.VMEM((NCH, S + 2 * HALO, 128), f32),
                pltpu.VMEM((NCH, S + 2 * HALO, 128), f32),
                pltpu.VMEM((T + HALO, D), f32),
                pltpu.VMEM((T + HALO, D), f32),
                pltpu.VMEM((NCH, T + 2 * HALO, 128), f32),
                pltpu.VMEM((2, T // 2, D), u32),
                pltpu.VMEM((S // 2 + HALO // 2, D), u32),
                pltpu.SemaphoreType.DMA((57,)),
                pltpu.SemaphoreType.DMA((2,)),
            ],
            compiler_params=pltpu.CompilerParams(vmem_limit_bytes=120 * 1024 * 1024),
        )(x, A_wqkv, A_wo, B_w1, B_w2, B_w3, B_w4, c, w_mod)
        return out.reshape(1, S, D)
    return fn


_fn = make()


def pallas_adaLN_cond__sliding_local_dilated__mixer_s_mlp__prompt_kernel(A_x, A_wqkv, A_wo, B_x, B_w1, B_w2, B_w3, B_w4, c, w_mod):
    return _fn(A_x, A_wqkv, A_wo, B_x, B_w1, B_w2, B_w3, B_w4, c, w_mod)
```

```python
import functools
import jax
import jax.numpy as jnp
from jax import lax
import jax.experimental.pallas as pl
import jax.experimental.pallas.tpu as pltpu

S, D, F = 2048, 1024, 3584
H, DH, W, DIL = 32, 32, 8, 2
NCH = D // 128
EPS = 1e-5
SCALE = DH ** -0.5
f32, bf16, u32 = jnp.float32, jnp.bfloat16, jnp.uint32
HALO = 16


def _ln(x):
    m = jnp.mean(x, axis=-1, keepdims=True)
    xc = x - m
    v = jnp.mean(xc * xc, axis=-1, keepdims=True)
    return xc * lax.rsqrt(v + EPS)


def _gelu(x):
    c0 = 0.7978845608028654
    c1 = c0 * 0.044715
    t = jnp.tanh(x * (c0 + c1 * (x * x)))
    hx = 0.5 * x
    return hx + hx * t


def _dot(a, b):
    return jnp.dot(a, b, preferred_element_type=f32)


def _bf(w):
    return pltpu.bitcast(w, bf16)


def _lane_xor(x, s):
    lane = lax.broadcasted_iota(jnp.int32, x.shape, 1)
    return jnp.take_along_axis(x, lane ^ s, axis=1)


def _exchange8_multi(XS):
    XS = [list(X) for X in XS]
    lane = lax.broadcasted_iota(jnp.int32, XS[0][0].shape, 1)
    for t in range(3):
        s = 1 << (t + 2)
        m = (lane & s) != 0
        for X in XS:
            for p in range(8):
                if p & (1 << t):
                    continue
                p2 = p | (1 << t)
                tmp = _lane_xor(jnp.where(m, X[p], X[p2]), s)
                X[p], X[p2] = jnp.where(m, tmp, X[p]), jnp.where(m, X[p2], tmp)
    return XS


def _group4_sum(acc):
    lane = lax.broadcasted_iota(jnp.int32, acc.shape, 1)
    acc = acc + jnp.where((lane & 1) != 0, pltpu.roll(acc, 1, 1), pltpu.roll(acc, 127, 1))
    acc = acc + jnp.where((lane & 2) != 0, pltpu.roll(acc, 2, 1), pltpu.roll(acc, 126, 1))
    return acc


def make(T=128, M0=512, TA=192, RB=8, AR=48, CP0=256, EG=4, IL0=512, only='', upto=9,
         rel4=(-1, -1, -1, 0, 1, 2, 3, 4), rel23=(8, 9, 10, 11, 12, 13, 14, 15)):
    NT = S // T
    NTA = (S - M0) // TA
    assert NTA == 8 and NTA * TA + M0 == S
    XP = 32
    NXP = TA // XP
    CPR = (M0 - CP0) // NTA
    S_C, S_X0, S_SA, S_CA, S_WQ, S_XA, S_WO, S_MB, S_W = 0, 1, 5, 13, 21, 29, 37, 45, 53

    def kernel(x_hbm, wqkv_hbm, wo_hbm, w1_hbm, w2_hbm, w3_hbm, w4_hbm, c_hbm, wmod_hbm,
               o_hbm,
               x_v, wqkv_raw, wqkv_v, wo_raw, wo_v, w1_v, w2_v, w3_v, w4_v, c_v, sc_v, wmA_v, wmB_v,
               modA, modB, st_m, st_r, xhatA, q0, k0, v0, qbuf, kbuf, vbuf, xmid, hb, h1buf, obuf, o_scr, hsbuf,
               sems, osems):
        def cp(src, dst, k):
            return pltpu.make_async_copy(src, dst, sems.at[k])

        xu = x_hbm.bitcast(u32)
        wqkvu = wqkv_hbm.bitcast(u32)
        wou = wo_hbm.bitcast(u32)
        wmodu = wmod_hbm.bitcast(u32)

        def lane_ds(k, n):
            if isinstance(k, int):
                return pl.ds(k * n, n)
            return pl.ds(pl.multiple_of(k * n, 128), n)

        def row_ds(base, k, n):
            if isinstance(k, int):
                return pl.ds(base + k * n, n)
            return pl.ds(pl.multiple_of(base + k * n, 8), n)

        c_c = cp(c_hbm, c_v, S_C)

        def c_x0(b):
            return cp(xu.at[row_ds(0, b, 64)], x_v.at[row_ds(0, b, 64)], S_X0 + b)

        def c_sa(k):
            return cp(wmodu.at[:, lane_ds(k, 128)], wmA_v.at[k, :, 0:128], S_SA + k)

        def c_ca(k):
            if isinstance(k, int):
                src = wmodu.at[:, pl.ds(D + k * 128, 128)]
            else:
                src = wmodu.at[:, pl.ds(pl.multiple_of(D + k * 128, 128), 128)]
            return cp(src, wmA_v.at[k, :, 128:256], S_CA + k)

        def c_wq(k):
            return cp(wqkvu.at[row_ds(0, k, 64)], wqkv_raw.at[row_ds(0, k, 64)], S_WQ + k)

        def c_xa(p):
            return cp(xu.at[row_ds(M0 // 2, p, TA // 2)], x_v.at[row_ds(M0 // 2, p, TA // 2)], S_XA + p)

        def c_wo(p):
            return cp(wou.at[:, lane_ds(p, 128)], wo_raw.at[p, 8:8 + D // 2], S_WO + p)

        def c_mb(p):
            if isinstance(p, int):
                src = wmodu.at[:, pl.ds(2 * D + p * 512, 512)]
            else:
                src = wmodu.at[:, pl.ds(pl.multiple_of(2 * D + p * 512, 128), 512)]
            return cp(src, wmB_v.at[p], S_MB + p)

        c_w = [cp(w1_hbm.bitcast(u32), w1_v, S_W), cp(w2_hbm.bitcast(u32), w2_v, S_W + 1),
               cp(w3_hbm.bitcast(u32), w3_v, S_W + 2), cp(w4_hbm.bitcast(u32), w4_v, S_W + 3)]

        if only == '':
            c_c.start()
            c_wq(0).start()
            for b in range(4):
                c_x0(b).start()
            for k in range(8):
                c_sa(k).start()
                c_ca(k).start()
                if k > 0:
                    c_wq(k).start()
                if k == 2:
                    c_xa(0).start()
            for p in range(8):
                if upto < 2:
                    break
                if p < 7:
                    c_xa(p + 1).start()
                c_wo(p).start()
                c_mb(p).start()
            for c in c_w:
                if upto >= 3:
                    c.start()

        x_v[S // 2:S // 2 + HALO // 2, :] = jnp.zeros((HALO // 2, D), u32)
        for j in range(NCH):
            z = jnp.zeros((HALO, 128), f32)
            qbuf[j, S:S + HALO, :] = z
            kbuf[j, HALO + S:2 * HALO + S, :] = z
            vbuf[j, HALO + S:2 * HALO + S, :] = z
            k0[j, 0:HALO, :] = z
            v0[j, 0:HALO, :] = z
            wo_raw[j, 0:8, :] = jnp.zeros((8, 128), u32)
            wo_raw[j, 8 + D // 2:16 + D // 2, :] = jnp.zeros((8, 128), u32)

        def phase0():
            c_c.wait()
            c = c_v[...].astype(f32)
            sc_v[...] = pltpu.bitcast(jnp.broadcast_to((c * jax.nn.sigmoid(c)).astype(bf16), (16, D)), u32)

            def stats(b):
                c_x0(b).wait()
                xb = _bf(x_v[b * 64:(b + 1) * 64, :])
                m = _dot(xb, jnp.ones((D, 128), bf16)) * (1.0 / D)
                acc = None
                for j in range(NCH):
                    xc = xb[:, j * 128:(j + 1) * 128].astype(f32) - m
                    acc = xc * xc if acc is None else acc + xc * xc
                var = jnp.sum(acc, axis=-1, keepdims=True) * (1.0 / D)
                st_m[b * 128:(b + 1) * 128, :] = m
                st_r[b * 128:(b + 1) * 128, :] = jnp.broadcast_to(lax.rsqrt(var + EPS), (128, 128))

            def exch_groups(groups):
                for g0 in range(0, len(groups), EG):
                    gs = groups[g0:g0 + EG]
                    XS = [[wqkv_raw[pl.ds(k * 64 + rg * 8, 8), b * D + a * 128:b * D + (a + 1) * 128] for a in range(NCH)]
                          for (k, b, rg) in gs]
                    YS = _exchange8_multi(XS)
                    for (k, b, rg), Y in zip(gs, YS):
                        wqkv_v[pl.ds(k * 64 + rg * 8, 8), b * D:(b + 1) * D] = jnp.concatenate(Y, axis=1)

            def exch(k, b):
                exch_groups([(k, b, rg) for rg in range(8)])

            def exch3(k):
                exch_groups([(k, b, rg) for b in range(3) for rg in range(8)])

            def modh(k):
                modc = _dot(_bf(sc_v[...]), _bf(wmA_v[k]))
                modA[k] = modc[0:8]
                sa_c = modc[0:1, 0:128]
                ca_c = modc[0:1, 128:256]
                xk = _bf(x_v[0:M0 // 2, k * 128:(k + 1) * 128]).astype(f32)
                return (((xk - st_m[...]) * st_r[...]) * (1.0 + ca_c) + sa_c).astype(bf16)

            c_wq(0).wait()
            exch(0, 0)
            stats(0)
            exch(0, 1)
            stats(1)
            exch(0, 2)
            stats(2)
            stats(3)
            c_sa(0).wait(); c_ca(0).wait()
            h = modh(0)

            for kc in range(8):
                if kc < 7:
                    c_sa(kc + 1).wait(); c_ca(kc + 1).wait(); c_wq(kc + 1).wait()
                if kc == 2:
                    c_xa(0).wait()

                pieces = []
                st = {}
                if kc < 7:
                    k1 = kc + 1

                    def p_mv():
                        modc = _dot(_bf(sc_v[...]), _bf(wmA_v[k1]))
                        modA[k1] = modc[0:8]
                        st['sa'] = modc[0:1, 0:128]
                        st['ca'] = modc[0:1, 128:256]
                        st['h'] = []

                    def p_h(rb):
                        def f():
                            xk = _bf(x_v[rb * 64:(rb + 1) * 64, k1 * 128:(k1 + 1) * 128]).astype(f32)
                            hh = ((xk - st_m[rb * 128:(rb + 1) * 128, :]) * st_r[rb * 128:(rb + 1) * 128, :]) * (1.0 + st['ca']) + st['sa']
                            st['h'].append(hh.astype(bf16))
                        return f

                    def p_ex(g0):
                        groups = [(k1, b, rg) for b in range(3) for rg in range(8)]
                        return lambda: exch_groups(groups[g0:g0 + EG])
                    exs = [p_ex(g0) for g0 in range(0, 24, EG)]
                    hs_ = [p_h(rb) for rb in range(M0 // 128)]
                else:
                    exs, hs_ = [], []

                def p_ln():
                    r0 = kc * (XP // 2) if kc < 2 else M0 // 2 + (kc - 2) * (XP // 2)
                    pc = kc if kc < 2 else kc - 2
                    xp = _bf(x_v[r0:r0 + XP // 2, :]).astype(f32)
                    xhatA[pc * XP:(pc + 1) * XP, :] = _ln(xp)
                if kc < 7:
                    pieces.append(p_mv)
                pieces.append(p_ln)
                a, bq = list(exs), list(hs_)
                while a or bq:
                    if a:
                        pieces.append(a.pop(0))
                    if bq and len(bq) >= len(a) - 1:
                        pieces.append(bq.pop(0))
                nsub = 3 * D // IL0
                slots = [[] for _ in range(nsub)]
                for i, pc_ in enumerate(pieces):
                    slots[min(nsub - 2, (i * (nsub - 1)) // len(pieces))].append(pc_)
                for sd in range(nsub):
                    c0 = sd * IL0
                    b = c0 // D
                    res = _dot(h, _bf(wqkv_v[kc * 64:(kc + 1) * 64, c0:c0 + IL0]))
                    buf = (q0, k0, v0)[b]
                    o = 0 if b == 0 else HALO
                    for jj in range(IL0 // 128):
                        j = (c0 % D) // 128 + jj
                        if kc == 0:
                            buf[j, o:o + M0, :] = res[:, jj * 128:(jj + 1) * 128]
                        else:
                            buf[j, o:o + M0, :] += res[:, jj * 128:(jj + 1) * 128]
                    for f in slots[sd]:
                        f()
                if kc < 7:
                    h = jnp.concatenate(st['h'], axis=0)

        if only == '' and upto >= 1:
            phase0()
        if upto == 0:
            c_c.wait(); c_wq(0).wait()
            for b in range(4):
                c_x0(b).wait()
            for k in range(8):
                c_sa(k).wait(); c_ca(k).wait()
                if k > 0:
                    c_wq(k).wait()
            c_xa(0).wait()

        def attention(qb, kb, vb, base, off, M, mask_rows, baseh=None):
            row0 = base + off

            def kvds(r, w):
                return pl.ds(base + (off + HALO + r - DIL * w), RB)

            o_rows = []
            for r in range(0, M, RB):
                q = [qb[j, pl.ds(base + (off + r), RB), :] for j in range(NCH)]
                s = []
                for w in range(W):
                    acc = None
                    for j in range(NCH):
                        p = q[j] * kb[j, kvds(r, w), :]
                        acc = p if acc is None else acc + p
                    acc = _group4_sum(acc)
                    if mask_rows and r < DIL * (W - 1) and w > 0:
                        rows = row0 + r + lax.broadcasted_iota(jnp.int32, (RB, 128), 0)
                        acc = jnp.where(rows >= DIL * w, acc, -1e30)
                    s.append(acc)
                m = functools.reduce(jnp.maximum, s)
                e = [jnp.exp((sw - m) * SCALE) for sw in s]
                den = functools.reduce(lambda a, b: a + b, e)
                rinv = 1.0 / den
                oc = []
                for j in range(NCH):
                    acc = None
                    for w in range(W):
                        p = e[w] * vb[j, kvds(r, w), :]
                        acc = p if acc is None else acc + p
                    oc.append(acc * rinv)
                o_rows.append(jnp.concatenate(oc, axis=1))
            o = jnp.concatenate(o_rows, axis=0).astype(bf16)
            if isinstance(row0, int):
                o_scr[row0 // 2:(row0 + M) // 2, :] = pltpu.bitcast(o, u32)
            elif baseh is not None:
                o_scr[pl.ds(baseh + off // 2, M // 2), :] = pltpu.bitcast(o, u32)
            else:
                o_scr[pl.ds(pl.multiple_of(row0 // 2, 8), M // 2), :] = pltpu.bitcast(o, u32)

        sub = lax.broadcasted_iota(jnp.int32, (8, 128), 0)

        def abody(p, carry):
            @pl.when(p < 7)
            def _():
                c_xa(p + 1).wait()
            c_wo(p).wait()
            c_mb(p).wait()
            sa = jnp.concatenate([modA[j, 0:1, 0:128] for j in range(NCH)], axis=1)
            ca = jnp.concatenate([modA[j, 0:1, 128:256] for j in range(NCH)], axis=1)
            h = (xhatA[0:TA, :] * (1.0 + ca) + sa).astype(bf16)
            r = pl.multiple_of(M0 + p * TA, 8)
            qkv = _dot(h, _bf(wqkv_v[0:D // 2, :]))
            for j in range(NCH):
                qbuf[j, pl.ds(r, TA), :] = qkv[:, j * 128:(j + 1) * 128]
                kbuf[j, pl.ds(r + HALO, TA), :] = qkv[:, D + j * 128:D + (j + 1) * 128]
                vbuf[j, pl.ds(r + HALO, TA), :] = qkv[:, 2 * D + j * 128:2 * D + (j + 1) * 128]
            nr = pl.multiple_of(M0 // 2 + jnp.minimum(p + 1, NTA - 1) * (TA // 2), 8)
            xhatA[0:TA, :] = _ln(_bf(x_v[pl.ds(nr, TA // 2), :]).astype(f32))
            modB[p] = _dot(_bf(sc_v[...]), _bf(wmB_v[p]))[0:8]
            for tv in range(D // 2 // 8):
                j = tv >> 3
                hh = (tv >> 1) & 3
                a2 = tv & 1
                parts = []
                for al in range(4):
                    a = a2 * 4 + al
                    src = a * 64 + hh * 16 + j * 2
                    st = src - 2 * al + 8
                    parts.append(wo_raw[p, st:st + 8, :])
                v = jnp.where(sub < 2, parts[0], parts[1])
                v2 = jnp.where(sub < 6, parts[2], parts[3])
                wo_v[p, 8 * tv:8 * tv + 8, :] = jnp.where(sub < 4, v, v2)
            attention(q0, k0, v0, pl.multiple_of(p * AR, 16), 0, AR, True, pl.multiple_of(p * (AR // 2), 8))
            cr = pl.multiple_of(CP0 + p * CPR, 8)
            for j in range(NCH):
                qbuf[j, pl.ds(cr, CPR), :] = q0[j, pl.ds(cr, CPR), :]
                kbuf[j, pl.ds(cr + HALO, CPR), :] = k0[j, pl.ds(cr + HALO, CPR), :]
                vbuf[j, pl.ds(cr + HALO, CPR), :] = v0[j, pl.ds(cr + HALO, CPR), :]
            return carry
        if only in ('', 'A') and upto >= 2:
            lax.fori_loop(0, NTA, abody, 0)

        if only == '' and upto >= 3:
            for c in c_w:
                c.wait()

        def rows_u32(ref, row0, M):
            if isinstance(row0, int):
                return _bf(ref[row0 // 2:(row0 + M) // 2, :])
            if isinstance(row0, tuple):
                return _bf(ref[pl.ds(row0[0] + row0[1] // 2, M // 2), :])
            return _bf(ref[pl.ds(pl.multiple_of(row0 // 2, 8), M // 2), :])

        def wo_dot(row0, M):
            o = rows_u32(o_scr, row0, M)
            return jnp.concatenate([_dot(o, _bf(wo_v[n])) for n in range(NCH)], axis=1)

        def row(k):
            return jnp.concatenate([modB[2 * (k - 2), 0:1, :], modB[2 * (k - 2) + 1, 0:1, :]], axis=1)

        def ln23(row0, M, A):
            ga = row(2); sb = row(3); cb = row(4)
            x = rows_u32(x_v, row0, M).astype(f32)
            xm = x + ga * A
            hB = _ln(xm) * (1.0 + cb) + sb
            n3 = _ln(hB).astype(bf16)
            return xm, hB, n3

        shifts = [-1, -1, 1, 1, -2, -2, 2, 2]

        def g_val():
            return jnp.concatenate(
                [h1buf[j, HALO + shifts[j]:HALO + shifts[j] + T, :] for j in range(NCH)], axis=1).astype(bf16)

        def out_copy(tile, slot):
            r0 = pl.multiple_of(tile * (T // 2), 8)
            return pltpu.make_async_copy(obuf.at[slot], o_hbm.bitcast(u32).at[pl.ds(r0, T // 2)], osems.at[slot])

        def ln4(hs):
            gb = row(5)
            x1 = hb[0:T, :] + hs
            base = xmid[0:T, :] + gb * x1
            n4 = _ln(x1).astype(bf16)
            return base, n4

        def bfirst():
            for j in range(NCH):
                h1buf[j, 0:HALO, :] = jnp.zeros((HALO, 128), f32)
            if NTA * AR < 2 * T + HALO:
                attention(q0, k0, v0, 0, NTA * AR, 2 * T + HALO - NTA * AR, False)
            h0 = (T + HALO) // 2 // 16 * 16 + (16 if T == 128 else 0)
            halves = [(0, h0), (h0, T + HALO - h0)]
            As = [wo_dot(r0, m) for r0, m in halves]
            for (r0, m), A in zip(halves, As):
                xm, hB, n3 = ln23(r0, m, A)
                h1 = _gelu(_dot(n3, _bf(w1_v[...])))
                xmid[r0:r0 + m, :] = xm
                hb[r0:r0 + m, :] = hB
                for j in range(NCH):
                    h1buf[j, HALO + r0:HALO + r0 + m, :] = h1[:, j * 128:(j + 1) * 128]

            hsbuf[0:T, :] = _dot(g_val(), _bf(w2_v[...]))

        if only in ('', 'BF') and upto >= 3:
            bfirst()

        def carries(xm, hB, h1, notlast):
            xmid[0:HALO, :] = xmid[T:T + HALO, :]
            hb[0:HALO, :] = hb[T:T + HALO, :]
            for j in range(NCH):
                h1buf[j, 0:2 * HALO, :] = h1buf[j, T:T + 2 * HALO, :]
            xmid[HALO:HALO + T, :] = xm
            hb[HALO:HALO + T, :] = hB
            for j in range(NCH):
                h1j = h1[:, j * 128:(j + 1) * 128]
                h1buf[j, 2 * HALO:HALO + T, :] = h1j[0:T - HALO]
                h1buf[j, HALO + T:2 * HALO + T, :] = jnp.where(notlast, h1j[T - HALO:T], 0.0)

        RP = 16

        def bbody(i, carry):
            slot = (i - 1) % 2

            @pl.when(i >= 3)
            def _():
                out_copy(i - 3, slot).wait()

            row0h = pl.multiple_of(i * (T // 2), T // 2)
            nxt = jnp.minimum(i + 1, NT - 1)
            abase = pl.multiple_of(nxt * T, T)
            abaseh = pl.multiple_of(nxt * (T // 2), T // 2)
            z1 = pl.multiple_of((i >> 8) * 8, 8)
            z2 = pl.multiple_of((i >> 9) * 8, 8)
            ga = row(2); sb = row(3); cb = row(4); gb = row(5)
            bases, n4p, xms, hBs, n3p, As = [], [], [], [], [], []

            def p4(r):
                r0 = r * RP
                x1 = hb[r0:r0 + RP, :] + hsbuf[pl.ds(z2 + r0, RP), :]
                bases.append(xmid[r0:r0 + RP, :] + gb * x1)
                n4p.append(_ln(x1).astype(bf16))

            def p23(r, A):
                r0 = r * RP
                x = rows_u32(x_v, (row0h, HALO + r0), RP).astype(f32)
                xm = x + ga * A[r0:r0 + RP]
                hB = _ln(xm) * (1.0 + cb) + sb
                xms.append(xm); hBs.append(hB)
                n3p.append(_ln(hB).astype(bf16))

            for r in range(T // RP):
                if rel4[r] < 0:
                    p4(r)
            o = rows_u32(o_scr, (row0h, HALO), T)
            for n in range(NCH):
                An = _dot(o, _bf(wo_v[n]))
                As.append(An)
                r4 = [r for r in range(T // RP) if rel4[r] == n]
                if r4:
                    hsbuf[pl.ds(z1 + T, 8), 0:128] = An[0:8, 0:128]
                for r in r4:
                    p4(r)
            A = jnp.concatenate(As, axis=1)
            base = jnp.concatenate(bases, axis=0)
            n4 = jnp.concatenate(n4p, axis=0)
            U = _dot(n4, _bf(w3_v[...]))
            u = _gelu(U).astype(bf16)
            for c in range(F // 128):
                r23 = [r for r in range(T // RP) if rel23[r] == NCH + c]
                if r23:
                    x_v[pl.ds(z1 + S // 2 + HALO // 2, 8), 0:128] = pltpu.bitcast(U[0:8, c * 128:(c + 1) * 128], u32)
                for r in r23:
                    p23(r, A)
            assert len(n3p) == T // RP and len(n4p) == T // RP
            xm = jnp.concatenate(xms, axis=0)
            hB = jnp.concatenate(hBs, axis=0)
            n3 = jnp.concatenate(n3p, axis=0)
            h1 = _gelu(_dot(n3, _bf(w1_v[...])))
            carries(xm, hB, h1, i < NT - 1)
            attention(qbuf, kbuf, vbuf, abase, HALO, T, False, abaseh)
            h2 = _dot(u, _bf(w4_v[...]))
            obuf[slot] = pltpu.bitcast((base + gb * h2).astype(bf16), u32)
            hsbuf[0:T, :] = _dot(g_val(), _bf(w2_v[...]))
            out_copy(i - 1, slot).start()
            return carry

        if only in ('', 'B') and upto >= 4:
            lax.fori_loop(1, NT, bbody, 0)
        if only == 'B' or upto == 4:
            out_copy(NT - 3, (NT - 1) % 2).wait()
            out_copy(NT - 2, NT % 2).wait()

        def blast():
            slot = (NT - 1) % 2
            out_copy(NT - 3, slot).wait()
            base, n4 = ln4(hsbuf[0:T, :])
            u = _gelu(_dot(n4, _bf(w3_v[...]))).astype(bf16)
            h2 = _dot(u, _bf(w4_v[...]))
            obuf[slot] = pltpu.bitcast((base + row(5) * h2).astype(bf16), u32)
            out_copy(NT - 1, slot).start()
            out_copy(NT - 2, 1 - slot).wait()
            out_copy(NT - 1, slot).wait()

        if only in ('', 'BL') and upto >= 5:
            blast()

    @jax.jit
    def fn(A_x, A_wqkv, A_wo, B_x, B_w1, B_w2, B_w3, B_w4, c, w_mod):
        x = A_x.reshape(S, D)
        any_spec = pl.BlockSpec(memory_space=pl.ANY)
        out = pl.pallas_call(
            kernel,
            in_specs=[any_spec] * 9,
            out_specs=any_spec,
            out_shape=jax.ShapeDtypeStruct((S, D), bf16),
            scratch_shapes=[
                pltpu.VMEM((S // 2 + HALO // 2 + 8, D), u32),
                pltpu.VMEM((D // 2, 3 * D), u32),
                pltpu.VMEM((D // 2, 3 * D), u32),
                pltpu.VMEM((NCH, D // 2 + 16, 128), u32),
                pltpu.VMEM((NCH, D // 2, 128), u32),
                pltpu.VMEM((D // 2, D), u32),
                pltpu.VMEM((D // 2, D), u32),
                pltpu.VMEM((D // 2, F), u32),
                pltpu.VMEM((F // 2, D), u32),
                pltpu.VMEM((1, D), bf16),
                pltpu.VMEM((8, D), u32),
                pltpu.VMEM((8, D // 2, 256), u32),
                pltpu.VMEM((8, D // 2, 512), u32),
                pltpu.VMEM((8, 8, 256), f32),
                pltpu.VMEM((8, 8, 512), f32),
                pltpu.VMEM((M0, 128), f32),
                pltpu.VMEM((M0, 128), f32),
                pltpu.VMEM((TA, D), f32),
                pltpu.VMEM((NCH, M0, 128), f32),
                pltpu.VMEM((NCH, M0 + HALO, 128), f32),
                pltpu.VMEM((NCH, M0 + HALO, 128), f32),
                pltpu.VMEM((NCH, S + HALO, 128), f32),
                pltpu.VMEM((NCH, S + 2 * HALO, 128), f32),
                pltpu.VMEM((NCH, S + 2 * HALO, 128), f32),
                pltpu.VMEM((T + HALO, D), f32),
                pltpu.VMEM((T + HALO, D), f32),
                pltpu.VMEM((NCH, T + 2 * HALO, 128), f32),
                pltpu.VMEM((2, T // 2, D), u32),
                pltpu.VMEM((S // 2 + HALO // 2, D), u32),
                pltpu.VMEM((T + 8, D), f32),
                pltpu.SemaphoreType.DMA((57,)),
                pltpu.SemaphoreType.DMA((2,)),
            ],
            compiler_params=pltpu.CompilerParams(vmem_limit_bytes=120 * 1024 * 1024),
        )(x, A_wqkv, A_wo, B_w1, B_w2, B_w3, B_w4, c, w_mod)
        return out.reshape(1, S, D)
    return fn


_fn = make()


def pallas_adaLN_cond__sliding_local_dilated__mixer_s_mlp__prompt_kernel(A_x, A_wqkv, A_wo, B_x, B_w1, B_w2, B_w3, B_w4, c, w_mod):
    return _fn(A_x, A_wqkv, A_wo, B_x, B_w1, B_w2, B_w3, B_w4, c, w_mod)
```

```python
import functools
import jax
import jax.numpy as jnp
from jax import lax
import jax.experimental.pallas as pl
import jax.experimental.pallas.tpu as pltpu

S, D, F = 2048, 1024, 3584
H, DH, W, DIL = 32, 32, 8, 2
NCH = D // 128
EPS = 1e-5
SCALE = DH ** -0.5
f32, bf16, u32 = jnp.float32, jnp.bfloat16, jnp.uint32
HALO = 16


def _ln(x):
    m = jnp.mean(x, axis=-1, keepdims=True)
    xc = x - m
    v = jnp.mean(xc * xc, axis=-1, keepdims=True)
    return xc * lax.rsqrt(v + EPS)


def _gelu(x):
    c0 = 0.7978845608028654
    c1 = c0 * 0.044715
    t = jnp.tanh(x * (c0 + c1 * (x * x)))
    hx = 0.5 * x
    return hx + hx * t


def _dot(a, b):
    return jnp.dot(a, b, preferred_element_type=f32)


def _bf(w):
    return pltpu.bitcast(w, bf16)


def _lane_xor(x, s):
    lane = lax.broadcasted_iota(jnp.int32, x.shape, 1)
    return jnp.take_along_axis(x, lane ^ s, axis=1)


def _exchange8_multi(XS):
    XS = [list(X) for X in XS]
    lane = lax.broadcasted_iota(jnp.int32, XS[0][0].shape, 1)
    for t in range(3):
        s = 1 << (t + 2)
        m = (lane & s) != 0
        for X in XS:
            for p in range(8):
                if p & (1 << t):
                    continue
                p2 = p | (1 << t)
                tmp = _lane_xor(jnp.where(m, X[p], X[p2]), s)
                X[p], X[p2] = jnp.where(m, tmp, X[p]), jnp.where(m, X[p2], tmp)
    return XS


def _group4_sum(acc):
    lane = lax.broadcasted_iota(jnp.int32, acc.shape, 1)
    acc = acc + jnp.where((lane & 1) != 0, pltpu.roll(acc, 1, 1), pltpu.roll(acc, 127, 1))
    acc = acc + jnp.where((lane & 2) != 0, pltpu.roll(acc, 2, 1), pltpu.roll(acc, 126, 1))
    return acc


def make(T=128, M0=512, TA=192, RB=8, AR=48, CP0=256, EG=4, only='', upto=9,
         relL=(1, 3, 5, 7, 9, 11, 13, 15, 17, 18, 19, 20), relM=(0, 1, 2, 3, 4, 6, 8, 10, 12, 14, 16, 18, 19, 20, 21, 22),
         relW=(0, 2, 4, 6, 8, 10, 12, 14), RL=16, KQ=4,
         rel4=(-1, -1, -1, 0, 1, 2, 3, 4), rel23=(8, 9, 10, 11, 12, 13, 14, 15),
         order0=None, KQ0=1, tok0=None, LN0=3):
    NT = S // T
    if order0 is None:
        order0 = 'x00 T0 m0 x01 T1 h0 h1 h2 h3 H0 x10 H1 x11 H2 x20 l H3 x21'
    order0 = order0.split()
    NTA = (S - M0) // TA
    assert NTA == 8 and NTA * TA + M0 == S
    XP = 32
    NXP = TA // XP
    CPR = (M0 - CP0) // NTA
    S_C, S_X0, S_SA, S_CA, S_WQ, S_XA, S_WO, S_MB, S_W = 0, 1, 5, 13, 21, 29, 37, 45, 53

    def kernel(x_hbm, wqkv_hbm, wo_hbm, w1_hbm, w2_hbm, w3_hbm, w4_hbm, c_hbm, wmod_hbm,
               o_hbm,
               x_v, wqkv_raw, wq_v, wk_v, wv_v, wo_raw, wo_v, w1_v, w2_v, w3_v, w4_v, c_v, cE, cO, wmA_v, wmB_v,
               modA, modB, st_m, st_r, xhatA, hA, hP, q0, k0, v0, qbuf, kbuf, vbuf, xmid, hb, h1buf, obuf, o_scr, hsbuf,
               sems, osems):
        def cp(src, dst, k):
            return pltpu.make_async_copy(src, dst, sems.at[k])

        xu = x_hbm.bitcast(u32)
        wqkvu = wqkv_hbm.bitcast(u32)
        wou = wo_hbm.bitcast(u32)
        wmodu = wmod_hbm.bitcast(u32)

        def lane_ds(k, n):
            if isinstance(k, int):
                return pl.ds(k * n, n)
            return pl.ds(pl.multiple_of(k * n, 128), n)

        def row_ds(base, k, n):
            if isinstance(k, int):
                return pl.ds(base + k * n, n)
            return pl.ds(pl.multiple_of(base + k * n, 8), n)

        c_c = cp(c_hbm, c_v, S_C)

        def c_x0(b):
            return cp(xu.at[row_ds(0, b, 64)], x_v.at[row_ds(0, b, 64)], S_X0 + b)

        def c_sa(k):
            return cp(wmodu.at[:, lane_ds(k, 128)], wmA_v.at[k, 0:D // 2, 0:128], S_SA + k)

        def c_ca(k):
            if isinstance(k, int):
                src = wmodu.at[:, pl.ds(D + k * 128, 128)]
            else:
                src = wmodu.at[:, pl.ds(pl.multiple_of(D + k * 128, 128), 128)]
            return cp(src, wmA_v.at[k, 0:D // 2, 128:256], S_CA + k)

        def c_wq(k):
            return cp(wqkvu.at[row_ds(0, k, 64)], wqkv_raw.at[row_ds(0, k, 64)], S_WQ + k)

        def c_xa(p):
            return cp(xu.at[row_ds(M0 // 2, p, TA // 2)], x_v.at[row_ds(M0 // 2, p, TA // 2)], S_XA + p)

        def c_wo(p):
            return cp(wou.at[:, lane_ds(p, 128)], wo_raw.at[p, 8:8 + D // 2], S_WO + p)

        def c_mb(p):
            if isinstance(p, int):
                src = wmodu.at[:, pl.ds(2 * D + p * 512, 512)]
            else:
                src = wmodu.at[:, pl.ds(pl.multiple_of(2 * D + p * 512, 128), 512)]
            return cp(src, wmB_v.at[p, 0:D // 2], S_MB + p)

        c_w = [cp(w1_hbm.bitcast(u32), w1_v, S_W), cp(w2_hbm.bitcast(u32), w2_v, S_W + 1),
               cp(w3_hbm.bitcast(u32), w3_v, S_W + 2), cp(w4_hbm.bitcast(u32), w4_v, S_W + 3)]

        if only == '':
            c_c.start()
            c_wq(0).start()
            for b in range(4):
                c_x0(b).start()
            for k in range(8):
                c_sa(k).start()
                c_ca(k).start()
                if k > 0:
                    c_wq(k).start()
                if k == 2:
                    c_xa(0).start()
            for p in range(8):
                if upto < 2:
                    break
                if p < 7:
                    c_xa(p + 1).start()
                c_wo(p).start()
                c_mb(p).start()
            for c in c_w:
                if upto >= 3:
                    c.start()

        x_v[S // 2:S // 2 + HALO // 2, :] = jnp.zeros((HALO // 2, D), u32)
        for j in range(NCH):
            z = jnp.zeros((HALO, 128), f32)
            qbuf[j, S:S + HALO, :] = z
            kbuf[j, HALO + S:2 * HALO + S, :] = z
            vbuf[j, HALO + S:2 * HALO + S, :] = z
            k0[j, 0:HALO, :] = z
            v0[j, 0:HALO, :] = z
            wo_raw[j, 0:8, :] = jnp.zeros((8, 128), u32)
            wo_raw[j, 8 + D // 2:16 + D // 2, :] = jnp.zeros((8, 128), u32)

        def mv_part(w, r0, acc):
            n = w.shape[0]
            lo = pltpu.bitcast(w << 16, f32)
            hi = pltpu.bitcast(w & jnp.uint32(0xFFFF0000), f32)
            pr = lo * cE[r0:r0 + n, :] + hi * cO[r0:r0 + n, :]
            for t in range(n // 8):
                acc = pr[8 * t:8 * t + 8] if acc is None else acc + pr[8 * t:8 * t + 8]
            return acc

        wparts = (wq_v, wk_v, wv_v)
        bufs0 = (q0, k0, v0)

        def exch_groups(groups):
            for g0 in range(0, len(groups), EG):
                gs = groups[g0:g0 + EG]
                XS = [[wqkv_raw[row_ds(rg * 8, k * 8, 8), b * D + a * 128:b * D + (a + 1) * 128] for a in range(NCH)]
                      for (k, b, rg) in gs]
                YS = _exchange8_multi(XS)
                for (k, b, rg), Y in zip(gs, YS):
                    wparts[b][row_ds(rg * 8, k * 8, 8), :] = jnp.concatenate(Y, axis=1)

        def h_piece(k, rb, sa, ca):
            xk = _bf(x_v[rb * 64:(rb + 1) * 64, lane_ds(k, 128)]).astype(f32)
            hh = ((xk - st_m[rb * 128:(rb + 1) * 128, :]) * st_r[rb * 128:(rb + 1) * 128, :]) * (1.0 + ca) + sa
            return hh.astype(bf16)

        def subdot(lhs, kc, sd, init=False):
            b, hf = sd // 2, sd % 2
            res = _dot(lhs, _bf(wparts[b][row_ds(0, kc, 64), hf * 512:(hf + 1) * 512]))
            o = 0 if b == 0 else HALO
            for jj in range(4):
                j = hf * 4 + jj
                if init:
                    bufs0[b][j, o:o + M0, :] = res[:, jj * 128:(jj + 1) * 128]
                else:
                    bufs0[b][j, o:o + M0, :] += res[:, jj * 128:(jj + 1) * 128]
            return res

        def phase0():
            c_c.wait()
            c = c_v[...].astype(f32)
            scf = (c * jax.nn.sigmoid(c)).astype(bf16).astype(f32)
            rr = lax.broadcasted_iota(jnp.int32, (128, 128), 0)
            ll = lax.broadcasted_iota(jnp.int32, (128, 128), 1)
            sel = ll == jnp.where(rr < 64, 2 * rr, 2 * rr - 127)
            for j in range(NCH):
                dg = jnp.where(sel, jnp.broadcast_to(scf[:, j * 128:(j + 1) * 128], (128, 128)), 0.0).astype(bf16)
                rep = _dot(dg, jnp.ones((128, 128), bf16))
                cE[j * 64:(j + 1) * 64, :] = rep[0:64]
                cO[j * 64:(j + 1) * 64, :] = rep[64:128]
                v0[j, HALO:HALO + M0, :] = jnp.zeros((M0, 128), f32)

            def stats(b):
                c_x0(b).wait()
                xb = _bf(x_v[b * 64:(b + 1) * 64, :])
                m = _dot(xb, jnp.ones((D, 128), bf16)) * (1.0 / D)
                acc = None
                for j in range(NCH):
                    xc = xb[:, j * 128:(j + 1) * 128].astype(f32) - m
                    acc = xc * xc if acc is None else acc + xc * xc
                var = jnp.sum(acc, axis=-1, keepdims=True) * (1.0 / D)
                st_m[b * 128:(b + 1) * 128, :] = m
                st_r[b * 128:(b + 1) * 128, :] = jnp.broadcast_to(lax.rsqrt(var + EPS), (128, 128))

            def exch(k, b):
                exch_groups([(k, b, rg) for rg in range(8)])

            c_wq(0).wait()
            exch(0, 0)
            stats(0)
            exch(0, 1)
            stats(1)
            exch(0, 2)
            stats(2)
            stats(3)
            c_sa(0).wait(); c_ca(0).wait()
            sa = jnp.sum(mv_part(wmA_v[0, 0:D // 2, 0:128], 0, None), axis=0, keepdims=True)
            ca = jnp.sum(mv_part(wmA_v[0, 0:D // 2, 128:256], 0, None), axis=0, keepdims=True)
            modA[0, 0:1, 0:128] = sa
            modA[0, 0:1, 128:256] = ca
            h = jnp.concatenate([h_piece(0, rb, sa, ca) for rb in range(M0 // 128)], axis=0)
            hP[...] = pltpu.bitcast(h, u32)
            for sd in range(4):
                subdot(h, 0, sd, True)

            def region(r, carry):
                c_sa(r).wait(); c_ca(r).wait(); c_wq(r).wait()

                @pl.when(r == LN0)
                def _():
                    c_xa(0).wait()
                z1 = pl.multiple_of((r >> 8) * 8, 8)
                z2 = pl.multiple_of((r >> 9) * 8, 8)
                hp = _bf(hP[...])
                st = {'acc': [None, None], 'hl': [], 'res': None}

                def mvp(kq):
                    n = D // 2 // KQ0
                    for q in range(2):
                        st['acc'][q] = mv_part(wmA_v[r, pl.ds(z2 + kq * n, n), q * 128:(q + 1) * 128], kq * n, st['acc'][q])
                    if kq == KQ0 - 1:
                        st['sa'] = jnp.sum(st['acc'][0], axis=0, keepdims=True)
                        st['ca'] = jnp.sum(st['acc'][1], axis=0, keepdims=True)
                        modA[r, 0:1, 0:128] = st['sa']
                        modA[r, 0:1, 128:256] = st['ca']

                def hpc(rb):
                    st['hl'].append(h_piece(r, rb, st['sa'], st['ca']))
                    if rb == M0 // 128 - 1:
                        st['h'] = jnp.concatenate(st['hl'], axis=0)
                        hP[...] = pltpu.bitcast(st['h'], u32)

                def lnp():
                    pc = jnp.maximum(r - LN0, 0)
                    r0 = pl.multiple_of(jnp.where(r >= LN0, M0 // 2 + pc * (XP // 2), 0), 8)
                    xp = _bf(x_v[pl.ds(r0, XP // 2), :]).astype(f32)
                    xhatA[pl.ds(pl.multiple_of(pc * XP, 8), XP), :] = _ln(xp)

                for it in order0:
                    if it[0] == 'T':
                        st['res'] = subdot(hp, r - 1, 4 + int(it[1]))
                    elif it[0] == 'H':
                        st['res'] = subdot(st['h'], r, int(it[1]))
                    elif it[0] == 'm':
                        mvp(int(it[1]))
                    elif it[0] == 'h':
                        hpc(int(it[1]))
                    elif it[0] == 'x':
                        b, hf = int(it[1]), int(it[2])
                        exch_groups([(r, b, rg) for rg in range(4 * hf, 4 * hf + 4)])
                    elif it[0] == 'l':
                        lnp()
                    elif it[0] == 'k':
                        cc = int(it[1])
                        wmA_v[r, pl.ds(z1 + D // 2, 8), 0:128] = pltpu.bitcast(st['res'][0:8, cc * 128:(cc + 1) * 128], u32)
                return carry

            lax.fori_loop(1, 8, region, 0)
            h7 = _bf(hP[...])
            for pc in range(8 - LN0, NXP):
                r0 = M0 // 2 + pc * (XP // 2)
                xhatA[pc * XP:(pc + 1) * XP, :] = _ln(_bf(x_v[r0:r0 + XP // 2, :]).astype(f32))
            subdot(h7, 7, 4)
            subdot(h7, 7, 5)
            sa = jnp.concatenate([modA[j, 0:1, 0:128] for j in range(NCH)], axis=1)
            ca = jnp.concatenate([modA[j, 0:1, 128:256] for j in range(NCH)], axis=1)
            hA[...] = pltpu.bitcast((xhatA[0:TA, :] * (1.0 + ca) + sa).astype(bf16), u32)

        if only == '' and upto >= 1:
            phase0()
        if upto == 0:
            c_c.wait(); c_wq(0).wait()
            for b in range(4):
                c_x0(b).wait()
            for k in range(8):
                c_sa(k).wait(); c_ca(k).wait()
                if k > 0:
                    c_wq(k).wait()
            c_xa(0).wait()

        def attention(qb, kb, vb, base, off, M, mask_rows, baseh=None):
            row0 = base + off

            def kvds(r, w):
                return pl.ds(base + (off + HALO + r - DIL * w), RB)

            o_rows = []
            for r in range(0, M, RB):
                q = [qb[j, pl.ds(base + (off + r), RB), :] for j in range(NCH)]
                s = []
                for w in range(W):
                    acc = None
                    for j in range(NCH):
                        p = q[j] * kb[j, kvds(r, w), :]
                        acc = p if acc is None else acc + p
                    acc = _group4_sum(acc)
                    if mask_rows and r < DIL * (W - 1) and w > 0:
                        rows = row0 + r + lax.broadcasted_iota(jnp.int32, (RB, 128), 0)
                        acc = jnp.where(rows >= DIL * w, acc, -1e30)
                    s.append(acc)
                m = functools.reduce(jnp.maximum, s)
                e = [jnp.exp((sw - m) * SCALE) for sw in s]
                den = functools.reduce(lambda a, b: a + b, e)
                rinv = 1.0 / den
                oc = []
                for j in range(NCH):
                    acc = None
                    for w in range(W):
                        p = e[w] * vb[j, kvds(r, w), :]
                        acc = p if acc is None else acc + p
                    oc.append(acc * rinv)
                o_rows.append(jnp.concatenate(oc, axis=1))
            o = jnp.concatenate(o_rows, axis=0).astype(bf16)
            if isinstance(row0, int):
                o_scr[row0 // 2:(row0 + M) // 2, :] = pltpu.bitcast(o, u32)
            elif baseh is not None:
                o_scr[pl.ds(baseh + off // 2, M // 2), :] = pltpu.bitcast(o, u32)
            else:
                o_scr[pl.ds(pl.multiple_of(row0 // 2, 8), M // 2), :] = pltpu.bitcast(o, u32)

        sub = lax.broadcasted_iota(jnp.int32, (8, 128), 0)

        def abody(p, carry):
            @pl.when(p < 7)
            def _():
                c_xa(p + 1).wait()
            c_wo(p).wait()
            c_mb(p).wait()
            def copies():
                cr = pl.multiple_of(CP0 + p * CPR, 8)
                for j in range(NCH):
                    qbuf[j, pl.ds(cr, CPR), :] = q0[j, pl.ds(cr, CPR), :]
                    kbuf[j, pl.ds(cr + HALO, CPR), :] = k0[j, pl.ds(cr + HALO, CPR), :]
                    vbuf[j, pl.ds(cr + HALO, CPR), :] = v0[j, pl.ds(cr + HALO, CPR), :]
            copies()

            def pW(q, z):
                for tv in range(8 * q, 8 * q + 8):
                    j = tv >> 3
                    hh = (tv >> 1) & 3
                    a2 = tv & 1
                    parts = []
                    for al in range(4):
                        a = a2 * 4 + al
                        src = a * 64 + hh * 16 + j * 2
                        st = src - 2 * al + 8
                        parts.append(wo_raw[p, pl.ds(z + st, 8), :])
                    v = jnp.where(sub < 2, parts[0], parts[1])
                    v2 = jnp.where(sub < 6, parts[2], parts[3])
                    wo_v[p, 8 * tv:8 * tv + 8, :] = jnp.where(sub < 4, v, v2)

            def sa_ca():
                sa = jnp.concatenate([modA[j, 0:1, 0:128] for j in range(NCH)], axis=1)
                ca = jnp.concatenate([modA[j, 0:1, 128:256] for j in range(NCH)], axis=1)
                return sa, ca
            h = _bf(hA[...])
            r = pl.multiple_of(M0 + p * TA, 8)
            qkv = []
            for b, (buf, o) in enumerate(((qbuf, 0), (kbuf, HALO), (vbuf, HALO))):
                res = _dot(h, _bf(wparts[b][...]))
                qkv.append(res)
                for j in range(NCH):
                    buf[j, pl.ds(r + o, TA), :] = res[:, j * 128:(j + 1) * 128]
            z1 = pl.multiple_of((p >> 8) * 8, 8)
            z2 = pl.multiple_of((p >> 9) * 8, 8)
            nrh = pl.multiple_of(M0 // 2 + jnp.minimum(p + 1, NTA - 1) * (TA // 2), 8)

            def pL(q):
                xn = _ln(_bf(x_v[pl.ds(nrh + q * (RL // 2), RL // 2), :]).astype(f32))
                sa, ca = sa_ca()
                hA[q * (RL // 2):(q + 1) * (RL // 2), :] = pltpu.bitcast((xn * (1.0 + ca) + sa).astype(bf16), u32)

            macc = {}

            def pM(qq):
                q, kq = qq // KQ, qq % KQ
                n = D // 2 // KQ
                macc[q] = mv_part(wmB_v[p, pl.ds(z2 + kq * n, n), q * 128:(q + 1) * 128], kq * n, macc.get(q))
                if kq == KQ - 1:
                    modB[p, 0:1, q * 128:(q + 1) * 128] = jnp.sum(macc[q], axis=0, keepdims=True)

            for c in range(-1, 3 * NCH):
                ql = [q for q in range(TA // RL) if relL[q] == c]
                qm = [q for q in range(4 * KQ) if relM[q] == c]
                qw = [q for q in range(8) if relW[q] == c]
                if c >= 0:
                    tk = pltpu.bitcast(qkv[c // NCH][0:8, (c % NCH) * 128:(c % NCH + 1) * 128], u32)
                    if ql:
                        x_v[pl.ds(z1 + S // 2 + HALO // 2, 8), 0:128] = tk
                    if qm:
                        wmB_v[p, pl.ds(z1 + D // 2, 8), 0:128] = tk
                    if qw:
                        wo_raw[p, pl.ds(z1 + D // 2 + 16, 8), :] = tk
                for q in ql:
                    pL(q)
                for q in qm:
                    pM(q)
                for q in qw:
                    pW(q, z2 if c >= 0 else 0)
            attention(q0, k0, v0, pl.multiple_of(p * AR, 16), 0, AR, True, pl.multiple_of(p * (AR // 2), 8))
            return carry
        if only in ('', 'A') and upto >= 2:
            lax.fori_loop(0, NTA, abody, 0)

        if only == '' and upto >= 3:
            for c in c_w:
                c.wait()

        def rows_u32(ref, row0, M):
            if isinstance(row0, int):
                return _bf(ref[row0 // 2:(row0 + M) // 2, :])
            if isinstance(row0, tuple):
                return _bf(ref[pl.ds(row0[0] + row0[1] // 2, M // 2), :])
            return _bf(ref[pl.ds(pl.multiple_of(row0 // 2, 8), M // 2), :])

        def wo_dot(row0, M):
            o = rows_u32(o_scr, row0, M)
            return jnp.concatenate([_dot(o, _bf(wo_v[n])) for n in range(NCH)], axis=1)

        def row(k):
            return jnp.concatenate([modB[2 * (k - 2), 0:1, :], modB[2 * (k - 2) + 1, 0:1, :]], axis=1)

        def ln23(row0, M, A):
            ga = row(2); sb = row(3); cb = row(4)
            x = rows_u32(x_v, row0, M).astype(f32)
            xm = x + ga * A
            hB = _ln(xm) * (1.0 + cb) + sb
            n3 = _ln(hB).astype(bf16)
            return xm, hB, n3

        shifts = [-1, -1, 1, 1, -2, -2, 2, 2]

        def g_val():
            return jnp.concatenate(
                [h1buf[j, HALO + shifts[j]:HALO + shifts[j] + T, :] for j in range(NCH)], axis=1).astype(bf16)

        def out_copy(tile, slot):
            r0 = pl.multiple_of(tile * (T // 2), 8)
            return pltpu.make_async_copy(obuf.at[slot], o_hbm.bitcast(u32).at[pl.ds(r0, T // 2)], osems.at[slot])

        def ln4(hs):
            gb = row(5)
            x1 = hb[0:T, :] + hs
            base = xmid[0:T, :] + gb * x1
            n4 = _ln(x1).astype(bf16)
            return base, n4

        def bfirst():
            for j in range(NCH):
                h1buf[j, 0:HALO, :] = jnp.zeros((HALO, 128), f32)
            if NTA * AR < 2 * T + HALO:
                attention(q0, k0, v0, 0, NTA * AR, 2 * T + HALO - NTA * AR, False)
            h0 = (T + HALO) // 2 // 16 * 16 + (16 if T == 128 else 0)
            halves = [(0, h0), (h0, T + HALO - h0)]
            As = [wo_dot(r0, m) for r0, m in halves]
            for (r0, m), A in zip(halves, As):
                xm, hB, n3 = ln23(r0, m, A)
                h1 = _gelu(_dot(n3, _bf(w1_v[...])))
                xmid[r0:r0 + m, :] = xm
                hb[r0:r0 + m, :] = hB
                for j in range(NCH):
                    h1buf[j, HALO + r0:HALO + r0 + m, :] = h1[:, j * 128:(j + 1) * 128]

            hsbuf[0:T, :] = _dot(g_val(), _bf(w2_v[...]))

        if only in ('', 'BF') and upto >= 3:
            bfirst()

        def carries(xm, hB, h1, notlast):
            xmid[0:HALO, :] = xmid[T:T + HALO, :]
            hb[0:HALO, :] = hb[T:T + HALO, :]
            for j in range(NCH):
                h1buf[j, 0:2 * HALO, :] = h1buf[j, T:T + 2 * HALO, :]
            xmid[HALO:HALO + T, :] = xm
            hb[HALO:HALO + T, :] = hB
            for j in range(NCH):
                h1j = h1[:, j * 128:(j + 1) * 128]
                h1buf[j, 2 * HALO:HALO + T, :] = h1j[0:T - HALO]
                h1buf[j, HALO + T:2 * HALO + T, :] = jnp.where(notlast, h1j[T - HALO:T], 0.0)

        RP = 16

        def bbody(i, carry):
            slot = (i - 1) % 2

            @pl.when(i >= 3)
            def _():
                out_copy(i - 3, slot).wait()

            row0h = pl.multiple_of(i * (T // 2), T // 2)
            nxt = jnp.minimum(i + 1, NT - 1)
            abase = pl.multiple_of(nxt * T, T)
            abaseh = pl.multiple_of(nxt * (T // 2), T // 2)
            z1 = pl.multiple_of((i >> 8) * 8, 8)
            z2 = pl.multiple_of((i >> 9) * 8, 8)
            ga = row(2); sb = row(3); cb = row(4); gb = row(5)
            bases, n4p, xms, hBs, n3p, As = [], [], [], [], [], []

            def p4(r):
                r0 = r * RP
                x1 = hb[r0:r0 + RP, :] + hsbuf[pl.ds(z2 + r0, RP), :]
                bases.append(xmid[r0:r0 + RP, :] + gb * x1)
                n4p.append(_ln(x1).astype(bf16))

            def p23(r, A):
                r0 = r * RP
                x = rows_u32(x_v, (row0h, HALO + r0), RP).astype(f32)
                xm = x + ga * A[r0:r0 + RP]
                hB = _ln(xm) * (1.0 + cb) + sb
                xms.append(xm); hBs.append(hB)
                n3p.append(_ln(hB).astype(bf16))

            for r in range(T // RP):
                if rel4[r] < 0:
                    p4(r)
            o = rows_u32(o_scr, (row0h, HALO), T)
            for n in range(NCH):
                An = _dot(o, _bf(wo_v[n]))
                As.append(An)
                r4 = [r for r in range(T // RP) if rel4[r] == n]
                if r4:
                    hsbuf[pl.ds(z1 + T, 8), 0:128] = An[0:8, 0:128]
                for r in r4:
                    p4(r)
            A = jnp.concatenate(As, axis=1)
            base = jnp.concatenate(bases, axis=0)
            n4 = jnp.concatenate(n4p, axis=0)
            U = _dot(n4, _bf(w3_v[...]))
            u = _gelu(U).astype(bf16)
            for c in range(F // 128):
                r23 = [r for r in range(T // RP) if rel23[r] == NCH + c]
                if r23:
                    x_v[pl.ds(z1 + S // 2 + HALO // 2, 8), 0:128] = pltpu.bitcast(U[0:8, c * 128:(c + 1) * 128], u32)
                for r in r23:
                    p23(r, A)
            assert len(n3p) == T // RP and len(n4p) == T // RP
            xm = jnp.concatenate(xms, axis=0)
            hB = jnp.concatenate(hBs, axis=0)
            n3 = jnp.concatenate(n3p, axis=0)
            h1 = _gelu(_dot(n3, _bf(w1_v[...])))
            carries(xm, hB, h1, i < NT - 1)
            attention(qbuf, kbuf, vbuf, abase, HALO, T, False, abaseh)
            h2 = _dot(u, _bf(w4_v[...]))
            obuf[slot] = pltpu.bitcast((base + gb * h2).astype(bf16), u32)
            hsbuf[0:T, :] = _dot(g_val(), _bf(w2_v[...]))
            out_copy(i - 1, slot).start()
            return carry

        if only in ('', 'B') and upto >= 4:
            lax.fori_loop(1, NT, bbody, 0)
        if only == 'B' or upto == 4:
            out_copy(NT - 3, (NT - 1) % 2).wait()
            out_copy(NT - 2, NT % 2).wait()

        def blast():
            slot = (NT - 1) % 2
            out_copy(NT - 3, slot).wait()
            base, n4 = ln4(hsbuf[0:T, :])
            u = _gelu(_dot(n4, _bf(w3_v[...]))).astype(bf16)
            h2 = _dot(u, _bf(w4_v[...]))
            obuf[slot] = pltpu.bitcast((base + row(5) * h2).astype(bf16), u32)
            out_copy(NT - 1, slot).start()
            out_copy(NT - 2, 1 - slot).wait()
            out_copy(NT - 1, slot).wait()

        if only in ('', 'BL') and upto >= 5:
            blast()

    @jax.jit
    def fn(A_x, A_wqkv, A_wo, B_x, B_w1, B_w2, B_w3, B_w4, c, w_mod):
        x = A_x.reshape(S, D)
        any_spec = pl.BlockSpec(memory_space=pl.ANY)
        out = pl.pallas_call(
            kernel,
            in_specs=[any_spec] * 9,
            out_specs=any_spec,
            out_shape=jax.ShapeDtypeStruct((S, D), bf16),
            scratch_shapes=[
                pltpu.VMEM((S // 2 + HALO // 2 + 8, D), u32),
                pltpu.VMEM((D // 2, 3 * D), u32),
                pltpu.VMEM((D // 2, D), u32),
                pltpu.VMEM((D // 2, D), u32),
                pltpu.VMEM((D // 2, D), u32),
                pltpu.VMEM((NCH, D // 2 + 24, 128), u32),
                pltpu.VMEM((NCH, D // 2, 128), u32),
                pltpu.VMEM((D // 2, D), u32),
                pltpu.VMEM((D // 2, D), u32),
                pltpu.VMEM((D // 2, F), u32),
                pltpu.VMEM((F // 2, D), u32),
                pltpu.VMEM((1, D), bf16),
                pltpu.VMEM((D // 2, 128), f32),
                pltpu.VMEM((D // 2, 128), f32),
                pltpu.VMEM((8, D // 2 + 8, 256), u32),
                pltpu.VMEM((8, D // 2 + 8, 512), u32),
                pltpu.VMEM((8, 8, 256), f32),
                pltpu.VMEM((8, 8, 512), f32),
                pltpu.VMEM((M0, 128), f32),
                pltpu.VMEM((M0, 128), f32),
                pltpu.VMEM((TA, D), f32),
                pltpu.VMEM((TA // 2, D), u32),
                pltpu.VMEM((M0 // 2, 128), u32),
                pltpu.VMEM((NCH, M0, 128), f32),
                pltpu.VMEM((NCH, M0 + HALO, 128), f32),
                pltpu.VMEM((NCH, M0 + HALO, 128), f32),
                pltpu.VMEM((NCH, S + HALO, 128), f32),
                pltpu.VMEM((NCH, S + 2 * HALO, 128), f32),
                pltpu.VMEM((NCH, S + 2 * HALO, 128), f32),
                pltpu.VMEM((T + HALO, D), f32),
                pltpu.VMEM((T + HALO, D), f32),
                pltpu.VMEM((NCH, T + 2 * HALO, 128), f32),
                pltpu.VMEM((2, T // 2, D), u32),
                pltpu.VMEM((S // 2 + HALO // 2, D), u32),
                pltpu.VMEM((T + 8, D), f32),
                pltpu.SemaphoreType.DMA((57,)),
                pltpu.SemaphoreType.DMA((2,)),
            ],
            compiler_params=pltpu.CompilerParams(vmem_limit_bytes=120 * 1024 * 1024),
        )(x, A_wqkv, A_wo, B_w1, B_w2, B_w3, B_w4, c, w_mod)
        return out.reshape(1, S, D)
    return fn


_fn = make()


def pallas_adaLN_cond__sliding_local_dilated__mixer_s_mlp__prompt_kernel(A_x, A_wqkv, A_wo, B_x, B_w1, B_w2, B_w3, B_w4, c, w_mod):
    return _fn(A_x, A_wqkv, A_wo, B_x, B_w1, B_w2, B_w3, B_w4, c, w_mod)
```

```python
import functools
import jax
import jax.numpy as jnp
from jax import lax
import jax.experimental.pallas as pl
import jax.experimental.pallas.tpu as pltpu

S, D, F = 2048, 1024, 3584
H, DH, W, DIL = 32, 32, 8, 2
NCH = D // 128
EPS = 1e-5
SCALE = DH ** -0.5
f32, bf16, u32 = jnp.float32, jnp.bfloat16, jnp.uint32
HALO = 16


def _ln(x):
    m = jnp.mean(x, axis=-1, keepdims=True)
    xc = x - m
    v = jnp.mean(xc * xc, axis=-1, keepdims=True)
    return xc * lax.rsqrt(v + EPS)


def _gelu(x):
    c0 = 0.7978845608028654
    c1 = c0 * 0.044715
    t = jnp.tanh(x * (c0 + c1 * (x * x)))
    hx = 0.5 * x
    return hx + hx * t


def _dot(a, b):
    return jnp.dot(a, b, preferred_element_type=f32)


def _bf(w):
    return pltpu.bitcast(w, bf16)


def _lane_xor(x, s):
    lane = lax.broadcasted_iota(jnp.int32, x.shape, 1)
    return jnp.take_along_axis(x, lane ^ s, axis=1)


def _exchange8_multi(XS):
    XS = [list(X) for X in XS]
    lane = lax.broadcasted_iota(jnp.int32, XS[0][0].shape, 1)
    for t in range(3):
        s = 1 << (t + 2)
        m = (lane & s) != 0
        for X in XS:
            for p in range(8):
                if p & (1 << t):
                    continue
                p2 = p | (1 << t)
                tmp = _lane_xor(jnp.where(m, X[p], X[p2]), s)
                X[p], X[p2] = jnp.where(m, tmp, X[p]), jnp.where(m, X[p2], tmp)
    return XS


def _group4_sum(acc):
    lane = lax.broadcasted_iota(jnp.int32, acc.shape, 1)
    acc = acc + jnp.where((lane & 1) != 0, pltpu.roll(acc, 1, 1), pltpu.roll(acc, 127, 1))
    acc = acc + jnp.where((lane & 2) != 0, pltpu.roll(acc, 2, 1), pltpu.roll(acc, 126, 1))
    return acc


def make(T=128, M0=512, TA=192, RB=8, AR=32, CP0=256, EG=4, only='', upto=9,
         relL=(1, 3, 5, 7, 9, 11, 13, 15, 17, 18, 19, 20), relM=(0, 1, 2, 3, 4, 6, 8, 10, 12, 14, 16, 18, 19, 20, 21, 22),
         relW=(0, 2, 4, 6, 8, 10, 12, 14), RL=16, KQ=4,
         rel4=(-1, -1, -1, 0, 1, 2, 3, 4), rel23=(8, 9, 10, 11, 12, 13, 14, 15),
         order0=None, KQ0=1, tok0=None, LN0=3, stage='', padr=0, dbg=''):
    NT = S // T
    if order0 is None:
        order0 = 'x00 T0 m0 x01 T1 h0 h1 h2 h3 H0 x10 H1 x11 H2 x20 l H3 x21'
    order0 = order0.split()
    NTA = (S - M0) // TA
    assert NTA == 8 and NTA * TA + M0 == S
    XP = 32
    NXP = TA // XP
    CPR = (M0 - CP0) // NTA
    S_C, S_X0, S_SA, S_CA, S_WQ, S_XA, S_WO, S_MB, S_W = 0, 1, 5, 13, 21, 29, 37, 45, 53

    def kernel(x_hbm, wqkv_hbm, wo_hbm, w1_hbm, w2_hbm, w3_hbm, w4_hbm, c_hbm, wmod_hbm,
               o_hbm,
               x_v, wqkv_raw, wq_v, wk_v, wv_v, wo_raw, wo_v, w1_v, w2_v, w3_v, w4_v, cE, cO, wmA_v, wmB_v,
               modA, modB, st_m, st_r, xhatA, hA, hP, q0, k0, v0, qbuf, kbuf, vbuf, xmid, hb, h1buf, obuf, o_scr, hsbuf, n4b, ub, n3b, gbf, c_v, *rest):
        sems, osems = rest[-2:]

        def cp(src, dst, k):
            return pltpu.make_async_copy(src, dst, sems.at[k])

        xu = x_hbm.bitcast(u32)
        wqkvu = wqkv_hbm.bitcast(u32)
        wou = wo_hbm.bitcast(u32)
        wmodu = wmod_hbm.bitcast(u32)

        def lane_ds(k, n):
            if isinstance(k, int):
                return pl.ds(k * n, n)
            return pl.ds(pl.multiple_of(k * n, 128), n)

        def row_ds(base, k, n):
            if isinstance(k, int):
                return pl.ds(base + k * n, n)
            return pl.ds(pl.multiple_of(base + k * n, 8), n)

        c_c = cp(c_hbm, c_v, S_C)

        def c_x0(b):
            return cp(xu.at[row_ds(0, b, 64)], x_v.at[row_ds(0, b, 64)], S_X0 + b)

        def c_sa(k):
            return cp(wmodu.at[:, lane_ds(k, 128)], wmA_v.at[k, 0:D // 2, 0:128], S_SA + k)

        def c_ca(k):
            if isinstance(k, int):
                src = wmodu.at[:, pl.ds(D + k * 128, 128)]
            else:
                src = wmodu.at[:, pl.ds(pl.multiple_of(D + k * 128, 128), 128)]
            return cp(src, wmA_v.at[k, 0:D // 2, 128:256], S_CA + k)

        def c_wq(k):
            return cp(wqkvu.at[row_ds(0, k, 64)], wqkv_raw.at[row_ds(0, k, 64)], S_WQ + k)

        def c_xa(p):
            return cp(xu.at[row_ds(M0 // 2, p, TA // 2)], x_v.at[row_ds(M0 // 2, p, TA // 2)], S_XA + p)

        def c_wo(p):
            return cp(wou.at[:, lane_ds(p, 128)], wo_raw.at[p, 8:8 + D // 2], S_WO + p)

        def c_mb(p):
            if isinstance(p, int):
                src = wmodu.at[:, pl.ds(2 * D + p * 512, 512)]
            else:
                src = wmodu.at[:, pl.ds(pl.multiple_of(2 * D + p * 512, 128), 512)]
            return cp(src, wmB_v.at[p, 0:D // 2], S_MB + p)

        c_w = [cp(w1_hbm.bitcast(u32), w1_v, S_W), cp(w2_hbm.bitcast(u32), w2_v, S_W + 1),
               cp(w3_hbm.bitcast(u32), w3_v, S_W + 2), cp(w4_hbm.bitcast(u32), w4_v, S_W + 3)]

        if only == '':
            c_c.start()
            c_wq(0).start()
            for b in range(4):
                c_x0(b).start()
            for k in range(8):
                c_sa(k).start()
                c_ca(k).start()
                if k > 0:
                    c_wq(k).start()
                if k == 2:
                    c_xa(0).start()
            for p in range(8):
                if upto < 2:
                    break
                if p < 7:
                    c_xa(p + 1).start()
                c_wo(p).start()
                c_mb(p).start()
            for c in c_w:
                if upto >= 3:
                    c.start()

        x_v[S // 2:S // 2 + HALO // 2, :] = jnp.zeros((HALO // 2, D), u32)
        for j in range(NCH):
            z = jnp.zeros((HALO, 128), f32)
            qbuf[j, S:S + HALO, :] = z
            kbuf[j, HALO + S:2 * HALO + S, :] = z
            vbuf[j, HALO + S:2 * HALO + S, :] = z
            k0[j, 0:HALO, :] = z
            v0[j, 0:HALO, :] = z
            wo_raw[j, 0:8, :] = jnp.zeros((8, 128), u32)
            wo_raw[j, 8 + D // 2:16 + D // 2, :] = jnp.zeros((8, 128), u32)

        def mv_part(w, r0, acc):
            n = w.shape[0]
            lo = pltpu.bitcast(w << 16, f32)
            hi = pltpu.bitcast(w & jnp.uint32(0xFFFF0000), f32)
            pr = lo * cE[r0:r0 + n, :] + hi * cO[r0:r0 + n, :]
            for t in range(n // 8):
                acc = pr[8 * t:8 * t + 8] if acc is None else acc + pr[8 * t:8 * t + 8]
            return acc

        wparts = (wq_v, wk_v, wv_v)
        bufs0 = (q0, k0, v0)

        def exch_groups(groups):
            for g0 in range(0, len(groups), EG):
                gs = groups[g0:g0 + EG]
                XS = [[wqkv_raw[row_ds(rg * 8, k * 8, 8), b * D + a * 128:b * D + (a + 1) * 128] for a in range(NCH)]
                      for (k, b, rg) in gs]
                YS = _exchange8_multi(XS)
                for (k, b, rg), Y in zip(gs, YS):
                    wparts[b][row_ds(rg * 8, k * 8, 8), :] = jnp.concatenate(Y, axis=1)

        def h_piece(k, rb, sa, ca):
            xk = _bf(x_v[rb * 64:(rb + 1) * 64, lane_ds(k, 128)]).astype(f32)
            hh = ((xk - st_m[rb * 128:(rb + 1) * 128, :]) * st_r[rb * 128:(rb + 1) * 128, :]) * (1.0 + ca) + sa
            return hh.astype(bf16)

        def subdot(lhs, kc, sd, init=False):
            b, hf = sd // 2, sd % 2
            res = _dot(lhs, _bf(wparts[b][row_ds(0, kc, 64), hf * 512:(hf + 1) * 512]))
            o = 0 if b == 0 else HALO
            for jj in range(4):
                j = hf * 4 + jj
                if init:
                    bufs0[b][j, o:o + M0, :] = res[:, jj * 128:(jj + 1) * 128]
                else:
                    bufs0[b][j, o:o + M0, :] += res[:, jj * 128:(jj + 1) * 128]
            return res

        def phase0():
            c_c.wait()
            c = c_v[...].astype(f32)
            scf = (c * jax.nn.sigmoid(c)).astype(bf16).astype(f32)
            rr = lax.broadcasted_iota(jnp.int32, (128, 128), 0)
            ll = lax.broadcasted_iota(jnp.int32, (128, 128), 1)
            sel = ll == jnp.where(rr < 64, 2 * rr, 2 * rr - 127)
            for j in range(NCH):
                dg = jnp.where(sel, jnp.broadcast_to(scf[:, j * 128:(j + 1) * 128], (128, 128)), 0.0).astype(bf16)
                rep = _dot(dg, jnp.ones((128, 128), bf16))
                cE[j * 64:(j + 1) * 64, :] = rep[0:64]
                cO[j * 64:(j + 1) * 64, :] = rep[64:128]
                v0[j, HALO:HALO + M0, :] = jnp.zeros((M0, 128), f32)

            def stats(b):
                c_x0(b).wait()
                xb = _bf(x_v[b * 64:(b + 1) * 64, :])
                m = _dot(xb, jnp.ones((D, 128), bf16)) * (1.0 / D)
                acc = None
                for j in range(NCH):
                    xc = xb[:, j * 128:(j + 1) * 128].astype(f32) - m
                    acc = xc * xc if acc is None else acc + xc * xc
                var = jnp.sum(acc, axis=-1, keepdims=True) * (1.0 / D)
                st_m[b * 128:(b + 1) * 128, :] = m
                st_r[b * 128:(b + 1) * 128, :] = jnp.broadcast_to(lax.rsqrt(var + EPS), (128, 128))

            def exch(k, b):
                exch_groups([(k, b, rg) for rg in range(8)])

            c_wq(0).wait()
            exch(0, 0)
            stats(0)
            exch(0, 1)
            stats(1)
            exch(0, 2)
            stats(2)
            stats(3)
            c_sa(0).wait(); c_ca(0).wait()
            sa = jnp.sum(mv_part(wmA_v[0, 0:D // 2, 0:128], 0, None), axis=0, keepdims=True)
            ca = jnp.sum(mv_part(wmA_v[0, 0:D // 2, 128:256], 0, None), axis=0, keepdims=True)
            modA[0, 0:1, 0:128] = sa
            modA[0, 0:1, 128:256] = ca
            h = jnp.concatenate([h_piece(0, rb, sa, ca) for rb in range(M0 // 128)], axis=0)
            hP[...] = pltpu.bitcast(h, u32)
            for sd in range(4):
                subdot(h, 0, sd, True)

            def region(r, carry):
                c_sa(r).wait(); c_ca(r).wait(); c_wq(r).wait()

                @pl.when(r == LN0)
                def _():
                    c_xa(0).wait()
                z1 = pl.multiple_of((r >> 8) * 8, 8)
                z2 = pl.multiple_of((r >> 9) * 8, 8)
                hp = _bf(hP[...])
                st = {'acc': [None, None], 'hl': [], 'res': None}

                def mvp(kq):
                    n = D // 2 // KQ0
                    for q in range(2):
                        st['acc'][q] = mv_part(wmA_v[r, pl.ds(z2 + kq * n, n), q * 128:(q + 1) * 128], kq * n, st['acc'][q])
                    if kq == KQ0 - 1:
                        st['sa'] = jnp.sum(st['acc'][0], axis=0, keepdims=True)
                        st['ca'] = jnp.sum(st['acc'][1], axis=0, keepdims=True)
                        modA[r, 0:1, 0:128] = st['sa']
                        modA[r, 0:1, 128:256] = st['ca']

                def hpc(rb):
                    st['hl'].append(h_piece(r, rb, st['sa'], st['ca']))
                    if rb == M0 // 128 - 1:
                        st['h'] = jnp.concatenate(st['hl'], axis=0)
                        hP[...] = pltpu.bitcast(st['h'], u32)

                def lnp():
                    pc = jnp.maximum(r - LN0, 0)
                    r0 = pl.multiple_of(jnp.where(r >= LN0, M0 // 2 + pc * (XP // 2), 0), 8)
                    xp = _bf(x_v[pl.ds(r0, XP // 2), :]).astype(f32)
                    xhatA[pl.ds(pl.multiple_of(pc * XP, 8), XP), :] = _ln(xp)

                for it in order0:
                    if it[0] == 'T':
                        st['res'] = subdot(hp, r - 1, 4 + int(it[1]))
                    elif it[0] == 'H':
                        st['res'] = subdot(st['h'], r, int(it[1]))
                    elif it[0] == 'm':
                        mvp(int(it[1]))
                    elif it[0] == 'h':
                        hpc(int(it[1]))
                    elif it[0] == 'x':
                        b, hf = int(it[1]), int(it[2])
                        exch_groups([(r, b, rg) for rg in range(4 * hf, 4 * hf + 4)])
                    elif it[0] == 'l':
                        lnp()
                    elif it[0] == 'k':
                        cc = int(it[1])
                        wmA_v[r, pl.ds(z1 + D // 2, 8), 0:128] = pltpu.bitcast(st['res'][0:8, cc * 128:(cc + 1) * 128], u32)
                return carry

            lax.fori_loop(1, 8, region, 0)
            h7 = _bf(hP[...])
            for pc in range(8 - LN0, NXP):
                r0 = M0 // 2 + pc * (XP // 2)
                xhatA[pc * XP:(pc + 1) * XP, :] = _ln(_bf(x_v[r0:r0 + XP // 2, :]).astype(f32))
            subdot(h7, 7, 4)
            subdot(h7, 7, 5)
            sa = jnp.concatenate([modA[j, 0:1, 0:128] for j in range(NCH)], axis=1)
            ca = jnp.concatenate([modA[j, 0:1, 128:256] for j in range(NCH)], axis=1)
            hA[...] = pltpu.bitcast((xhatA[0:TA, :] * (1.0 + ca) + sa).astype(bf16), u32)

        if only == '' and upto >= 1:
            phase0()
        if upto == 0:
            c_c.wait(); c_wq(0).wait()
            for b in range(4):
                c_x0(b).wait()
            for k in range(8):
                c_sa(k).wait(); c_ca(k).wait()
                if k > 0:
                    c_wq(k).wait()
            c_xa(0).wait()

        def attention(qb, kb, vb, base, off, M, mask_rows, baseh=None):
            row0 = base + off

            def kvds(r, w):
                return pl.ds(base + (off + HALO + r - DIL * w), RB)

            o_rows = []
            for r in range(0, M, RB):
                q = [qb[j, pl.ds(base + (off + r), RB), :] for j in range(NCH)]
                s = []
                for w in range(W):
                    acc = None
                    for j in range(NCH):
                        p = q[j] * kb[j, kvds(r, w), :]
                        acc = p if acc is None else acc + p
                    acc = _group4_sum(acc)
                    if mask_rows and r < DIL * (W - 1) and w > 0:
                        rows = row0 + r + lax.broadcasted_iota(jnp.int32, (RB, 128), 0)
                        acc = jnp.where(rows >= DIL * w, acc, -1e30)
                    s.append(acc)
                m = functools.reduce(jnp.maximum, s)
                e = [jnp.exp((sw - m) * SCALE) for sw in s]
                den = functools.reduce(lambda a, b: a + b, e)
                rinv = 1.0 / den
                oc = []
                for j in range(NCH):
                    acc = None
                    for w in range(W):
                        p = e[w] * vb[j, kvds(r, w), :]
                        acc = p if acc is None else acc + p
                    oc.append(acc * rinv)
                o_rows.append(jnp.concatenate(oc, axis=1))
            o = jnp.concatenate(o_rows, axis=0).astype(bf16)
            if isinstance(row0, int):
                o_scr[row0 // 2:(row0 + M) // 2, :] = pltpu.bitcast(o, u32)
            elif baseh is not None:
                o_scr[pl.ds(baseh + off // 2, M // 2), :] = pltpu.bitcast(o, u32)
            else:
                o_scr[pl.ds(pl.multiple_of(row0 // 2, 8), M // 2), :] = pltpu.bitcast(o, u32)

        sub = lax.broadcasted_iota(jnp.int32, (8, 128), 0)

        def abody(p, carry):
            @pl.when(p < 7)
            def _():
                c_xa(p + 1).wait()
            c_wo(p).wait()
            c_mb(p).wait()
            def copies():
                cr = pl.multiple_of(CP0 + p * CPR, 8)
                for j in range(NCH):
                    qbuf[j, pl.ds(cr, CPR), :] = q0[j, pl.ds(cr, CPR), :]
                    kbuf[j, pl.ds(cr + HALO, CPR), :] = k0[j, pl.ds(cr + HALO, CPR), :]
                    vbuf[j, pl.ds(cr + HALO, CPR), :] = v0[j, pl.ds(cr + HALO, CPR), :]
            copies()

            def pW(q, z):
                for tv in range(8 * q, 8 * q + 8):
                    j = tv >> 3
                    hh = (tv >> 1) & 3
                    a2 = tv & 1
                    parts = []
                    for al in range(4):
                        a = a2 * 4 + al
                        src = a * 64 + hh * 16 + j * 2
                        st = src - 2 * al + 8
                        parts.append(wo_raw[p, pl.ds(z + st, 8), :])
                    v = jnp.where(sub < 2, parts[0], parts[1])
                    v2 = jnp.where(sub < 6, parts[2], parts[3])
                    wo_v[p, 8 * tv:8 * tv + 8, :] = jnp.where(sub < 4, v, v2)

            def sa_ca():
                sa = jnp.concatenate([modA[j, 0:1, 0:128] for j in range(NCH)], axis=1)
                ca = jnp.concatenate([modA[j, 0:1, 128:256] for j in range(NCH)], axis=1)
                return sa, ca
            h = _bf(hA[...])
            r = pl.multiple_of(M0 + p * TA, 8)
            qkv = []
            for b, (buf, o) in enumerate(((qbuf, 0), (kbuf, HALO), (vbuf, HALO))):
                res = _dot(h, _bf(wparts[b][...]))
                qkv.append(res)
                for j in range(NCH):
                    buf[j, pl.ds(r + o, TA), :] = res[:, j * 128:(j + 1) * 128]
            z1 = pl.multiple_of((p >> 8) * 8, 8)
            z2 = pl.multiple_of((p >> 9) * 8, 8)
            nrh = pl.multiple_of(M0 // 2 + jnp.minimum(p + 1, NTA - 1) * (TA // 2), 8)

            def pL(q):
                xn = _ln(_bf(x_v[pl.ds(nrh + q * (RL // 2), RL // 2), :]).astype(f32))
                sa, ca = sa_ca()
                hA[q * (RL // 2):(q + 1) * (RL // 2), :] = pltpu.bitcast((xn * (1.0 + ca) + sa).astype(bf16), u32)

            macc = {}

            def pM(qq):
                q, kq = qq // KQ, qq % KQ
                n = D // 2 // KQ
                macc[q] = mv_part(wmB_v[p, pl.ds(z2 + kq * n, n), q * 128:(q + 1) * 128], kq * n, macc.get(q))
                if kq == KQ - 1:
                    modB[p, 0:1, q * 128:(q + 1) * 128] = jnp.sum(macc[q], axis=0, keepdims=True)

            for c in range(-1, 3 * NCH):
                ql = [q for q in range(TA // RL) if relL[q] == c]
                qm = [q for q in range(4 * KQ) if relM[q] == c]
                qw = [q for q in range(8) if relW[q] == c]
                if c >= 0:
                    tk = pltpu.bitcast(qkv[c // NCH][0:8, (c % NCH) * 128:(c % NCH + 1) * 128], u32)
                    if ql:
                        x_v[pl.ds(z1 + S // 2 + HALO // 2, 8), 0:128] = tk
                    if qm:
                        wmB_v[p, pl.ds(z1 + D // 2, 8), 0:128] = tk
                    if qw:
                        wo_raw[p, pl.ds(z1 + D // 2 + 16, 8), :] = tk
                for q in ql:
                    pL(q)
                for q in qm:
                    pM(q)
                for q in qw:
                    pW(q, z2 if c >= 0 else 0)
            attention(q0, k0, v0, pl.multiple_of(p * AR, 16), 0, AR, True, pl.multiple_of(p * (AR // 2), 8))
            return carry
        if only in ('', 'A') and upto >= 2:
            lax.fori_loop(0, NTA, abody, 0)

        if only == '' and upto >= 3:
            for c in c_w:
                c.wait()

        def rows_u32(ref, row0, M):
            if isinstance(row0, int):
                return _bf(ref[row0 // 2:(row0 + M) // 2, :])
            if isinstance(row0, tuple):
                return _bf(ref[pl.ds(row0[0] + row0[1] // 2, M // 2), :])
            return _bf(ref[pl.ds(pl.multiple_of(row0 // 2, 8), M // 2), :])

        def wo_dot(row0, M):
            o = rows_u32(o_scr, row0, M)
            return jnp.concatenate([_dot(o, _bf(wo_v[n])) for n in range(NCH)], axis=1)

        def row(k):
            return jnp.concatenate([modB[2 * (k - 2), 0:1, :], modB[2 * (k - 2) + 1, 0:1, :]], axis=1)

        def ln23(row0, M, A):
            ga = row(2); sb = row(3); cb = row(4)
            x = rows_u32(x_v, row0, M).astype(f32)
            xm = x + ga * A
            hB = _ln(xm) * (1.0 + cb) + sb
            n3 = _ln(hB).astype(bf16)
            return xm, hB, n3

        shifts = [-1, -1, 1, 1, -2, -2, 2, 2]

        def g_val():
            return jnp.concatenate(
                [h1buf[j, HALO + shifts[j]:HALO + shifts[j] + T, :] for j in range(NCH)], axis=1).astype(bf16)

        def out_copy(r0, n, k):
            return pltpu.make_async_copy(obuf.at[pl.ds(r0, n)], o_hbm.bitcast(u32).at[pl.ds(r0, n)], osems.at[k])

        def ln4(hs):
            gb = row(5)
            x1 = hb[0:T, :] + hs
            base = xmid[0:T, :] + gb * x1
            n4 = _ln(x1).astype(bf16)
            return base, n4

        def bfirst():
            for j in range(NCH):
                h1buf[j, 0:HALO, :] = jnp.zeros((HALO, 128), f32)
            if NTA * AR < 2 * T + HALO:
                attention(q0, k0, v0, 0, NTA * AR, 2 * T + HALO - NTA * AR, False)
            h0 = (T + HALO) // 2 // 16 * 16 + (16 if T == 128 else 0)
            halves = [(0, h0), (h0, T + HALO - h0)]
            As = [wo_dot(r0, m) for r0, m in halves]
            for (r0, m), A in zip(halves, As):
                xm, hB, n3 = ln23(r0, m, A)
                h1 = _gelu(_dot(n3, _bf(w1_v[...])))
                xmid[r0:r0 + m, :] = xm
                hb[r0:r0 + m, :] = hB
                for j in range(NCH):
                    h1buf[j, HALO + r0:HALO + r0 + m, :] = h1[:, j * 128:(j + 1) * 128]

            hsbuf[0:T, :] = _dot(g_val(), _bf(w2_v[...]))

        if only in ('', 'BF') and upto >= 3:
            bfirst()

        def carries(xm, hB, h1, notlast):
            xmid[0:HALO, :] = xmid[T:T + HALO, :]
            hb[0:HALO, :] = hb[T:T + HALO, :]
            for j in range(NCH):
                h1buf[j, 0:2 * HALO, :] = h1buf[j, T:T + 2 * HALO, :]
            xmid[HALO:HALO + T, :] = xm
            hb[HALO:HALO + T, :] = hB
            for j in range(NCH):
                h1j = h1[:, j * 128:(j + 1) * 128]
                h1buf[j, 2 * HALO:HALO + T, :] = h1j[0:T - HALO]
                h1buf[j, HALO + T:2 * HALO + T, :] = jnp.where(notlast, h1j[T - HALO:T], 0.0)

        RP = 16

        def bbody(i, carry):
            row0h = pl.multiple_of(i * (T // 2), T // 2)
            nxt = jnp.minimum(i + 1, NT - 1)
            abase = pl.multiple_of(nxt * T, T)
            abaseh = pl.multiple_of(nxt * (T // 2), T // 2)
            z1 = pl.multiple_of((i >> 8) * 8, 8)
            z2 = pl.multiple_of((i >> 9) * 8, 8)
            ga = row(2); sb = row(3); cb = row(4); gb = row(5)
            bases, n4p, xms, hBs, n3p, As = [], [], [], [], [], []

            def staged(key, ref, val):
                if key in stage:
                    ref[...] = pltpu.bitcast(val, u32)
                    return _bf(ref[...])
                if key.upper() in stage:
                    ref[pl.ds(z2, T // 2), :] = pltpu.bitcast(val, u32)
                    return _bf(ref[pl.ds(z2, T // 2), :])
                return val

            def p4(r):
                r0 = r * RP
                x1 = hb[r0:r0 + RP, :] + hsbuf[pl.ds(z2 + r0, RP), :]
                bases.append(xmid[r0:r0 + RP, :] + gb * x1)
                n4p.append(_ln(x1).astype(bf16))

            def p23(r, A):
                r0 = r * RP
                x = rows_u32(x_v, (row0h, HALO + r0), RP).astype(f32)
                xm = x + ga * A[r0:r0 + RP]
                hB = _ln(xm) * (1.0 + cb) + sb
                xms.append(xm); hBs.append(hB)
                n3p.append(_ln(hB).astype(bf16))

            for r in range(T // RP):
                if rel4[r] < 0:
                    p4(r)
            o = rows_u32(o_scr, (row0h, HALO), T)
            for n in range(NCH):
                An = _dot(o, _bf(wo_v[n]))
                As.append(An)
                r4 = [r for r in range(T // RP) if rel4[r] == n]
                if r4:
                    hsbuf[pl.ds(z1 + T, 8), 0:128] = An[0:8, 0:128]
                for r in r4:
                    p4(r)
            A = jnp.concatenate(As, axis=1)
            base = jnp.concatenate(bases, axis=0)
            n4 = jnp.concatenate(n4p, axis=0)
            n4 = staged('4', n4b, n4)
            U = _dot(n4, _bf(w3_v[...]))
            u = staged('u', ub, _gelu(U).astype(bf16))
            for c in range(F // 128):
                r23 = [r for r in range(T // RP) if rel23[r] == NCH + c]
                if r23:
                    x_v[pl.ds(z1 + S // 2 + HALO // 2, 8), 0:128] = pltpu.bitcast(U[0:8, c * 128:(c + 1) * 128], u32)
                for r in r23:
                    p23(r, A)
            assert len(n3p) == T // RP and len(n4p) == T // RP
            xm = jnp.concatenate(xms, axis=0)
            hB = jnp.concatenate(hBs, axis=0)
            n3 = staged('3', n3b, jnp.concatenate(n3p, axis=0))
            h1 = _gelu(_dot(n3, _bf(w1_v[...])))
            carries(xm, hB, h1, i < NT - 1)
            if 'noatt' not in dbg:
                attention(qbuf, kbuf, vbuf, abase, HALO, T, False, abaseh)
            h2 = _dot(u, _bf(w4_v[...]))
            obuf[pl.ds(pl.multiple_of((i - 1) * (T // 2), T // 2), T // 2), :] = pltpu.bitcast((base + gb * h2).astype(bf16), u32)
            hsbuf[0:T, :] = _dot(staged('g', gbf, g_val()), _bf(w2_v[...]))
            return carry

        if only in ('', 'B') and upto >= 4:
            lax.fori_loop(1, NT, bbody, 0)

        def blast():
            r0 = (NT - 1) * (T // 2)
            out_copy(0, r0, 0).start()
            base, n4 = ln4(hsbuf[0:T, :])
            u = _gelu(_dot(n4, _bf(w3_v[...]))).astype(bf16)
            h2 = _dot(u, _bf(w4_v[...]))
            obuf[r0:r0 + T // 2, :] = pltpu.bitcast((base + row(5) * h2).astype(bf16), u32)
            out_copy(r0, T // 2, 1).start()
            out_copy(0, r0, 0).wait()
            out_copy(r0, T // 2, 1).wait()

        if only in ('', 'BL') and upto >= 5:
            blast()

    @jax.jit
    def fn(A_x, A_wqkv, A_wo, B_x, B_w1, B_w2, B_w3, B_w4, c, w_mod):
        x = A_x.reshape(S, D)
        any_spec = pl.BlockSpec(memory_space=pl.ANY)
        out = pl.pallas_call(
            kernel,
            in_specs=[any_spec] * 9,
            out_specs=any_spec,
            out_shape=jax.ShapeDtypeStruct((S, D), bf16),
            scratch_shapes=[
                pltpu.VMEM((S // 2 + HALO // 2 + 8, D), u32),
                pltpu.VMEM((D // 2, 3 * D), u32),
                pltpu.VMEM((D // 2, D), u32),
                pltpu.VMEM((D // 2, D), u32),
                pltpu.VMEM((D // 2, D), u32),
                pltpu.VMEM((NCH, D // 2 + 32, 128), u32),
                pltpu.VMEM((NCH, D // 2, 128), u32),
                pltpu.VMEM((D // 2, D), u32),
                pltpu.VMEM((D // 2, D), u32),
                pltpu.VMEM((D // 2, F), u32),
                pltpu.VMEM((F // 2, D), u32),
                pltpu.VMEM((D // 2, 128), f32),
                pltpu.VMEM((D // 2, 128), f32),
                pltpu.VMEM((8, D // 2 + 16, 256), u32),
                pltpu.VMEM((8, D // 2 + 8, 512), u32),
                pltpu.VMEM((8, 8, 256), f32),
                pltpu.VMEM((8, 8, 512), f32),
                pltpu.VMEM((M0, 128), f32),
                pltpu.VMEM((M0, 128), f32),
                pltpu.VMEM((TA, D), f32),
                pltpu.VMEM((TA // 2, D), u32),
                pltpu.VMEM((M0 // 2, 128), u32),
                pltpu.VMEM((NCH, M0, 128), f32),
                pltpu.VMEM((NCH, M0 + HALO, 128), f32),
                pltpu.VMEM((NCH, M0 + HALO, 128), f32),
                pltpu.VMEM((NCH, S + HALO, 128), f32),
                pltpu.VMEM((NCH, S + 2 * HALO, 128), f32),
                pltpu.VMEM((NCH, S + 2 * HALO, 128), f32),
                pltpu.VMEM((T + HALO, D), f32),
                pltpu.VMEM((T + HALO, D), f32),
                pltpu.VMEM((NCH, T + 2 * HALO, 128), f32),
                pltpu.VMEM((S // 2, D), u32),
                pltpu.VMEM((S // 2 + HALO // 2, D), u32),
                pltpu.VMEM((T + 8, D), f32),
                pltpu.VMEM((T // 2, D), u32),
                pltpu.VMEM((T // 2, F), u32),
                pltpu.VMEM((T // 2, D), u32),
                pltpu.VMEM((T // 2, D), u32),
                pltpu.VMEM((1, D), bf16),
            ] + ([pltpu.VMEM((padr, 128), f32)] if padr else []) + [
                pltpu.SemaphoreType.DMA((57,)),
                pltpu.SemaphoreType.DMA((2,)),
            ],
            compiler_params=pltpu.CompilerParams(vmem_limit_bytes=120 * 1024 * 1024),
        )(x, A_wqkv, A_wo, B_w1, B_w2, B_w3, B_w4, c, w_mod)
        return out.reshape(1, S, D)
    return fn


_fn = make()


def pallas_adaLN_cond__sliding_local_dilated__mixer_s_mlp__prompt_kernel(A_x, A_wqkv, A_wo, B_x, B_w1, B_w2, B_w3, B_w4, c, w_mod):
    return _fn(A_x, A_wqkv, A_wo, B_x, B_w1, B_w2, B_w3, B_w4, c, w_mod)
```

```python
import functools
import jax
import jax.numpy as jnp
from jax import lax
import jax.experimental.pallas as pl
import jax.experimental.pallas.tpu as pltpu

S, D, F = 2048, 1024, 3584
H, DH, W, DIL = 32, 32, 8, 2
NCH = D // 128
EPS = 1e-5
SCALE = DH ** -0.5
f32, bf16, u32 = jnp.float32, jnp.bfloat16, jnp.uint32
HALO = 16


def _ln(x):
    m = jnp.mean(x, axis=-1, keepdims=True)
    xc = x - m
    v = jnp.mean(xc * xc, axis=-1, keepdims=True)
    return xc * lax.rsqrt(v + EPS)


def _gelu(x):
    c0 = 0.7978845608028654
    c1 = c0 * 0.044715
    t = jnp.tanh(x * (c0 + c1 * (x * x)))
    hx = 0.5 * x
    return hx + hx * t


def _dot(a, b):
    return jnp.dot(a, b, preferred_element_type=f32)


def _bf(w):
    return pltpu.bitcast(w, bf16)


def _lane_xor(x, s):
    lane = lax.broadcasted_iota(jnp.int32, x.shape, 1)
    return jnp.take_along_axis(x, lane ^ s, axis=1)


def _exchange8_multi(XS):
    XS = [list(X) for X in XS]
    lane = lax.broadcasted_iota(jnp.int32, XS[0][0].shape, 1)
    for t in range(3):
        s = 1 << (t + 2)
        m = (lane & s) != 0
        for X in XS:
            for p in range(8):
                if p & (1 << t):
                    continue
                p2 = p | (1 << t)
                tmp = _lane_xor(jnp.where(m, X[p], X[p2]), s)
                X[p], X[p2] = jnp.where(m, tmp, X[p]), jnp.where(m, X[p2], tmp)
    return XS


def _group4_sum(acc):
    lane = lax.broadcasted_iota(jnp.int32, acc.shape, 1)
    acc = acc + jnp.where((lane & 1) != 0, pltpu.roll(acc, 1, 1), pltpu.roll(acc, 127, 1))
    acc = acc + jnp.where((lane & 2) != 0, pltpu.roll(acc, 2, 1), pltpu.roll(acc, 126, 1))
    return acc


def make(T=128, PR=512, RB=8, EG=4, upto=9, AT0=0, AP=16,
         DO='c X0 Wq sa ca X1 Wk Wv X2 X3 X4 X5 X6 X7 X8 X9 X10 X11 X12 X13 X14 X15',
         PS=None, PSX=None, RL=1, D0='1234567', LP=16, BL=2, ZB=1,
         order0='T0 T1 x00 x01 m0 T2 T3 x10 x11 h0 T4 T5 x20 x21 H0 H1 H2 H3 H4 H5', NDEF=6, BA=None,
         side=None, KQ=4, KQ0=1, NM=5, NR=8, AG=1,
         rel4=(-1, -1, -1, 0, 1, 2, 3, 4), rel23=(8, 9, 10, 11, 12, 13, 14, 15),
         padr=0, dbg='', UB=0, BAR=()):
    NT = S // T
    NP = S // PR
    order0 = order0.split()
    TL = S - PR
    if PS is None:
        PS = ('wc C wX0 L0 wWq e0 wsa S wca A h0 wX1 u0:0 L1 wWk u1:0 e1 wWv u0:1 u1:1 e2 wX2 u0:2 u1:2 L2 u2:01 '
              'wX3 wX4 u2:2 L3 u3:012 L4 wX5 wX6 wX7 u4:012 L5 u5:012 L6 L7 u6:012 wX8 wX9 wX10 wX11 wX12 '
              'u7:012 L8 u8:012 L9 u9:012 L10 L11 L12 wX13 wX14 wX15 DW ua:012 L13 L14 L15 ub:012')
    if BA is None:
        BA = ('a0 a1 T0 T1 t0 a2 a3 W w0 w1 w2 w3 w4 w5 w6 w7 T2 t0 a4 a5 T3 t0 a6 a7 T4 t0 a8 a9 T5 t0 a10 o0 t0 a11 t4 a12 '
              'o1 t0 a13 t4 a14 M m0 m1 l0 l1 u0 t0 a15 t4 a16 u1')
    if PSX:
        for k_, v_ in PSX.items():
            assert (' ' + k_ + ' ') in PS
            PS = PS.replace(' ' + k_ + ' ', ' ' + k_ + ' ' + v_ + ' ')
    S_C, S_X, S_SA, S_CA, S_W0, S_WQ, S_WO, S_MB, S_W = 0, 1, 17, 25, 33, 36, 44, 52, 60
    NSEM = 64
    DEF = list(range(6 - NDEF, 6))
    tags = ['T%d' % sd for sd in DEF] + ['%dH%d' % (p, sd) for p in range(NP) for sd in range(6 if p < NP - 1 else 6 - NDEF)]
    if side is None:
        side = 'W:7,9,11,13,15,17,19,21 M:4,5,6,7,8,9,10,11,12,13,14,15,16,17,18,19,20,21,22,22'
    if isinstance(side, str):
        sd_ = {}
        for grp in side.split():
            kind, lst = grp.split(':')
            for k, t in enumerate(lst.split(',')):
                sd_.setdefault(tags[int(t)], []).append(kind + str(k))
        side = sd_
    assert sum(1 for v in side.values() for j in v if j[0] in 'Aa') * AP == AT0

    def kernel(x_hbm, wqkv_hbm, wo_hbm, w1_hbm, w2_hbm, w3_hbm, w4_hbm, c_hbm, wmod_hbm,
               o_hbm,
               x_v, wqkv_raw, wq_v, wk_v, wv_v, wo_raw, wo_v, w1_v, w2_v, w3_v, w4_v, cE, cO, wmA_v, wmB_v,
               modA, modB, xhat, hP, h0, qbuf, kbuf, vbuf, xmid, hb, h1buf, obuf, o_scr, hsbuf, n4b, c_v, *rest):
        zsm, sems, osems = rest[-3:]

        def cp(src, dst, k):
            return pltpu.make_async_copy(src, dst, sems.at[k])

        xu = x_hbm.bitcast(u32)
        wqkvu = wqkv_hbm.bitcast(u32)
        wou = wo_hbm.bitcast(u32)
        wmodu = wmod_hbm.bitcast(u32)

        def lane_ds(k, n, base=0):
            if isinstance(k, int):
                return pl.ds(base + k * n, n)
            return pl.ds(pl.multiple_of(base + k * n, 128), n)

        def row_ds(base, k, n):
            if isinstance(k, int):
                return pl.ds(base + k * n, n)
            return pl.ds(pl.multiple_of(base + k * n, 8), n)

        c_c = cp(c_hbm, c_v, S_C)

        def c_x(b):
            return cp(xu.at[b * 64:(b + 1) * 64], x_v.at[b * 64:(b + 1) * 64], S_X + b)

        def c_sa(k):
            return cp(wmodu.at[:, lane_ds(k, 128)], wmA_v.at[k, 0:D // 2, 0:128], S_SA + k)

        def c_ca(k):
            return cp(wmodu.at[:, lane_ds(k, 128, D)], wmA_v.at[k, 0:D // 2, 128:256], S_CA + k)

        def c_w0(b):
            return cp(wqkvu.at[0:64, b * D:(b + 1) * D], wqkv_raw.at[0:64, b * D:(b + 1) * D], S_W0 + b)

        def c_wq(k):
            return cp(wqkvu.at[row_ds(0, k, 64)], wqkv_raw.at[row_ds(0, k, 64)], S_WQ + k)

        def c_wo(p):
            return cp(wou.at[:, lane_ds(p, 128)], wo_raw.at[p, 8:8 + D // 2], S_WO + p)

        def c_mb(t, g):
            return cp(wmodu.at[:, lane_ds(t, 128, 2 * D)], wmB_v.at[t, 0:D // 2], S_MB + g)

        c_w = [cp(w1_hbm.bitcast(u32), w1_v, S_W), cp(w2_hbm.bitcast(u32), w2_v, S_W + 1),
               cp(w3_hbm.bitcast(u32), w3_v, S_W + 2), cp(w4_hbm.bitcast(u32), w4_v, S_W + 3)]

        def named(nm):
            if nm == 'c':
                return c_c
            if nm == 'sa':
                return c_sa(0)
            if nm == 'ca':
                return c_ca(0)
            if nm[0] == 'W':
                return c_w0('qkv'.index(nm[1]))
            return c_x(int(nm[1:]))

        for nm in DO.split():
            named(nm).start()
        def start_group(g):
            if g == 'W':
                if upto >= 3:
                    c_wo(7).start()
                    for t in range(6 * NM, 32):
                        c_mb(t, 6).start()
                    for c in c_w:
                        c.start()
            elif upto >= 2 and 'nodma2' not in dbg:
                r = int(g)
                c_sa(r).start()
                c_ca(r).start()
                c_wq(r).start()
                c_wo(r - 1).start()
                if r >= 2:
                    for i in range(NM):
                        c_mb(NM * (r - 2) + i, r - 2).start()

        for g in D0:
            start_group(g)
        assert sorted(list(D0) + [it[1] for it in PS.split() if it[0] == 'D']) == list('1234567W')

        def _zinit(i, carry):
            zsm[2 + i] = i >> 8
            return carry

        lax.fori_loop(0, 3, _zinit, 0)
        zp3 = pl.multiple_of(zsm[4] * 8, 8)
        zp1 = pl.multiple_of(zsm[2] * 8, 8)
        zp2 = pl.multiple_of(zsm[3] * 8, 8)

        x_v[S // 2:S // 2 + HALO // 2, :] = jnp.zeros((HALO // 2, D), u32)
        for j in range(NCH):
            z = jnp.zeros((HALO, 128), f32)
            qbuf[j, S:S + HALO, :] = z
            kbuf[j, HALO + S:2 * HALO + S, :] = z
            vbuf[j, HALO + S:2 * HALO + S, :] = z
            kbuf[j, 0:HALO, :] = z
            vbuf[j, 0:HALO, :] = z
            wo_raw[j, 0:8, :] = jnp.zeros((8, 128), u32)
            wo_raw[j, 8 + D // 2:16 + D // 2, :] = jnp.zeros((8, 128), u32)

        def mv_part(w, r0, acc):
            n = w.shape[0]
            lo = pltpu.bitcast(w << 16, f32)
            hi = pltpu.bitcast(w & jnp.uint32(0xFFFF0000), f32)
            pr = lo * cE[r0:r0 + n, :] + hi * cO[r0:r0 + n, :]
            for t in range(n // 8):
                acc = pr[8 * t:8 * t + 8] if acc is None else acc + pr[8 * t:8 * t + 8]
            return acc

        wparts = (wq_v, wk_v, wv_v)
        bufs = (qbuf, kbuf, vbuf)

        def exch_groups(grps):
            for g0 in range(0, len(grps), EG):
                gs = grps[g0:g0 + EG]
                XS = [[wqkv_raw[row_ds(rg * 8, k * 8, 8), b * D + a * 128:b * D + (a + 1) * 128] for a in range(NCH)]
                      for (k, b, rg) in gs]
                YS = _exchange8_multi(XS)
                for (k, b, rg), Y in zip(gs, YS):
                    wparts[b][row_ds(rg * 8, k * 8, 8), :] = jnp.concatenate(Y, axis=1)

        def subdot(lhs, row0, kc, sd, init=False, valid=None):
            b, hf = sd // 2, sd % 2
            n = lhs.shape[0]
            res = _dot(lhs, _bf(wparts[b][row_ds(0, kc, 64), hf * 512:(hf + 1) * 512]))
            o = row0 + (0 if b == 0 else HALO)
            for jj in range(4):
                j = hf * 4 + jj
                if init:
                    bufs[b][j, o:o + n, :] = res[:, jj * 128:(jj + 1) * 128]
                elif valid is not None:
                    bufs[b][j, o:o + n, :] = jnp.where(valid, bufs[b][j, o:o + n, :], 0.0) + res[:, jj * 128:(jj + 1) * 128]
                else:
                    bufs[b][j, o:o + n, :] += res[:, jj * 128:(jj + 1) * 128]
            return res

        def prologue():
            st = {}

            def crep():
                c = c_v[...].astype(f32)
                scf = (c * jax.nn.sigmoid(c)).astype(bf16).astype(f32)
                rr = lax.broadcasted_iota(jnp.int32, (128, 128), 0)
                ll = lax.broadcasted_iota(jnp.int32, (128, 128), 1)
                sel = ll == jnp.where(rr < 64, 2 * rr, 2 * rr - 127)
                for j in range(NCH):
                    dg = jnp.where(sel, jnp.broadcast_to(scf[:, j * 128:(j + 1) * 128], (128, 128)), 0.0).astype(bf16)
                    rep = _dot(dg, jnp.ones((128, 128), bf16))
                    cE[j * 64:(j + 1) * 64, :] = rep[0:64]
                    cO[j * 64:(j + 1) * 64, :] = rep[64:128]

            def h_store(r0, xh0):
                h = (xh0 * (1.0 + st['ca']) + st['sa']).astype(bf16)
                if r0 < TL:
                    h0[r0 // 2:(r0 + LP) // 2, :] = pltpu.bitcast(h, u32)
                else:
                    hP[(r0 - TL) // 2:(r0 - TL + LP) // 2, :] = pltpu.bitcast(h, u32)

            def ln_piece(b, i):
                r0 = b * 128 + i * LP
                if RL:
                    m = jnp.mean(_bf(x_v[pl.ds(zp1 + r0 // 2, LP // 2), :]).astype(f32), axis=-1, keepdims=True)
                    xc = _bf(x_v[pl.ds(zp2 + r0 // 2, LP // 2), :]).astype(f32) - m
                    v = jnp.mean(xc * xc, axis=-1, keepdims=True)
                    xh = (_bf(x_v[r0 // 2:(r0 + LP) // 2, :]).astype(f32) - m) * lax.rsqrt(v + EPS)
                else:
                    xh = _ln(_bf(x_v[pl.ds(zp1 + r0 // 2, LP // 2), :]).astype(f32))
                direct = 'ca' in st and 'sa' in st
                for j in range(1 if direct else 0, NCH):
                    xhat[j, r0:r0 + LP, :] = xh[:, j * 128:(j + 1) * 128]
                if direct:
                    h_store(r0, xh[:, 0:128])

            def ln_block(b):
                for i in range(128 // LP):
                    ln_piece(b, i)

            def hblk(b):
                for i in range(128 // LP):
                    r0 = b * 128 + i * LP
                    h_store(r0, xhat[0, r0:r0 + LP, :])

            for it in PS.split():
                if it[0] == 'w':
                    named(it[1:]).wait()
                elif it[0] == 'D':
                    start_group(it[1])
                elif it == 'C':
                    crep()
                elif it[0] == 'L':
                    ln_block(int(it[1:]))
                elif it[0] == 'h':
                    hblk(int(it[1:]))
                elif it == 'S':
                    st['sa'] = jnp.sum(mv_part(wmA_v[0, 0:D // 2, 0:128], 0, None), axis=0, keepdims=True)
                elif it == 'A':
                    st['ca'] = jnp.sum(mv_part(wmA_v[0, 0:D // 2, 128:256], 0, None), axis=0, keepdims=True)
                elif it[0] == 'e':
                    exch_groups([(0, int(it[1]), rg) for rg in range(8)])
                elif it[0] == 'p':
                    b_, i_ = it[1:].split(':')
                    ln_piece(int(b_), int(i_))
                elif it[0] == 't':
                    x_v[pl.ds(zp3 + S // 2 + HALO // 2, 8), 0:128] = pltpu.bitcast(st['res'][0:8, 0:128], u32)
                elif it[0] == 's':
                    blks, sd = it[1:].split(':')
                    b0, nb = int(blks[0], 16), len(blks)
                    st['res'] = subdot(_bf(h0[b0 * 64:(b0 + nb) * 64, :]), b0 * 128, 0, int(sd), True)
                elif it[0] == 'u':
                    blks, parts = it[1:].split(':')
                    b0, nb = int(blks[0], 16), len(blks)
                    lhs = _bf(h0[b0 * 64:(b0 + nb) * 64, :])
                    for p in parts:
                        subdot(lhs, b0 * 128, 0, 2 * int(p), True)
                        st['res'] = subdot(lhs, b0 * 128, 0, 2 * int(p) + 1, True)

        prologue()

        def attention(qb, kb, vb, base, off, M, mask_rows, baseh=None):
            row0 = base + off

            def kvds(r, w):
                return pl.ds(base + (off + HALO + r - DIL * w), RB)

            o_rows = []
            for r in range(0, M, RB):
                q = [qb[j, pl.ds(base + (off + r), RB), :] for j in range(NCH)]
                s = []
                for w in range(W):
                    acc = None
                    for j in range(NCH):
                        p = q[j] * kb[j, kvds(r, w), :]
                        acc = p if acc is None else acc + p
                    acc = _group4_sum(acc)
                    if mask_rows and off + r < DIL * (W - 1) and w > 0:
                        rows = row0 + r + lax.broadcasted_iota(jnp.int32, (RB, 128), 0)
                        acc = jnp.where(rows >= DIL * w, acc, -1e30)
                    s.append(acc)
                m = functools.reduce(jnp.maximum, s)
                e = [jnp.exp((sw - m) * SCALE) for sw in s]
                den = functools.reduce(lambda a, b: a + b, e)
                rinv = 1.0 / den
                oc = []
                for j in range(NCH):
                    acc = None
                    for w in range(W):
                        p = e[w] * vb[j, kvds(r, w), :]
                        acc = p if acc is None else acc + p
                    oc.append(acc * rinv)
                o_rows.append(jnp.concatenate(oc, axis=1))
            o = jnp.concatenate(o_rows, axis=0).astype(bf16)
            if isinstance(row0, int):
                o_scr[row0 // 2:(row0 + M) // 2, :] = pltpu.bitcast(o, u32)
            elif baseh is not None:
                o_scr[pl.ds(baseh + off // 2, M // 2), :] = pltpu.bitcast(o, u32)
            else:
                o_scr[pl.ds(pl.multiple_of(row0 // 2, 8), M // 2), :] = pltpu.bitcast(o, u32)


        def attention2(off, M, G):
            o_rows = []
            for r0 in range(0, M, RB * G):
                rs = [off + r0 + g * RB for g in range(G) if r0 + g * RB < M]
                lane = lax.broadcasted_iota(jnp.int32, (RB, 128), 1)
                S_ = {}
                for r in rs:
                    q = [qbuf[j, r:r + RB, :] for j in range(NCH)]
                    for w in range(W):
                        acc = None
                        for j in range(NCH):
                            k0 = HALO + r - DIL * w
                            p = q[j] * kbuf[j, k0:k0 + RB, :]
                            acc = p if acc is None else acc + p
                        S_[r, w] = acc
                keys = list(S_)
                for sh in (1, 2):
                    R = {k: (pltpu.roll(S_[k], sh, 1), pltpu.roll(S_[k], 128 - sh, 1)) for k in keys}
                    for k in keys:
                        S_[k] = S_[k] + jnp.where((lane & sh) != 0, R[k][0], R[k][1])
                for r in rs:
                    s = []
                    for w in range(W):
                        acc = S_[r, w]
                        if r < DIL * (W - 1) and w > 0:
                            rows = r + lax.broadcasted_iota(jnp.int32, (RB, 128), 0)
                            acc = jnp.where(rows >= DIL * w, acc, -1e30)
                        s.append(acc)
                    m = functools.reduce(jnp.maximum, s)
                    e = [jnp.exp((sw - m) * SCALE) for sw in s]
                    den = functools.reduce(lambda a, b: a + b, e)
                    rinv = 1.0 / den
                    oc = []
                    for j in range(NCH):
                        acc = None
                        for w in range(W):
                            k0 = HALO + r - DIL * w
                            p = e[w] * vbuf[j, k0:k0 + RB, :]
                            acc = p if acc is None else acc + p
                        oc.append(acc * rinv)
                    o_rows.append(jnp.concatenate(oc, axis=1))
            o = jnp.concatenate(o_rows, axis=0).astype(bf16)
            o_scr[off // 2:(off + M) // 2, :] = pltpu.bitcast(o, u32)
            return o

        sub = lax.broadcasted_iota(jnp.int32, (8, 128), 0)

        def pW(p, q, z):
            for tv in range(8 * q, 8 * q + 8):
                j = tv >> 3
                hh = (tv >> 1) & 3
                a2 = tv & 1
                parts = []
                for al in range(4):
                    a = a2 * 4 + al
                    src = a * 64 + hh * 16 + j * 2
                    st = src - 2 * al + 8
                    if isinstance(z, int):
                        parts.append(wo_raw[p, z + st:z + st + 8, :])
                    else:
                        parts.append(wo_raw[p, pl.ds(z + st, 8), :])
                v = jnp.where(sub < 2, parts[0], parts[1])
                v2 = jnp.where(sub < 6, parts[2], parts[3])
                wo_v[p, 8 * tv:8 * tv + 8, :] = jnp.where(sub < 4, v, v2)

        def pM(t, kq, z, macc, key):
            n = D // 2 // KQ
            rows = pl.ds(z + kq * n, n)
            macc[key] = mv_part(wmB_v[t, rows, :], kq * n, macc.get(key))
            if kq == KQ - 1:
                modB[t, 0:1, :] = jnp.sum(macc[key], axis=0, keepdims=True)

        def region_waits(r):
            c_sa(r).wait(); c_ca(r).wait(); c_wq(r).wait(); c_wo(r - 1).wait()

            @pl.when(r >= 2)
            def _():
                for i in range(NM):
                    c_mb(NM * (r - 2) + i, r - 2).wait()

        if 'prewait' in dbg:
            for r in range(1, 8):
                region_waits(r)

        def region(r, carry):
            if 'prewait' not in dbg and 'nodma2' not in dbg:
                region_waits(r)
            z1 = pl.multiple_of((r >> 8) * 8, 8)
            z2 = pl.multiple_of((r >> 9) * 8, 8)
            pm = [jnp.where(r >= 2, NM * (r - 2) + i, 32) for i in range(NM)]
            hp = _bf(hP[...])
            st = {'acc': [None, None], 'res': None}
            macc = {}

            def mvp(kq):
                n = D // 2 // KQ0
                for q in range(2):
                    st['acc'][q] = mv_part(wmA_v[r, pl.ds(z2 + kq * n, n), q * 128:(q + 1) * 128], kq * n, st['acc'][q])
                if kq == KQ0 - 1:
                    st['sa'] = jnp.sum(st['acc'][0], axis=0, keepdims=True)
                    st['ca'] = jnp.sum(st['acc'][1], axis=0, keepdims=True)
                    modA[r, 0:1, 0:128] = st['sa']
                    modA[r, 0:1, 128:256] = st['ca']

            def hpass(p):
                xh = xhat[r, p * PR:(p + 1) * PR, :]
                st['h'] = (xh * (1.0 + st['ca']) + st['sa']).astype(bf16)
                st['row'] = p * PR
                if p == NP - 1:
                    hP[...] = pltpu.bitcast(st['h'], u32)

            def do_side(tag):
                jobs = side.get(tag, ())
                if not jobs:
                    return
                tk = pltpu.bitcast(st['res'][0:8, 0:128], u32)
                kinds = set(j[0] for j in jobs)
                if 'W' in kinds:
                    wo_raw[r - 1, pl.ds(z1 + D // 2 + 16, 8), :] = tk
                if 'M' in kinds:
                    wmB_v[32, pl.ds(z1 + D // 2, 8), :] = tk
                if 'A' in kinds:
                    qbuf[0, pl.ds(z1 + S + HALO, 8), :] = pltpu.bitcast(tk, f32)
                for j in jobs:
                    k = int(j[1:])
                    if j[0] == 'W':
                        pW(r - 1, k, z2)
                    elif j[0] == 'w':
                        pW(r - 1, k, 0)
                    elif j[0] == 'M':
                        pM(pm[k // KQ], k % KQ, z2, macc, k // KQ)
                    elif j[0] in 'Aa':
                        attention(qbuf, kbuf, vbuf, 0, k * AP, AP, True)

            for it in order0:
                if it[0] == 'T':
                    st['res'] = subdot(hp, TL, r - 1, int(it[1]), valid=r >= 2)
                    do_side(it)
                elif it[0] == 'H':
                    st['res'] = subdot(st['h'], st['row'], r, int(it[1]))
                    do_side('0' + it)
                elif it[0] == 'm':
                    mvp(int(it[1]))
                elif it[0] == 'h':
                    hpass(int(it[1]))
                elif it[0] == 'x':
                    b, hf = int(it[1]), int(it[2])
                    exch_groups([(r, b, rg) for rg in range(4 * hf, 4 * hf + 4)])
            for p in range(1, NP):
                hpass(p)
                for sd in range(6 if p < NP - 1 else 6 - NDEF):
                    st['res'] = subdot(st['h'], st['row'], r, sd)
                    do_side('%dH%d' % (p, sd))
            zsm[0] = r >> 8
            zsm[1] = r >> 9
            return carry

        if upto >= 2:
            lax.fori_loop(1, NR, region, 0)
            zero = zsm[0]
            zero2 = zsm[1]

        if upto >= 3:
            c_wo(7).wait()
            for t in range(6 * NM, 32):
                c_mb(t, 6).wait()
            for c in c_w:
                c.wait()

        def rows_u32(ref, row0, M):
            if isinstance(row0, int):
                return _bf(ref[row0 // 2:(row0 + M) // 2, :])
            if isinstance(row0, tuple):
                return _bf(ref[pl.ds(row0[0] + row0[1] // 2, M // 2), :])
            return _bf(ref[pl.ds(pl.multiple_of(row0 // 2, 8), M // 2), :])

        def wo_dot(row0, M):
            o = rows_u32(o_scr, row0, M)
            return jnp.concatenate([_dot(o, _bf(wo_v[n])) for n in range(NCH)], axis=1)

        def row(k):
            return jnp.concatenate([modB[8 * (k - 2) + j, 0:1, :] for j in range(NCH)], axis=1)

        def ln23(row0, M, A):
            ga = row(2); sb = row(3); cb = row(4)
            x = rows_u32(x_v, row0, M).astype(f32)
            xm = x + ga * A
            hB = _ln(xm) * (1.0 + cb) + sb
            n3 = _ln(hB).astype(bf16)
            return xm, hB, n3

        shifts = [-1, -1, 1, 1, -2, -2, 2, 2]

        def g_val():
            return jnp.concatenate(
                [h1buf[j, HALO + shifts[j]:HALO + shifts[j] + T, :] for j in range(NCH)], axis=1).astype(bf16)

        def out_copy(r0, n, k):
            return pltpu.make_async_copy(obuf.at[pl.ds(r0, n)], o_hbm.bitcast(u32).at[pl.ds(r0, n)], osems.at[k])

        def ln4(hs):
            gb = row(5)
            x1 = hb[0:T, :] + hs
            base = xmid[0:T, :] + gb * x1
            n4 = _ln(x1).astype(bf16)
            return base, n4

        def bfirst():
            for j in range(NCH):
                h1buf[j, 0:HALO, :] = jnp.zeros((HALO, 128), f32)
            h7 = _bf(hP[...])
            zb = pl.multiple_of(zero * 8, 8) if ZB else 0
            h0 = (T + HALO) // 2 // 16 * 16 + (16 if T == 128 else 0)
            halves = [(0, h0), (h0, T + HALO - h0)]
            nA = (2 * T + HALO - AT0) // AP
            st = {'res': None, 'As': [], 'n3': [], 'h1': [], 'macc': {}}

            def att(k):
                if AG:
                    st['o'] = attention2(AT0 + k * AP, AP, AG)
                else:
                    attention(qbuf, kbuf, vbuf, 0, AT0 + k * AP, AP, True)

            def tok_q(cc=0):
                qbuf[0, pl.ds(zb + S + HALO, 8), :] = st['res'][0:8, cc * 128:(cc + 1) * 128]

            for it in BA.split():
                k = int(it[1:]) if len(it) > 1 and it[1:].isdigit() else None
                if not ZB and it[0] in 'tWM':
                    continue
                if it[0] == 'T':
                    st['res'] = subdot(h7, TL, 7, k)
                elif it[0] == 'a':
                    att(k)
                elif it[0] == 't':
                    tok_q(k or 0)
                elif it[0] == 'w':
                    pW(7, k, zb)
                elif it[0] == 'm':
                    for kq in range(KQ):
                        pM(6 * NM + k, kq, zb, st['macc'], k)
                elif it[0] == 'M':
                    wmB_v[32, pl.ds(zb + D // 2, 8), :] = pltpu.bitcast(st['res'][0:8, 0:128], u32)
                elif it[0] == 'W':
                    wo_raw[7, pl.ds(zb + D // 2 + 16, 8), :] = pltpu.bitcast(st['res'][0:8, 0:128], u32)
                elif it[0] == 'o':
                    st['res'] = wo_dot(*halves[k])
                    st['As'].append(st['res'])
                elif it[0] == 'l':
                    r0, m = halves[k]
                    xm, hB, n3 = ln23(r0, m, st['As'][k])
                    xmid[r0:r0 + m, :] = xm
                    hb[r0:r0 + m, :] = hB
                    st['n3'].append(n3)
                elif it[0] == 'u':
                    r0, m = halves[k]
                    st['res'] = _dot(st['n3'][k], _bf(w1_v[...]))
                    h1 = _gelu(st['res'])
                    for j in range(NCH):
                        h1buf[j, HALO + r0:HALO + r0 + m, :] = h1[:, j * 128:(j + 1) * 128]
            hsbuf[0:T, :] = _dot(g_val(), _bf(w2_v[...]))

        if upto >= 3:
            bfirst()

        def carries(xm, hB, h1, notlast):
            xmid[0:HALO, :] = xmid[T:T + HALO, :]
            hb[0:HALO, :] = hb[T:T + HALO, :]
            for j in range(NCH):
                h1buf[j, 0:2 * HALO, :] = h1buf[j, T:T + 2 * HALO, :]
            xmid[HALO:HALO + T, :] = xm
            hb[HALO:HALO + T, :] = hB
            for j in range(NCH):
                h1j = h1[:, j * 128:(j + 1) * 128]
                h1buf[j, 2 * HALO:HALO + T, :] = h1j[0:T - HALO]
                h1buf[j, HALO + T:2 * HALO + T, :] = jnp.where(notlast, h1j[T - HALO:T], 0.0)

        RP = 16

        def bbody(i, carry):
            static = isinstance(i, int)
            if static:
                row0h = i * (T // 2)
                abase = (i + 1) * T
                abaseh = (i + 1) * (T // 2)
                z1 = pl.multiple_of(zero * 8, 8)
                z2 = pl.multiple_of(zero2 * 8, 8)
            else:
                row0h = pl.multiple_of(i * (T // 2), T // 2)
                nxt = jnp.minimum(i + 1, NT - 1)
                abase = pl.multiple_of(nxt * T, T)
                abaseh = pl.multiple_of(nxt * (T // 2), T // 2)
                z1 = pl.multiple_of((i >> 8) * 8, 8)
                z2 = pl.multiple_of((i >> 9) * 8, 8)
            ga = row(2); sb = row(3); cb = row(4); gb = row(5)
            bases, n4p, xms, hBs, n3p, As = [], [], [], [], [], []

            def p4(r):
                r0 = r * RP
                x1 = hb[r0:r0 + RP, :] + hsbuf[pl.ds(z2 + r0, RP), :]
                bases.append(xmid[r0:r0 + RP, :] + gb * x1)
                n4p.append(_ln(x1).astype(bf16))

            def p23(r, A):
                r0 = r * RP
                x = rows_u32(x_v, (row0h, HALO + r0), RP).astype(f32)
                xm = x + ga * A[r0:r0 + RP]
                hB = _ln(xm) * (1.0 + cb) + sb
                xms.append(xm); hBs.append(hB)
                n3p.append(_ln(hB).astype(bf16))

            for r in range(T // RP):
                if rel4[r] < 0:
                    p4(r)
            o = rows_u32(o_scr, (row0h, HALO), T)
            for n in range(NCH):
                An = _dot(o, _bf(wo_v[n]))
                As.append(An)
                r4 = [r for r in range(T // RP) if rel4[r] == n]
                if r4:
                    hsbuf[pl.ds(z1 + T, 8), 0:128] = An[0:8, 0:128]
                for r in r4:
                    p4(r)
            A = jnp.concatenate(As, axis=1)
            base = jnp.concatenate(bases, axis=0)
            n4 = jnp.concatenate(n4p, axis=0)
            U = _dot(n4, _bf(w3_v[...]))
            u = _gelu(U).astype(bf16)
            for c in range(F // 128):
                r23 = [r for r in range(T // RP) if rel23[r] == NCH + c]
                if r23:
                    x_v[pl.ds(z1 + S // 2 + HALO // 2, 8), 0:128] = pltpu.bitcast(U[0:8, c * 128:(c + 1) * 128], u32)
                for r in r23:
                    p23(r, A)
            assert len(n3p) == T // RP and len(n4p) == T // RP
            xm = jnp.concatenate(xms, axis=0)
            hB = jnp.concatenate(hBs, axis=0)
            n3 = jnp.concatenate(n3p, axis=0)
            h1 = _gelu(_dot(n3, _bf(w1_v[...])))
            carries(xm, hB, h1, i < NT - 1)
            if static:
                if i < NT - 1:
                    attention(qbuf, kbuf, vbuf, abase, HALO, T, False, abaseh)
            elif 'noatt' not in dbg:
                attention(qbuf, kbuf, vbuf, abase, HALO, T, False, abaseh)
            h2 = _dot(u, _bf(w4_v[...]))
            if static:
                obuf[(i - 1) * (T // 2):i * (T // 2), :] = pltpu.bitcast((base + gb * h2).astype(bf16), u32)
            else:
                obuf[pl.ds(pl.multiple_of((i - 1) * (T // 2), T // 2), T // 2), :] = pltpu.bitcast((base + gb * h2).astype(bf16), u32)
            hsbuf[0:T, :] = _dot(g_val(), _bf(w2_v[...]))
            return carry

        if upto >= 4:
            if UB:
                for i in range(1, 1 + UB):
                    bbody(i, 0)
                    if i in BAR:
                        out_copy_i(i).start()
                if 1 + UB < NT:
                    lax.fori_loop(1 + UB, NT, bbody, 0)
            else:
                lax.fori_loop(1, NT, bbody, 0)

        def blast():
            r0 = (NT - 1) * (T // 2)
            out_copy(0, r0, 0).start()
            base, n4 = ln4(hsbuf[0:T, :])
            if BL:
                FC = F // BL
                xmid[0:T, :] = base
                n4b[...] = pltpu.bitcast(n4, u32)
                hsbuf[0:T, :] = jnp.zeros((T, D), f32)

                def body(c, carry):
                    w3c = w3_v[:, pl.ds(pl.multiple_of(c * FC, 128), FC)]
                    u = _gelu(_dot(_bf(n4b[...]), _bf(w3c))).astype(bf16)
                    w4c = w4_v[pl.ds(pl.multiple_of(c * (FC // 2), 32), FC // 2), :]
                    hsbuf[0:T, :] += _dot(u, _bf(w4c))
                    return carry

                lax.fori_loop(0, BL, body, 0)
                obuf[r0:r0 + T // 2, :] = pltpu.bitcast((xmid[0:T, :] + row(5) * hsbuf[0:T, :]).astype(bf16), u32)
            else:
                u = _gelu(_dot(n4, _bf(w3_v[...]))).astype(bf16)
                h2 = _dot(u, _bf(w4_v[...]))
                obuf[r0:r0 + T // 2, :] = pltpu.bitcast((base + row(5) * h2).astype(bf16), u32)
            out_copy(r0, T // 2, 1).start()
            out_copy(0, r0, 0).wait()
            out_copy(r0, T // 2, 1).wait()

        if upto >= 5:
            blast()

    @jax.jit
    def fn(A_x, A_wqkv, A_wo, B_x, B_w1, B_w2, B_w3, B_w4, c, w_mod):
        x = A_x.reshape(S, D)
        any_spec = pl.BlockSpec(memory_space=pl.ANY)
        out = pl.pallas_call(
            kernel,
            in_specs=[any_spec] * 9,
            out_specs=any_spec,
            out_shape=jax.ShapeDtypeStruct((S, D), bf16),
            scratch_shapes=[
                pltpu.VMEM((S // 2 + HALO // 2 + 8, D), u32),
                pltpu.VMEM((D // 2, 3 * D), u32),
                pltpu.VMEM((D // 2, D), u32),
                pltpu.VMEM((D // 2, D), u32),
                pltpu.VMEM((D // 2, D), u32),
                pltpu.VMEM((NCH, D // 2 + 32, 128), u32),
                pltpu.VMEM((NCH, D // 2, 128), u32),
                pltpu.VMEM((D // 2, D), u32),
                pltpu.VMEM((D // 2, D), u32),
                pltpu.VMEM((D // 2, F), u32),
                pltpu.VMEM((F // 2, D), u32),
                pltpu.VMEM((D // 2, 128), f32),
                pltpu.VMEM((D // 2, 128), f32),
                pltpu.VMEM((8, D // 2 + 16, 256), u32),
                pltpu.VMEM((33, D // 2 + 32, 128), u32),
                pltpu.VMEM((8, 8, 256), f32),
                pltpu.VMEM((36, 8, 128), f32),
                pltpu.VMEM((NCH, S + 32, 128), f32),
                pltpu.VMEM((PR // 2, 128), u32),
                pltpu.VMEM((S // 2, 128), u32),
                pltpu.VMEM((NCH, S + 32, 128), f32),
                pltpu.VMEM((NCH, S + 2 * HALO, 128), f32),
                pltpu.VMEM((NCH, S + 2 * HALO, 128), f32),
                pltpu.VMEM((T + HALO, D), f32),
                pltpu.VMEM((T + HALO, D), f32),
                pltpu.VMEM((NCH, T + 2 * HALO, 128), f32),
                pltpu.VMEM((S // 2, D), u32),
                pltpu.VMEM((S // 2 + HALO // 2, D), u32),
                pltpu.VMEM((T + 32, D), f32),
                pltpu.VMEM((T // 2, D), u32),
                pltpu.VMEM((1, D), bf16),
            ] + ([pltpu.VMEM((padr, 128), f32)] if padr else []) + [
                pltpu.SMEM((8,), jnp.int32),
                pltpu.SemaphoreType.DMA((NSEM,)),
                pltpu.SemaphoreType.DMA((2,)),
            ],
            compiler_params=pltpu.CompilerParams(vmem_limit_bytes=120 * 1024 * 1024),
        )(x, A_wqkv, A_wo, B_w1, B_w2, B_w3, B_w4, c, w_mod)
        return out.reshape(1, S, D)
    return fn


_fn = make()


def pallas_adaLN_cond__sliding_local_dilated__mixer_s_mlp__prompt_kernel(A_x, A_wqkv, A_wo, B_x, B_w1, B_w2, B_w3, B_w4, c, w_mod):
    return _fn(A_x, A_wqkv, A_wo, B_x, B_w1, B_w2, B_w3, B_w4, c, w_mod)
```

```python
import functools
import jax
import jax.numpy as jnp
from jax import lax
import jax.experimental.pallas as pl
import jax.experimental.pallas.tpu as pltpu

S, D, F = 2048, 1024, 3584
H, DH, W, DIL = 32, 32, 8, 2
NCH = D // 128
EPS = 1e-5
SCALE = DH ** -0.5
f32, bf16, u32 = jnp.float32, jnp.bfloat16, jnp.uint32
HALO = 16


def _ln(x):
    m = jnp.mean(x, axis=-1, keepdims=True)
    xc = x - m
    v = jnp.mean(xc * xc, axis=-1, keepdims=True)
    return xc * lax.rsqrt(v + EPS)


def _gelu(x):
    c0 = 0.7978845608028654
    c1 = c0 * 0.044715
    t = jnp.tanh(x * (c0 + c1 * (x * x)))
    hx = 0.5 * x
    return hx + hx * t


def _dot(a, b):
    return jnp.dot(a, b, preferred_element_type=f32)


def _bf(w):
    return pltpu.bitcast(w, bf16)


def _lane_xor(x, s):
    lane = lax.broadcasted_iota(jnp.int32, x.shape, 1)
    return jnp.take_along_axis(x, lane ^ s, axis=1)


def _exchange8_multi(XS):
    XS = [list(X) for X in XS]
    lane = lax.broadcasted_iota(jnp.int32, XS[0][0].shape, 1)
    for t in range(3):
        s = 1 << (t + 2)
        m = (lane & s) != 0
        for X in XS:
            for p in range(8):
                if p & (1 << t):
                    continue
                p2 = p | (1 << t)
                tmp = _lane_xor(jnp.where(m, X[p], X[p2]), s)
                X[p], X[p2] = jnp.where(m, tmp, X[p]), jnp.where(m, X[p2], tmp)
    return XS


def _group4_sum(acc):
    lane = lax.broadcasted_iota(jnp.int32, acc.shape, 1)
    acc = acc + jnp.where((lane & 1) != 0, pltpu.roll(acc, 1, 1), pltpu.roll(acc, 127, 1))
    acc = acc + jnp.where((lane & 2) != 0, pltpu.roll(acc, 2, 1), pltpu.roll(acc, 126, 1))
    return acc


def make(T=128, PR=512, RB=8, EG=4, upto=9, AT0=0, AP=16,
         DO='c X0 Wq sa ca X1 Wk Wv X2 X3 X4 X5 X6 X7 X8 X9 X10 X12 X13 X11 X14 X15',
         PS=None, PSX=None, RL=1, D0='1234567', LP=16, BL=2, ZB=1,
         order0='T0 T1 X x00 x01 m0 T2 T3 X x10 x11 h0 T4 T5 X x20 H0 X x21 H1 H2 H3 H4 H5', NDEF=6, BA=None,
         side=None, KQ=4, KQ0=1, NM=5, NR=8, AG=1,
         rel4=(-1, -1, -1, 0, 1, 2, 3, 4), rel23=(8, 9, 10, 11, 12, 13, 14, 15),
         padr=0, dbg='', UB=0, BAR=(), GL=0, MU=1, WS=1):
    HS, HO = (2, 0) if MU else (0, S // 2)
    NT = S // T
    NP = S // PR
    order0 = order0.split()
    TL = S - PR
    if PS is None:
        PS = ('wc C wX0 L0 wWq e0 wsa S wca A h0 wX1 u0:0 L1 wWk u1:0 e1 wWv u0:1 u1:1 e2 wX2 u0:2 u1:2 L2 u2:0 '
              'wX3 wX4 u2:12 L3 u3:012 L4 u4:0 wX5 wX6 wX7 u4:12 L5 u5:012 L6 u6:012 L7 u7:0 '
              'wX8 wX9 wX10 wX12 wX13 u7:12 L8 u8:012 L9 u9:012 L10 ua:0 L12 L13 wX11 wX14 wX15 DW ua:12 L11 ub:012 L14 L15')
    if BA is None:
        BA = ('a0 a1 T0 T1 t0 a2 a3 W w0 w1 w2 w3 w4 w5 w6 w7 T2 t0 a4 a5 T3 t0 a6 a7 T4 t0 a8 a9 T5 t0 a10 o0 t0 a11 t4 a12 '
              'o1 t0 a13 t4 a14 M m0 m1 l0 l1 u0 t0 a15 t4 a16 u1')
    if WS and 'v0' not in BA:
        BA = BA.replace('W w0 w1 w2 w3 w4 w5 w6 w7', 'W v0 v1 v2 v3 v4 v5 v6 v7 w0 w1 w2 w3 w4 w5 w6 w7')
    if PSX:
        for k_, v_ in PSX.items():
            assert (' ' + k_ + ' ') in PS
            PS = PS.replace(' ' + k_ + ' ', ' ' + k_ + ' ' + v_ + ' ')
    S_C, S_X, S_SA, S_CA, S_W0, S_WQ, S_WO, S_MB, S_W = 0, 1, 17, 25, 33, 36, 44, 52, 60
    NSEM = 64
    DEF = list(range(6 - NDEF, 6))
    tags = ['T%d' % sd for sd in DEF] + ['%dH%d' % (p, sd) for p in range(NP) for sd in range(6 if p < NP - 1 else 6 - NDEF)]
    if side is None:
        side = 'W:7,9,11,13,15,17,19,21 M:4,5,6,7,8,9,10,11,12,13,14,15,16,17,18,19,20,21,22,22'
    if isinstance(side, str):
        sd_ = {}
        for grp in side.split():
            kind, lst = grp.split(':')
            for k, t in enumerate(lst.split(',')):
                sd_.setdefault(tags[int(t)], []).append(kind + str(k))
        side = sd_
    assert sum(1 for v in side.values() for j in v if j[0] in 'Aa') * AP == AT0

    def kernel(x_hbm, wqkv_hbm, wo_hbm, w1_hbm, w2_hbm, w3_hbm, w4_hbm, c_hbm, wmod_hbm,
               o_hbm,
               x_v, wqkv_raw, wq_v, wk_v, wv_v, wo_raw, wo_v, w1_v, w2_v, w3_v, w4_v, cE, cO, wmA_v, wmB_v,
               modA, modB, xhat, hP, h0, qbuf, kbuf, vbuf, xmid, hb, h1buf, obuf, o_scr, hsbuf, n4b, c_v, *rest):
        zsm, sems, osems = rest[-3:]

        def cp(src, dst, k):
            return pltpu.make_async_copy(src, dst, sems.at[k])

        xu = x_hbm.bitcast(u32)
        wqkvu = wqkv_hbm.bitcast(u32)
        wou = wo_hbm.bitcast(u32)
        wmodu = wmod_hbm.bitcast(u32)

        def lane_ds(k, n, base=0):
            if isinstance(k, int):
                return pl.ds(base + k * n, n)
            return pl.ds(pl.multiple_of(base + k * n, 128), n)

        def row_ds(base, k, n):
            if isinstance(k, int):
                return pl.ds(base + k * n, n)
            return pl.ds(pl.multiple_of(base + k * n, 8), n)

        c_c = cp(c_hbm, c_v, S_C)

        def c_x(b):
            return cp(xu.at[b * 64:(b + 1) * 64], x_v.at[b * 64:(b + 1) * 64], S_X + b)

        def c_sa(k):
            return cp(wmodu.at[:, lane_ds(k, 128)], wmA_v.at[k, 0:D // 2, 0:128], S_SA + k)

        def c_ca(k):
            return cp(wmodu.at[:, lane_ds(k, 128, D)], wmA_v.at[k, 0:D // 2, 128:256], S_CA + k)

        def c_w0(b):
            return cp(wqkvu.at[0:64, b * D:(b + 1) * D], wqkv_raw.at[0:64, b * D:(b + 1) * D], S_W0 + b)

        def c_wq(k):
            return cp(wqkvu.at[row_ds(0, k, 64)], wqkv_raw.at[row_ds(0, k, 64)], S_WQ + k)

        def c_wo(p):
            return cp(wou.at[:, lane_ds(p, 128)], wo_raw.at[p, 8:8 + D // 2], S_WO + p)

        def c_mb(t, g):
            return cp(wmodu.at[:, lane_ds(t, 128, 2 * D)], wmB_v.at[t, 0:D // 2], S_MB + g)

        c_w = [cp(w1_hbm.bitcast(u32), w1_v, S_W), cp(w2_hbm.bitcast(u32), w2_v, S_W + 1),
               cp(w3_hbm.bitcast(u32), w3_v, S_W + 2), cp(w4_hbm.bitcast(u32), w4_v, S_W + 3)]

        def named(nm):
            if nm == 'c':
                return c_c
            if nm == 'sa':
                return c_sa(0)
            if nm == 'ca':
                return c_ca(0)
            if nm[0] == 'W':
                return c_w0('qkv'.index(nm[1]))
            return c_x(int(nm[1:]))

        for nm in DO.split():
            named(nm).start()
        def start_group(g):
            if g == 'W':
                if upto >= 3:
                    c_wo(7).start()
                    for t in range(6 * NM, 32):
                        c_mb(t, 6).start()
                    for c in c_w:
                        c.start()
            elif upto >= 2 and 'nodma2' not in dbg:
                r = int(g)
                c_sa(r).start()
                c_ca(r).start()
                c_wq(r).start()
                c_wo(r - 1).start()
                if r >= 2:
                    for i in range(NM):
                        c_mb(NM * (r - 2) + i, r - 2).start()

        for g in D0:
            start_group(g)
        assert sorted(list(D0) + [it[1] for it in PS.split() if it[0] == 'D']) == list('1234567W')

        def _zinit(i, carry):
            zsm[2 + i] = i >> 8
            return carry

        lax.fori_loop(0, 3, _zinit, 0)
        zp3 = pl.multiple_of(zsm[4] * 8, 8)
        zp1 = pl.multiple_of(zsm[2] * 8, 8)
        zp2 = pl.multiple_of(zsm[3] * 8, 8)

        x_v[S // 2:S // 2 + HALO // 2, :] = jnp.zeros((HALO // 2, D), u32)
        for j in range(NCH):
            z = jnp.zeros((HALO, 128), f32)
            qbuf[j, S:S + HALO, :] = z
            kbuf[j, HALO + S:2 * HALO + S, :] = z
            vbuf[j, HALO + S:2 * HALO + S, :] = z
            kbuf[j, 0:HALO, :] = z
            vbuf[j, 0:HALO, :] = z
            wo_raw[j, 0:8, :] = jnp.zeros((8, 128), u32)
            wo_raw[j, 8 + D // 2:16 + D // 2, :] = jnp.zeros((8, 128), u32)

        def mv_part(w, r0, acc):
            n = w.shape[0]
            lo = pltpu.bitcast(w << 16, f32)
            hi = pltpu.bitcast(w & jnp.uint32(0xFFFF0000), f32)
            pr = lo * cE[r0:r0 + n, :] + hi * cO[r0:r0 + n, :]
            for t in range(n // 8):
                acc = pr[8 * t:8 * t + 8] if acc is None else acc + pr[8 * t:8 * t + 8]
            return acc

        wparts = (wq_v, wk_v, wv_v)
        bufs = (qbuf, kbuf, vbuf)

        def exch_groups(grps):
            for g0 in range(0, len(grps), EG):
                gs = grps[g0:g0 + EG]
                XS = [[wqkv_raw[row_ds(rg * 8, k * 8, 8), b * D + a * 128:b * D + (a + 1) * 128] for a in range(NCH)]
                      for (k, b, rg) in gs]
                YS = _exchange8_multi(XS)
                for (k, b, rg), Y in zip(gs, YS):
                    wparts[b][row_ds(rg * 8, k * 8, 8), :] = jnp.concatenate(Y, axis=1)

        def subdot(lhs, row0, kc, sd, init=False, valid=None):
            b, hf = sd // 2, sd % 2
            n = lhs.shape[0]
            res = _dot(lhs, _bf(wparts[b][row_ds(0, kc, 64), hf * 512:(hf + 1) * 512]))
            o = row0 + (0 if b == 0 else HALO)
            for jj in range(4):
                j = hf * 4 + jj
                if init:
                    bufs[b][j, o:o + n, :] = res[:, jj * 128:(jj + 1) * 128]
                elif valid is not None:
                    bufs[b][j, o:o + n, :] = jnp.where(valid, bufs[b][j, o:o + n, :], 0.0) + res[:, jj * 128:(jj + 1) * 128]
                else:
                    bufs[b][j, o:o + n, :] += res[:, jj * 128:(jj + 1) * 128]
            return res

        def prologue():
            st = {}

            def crep():
                c = c_v[...].astype(f32)
                scf = (c * jax.nn.sigmoid(c)).astype(bf16).astype(f32)
                rr = lax.broadcasted_iota(jnp.int32, (128, 128), 0)
                ll = lax.broadcasted_iota(jnp.int32, (128, 128), 1)
                sel = ll == jnp.where(rr < 64, 2 * rr, 2 * rr - 127)
                for j in range(NCH):
                    dg = jnp.where(sel, jnp.broadcast_to(scf[:, j * 128:(j + 1) * 128], (128, 128)), 0.0).astype(bf16)
                    rep = _dot(dg, jnp.ones((128, 128), bf16))
                    cE[j * 64:(j + 1) * 64, :] = rep[0:64]
                    cO[j * 64:(j + 1) * 64, :] = rep[64:128]

            def h_store(r0, xh0):
                h = (xh0 * (1.0 + st['ca']) + st['sa']).astype(bf16)
                if r0 < TL:
                    xhat[HS, HO + r0 // 2:HO + (r0 + LP) // 2, :] = pltpu.bitcast(h, f32)
                else:
                    hP[(r0 - TL) // 2:(r0 - TL + LP) // 2, :] = pltpu.bitcast(h, u32)

            def h0_lhs(b0, nb, gated):
                r0 = HO + b0 * 64
                if not gated:
                    return _bf(xhat[HS, r0:r0 + nb * 64, :])
                if GL:
                    return jnp.concatenate([_bf(xhat[HS, r0:r0 + nb * 64 - 8, :]), _bf(xhat[HS, pl.ds(zp3 + r0 + nb * 64 - 8, 8), :])], axis=0)
                return jnp.concatenate([_bf(xhat[HS, pl.ds(zp3 + r0, 8), :]), _bf(xhat[HS, r0 + 8:r0 + nb * 64, :])], axis=0)

            def ln_piece(b, i):
                r0 = b * 128 + i * LP
                direct = 'ca' in st and 'sa' in st
                if MU:
                    x = _bf(x_v[pl.ds(zp1 + r0 // 2, LP // 2), :]).astype(f32)
                    m = jnp.mean(x, axis=-1, keepdims=True)
                    if RL:
                        x = _bf(x_v[pl.ds(zp2 + r0 // 2, LP // 2), :]).astype(f32)
                    xc = x - m
                    rs = lax.rsqrt(jnp.mean(xc * xc, axis=-1, keepdims=True) + EPS)
                    xhat[0, r0:r0 + LP, :] = jnp.broadcast_to(m, (LP, 128))
                    xhat[1, r0:r0 + LP, :] = jnp.broadcast_to(rs, (LP, 128))
                    if direct:
                        h_store(r0, xc[:, 0:128] * rs)
                    return
                if RL:
                    m = jnp.mean(_bf(x_v[pl.ds(zp1 + r0 // 2, LP // 2), :]).astype(f32), axis=-1, keepdims=True)
                    xc = _bf(x_v[pl.ds(zp2 + r0 // 2, LP // 2), :]).astype(f32) - m
                    v = jnp.mean(xc * xc, axis=-1, keepdims=True)
                    xh = (_bf(x_v[r0 // 2:(r0 + LP) // 2, :]).astype(f32) - m) * lax.rsqrt(v + EPS)
                else:
                    xh = _ln(_bf(x_v[pl.ds(zp1 + r0 // 2, LP // 2), :]).astype(f32))
                for j in range(1 if direct else 0, NCH):
                    xhat[j, r0:r0 + LP, :] = xh[:, j * 128:(j + 1) * 128]
                if direct:
                    h_store(r0, xh[:, 0:128])

            def ln_block(b):
                for i in range(128 // LP):
                    ln_piece(b, i)

            def hblk(b):
                for i in range(128 // LP):
                    r0 = b * 128 + i * LP
                    if MU:
                        x = _bf(x_v[r0 // 2:(r0 + LP) // 2, 0:128]).astype(f32)
                        h_store(r0, (x - xhat[0, r0:r0 + LP, :]) * xhat[1, r0:r0 + LP, :])
                    else:
                        h_store(r0, xhat[0, r0:r0 + LP, :])

            for it in PS.split():
                if it[0] == 'w':
                    named(it[1:]).wait()
                elif it[0] == 'D':
                    start_group(it[1])
                elif it == 'C':
                    crep()
                elif it[0] == 'L':
                    ln_block(int(it[1:]))
                elif it[0] == 'h':
                    hblk(int(it[1:]))
                elif it == 'S':
                    st['sa'] = jnp.sum(mv_part(wmA_v[0, 0:D // 2, 0:128], 0, None), axis=0, keepdims=True)
                elif it == 'A':
                    st['ca'] = jnp.sum(mv_part(wmA_v[0, 0:D // 2, 128:256], 0, None), axis=0, keepdims=True)
                elif it[0] == 'e':
                    exch_groups([(0, int(it[1]), rg) for rg in range(8)])
                elif it[0] == 'p':
                    b_, i_ = it[1:].split(':')
                    ln_piece(int(b_), int(i_))
                elif it[0] == 't':
                    x_v[pl.ds(zp3 + S // 2 + HALO // 2, 8), 0:128] = pltpu.bitcast(st['res'][0:8, 0:128], u32)
                elif it[0] in 'sg':
                    blks, sd = it[1:].split(':')
                    b0, nb = int(blks[0], 16), len(blks)
                    st['res'] = subdot(h0_lhs(b0, nb, it[0] == 'g'), b0 * 128, 0, int(sd), True)
                elif it[0] == 'u':
                    blks, parts = it[1:].split(':')
                    b0, nb = int(blks[0], 16), len(blks)
                    lhs = h0_lhs(b0, nb, False)
                    for p in parts:
                        subdot(lhs, b0 * 128, 0, 2 * int(p), True)
                        st['res'] = subdot(lhs, b0 * 128, 0, 2 * int(p) + 1, True)

        prologue()

        def attention(qb, kb, vb, base, off, M, mask_rows, baseh=None):
            row0 = base + off

            def kvds(r, w):
                return pl.ds(base + (off + HALO + r - DIL * w), RB)

            o_rows = []
            for r in range(0, M, RB):
                q = [qb[j, pl.ds(base + (off + r), RB), :] for j in range(NCH)]
                s = []
                for w in range(W):
                    acc = None
                    for j in range(NCH):
                        p = q[j] * kb[j, kvds(r, w), :]
                        acc = p if acc is None else acc + p
                    acc = _group4_sum(acc)
                    if mask_rows and off + r < DIL * (W - 1) and w > 0:
                        rows = row0 + r + lax.broadcasted_iota(jnp.int32, (RB, 128), 0)
                        acc = jnp.where(rows >= DIL * w, acc, -1e30)
                    s.append(acc)
                m = functools.reduce(jnp.maximum, s)
                e = [jnp.exp((sw - m) * SCALE) for sw in s]
                den = functools.reduce(lambda a, b: a + b, e)
                rinv = 1.0 / den
                oc = []
                for j in range(NCH):
                    acc = None
                    for w in range(W):
                        p = e[w] * vb[j, kvds(r, w), :]
                        acc = p if acc is None else acc + p
                    oc.append(acc * rinv)
                o_rows.append(jnp.concatenate(oc, axis=1))
            o = jnp.concatenate(o_rows, axis=0).astype(bf16)
            if isinstance(row0, int):
                o_scr[row0 // 2:(row0 + M) // 2, :] = pltpu.bitcast(o, u32)
            elif baseh is not None:
                o_scr[pl.ds(baseh + off // 2, M // 2), :] = pltpu.bitcast(o, u32)
            else:
                o_scr[pl.ds(pl.multiple_of(row0 // 2, 8), M // 2), :] = pltpu.bitcast(o, u32)


        def attention2(off, M, G):
            o_rows = []
            for r0 in range(0, M, RB * G):
                rs = [off + r0 + g * RB for g in range(G) if r0 + g * RB < M]
                lane = lax.broadcasted_iota(jnp.int32, (RB, 128), 1)
                S_ = {}
                for r in rs:
                    q = [qbuf[j, r:r + RB, :] for j in range(NCH)]
                    for w in range(W):
                        acc = None
                        for j in range(NCH):
                            k0 = HALO + r - DIL * w
                            p = q[j] * kbuf[j, k0:k0 + RB, :]
                            acc = p if acc is None else acc + p
                        S_[r, w] = acc
                keys = list(S_)
                for sh in (1, 2):
                    R = {k: (pltpu.roll(S_[k], sh, 1), pltpu.roll(S_[k], 128 - sh, 1)) for k in keys}
                    for k in keys:
                        S_[k] = S_[k] + jnp.where((lane & sh) != 0, R[k][0], R[k][1])
                for r in rs:
                    s = []
                    for w in range(W):
                        acc = S_[r, w]
                        if r < DIL * (W - 1) and w > 0:
                            rows = r + lax.broadcasted_iota(jnp.int32, (RB, 128), 0)
                            acc = jnp.where(rows >= DIL * w, acc, -1e30)
                        s.append(acc)
                    m = functools.reduce(jnp.maximum, s)
                    e = [jnp.exp((sw - m) * SCALE) for sw in s]
                    den = functools.reduce(lambda a, b: a + b, e)
                    rinv = 1.0 / den
                    oc = []
                    for j in range(NCH):
                        acc = None
                        for w in range(W):
                            k0 = HALO + r - DIL * w
                            p = e[w] * vbuf[j, k0:k0 + RB, :]
                            acc = p if acc is None else acc + p
                        oc.append(acc * rinv)
                    o_rows.append(jnp.concatenate(oc, axis=1))
            o = jnp.concatenate(o_rows, axis=0).astype(bf16)
            o_scr[off // 2:(off + M) // 2, :] = pltpu.bitcast(o, u32)
            return o

        sub = lax.broadcasted_iota(jnp.int32, (8, 128), 0)

        def pW(p, q, z):
            for tv in range(8 * q, 8 * q + 8):
                j = tv >> 3
                hh = (tv >> 1) & 3
                a2 = tv & 1
                parts = []
                for al in range(4):
                    a = a2 * 4 + al
                    src = a * 64 + hh * 16 + j * 2
                    st = src - 2 * al + 8
                    if isinstance(z, int):
                        parts.append(wo_raw[p, z + st:z + st + 8, :])
                    else:
                        parts.append(wo_raw[p, pl.ds(z + st, 8), :])
                v = jnp.where(sub < 2, parts[0], parts[1])
                v2 = jnp.where(sub < 6, parts[2], parts[3])
                wo_v[p, 8 * tv:8 * tv + 8, :] = jnp.where(sub < 4, v, v2)

        def pM(t, kq, z, macc, key):
            n = D // 2 // KQ
            rows = pl.ds(z + kq * n, n)
            macc[key] = mv_part(wmB_v[t, rows, :], kq * n, macc.get(key))
            if kq == KQ - 1:
                modB[t, 0:1, :] = jnp.sum(macc[key], axis=0, keepdims=True)

        def region_waits(r):
            c_sa(r).wait(); c_ca(r).wait(); c_wq(r).wait()
            if not WS:
                c_wo(r - 1).wait()

            @pl.when(r >= 2)
            def _():
                if WS:
                    c_wo(r - 2).wait()
                for i in range(NM):
                    c_mb(NM * (r - 2) + i, r - 2).wait()

        if 'prewait' in dbg:
            for r in range(1, 8):
                region_waits(r)

        def region(r, carry):
            if 'prewait' not in dbg and 'nodma2' not in dbg:
                region_waits(r)
            z1 = pl.multiple_of((r >> 8) * 8, 8)
            z2 = pl.multiple_of((r >> 9) * 8, 8)
            pm = [jnp.where(r >= 2, NM * (r - 2) + i, 32) for i in range(NM)]
            pw = jnp.where(r >= 2, r - 2, NCH) if WS else r - 1
            hp = _bf(hP[...])
            st = {'acc': [None, None], 'res': None}
            macc = {}

            def mvp(kq):
                n = D // 2 // KQ0
                for q in range(2):
                    st['acc'][q] = mv_part(wmA_v[r, pl.ds(z2 + kq * n, n), q * 128:(q + 1) * 128], kq * n, st['acc'][q])
                if kq == KQ0 - 1:
                    st['sa'] = jnp.sum(st['acc'][0], axis=0, keepdims=True)
                    st['ca'] = jnp.sum(st['acc'][1], axis=0, keepdims=True)
                    modA[r, 0:1, 0:128] = st['sa']
                    modA[r, 0:1, 128:256] = st['ca']

            def hpass(p):
                if MU:
                    x = _bf(x_v[p * PR // 2:(p + 1) * PR // 2, lane_ds(r, 128)]).astype(f32)
                    xh = (x - xhat[0, p * PR:(p + 1) * PR, :]) * xhat[1, p * PR:(p + 1) * PR, :]
                else:
                    xh = xhat[r, p * PR:(p + 1) * PR, :]
                st['h'] = (xh * (1.0 + st['ca']) + st['sa']).astype(bf16)
                st['row'] = p * PR
                if p == NP - 1:
                    hP[...] = pltpu.bitcast(st['h'], u32)

            def do_side(tag):
                jobs = side.get(tag, ())
                if not jobs:
                    return
                tk = pltpu.bitcast(st['res'][0:8, 0:128], u32)
                kinds = set(j[0] for j in jobs)
                if 'W' in kinds:
                    wo_raw[pw, pl.ds(z1 + D // 2 + 16, 8), :] = tk
                if 'M' in kinds:
                    wmB_v[32, pl.ds(z1 + D // 2, 8), :] = tk
                if 'A' in kinds:
                    qbuf[0, pl.ds(z1 + S + HALO, 8), :] = pltpu.bitcast(tk, f32)
                for j in jobs:
                    k = int(j[1:])
                    if j[0] == 'W':
                        pW(pw, k, z2)
                    elif j[0] == 'w':
                        pW(pw, k, 0)
                    elif j[0] == 'M':
                        pM(pm[k // KQ], k % KQ, z2, macc, k // KQ)
                    elif j[0] in 'Aa':
                        attention(qbuf, kbuf, vbuf, 0, k * AP, AP, True)

            for it in order0:
                if it[0] == 'T':
                    st['res'] = subdot(hp, TL, r - 1, int(it[1]), valid=r >= 2)
                    do_side(it)
                elif it[0] == 'H':
                    st['res'] = subdot(st['h'], st['row'], r, int(it[1]))
                    do_side('0' + it)
                elif it[0] == 'm':
                    mvp(int(it[1]))
                elif it[0] == 'K':
                    q = int(it[1:] or 0) * 128
                    wmA_v[r, pl.ds(z1 + D // 2, 8), 0:128] = pltpu.bitcast(st['res'][q:q + 8, 0:128], u32)
                elif it[0] == 'X':
                    q = int(it[1:] or 0) * 128
                    wqkv_raw[pl.ds(z1 + D // 2, 8), 0:128] = pltpu.bitcast(st['res'][q:q + 8, 0:128], u32)
                elif it[0] == 'h':
                    hpass(int(it[1]))
                elif it[0] == 'y':
                    b, qf = int(it[1]), int(it[2])
                    exch_groups([(r, b, rg) for rg in range(2 * qf, 2 * qf + 2)])
                elif it[0] == 'x':
                    b, hf = int(it[1]), int(it[2])
                    exch_groups([(r, b, rg) for rg in range(4 * hf, 4 * hf + 4)])
            for p in range(1, NP):
                hpass(p)
                for sd in range(6 if p < NP - 1 else 6 - NDEF):
                    st['res'] = subdot(st['h'], st['row'], r, sd)
                    do_side('%dH%d' % (p, sd))
            zsm[0] = r >> 8
            zsm[1] = r >> 9
            return carry

        if upto >= 2:
            lax.fori_loop(1, NR, region, 0)
            zero = zsm[0]
            zero2 = zsm[1]

        if WS and upto >= 2:
            c_wo(6).wait()
        if upto >= 3:
            c_wo(7).wait()
            for t in range(6 * NM, 32):
                c_mb(t, 6).wait()
            for c in c_w:
                c.wait()

        def rows_u32(ref, row0, M):
            if isinstance(row0, int):
                return _bf(ref[row0 // 2:(row0 + M) // 2, :])
            if isinstance(row0, tuple):
                return _bf(ref[pl.ds(row0[0] + row0[1] // 2, M // 2), :])
            return _bf(ref[pl.ds(pl.multiple_of(row0 // 2, 8), M // 2), :])

        def wo_dot(row0, M):
            o = rows_u32(o_scr, row0, M)
            return jnp.concatenate([_dot(o, _bf(wo_v[n])) for n in range(NCH)], axis=1)

        def row(k):
            return jnp.concatenate([modB[8 * (k - 2) + j, 0:1, :] for j in range(NCH)], axis=1)

        def ln23(row0, M, A):
            ga = row(2); sb = row(3); cb = row(4)
            x = rows_u32(x_v, row0, M).astype(f32)
            xm = x + ga * A
            hB = _ln(xm) * (1.0 + cb) + sb
            n3 = _ln(hB).astype(bf16)
            return xm, hB, n3

        shifts = [-1, -1, 1, 1, -2, -2, 2, 2]

        def g_val():
            return jnp.concatenate(
                [h1buf[j, HALO + shifts[j]:HALO + shifts[j] + T, :] for j in range(NCH)], axis=1).astype(bf16)

        def out_copy(r0, n, k):
            return pltpu.make_async_copy(obuf.at[pl.ds(r0, n)], o_hbm.bitcast(u32).at[pl.ds(r0, n)], osems.at[k])

        def ln4(hs):
            gb = row(5)
            x1 = hb[0:T, :] + hs
            base = xmid[0:T, :] + gb * x1
            n4 = _ln(x1).astype(bf16)
            return base, n4

        def bfirst():
            for j in range(NCH):
                h1buf[j, 0:HALO, :] = jnp.zeros((HALO, 128), f32)
            h7 = _bf(hP[...])
            zb = pl.multiple_of(zero * 8, 8) if ZB else 0
            h0 = (T + HALO) // 2 // 16 * 16 + (16 if T == 128 else 0)
            halves = [(0, h0), (h0, T + HALO - h0)]
            nA = (2 * T + HALO - AT0) // AP
            st = {'res': None, 'As': [], 'n3': [], 'h1': [], 'macc': {}}

            def att(k):
                if AG:
                    st['o'] = attention2(AT0 + k * AP, AP, AG)
                else:
                    attention(qbuf, kbuf, vbuf, 0, AT0 + k * AP, AP, True)

            def tok_q(cc=0):
                qbuf[0, pl.ds(zb + S + HALO, 8), :] = st['res'][0:8, cc * 128:(cc + 1) * 128]

            for it in BA.split():
                k = int(it[1:]) if len(it) > 1 and it[1:].isdigit() else None
                if not ZB and it[0] in 'tWM':
                    continue
                if it[0] == 'T':
                    st['res'] = subdot(h7, TL, 7, k)
                elif it[0] == 'a':
                    att(k)
                elif it[0] == 't':
                    tok_q(k or 0)
                elif it[0] == 'w':
                    pW(7, k, zb)
                elif it[0] == 'v':
                    pW(6, k, zb)
                elif it[0] == 'm':
                    for kq in range(KQ):
                        pM(6 * NM + k, kq, zb, st['macc'], k)
                elif it[0] == 'M':
                    wmB_v[32, pl.ds(zb + D // 2, 8), :] = pltpu.bitcast(st['res'][0:8, 0:128], u32)
                elif it[0] == 'W':
                    wo_raw[7, pl.ds(zb + D // 2 + 16, 8), :] = pltpu.bitcast(st['res'][0:8, 0:128], u32)
                elif it[0] == 'o':
                    st['res'] = wo_dot(*halves[k])
                    st['As'].append(st['res'])
                elif it[0] == 'l':
                    r0, m = halves[k]
                    xm, hB, n3 = ln23(r0, m, st['As'][k])
                    xmid[r0:r0 + m, :] = xm
                    hb[r0:r0 + m, :] = hB
                    st['n3'].append(n3)
                elif it[0] == 'u':
                    r0, m = halves[k]
                    st['res'] = _dot(st['n3'][k], _bf(w1_v[...]))
                    h1 = _gelu(st['res'])
                    for j in range(NCH):
                        h1buf[j, HALO + r0:HALO + r0 + m, :] = h1[:, j * 128:(j + 1) * 128]
            hsbuf[0:T, :] = _dot(g_val(), _bf(w2_v[...]))

        if upto >= 3:
            bfirst()

        def carries(xm, hB, h1, notlast):
            xmid[0:HALO, :] = xmid[T:T + HALO, :]
            hb[0:HALO, :] = hb[T:T + HALO, :]
            for j in range(NCH):
                h1buf[j, 0:2 * HALO, :] = h1buf[j, T:T + 2 * HALO, :]
            xmid[HALO:HALO + T, :] = xm
            hb[HALO:HALO + T, :] = hB
            for j in range(NCH):
                h1j = h1[:, j * 128:(j + 1) * 128]
                h1buf[j, 2 * HALO:HALO + T, :] = h1j[0:T - HALO]
                h1buf[j, HALO + T:2 * HALO + T, :] = jnp.where(notlast, h1j[T - HALO:T], 0.0)

        RP = 16

        def bbody(i, carry):
            static = isinstance(i, int)
            if static:
                row0h = i * (T // 2)
                abase = (i + 1) * T
                abaseh = (i + 1) * (T // 2)
                z1 = pl.multiple_of(zero * 8, 8)
                z2 = pl.multiple_of(zero2 * 8, 8)
            else:
                row0h = pl.multiple_of(i * (T // 2), T // 2)
                nxt = jnp.minimum(i + 1, NT - 1)
                abase = pl.multiple_of(nxt * T, T)
                abaseh = pl.multiple_of(nxt * (T // 2), T // 2)
                z1 = pl.multiple_of((i >> 8) * 8, 8)
                z2 = pl.multiple_of((i >> 9) * 8, 8)
            ga = row(2); sb = row(3); cb = row(4); gb = row(5)
            bases, n4p, xms, hBs, n3p, As = [], [], [], [], [], []

            def p4(r):
                r0 = r * RP
                x1 = hb[r0:r0 + RP, :] + hsbuf[pl.ds(z2 + r0, RP), :]
                bases.append(xmid[r0:r0 + RP, :] + gb * x1)
                n4p.append(_ln(x1).astype(bf16))

            def p23(r, A):
                r0 = r * RP
                x = rows_u32(x_v, (row0h, HALO + r0), RP).astype(f32)
                xm = x + ga * A[r0:r0 + RP]
                hB = _ln(xm) * (1.0 + cb) + sb
                xms.append(xm); hBs.append(hB)
                n3p.append(_ln(hB).astype(bf16))

            for r in range(T // RP):
                if rel4[r] < 0:
                    p4(r)
            o = rows_u32(o_scr, (row0h, HALO), T)
            for n in range(NCH):
                An = _dot(o, _bf(wo_v[n]))
                As.append(An)
                r4 = [r for r in range(T // RP) if rel4[r] == n]
                if r4:
                    hsbuf[pl.ds(z1 + T, 8), 0:128] = An[0:8, 0:128]
                for r in r4:
                    p4(r)
            A = jnp.concatenate(As, axis=1)
            base = jnp.concatenate(bases, axis=0)
            n4 = jnp.concatenate(n4p, axis=0)
            U = _dot(n4, _bf(w3_v[...]))
            u = _gelu(U).astype(bf16)
            for c in range(F // 128):
                r23 = [r for r in range(T // RP) if rel23[r] == NCH + c]
                if r23:
                    x_v[pl.ds(z1 + S // 2 + HALO // 2, 8), 0:128] = pltpu.bitcast(U[0:8, c * 128:(c + 1) * 128], u32)
                for r in r23:
                    p23(r, A)
            assert len(n3p) == T // RP and len(n4p) == T // RP
            xm = jnp.concatenate(xms, axis=0)
            hB = jnp.concatenate(hBs, axis=0)
            n3 = jnp.concatenate(n3p, axis=0)
            h1 = _gelu(_dot(n3, _bf(w1_v[...])))
            carries(xm, hB, h1, i < NT - 1)
            if static:
                if i < NT - 1:
                    attention(qbuf, kbuf, vbuf, abase, HALO, T, False, abaseh)
            elif 'noatt' not in dbg:
                attention(qbuf, kbuf, vbuf, abase, HALO, T, False, abaseh)
            h2 = _dot(u, _bf(w4_v[...]))
            if static:
                obuf[(i - 1) * (T // 2):i * (T // 2), :] = pltpu.bitcast((base + gb * h2).astype(bf16), u32)
            else:
                obuf[pl.ds(pl.multiple_of((i - 1) * (T // 2), T // 2), T // 2), :] = pltpu.bitcast((base + gb * h2).astype(bf16), u32)
            hsbuf[0:T, :] = _dot(g_val(), _bf(w2_v[...]))
            return carry

        if upto >= 4:
            if UB:
                for i in range(1, 1 + UB):
                    bbody(i, 0)
                    if i in BAR:
                        out_copy_i(i).start()
                if 1 + UB < NT:
                    lax.fori_loop(1 + UB, NT, bbody, 0)
            else:
                lax.fori_loop(1, NT, bbody, 0)

        def blast():
            r0 = (NT - 1) * (T // 2)
            out_copy(0, r0, 0).start()
            base, n4 = ln4(hsbuf[0:T, :])
            if BL:
                FC = F // BL
                xmid[0:T, :] = base
                n4b[...] = pltpu.bitcast(n4, u32)
                hsbuf[0:T, :] = jnp.zeros((T, D), f32)

                def body(c, carry):
                    w3c = w3_v[:, pl.ds(pl.multiple_of(c * FC, 128), FC)]
                    u = _gelu(_dot(_bf(n4b[...]), _bf(w3c))).astype(bf16)
                    w4c = w4_v[pl.ds(pl.multiple_of(c * (FC // 2), 32), FC // 2), :]
                    hsbuf[0:T, :] += _dot(u, _bf(w4c))
                    return carry

                lax.fori_loop(0, BL, body, 0)
                obuf[r0:r0 + T // 2, :] = pltpu.bitcast((xmid[0:T, :] + row(5) * hsbuf[0:T, :]).astype(bf16), u32)
            else:
                u = _gelu(_dot(n4, _bf(w3_v[...]))).astype(bf16)
                h2 = _dot(u, _bf(w4_v[...]))
                obuf[r0:r0 + T // 2, :] = pltpu.bitcast((base + row(5) * h2).astype(bf16), u32)
            out_copy(r0, T // 2, 1).start()
            out_copy(0, r0, 0).wait()
            out_copy(r0, T // 2, 1).wait()

        if upto >= 5:
            blast()

    @jax.jit
    def fn(A_x, A_wqkv, A_wo, B_x, B_w1, B_w2, B_w3, B_w4, c, w_mod):
        x = A_x.reshape(S, D)
        any_spec = pl.BlockSpec(memory_space=pl.ANY)
        out = pl.pallas_call(
            kernel,
            in_specs=[any_spec] * 9,
            out_specs=any_spec,
            out_shape=jax.ShapeDtypeStruct((S, D), bf16),
            scratch_shapes=[
                pltpu.VMEM((S // 2 + HALO // 2 + 8, D), u32),
                pltpu.VMEM((D // 2 + 32, 3 * D), u32),
                pltpu.VMEM((D // 2, D), u32),
                pltpu.VMEM((D // 2, D), u32),
                pltpu.VMEM((D // 2, D), u32),
                pltpu.VMEM((NCH + WS, D // 2 + 32, 128), u32),
                pltpu.VMEM((NCH + WS, D // 2, 128), u32),
                pltpu.VMEM((D // 2, D), u32),
                pltpu.VMEM((D // 2, D), u32),
                pltpu.VMEM((D // 2, F), u32),
                pltpu.VMEM((F // 2, D), u32),
                pltpu.VMEM((D // 2, 128), f32),
                pltpu.VMEM((D // 2, 128), f32),
                pltpu.VMEM((8, D // 2 + 16, 256), u32),
                pltpu.VMEM((33, D // 2 + 32, 128), u32),
                pltpu.VMEM((8, 8, 256), f32),
                pltpu.VMEM((36, 8, 128), f32),
                pltpu.VMEM((3 if MU else NCH, S + 32, 128), f32),
                pltpu.VMEM((PR // 2, 128), u32),
                pltpu.VMEM((S // 2, 128), u32),
                pltpu.VMEM((NCH, S + 32, 128), f32),
                pltpu.VMEM((NCH, S + 2 * HALO, 128), f32),
                pltpu.VMEM((NCH, S + 2 * HALO, 128), f32),
                pltpu.VMEM((T + HALO, D), f32),
                pltpu.VMEM((T + HALO, D), f32),
                pltpu.VMEM((NCH, T + 2 * HALO, 128), f32),
                pltpu.VMEM((S // 2, D), u32),
                pltpu.VMEM((S // 2 + HALO // 2, D), u32),
                pltpu.VMEM((T + 32, D), f32),
                pltpu.VMEM((T // 2, D), u32),
                pltpu.VMEM((1, D), bf16),
            ] + ([pltpu.VMEM((padr, 128), f32)] if padr else []) + [
                pltpu.SMEM((8,), jnp.int32),
                pltpu.SemaphoreType.DMA((NSEM,)),
                pltpu.SemaphoreType.DMA((2,)),
            ],
            compiler_params=pltpu.CompilerParams(vmem_limit_bytes=120 * 1024 * 1024),
        )(x, A_wqkv, A_wo, B_w1, B_w2, B_w3, B_w4, c, w_mod)
        return out.reshape(1, S, D)
    return fn


_fn = make()


def pallas_adaLN_cond__sliding_local_dilated__mixer_s_mlp__prompt_kernel(A_x, A_wqkv, A_wo, B_x, B_w1, B_w2, B_w3, B_w4, c, w_mod):
    return _fn(A_x, A_wqkv, A_wo, B_x, B_w1, B_w2, B_w3, B_w4, c, w_mod)
```

```python
import functools
import jax
import jax.numpy as jnp
from jax import lax
import jax.experimental.pallas as pl
import jax.experimental.pallas.tpu as pltpu

S, D, F = 2048, 1024, 3584
H, DH, W, DIL = 32, 32, 8, 2
NCH = D // 128
EPS = 1e-5
SCALE = DH ** -0.5
f32, bf16, u32 = jnp.float32, jnp.bfloat16, jnp.uint32
HALO = 16


def _ln(x):
    m = jnp.mean(x, axis=-1, keepdims=True)
    xc = x - m
    v = jnp.mean(xc * xc, axis=-1, keepdims=True)
    return xc * lax.rsqrt(v + EPS)


def _gelu(x):
    c0 = 0.7978845608028654
    c1 = c0 * 0.044715
    t = jnp.tanh(x * (c0 + c1 * (x * x)))
    hx = 0.5 * x
    return hx + hx * t


def _dot(a, b):
    return jnp.dot(a, b, preferred_element_type=f32)


def _bf(w):
    return pltpu.bitcast(w, bf16)


def _lane_xor(x, s):
    lane = lax.broadcasted_iota(jnp.int32, x.shape, 1)
    return jnp.take_along_axis(x, lane ^ s, axis=1)


def _exchange8_multi(XS):
    XS = [list(X) for X in XS]
    lane = lax.broadcasted_iota(jnp.int32, XS[0][0].shape, 1)
    for t in range(3):
        s = 1 << (t + 2)
        m = (lane & s) != 0
        for X in XS:
            for p in range(8):
                if p & (1 << t):
                    continue
                p2 = p | (1 << t)
                tmp = _lane_xor(jnp.where(m, X[p], X[p2]), s)
                X[p], X[p2] = jnp.where(m, tmp, X[p]), jnp.where(m, X[p2], tmp)
    return XS


def _group4_sum(acc):
    lane = lax.broadcasted_iota(jnp.int32, acc.shape, 1)
    acc = acc + jnp.where((lane & 1) != 0, pltpu.roll(acc, 1, 1), pltpu.roll(acc, 127, 1))
    acc = acc + jnp.where((lane & 2) != 0, pltpu.roll(acc, 2, 1), pltpu.roll(acc, 126, 1))
    return acc


def make(T=128, PR=512, RB=8, EG=4, upto=9, AT0=0, AP=16,
         DO='c X0 Wq sa ca X1 Wk Wv X2 X3 X4 X5 X6 X7 X8 X9 X10 X12 X13 X11 X14 X15',
         PS=None, PSX=None, RL=1, D0='1234567', LP=16, BL=2, ZB=1,
         order0='T0 T1 X x00 x01 m0 T2 T3 X x10 x11 h0 T4 T5 X x20 H0 X x21 H1 H2 H3 H4 H5', NDEF=6, BA=None,
         side=None, KQ=4, KQ0=1, NM=5, NR=8, AG=1,
         rel4=(-1, -1, -1, 0, 1, 2, 3, 4), rel23=(8, 9, 10, 11, 12, 13, 14, 15),
         padr=0, dbg='', UB=0, BAR=(), GL=0, MU=1, WS=1, skip='', AB=9, WGS='1'*128, PD=0, ASCH='', DL=0, EX3=1, EX4=1, XT=()):
    HS, HO = (2, 0) if MU else (0, S // 2)
    NT = S // T
    NP = S // PR
    order0 = order0.split()
    TL = S - PR
    if PS is None:
        PS = ('wc C wX0 L0 wWq e0 wsa S wca A h0 wX1 u0:0 L1 wWk u1:0 e1 wWv u0:1 u1:1 e2 wX2 u0:2 u1:2 L2 u2:0 '
              'wX3 wX4 u2:12 L3 u3:012 L4 u4:0 wX5 wX6 wX7 u4:12 L5 u5:012 L6 u6:012 L7 u7:0 '
              'wX8 wX9 wX10 wX12 wX13 u7:12 L8 u8:012 L9 u9:012 L10 ua:0 L12 L13 wX11 wX14 wX15 DW ua:12 L11 ub:012 L14 L15')
    if BA is None:
        BA = ('a0 a1 T0 T1 t0 a2 a3 W w0 w1 w2 w3 w4 w5 w6 w7 T2 t0 a4 a5 T3 t0 a6 a7 T4 t0 a8 a9 T5 t0 a10 o0 t0 a11 t4 a12 '
              'o1 t0 a13 t4 a14 M m0 m1 l0 l1 u0 t0 a15 t4 a16 u1')
    if WS and 'v0' not in BA:
        BA = BA.replace('W w0 w1 w2 w3 w4 w5 w6 w7', 'W v0 v1 v2 v3 v4 v5 v6 v7 w0 w1 w2 w3 w4 w5 w6 w7')
    if PSX:
        for k_, v_ in PSX.items():
            assert (' ' + k_ + ' ') in PS
            PS = PS.replace(' ' + k_ + ' ', ' ' + k_ + ' ' + v_ + ' ')
    S_C, S_X, S_SA, S_CA, S_W0, S_WQ, S_WO, S_MB, S_W = 0, 1, 17, 25, 33, 36, 44, 52, 60
    NSEM = 64
    DEF = list(range(6 - NDEF, 6))
    tags = ['T%d' % sd for sd in DEF] + ['%dH%d' % (p, sd) for p in range(NP) for sd in range(6 if p < NP - 1 else 6 - NDEF)]
    if side is None:
        side = 'W:7,9,11,13,15,17,19,21 M:4,5,6,7,8,9,10,11,12,13,14,15,16,17,18,19,20,21,22,22'
    if isinstance(side, str):
        sd_ = {}
        for grp in side.split():
            kind, lst = grp.split(':')
            for k, t in enumerate(lst.split(',')):
                sd_.setdefault(tags[int(t)], []).append(kind + str(k))
        side = sd_
    assert sum(1 for v in side.values() for j in v if j[0] in 'Aa') * AP == AT0

    def kernel(x_hbm, wqkv_hbm, wo_hbm, w1_hbm, w2_hbm, w3_hbm, w4_hbm, c_hbm, wmod_hbm,
               o_hbm,
               x_v, wqkv_raw, wq_v, wk_v, wv_v, wo_raw, wo_v, w1_v, w2_v, w3_v, w4_v, cE, cO, wmA_v, wmB_v,
               modA, modB, xhat, hP, h0, qbuf, kbuf, vbuf, xmid, hb, h1buf, obuf, o_scr, hsbuf, n4b, n3b, c_v, *rest):
        zsm, sems, osems = rest[-3:]

        def cp(src, dst, k):
            return pltpu.make_async_copy(src, dst, sems.at[k])

        xu = x_hbm.bitcast(u32)
        wqkvu = wqkv_hbm.bitcast(u32)
        wou = wo_hbm.bitcast(u32)
        wmodu = wmod_hbm.bitcast(u32)

        def lane_ds(k, n, base=0):
            if isinstance(k, int):
                return pl.ds(base + k * n, n)
            return pl.ds(pl.multiple_of(base + k * n, 128), n)

        def row_ds(base, k, n):
            if isinstance(k, int):
                return pl.ds(base + k * n, n)
            return pl.ds(pl.multiple_of(base + k * n, 8), n)

        c_c = cp(c_hbm, c_v, S_C)

        def c_x(b):
            return cp(xu.at[b * 64:(b + 1) * 64], x_v.at[b * 64:(b + 1) * 64], S_X + b)

        def c_sa(k):
            return cp(wmodu.at[:, lane_ds(k, 128)], wmA_v.at[k, 0:D // 2, 0:128], S_SA + k)

        def c_ca(k):
            return cp(wmodu.at[:, lane_ds(k, 128, D)], wmA_v.at[k, 0:D // 2, 128:256], S_CA + k)

        def c_w0(b):
            return cp(wqkvu.at[0:64, b * D:(b + 1) * D], wqkv_raw.at[0:64, b * D:(b + 1) * D], S_W0 + b)

        def c_wq(k):
            return cp(wqkvu.at[row_ds(0, k, 64)], wqkv_raw.at[row_ds(0, k, 64)], S_WQ + k)

        def c_wo(p):
            return cp(wou.at[:, lane_ds(p, 128)], wo_raw.at[p, 8:8 + D // 2], S_WO + p)

        def c_mb(t, g):
            return cp(wmodu.at[:, lane_ds(t, 128, 2 * D)], wmB_v.at[t, 0:D // 2], S_MB + g)

        c_w = [cp(w1_hbm.bitcast(u32), w1_v, S_W), cp(w2_hbm.bitcast(u32), w2_v, S_W + 1),
               cp(w3_hbm.bitcast(u32), w3_v, S_W + 2), cp(w4_hbm.bitcast(u32), w4_v, S_W + 3)]

        def named(nm):
            if nm == 'c':
                return c_c
            if nm == 'sa':
                return c_sa(0)
            if nm == 'ca':
                return c_ca(0)
            if nm[0] == 'W':
                return c_w0('qkv'.index(nm[1]))
            return c_x(int(nm[1:]))

        for nm in DO.split():
            named(nm).start()
        def start_group(g):
            if g == 'W':
                if upto >= 3:
                    c_wo(7).start()
                    for t in range(6 * NM, 32):
                        c_mb(t, 6).start()
                    for c in c_w:
                        c.start()
            elif upto >= 2 and 'nodma2' not in dbg:
                r = int(g)
                c_sa(r).start()
                c_ca(r).start()
                c_wq(r).start()
                c_wo(r - 1).start()
                if r >= 2:
                    for i in range(NM):
                        c_mb(NM * (r - 2) + i, r - 2).start()

        for g in D0:
            start_group(g)
        assert sorted(list(D0) + [it[1] for it in PS.split() if it[0] == 'D']) == list('1234567W')

        def _zinit(i, carry):
            zsm[2 + i] = i >> 8
            return carry

        lax.fori_loop(0, 3, _zinit, 0)
        zp3 = pl.multiple_of(zsm[4] * 8, 8)
        zp1 = pl.multiple_of(zsm[2] * 8, 8)
        zp2 = pl.multiple_of(zsm[3] * 8, 8)

        x_v[S // 2:S // 2 + HALO // 2, :] = jnp.zeros((HALO // 2, D), u32)
        for j in range(NCH):
            z = jnp.zeros((HALO, 128), f32)
            qbuf[j, S:S + HALO, :] = z
            kbuf[j, HALO + S:2 * HALO + S, :] = z
            vbuf[j, HALO + S:2 * HALO + S, :] = z
            kbuf[j, 0:HALO, :] = z
            vbuf[j, 0:HALO, :] = z
            wo_raw[j, 0:8, :] = jnp.zeros((8, 128), u32)
            wo_raw[j, 8 + D // 2:16 + D // 2, :] = jnp.zeros((8, 128), u32)

        def mv_part(w, r0, acc):
            n = w.shape[0]
            lo = pltpu.bitcast(w << 16, f32)
            hi = pltpu.bitcast(w & jnp.uint32(0xFFFF0000), f32)
            pr = lo * cE[r0:r0 + n, :] + hi * cO[r0:r0 + n, :]
            for t in range(n // 8):
                acc = pr[8 * t:8 * t + 8] if acc is None else acc + pr[8 * t:8 * t + 8]
            return acc

        wparts = (wq_v, wk_v, wv_v)
        bufs = (qbuf, kbuf, vbuf)

        def exch_groups(grps):
            for g0 in range(0, len(grps), EG):
                gs = grps[g0:g0 + EG]
                XS = [[wqkv_raw[row_ds(rg * 8, k * 8, 8), b * D + a * 128:b * D + (a + 1) * 128] for a in range(NCH)]
                      for (k, b, rg) in gs]
                YS = _exchange8_multi(XS)
                for (k, b, rg), Y in zip(gs, YS):
                    wparts[b][row_ds(rg * 8, k * 8, 8), :] = jnp.concatenate(Y, axis=1)

        def subdot(lhs, row0, kc, sd, init=False, valid=None):
            b, hf = sd // 2, sd % 2
            n = lhs.shape[0]
            res = _dot(lhs, _bf(wparts[b][row_ds(0, kc, 64), hf * 512:(hf + 1) * 512]))
            o = row0 + (0 if b == 0 else HALO)
            for jj in range(4):
                j = hf * 4 + jj
                if init:
                    bufs[b][j, o:o + n, :] = res[:, jj * 128:(jj + 1) * 128]
                elif valid is not None:
                    bufs[b][j, o:o + n, :] = jnp.where(valid, bufs[b][j, o:o + n, :], 0.0) + res[:, jj * 128:(jj + 1) * 128]
                else:
                    bufs[b][j, o:o + n, :] += res[:, jj * 128:(jj + 1) * 128]
            return res

        def prologue():
            st = {}

            def crep():
                c = c_v[...].astype(f32)
                scf = (c * jax.nn.sigmoid(c)).astype(bf16).astype(f32)
                rr = lax.broadcasted_iota(jnp.int32, (128, 128), 0)
                ll = lax.broadcasted_iota(jnp.int32, (128, 128), 1)
                sel = ll == jnp.where(rr < 64, 2 * rr, 2 * rr - 127)
                for j in range(NCH):
                    dg = jnp.where(sel, jnp.broadcast_to(scf[:, j * 128:(j + 1) * 128], (128, 128)), 0.0).astype(bf16)
                    rep = _dot(dg, jnp.ones((128, 128), bf16))
                    cE[j * 64:(j + 1) * 64, :] = rep[0:64]
                    cO[j * 64:(j + 1) * 64, :] = rep[64:128]

            def h_store(r0, xh0):
                h = (xh0 * (1.0 + st['ca']) + st['sa']).astype(bf16)
                if r0 < TL:
                    xhat[HS, HO + r0 // 2:HO + (r0 + LP) // 2, :] = pltpu.bitcast(h, f32)
                else:
                    hP[(r0 - TL) // 2:(r0 - TL + LP) // 2, :] = pltpu.bitcast(h, u32)

            def h0_lhs(b0, nb, gated):
                r0 = HO + b0 * 64
                if not gated:
                    return _bf(xhat[HS, r0:r0 + nb * 64, :])
                if GL:
                    return jnp.concatenate([_bf(xhat[HS, r0:r0 + nb * 64 - 8, :]), _bf(xhat[HS, pl.ds(zp3 + r0 + nb * 64 - 8, 8), :])], axis=0)
                return jnp.concatenate([_bf(xhat[HS, pl.ds(zp3 + r0, 8), :]), _bf(xhat[HS, r0 + 8:r0 + nb * 64, :])], axis=0)

            def ln_piece(b, i):
                r0 = b * 128 + i * LP
                direct = 'ca' in st and 'sa' in st
                if MU:
                    x = _bf(x_v[pl.ds(zp1 + r0 // 2, LP // 2), :]).astype(f32)
                    m = jnp.mean(x, axis=-1, keepdims=True)
                    if RL:
                        x = _bf(x_v[pl.ds(zp2 + r0 // 2, LP // 2), :]).astype(f32)
                    xc = x - m
                    rs = lax.rsqrt(jnp.mean(xc * xc, axis=-1, keepdims=True) + EPS)
                    xhat[0, r0:r0 + LP, :] = jnp.broadcast_to(m, (LP, 128))
                    xhat[1, r0:r0 + LP, :] = jnp.broadcast_to(rs, (LP, 128))
                    if direct:
                        h_store(r0, xc[:, 0:128] * rs)
                    return
                if RL:
                    m = jnp.mean(_bf(x_v[pl.ds(zp1 + r0 // 2, LP // 2), :]).astype(f32), axis=-1, keepdims=True)
                    xc = _bf(x_v[pl.ds(zp2 + r0 // 2, LP // 2), :]).astype(f32) - m
                    v = jnp.mean(xc * xc, axis=-1, keepdims=True)
                    xh = (_bf(x_v[r0 // 2:(r0 + LP) // 2, :]).astype(f32) - m) * lax.rsqrt(v + EPS)
                else:
                    xh = _ln(_bf(x_v[pl.ds(zp1 + r0 // 2, LP // 2), :]).astype(f32))
                for j in range(1 if direct else 0, NCH):
                    xhat[j, r0:r0 + LP, :] = xh[:, j * 128:(j + 1) * 128]
                if direct:
                    h_store(r0, xh[:, 0:128])

            def ln_block(b):
                for i in range(128 // LP):
                    ln_piece(b, i)

            def hblk(b):
                for i in range(128 // LP):
                    r0 = b * 128 + i * LP
                    if MU:
                        x = _bf(x_v[r0 // 2:(r0 + LP) // 2, 0:128]).astype(f32)
                        h_store(r0, (x - xhat[0, r0:r0 + LP, :]) * xhat[1, r0:r0 + LP, :])
                    else:
                        h_store(r0, xhat[0, r0:r0 + LP, :])

            for it in PS.split():
                if it[0] == 'w':
                    named(it[1:]).wait()
                elif it[0] == 'D':
                    start_group(it[1])
                elif it == 'C':
                    crep()
                elif it[0] == 'L':
                    ln_block(int(it[1:]))
                elif it[0] == 'h':
                    hblk(int(it[1:]))
                elif it == 'S':
                    st['sa'] = jnp.sum(mv_part(wmA_v[0, 0:D // 2, 0:128], 0, None), axis=0, keepdims=True)
                elif it == 'A':
                    st['ca'] = jnp.sum(mv_part(wmA_v[0, 0:D // 2, 128:256], 0, None), axis=0, keepdims=True)
                elif it[0] == 'e':
                    exch_groups([(0, int(it[1]), rg) for rg in range(8)])
                elif it[0] == 'p':
                    b_, i_ = it[1:].split(':')
                    ln_piece(int(b_), int(i_))
                elif it[0] == 't':
                    x_v[pl.ds(zp3 + S // 2 + HALO // 2, 8), 0:128] = pltpu.bitcast(st['res'][0:8, 0:128], u32)
                elif it[0] in 'sg':
                    blks, sd = it[1:].split(':')
                    b0, nb = int(blks[0], 16), len(blks)
                    st['res'] = subdot(h0_lhs(b0, nb, it[0] == 'g'), b0 * 128, 0, int(sd), True)
                elif it[0] == 'u':
                    blks, parts = it[1:].split(':')
                    b0, nb = int(blks[0], 16), len(blks)
                    lhs = h0_lhs(b0, nb, False)
                    for p in parts:
                        subdot(lhs, b0 * 128, 0, 2 * int(p), True)
                        st['res'] = subdot(lhs, b0 * 128, 0, 2 * int(p) + 1, True)

        if 'P' not in skip:
            prologue()

        def attention(qb, kb, vb, base, off, M, mask_rows, baseh=None):
            row0 = base + off

            def kvds(r, w):
                return pl.ds(base + (off + HALO + r - DIL * w), RB)

            o_rows = []
            for r in range(0, M, RB):
                q = [qb[j, pl.ds(base + (off + r), RB), :] for j in range(NCH)]
                s = []
                for w in range(W):
                    acc = None
                    for j in range(NCH):
                        p = q[j] * kb[j, kvds(r, w), :]
                        acc = p if acc is None else acc + p
                    acc = _group4_sum(acc)
                    if mask_rows and off + r < DIL * (W - 1) and w > 0:
                        rows = row0 + r + lax.broadcasted_iota(jnp.int32, (RB, 128), 0)
                        acc = jnp.where(rows >= DIL * w, acc, -1e30)
                    s.append(acc)
                m = functools.reduce(jnp.maximum, s)
                e = [jnp.exp((sw - m) * SCALE) for sw in s]
                den = functools.reduce(lambda a, b: a + b, e)
                rinv = 1.0 / den
                oc = []
                for j in range(NCH):
                    acc = None
                    for w in range(W):
                        p = e[w] * vb[j, kvds(r, w), :]
                        acc = p if acc is None else acc + p
                    oc.append(acc * rinv)
                o_rows.append(jnp.concatenate(oc, axis=1))
            o = jnp.concatenate(o_rows, axis=0).astype(bf16)
            if isinstance(row0, int):
                o_scr[row0 // 2:(row0 + M) // 2, :] = pltpu.bitcast(o, u32)
            elif baseh is not None:
                o_scr[pl.ds(baseh + off // 2, M // 2), :] = pltpu.bitcast(o, u32)
            else:
                o_scr[pl.ds(pl.multiple_of(row0 // 2, 8), M // 2), :] = pltpu.bitcast(o, u32)


        def attention2(off, M, G, base=None, baseh=None):
            o_rows = []

            def rs_(a):
                return slice(a, a + RB) if base is None else pl.ds(base + a, RB)

            for r0 in range(0, M, RB * G):
                rs = [off + r0 + g * RB for g in range(G) if r0 + g * RB < M]
                lane = lax.broadcasted_iota(jnp.int32, (RB, 128), 1)
                S_ = {}
                for r in rs:
                    q = [qbuf[j, rs_(r), :] for j in range(NCH)]
                    for w in range(W):
                        acc = None
                        for j in range(NCH):
                            k0 = HALO + r - DIL * w
                            p = q[j] * kbuf[j, rs_(k0), :]
                            acc = p if acc is None else acc + p
                        S_[r, w] = acc
                keys = list(S_)
                for sh in (1, 2):
                    R = {k: (pltpu.roll(S_[k], sh, 1), pltpu.roll(S_[k], 128 - sh, 1)) for k in keys}
                    for k in keys:
                        S_[k] = S_[k] + jnp.where((lane & sh) != 0, R[k][0], R[k][1])
                for r in rs:
                    s = []
                    for w in range(W):
                        acc = S_[r, w]
                        if base is None and r < DIL * (W - 1) and w > 0:
                            rows = r + lax.broadcasted_iota(jnp.int32, (RB, 128), 0)
                            acc = jnp.where(rows >= DIL * w, acc, -1e30)
                        s.append(acc)
                    m = functools.reduce(jnp.maximum, s)
                    e = [jnp.exp((sw - m) * SCALE) for sw in s]
                    den = functools.reduce(lambda a, b: a + b, e)
                    rinv = 1.0 / den
                    oc = []
                    for j in range(NCH):
                        acc = None
                        for w in range(W):
                            k0 = HALO + r - DIL * w
                            p = e[w] * vbuf[j, rs_(k0), :]
                            acc = p if acc is None else acc + p
                        oc.append(acc * rinv)
                    o_rows.append(jnp.concatenate(oc, axis=1))
            o = jnp.concatenate(o_rows, axis=0).astype(bf16)
            if base is None:
                o_scr[off // 2:(off + M) // 2, :] = pltpu.bitcast(o, u32)
            else:
                o_scr[pl.ds(baseh + off // 2, M // 2), :] = pltpu.bitcast(o, u32)
            return o

        class Att:
            def __init__(self, base, baseh, off, M, wgs, PD, ztok):
                self.base, self.baseh, self.off, self.PD, self.ztok = base, baseh, off, PD, ztok
                self.nrb = M // RB
                self.wgs = list(wgs)
                assert sum(self.wgs) == self.nrb * W
                self.Q, self.SS, self.E, self.OC = {}, {}, {}, {}
                self.win = 0
                self.done = 0

            def scores(self, wl):
                lane = lax.broadcasted_iota(jnp.int32, (RB, 128), 1)
                accs = []
                for (rb, w) in wl:
                    r = self.off + rb * RB
                    if rb not in self.Q:
                        self.Q[rb] = [qbuf[j, pl.ds(self.base + r, RB), :] for j in range(NCH)]
                    acc = None
                    for j in range(NCH):
                        p = self.Q[rb][j] * kbuf[j, pl.ds(self.base + (HALO + r - DIL * w), RB), :]
                        acc = p if acc is None else acc + p
                    accs.append(acc)
                for sh in (1, 2):
                    R = [(pltpu.roll(a, sh, 1), pltpu.roll(a, 128 - sh, 1)) for a in accs]
                    accs = [a + jnp.where((lane & sh) != 0, x, y) for a, (x, y) in zip(accs, R)]
                for k, a in zip(wl, accs):
                    self.SS[k] = a
                    if k[1] == W - 1:
                        self.softmax(k[0])

            def softmax(self, rb):
                s = [self.SS[rb, w] for w in range(W)]
                m = functools.reduce(jnp.maximum, s)
                e = [jnp.exp((sw - m) * SCALE) for sw in s]
                den = functools.reduce(lambda a, b: a + b, e)
                self.E[rb] = (e, 1.0 / den)

            def pv(self):
                rb, j = divmod(self.done, NCH)
                self.done += 1
                r = self.off + rb * RB
                e, rinv = self.E[rb]
                acc = None
                for w in range(W):
                    p = e[w] * vbuf[j, pl.ds(self.base + (HALO + r - DIL * w), RB), :]
                    acc = p if acc is None else acc + p
                self.OC[rb, j] = acc * rinv
                if rb % 2 == 1 and j == NCH - 1:
                    o = jnp.concatenate([jnp.concatenate([self.OC[q, c] for c in range(NCH)], axis=1) for q in (rb - 1, rb)], axis=0)
                    o_scr[pl.ds(self.baseh + (self.off + (rb - 1) * RB) // 2, RB), :] = pltpu.bitcast(o.astype(bf16), u32)

            def token(self, v):
                vbuf[0, pl.ds(self.ztok + S + 2 * HALO, 8), :] = v

            def steps(self, n):
                for _ in range(n):
                    if not self.wgs:
                        return
                    g = self.wgs.pop(0)
                    wl = [divmod(self.win + t, W) for t in range(g)]
                    self.win += g
                    self.scores(wl)
                    tok = False
                    while self.done < self.nrb * NCH and self.done + W + self.PD <= self.win - 1 and self.done // NCH in self.E:
                        if not tok:
                            self.token(self.SS[wl[-1]])
                            tok = True
                        self.pv()

            def rest(self, n=999):
                while self.done < self.nrb * NCH and n > 0:
                    self.pv(); n -= 1

        sub = lax.broadcasted_iota(jnp.int32, (8, 128), 0)

        def pW(p, q, z):
            for tv in range(8 * q, 8 * q + 8):
                j = tv >> 3
                hh = (tv >> 1) & 3
                a2 = tv & 1
                parts = []
                for al in range(4):
                    a = a2 * 4 + al
                    src = a * 64 + hh * 16 + j * 2
                    st = src - 2 * al + 8
                    if isinstance(z, int):
                        parts.append(wo_raw[p, z + st:z + st + 8, :])
                    else:
                        parts.append(wo_raw[p, pl.ds(z + st, 8), :])
                v = jnp.where(sub < 2, parts[0], parts[1])
                v2 = jnp.where(sub < 6, parts[2], parts[3])
                wo_v[p, 8 * tv:8 * tv + 8, :] = jnp.where(sub < 4, v, v2)

        def pM(t, kq, z, macc, key):
            n = D // 2 // KQ
            rows = pl.ds(z + kq * n, n)
            macc[key] = mv_part(wmB_v[t, rows, :], kq * n, macc.get(key))
            if kq == KQ - 1:
                modB[t, 0:1, :] = jnp.sum(macc[key], axis=0, keepdims=True)

        def region_waits(r):
            c_sa(r).wait(); c_ca(r).wait(); c_wq(r).wait()
            if not WS:
                c_wo(r - 1).wait()

            @pl.when(r >= 2)
            def _():
                if WS:
                    c_wo(r - 2).wait()
                for i in range(NM):
                    c_mb(NM * (r - 2) + i, r - 2).wait()

        if 'prewait' in dbg:
            for r in range(1, 8):
                region_waits(r)

        def region(r, carry):
            if 'prewait' not in dbg and 'nodma2' not in dbg:
                region_waits(r)
            z1 = pl.multiple_of((r >> 8) * 8, 8)
            z2 = pl.multiple_of((r >> 9) * 8, 8)
            pm = [jnp.where(r >= 2, NM * (r - 2) + i, 32) for i in range(NM)]
            pw = jnp.where(r >= 2, r - 2, NCH) if WS else r - 1
            hp = _bf(hP[...])
            st = {'acc': [None, None], 'res': None}
            macc = {}

            def mvp(kq):
                n = D // 2 // KQ0
                for q in range(2):
                    st['acc'][q] = mv_part(wmA_v[r, pl.ds(z2 + kq * n, n), q * 128:(q + 1) * 128], kq * n, st['acc'][q])
                if kq == KQ0 - 1:
                    st['sa'] = jnp.sum(st['acc'][0], axis=0, keepdims=True)
                    st['ca'] = jnp.sum(st['acc'][1], axis=0, keepdims=True)
                    modA[r, 0:1, 0:128] = st['sa']
                    modA[r, 0:1, 128:256] = st['ca']

            def hpass(p):
                if MU:
                    x = _bf(x_v[p * PR // 2:(p + 1) * PR // 2, lane_ds(r, 128)]).astype(f32)
                    xh = (x - xhat[0, p * PR:(p + 1) * PR, :]) * xhat[1, p * PR:(p + 1) * PR, :]
                else:
                    xh = xhat[r, p * PR:(p + 1) * PR, :]
                st['h'] = (xh * (1.0 + st['ca']) + st['sa']).astype(bf16)
                st['row'] = p * PR
                if p == NP - 1:
                    hP[...] = pltpu.bitcast(st['h'], u32)

            def do_side(tag):
                jobs = side.get(tag, ())
                if not jobs:
                    return
                tk = pltpu.bitcast(st['res'][0:8, 0:128], u32)
                kinds = set(j[0] for j in jobs)
                if 'W' in kinds:
                    wo_raw[pw, pl.ds(z1 + D // 2 + 16, 8), :] = tk
                if 'M' in kinds:
                    wmB_v[32, pl.ds(z1 + D // 2, 8), :] = tk
                if 'A' in kinds:
                    qbuf[0, pl.ds(z1 + S + HALO, 8), :] = pltpu.bitcast(tk, f32)
                for j in jobs:
                    k = int(j[1:])
                    if j[0] == 'W':
                        pW(pw, k, z2)
                    elif j[0] == 'w':
                        pW(pw, k, 0)
                    elif j[0] == 'M':
                        pM(pm[k // KQ], k % KQ, z2, macc, k // KQ)
                    elif j[0] in 'Aa':
                        attention(qbuf, kbuf, vbuf, 0, k * AP, AP, True)

            for it in order0:
                if it[0] == 'T':
                    st['res'] = subdot(hp, TL, r - 1, int(it[1]), valid=r >= 2)
                    do_side(it)
                elif it[0] == 'H':
                    st['res'] = subdot(st['h'], st['row'], r, int(it[1]))
                    do_side('0' + it)
                elif it[0] == 'm':
                    mvp(int(it[1]))
                elif it[0] == 'K':
                    q = int(it[1:] or 0) * 128
                    wmA_v[r, pl.ds(z1 + D // 2, 8), 0:128] = pltpu.bitcast(st['res'][q:q + 8, 0:128], u32)
                elif it[0] == 'X':
                    q = int(it[1:] or 0) * 128
                    wqkv_raw[pl.ds(z1 + D // 2, 8), 0:128] = pltpu.bitcast(st['res'][q:q + 8, 0:128], u32)
                elif it[0] == 'h':
                    hpass(int(it[1]))
                elif it[0] == 'y':
                    b, qf = int(it[1]), int(it[2])
                    exch_groups([(r, b, rg) for rg in range(2 * qf, 2 * qf + 2)])
                elif it[0] == 'x':
                    b, hf = int(it[1]), int(it[2])
                    exch_groups([(r, b, rg) for rg in range(4 * hf, 4 * hf + 4)])
            for p in range(1, NP):
                hpass(p)
                for sd in range(6 if p < NP - 1 else 6 - NDEF):
                    st['res'] = subdot(st['h'], st['row'], r, sd)
                    do_side('%dH%d' % (p, sd))
            zsm[0] = r >> 8
            zsm[1] = r >> 9
            return carry

        if upto >= 2:
            if 'R' not in skip:
                lax.fori_loop(1, NR, region, 0)
            zero = zsm[0]
            zero2 = zsm[1]

        if WS and upto >= 2:
            c_wo(6).wait()
        if upto >= 3:
            c_wo(7).wait()
            for t in range(6 * NM, 32):
                c_mb(t, 6).wait()
            for c in c_w:
                c.wait()

        def rows_u32(ref, row0, M):
            if isinstance(row0, int):
                return _bf(ref[row0 // 2:(row0 + M) // 2, :])
            if isinstance(row0, tuple):
                return _bf(ref[pl.ds(row0[0] + row0[1] // 2, M // 2), :])
            return _bf(ref[pl.ds(pl.multiple_of(row0 // 2, 8), M // 2), :])

        def wo_dot(row0, M):
            o = rows_u32(o_scr, row0, M)
            return jnp.concatenate([_dot(o, _bf(wo_v[n])) for n in range(NCH)], axis=1)

        def row(k):
            return jnp.concatenate([modB[8 * (k - 2) + j, 0:1, :] for j in range(NCH)], axis=1)

        def ln23(row0, M, A):
            ga = row(2); sb = row(3); cb = row(4)
            x = rows_u32(x_v, row0, M).astype(f32)
            xm = x + ga * A
            hB = _ln(xm) * (1.0 + cb) + sb
            n3 = _ln(hB).astype(bf16)
            return xm, hB, n3

        shifts = [-1, -1, 1, 1, -2, -2, 2, 2]

        def g_val():
            return jnp.concatenate(
                [h1buf[j, HALO + shifts[j]:HALO + shifts[j] + T, :] for j in range(NCH)], axis=1).astype(bf16)

        def out_copy(r0, n, k):
            return pltpu.make_async_copy(obuf.at[pl.ds(r0, n)], o_hbm.bitcast(u32).at[pl.ds(r0, n)], osems.at[k])

        def ln4(hs):
            gb = row(5)
            x1 = hb[0:T, :] + hs
            base = xmid[0:T, :] + gb * x1
            n4 = _ln(x1).astype(bf16)
            return base, n4

        def bfirst():
            for j in range(NCH):
                h1buf[j, 0:HALO, :] = jnp.zeros((HALO, 128), f32)
            h7 = _bf(hP[...])
            zb = pl.multiple_of(zero * 8, 8) if ZB else 0
            h0 = (T + HALO) // 2 // 16 * 16 + (16 if T == 128 else 0)
            halves = [(0, h0), (h0, T + HALO - h0)]
            nA = (2 * T + HALO - AT0) // AP
            st = {'res': None, 'As': [], 'n3': [], 'h1': [], 'macc': {}}

            def att(k):
                if AG:
                    st['o'] = attention2(AT0 + k * AP, AP, AG)
                else:
                    attention(qbuf, kbuf, vbuf, 0, AT0 + k * AP, AP, True)

            def tok_q(cc=0):
                qbuf[0, pl.ds(zb + S + HALO, 8), :] = st['res'][0:8, cc * 128:(cc + 1) * 128]

            for it in BA.split():
                k = int(it[1:]) if len(it) > 1 and it[1:].isdigit() else None
                if not ZB and it[0] in 'tWM':
                    continue
                if it[0] == 'T':
                    st['res'] = subdot(h7, TL, 7, k)
                elif it[0] == 'a':
                    att(k)
                elif it[0] == 't':
                    tok_q(k or 0)
                elif it[0] == 'w':
                    pW(7, k, zb)
                elif it[0] == 'v':
                    pW(6, k, zb)
                elif it[0] == 'm':
                    for kq in range(KQ):
                        pM(6 * NM + k, kq, zb, st['macc'], k)
                elif it[0] == 'M':
                    wmB_v[32, pl.ds(zb + D // 2, 8), :] = pltpu.bitcast(st['res'][0:8, 0:128], u32)
                elif it[0] == 'W':
                    wo_raw[7, pl.ds(zb + D // 2 + 16, 8), :] = pltpu.bitcast(st['res'][0:8, 0:128], u32)
                elif it[0] == 'o':
                    st['res'] = wo_dot(*halves[k])
                    st['As'].append(st['res'])
                elif it[0] == 'l':
                    r0, m = halves[k]
                    xm, hB, n3 = ln23(r0, m, st['As'][k])
                    xmid[r0:r0 + m, :] = xm
                    hb[r0:r0 + m, :] = hB
                    st['n3'].append(n3)
                elif it[0] == 'u':
                    r0, m = halves[k]
                    st['res'] = _dot(st['n3'][k], _bf(w1_v[...]))
                    h1 = _gelu(st['res'])
                    for j in range(NCH):
                        h1buf[j, HALO + r0:HALO + r0 + m, :] = h1[:, j * 128:(j + 1) * 128]
            hsbuf[0:T, :] = _dot(g_val(), _bf(w2_v[...]))

        if upto >= 3 and 'F' not in skip:
            bfirst()

        def carries(xm, hB, h1, notlast):
            xmid[0:HALO, :] = xmid[T:T + HALO, :]
            hb[0:HALO, :] = hb[T:T + HALO, :]
            for j in range(NCH):
                h1buf[j, 0:2 * HALO, :] = h1buf[j, T:T + 2 * HALO, :]
            xmid[HALO:HALO + T, :] = xm
            hb[HALO:HALO + T, :] = hB
            for j in range(NCH):
                h1j = h1[:, j * 128:(j + 1) * 128]
                h1buf[j, 2 * HALO:HALO + T, :] = h1j[0:T - HALO]
                h1buf[j, HALO + T:2 * HALO + T, :] = jnp.where(notlast, h1j[T - HALO:T], 0.0)

        RP = 16

        def bbody(i, carry):
            static = isinstance(i, int)
            if static:
                row0h = i * (T // 2)
                abase = (i + 1) * T
                abaseh = (i + 1) * (T // 2)
                z1 = pl.multiple_of(zero * 8, 8)
                z2 = pl.multiple_of(zero2 * 8, 8)
            else:
                row0h = pl.multiple_of(i * (T // 2), T // 2)
                nxt = jnp.minimum(i + 1, NT - 1)
                abase = pl.multiple_of(nxt * T, T)
                abaseh = pl.multiple_of(nxt * (T // 2), T // 2)
                z1 = pl.multiple_of((i >> 8) * 8, 8)
                z2 = pl.multiple_of((i >> 9) * 8, 8)
            ga = row(2); sb = row(3); cb = row(4); gb = row(5)
            bases, n4p, xms, hBs, n3p, As = [], [], [], [], [], []
            att = None
            asch = {}
            if AB == 9:
                att = Att(abase, abaseh, HALO, T, [int(t) for t in WGS], PD, z1)
                for t in ASCH.split():
                    k_, v_ = t.split(':')
                    asch[k_] = int(v_)

            def astep(tag):
                if att is not None and tag in asch:
                    att.steps(asch[tag])

            def p4(r):
                r0 = r * RP
                x1 = hb[r0:r0 + RP, :] + hsbuf[pl.ds(z2 + r0, RP), :]
                bases.append(xmid[r0:r0 + RP, :] + gb * x1)
                n4v = _ln(x1).astype(bf16)
                if EX4:
                    n4b[r0 // 2:(r0 + RP) // 2, :] = pltpu.bitcast(n4v, u32)
                n4p.append(n4v)

            def p23(r, A):
                r0 = r * RP
                x = rows_u32(x_v, (row0h, HALO + r0), RP).astype(f32)
                xm = x + ga * A[r0:r0 + RP]
                hB = _ln(xm) * (1.0 + cb) + sb
                xms.append(xm); hBs.append(hB)
                n3v = _ln(hB).astype(bf16)
                if EX3:
                    n3b[r0 // 2:(r0 + RP) // 2, :] = pltpu.bitcast(n3v, u32)
                n3p.append(n3v)

            for r in range(T // RP):
                if rel4[r] < 0:
                    p4(r)
            o = rows_u32(o_scr, (row0h, HALO), T)
            for n in range(NCH):
                An = _dot(o, _bf(wo_v[n]))
                As.append(An)
                r4 = [r for r in range(T // RP) if rel4[r] == n]
                if r4:
                    hsbuf[pl.ds(z1 + T, 8), 0:128] = An[0:8, 0:128]
                for r in r4:
                    p4(r)
                astep('o%d' % n)
            A = jnp.concatenate(As, axis=1)
            base = jnp.concatenate(bases, axis=0)
            n4 = _bf(n4b[...]) if EX4 else jnp.concatenate(n4p, axis=0)
            U = _dot(n4, _bf(w3_v[...]))
            u = _gelu(U).astype(bf16)
            for c in range(F // 128):
                r23 = [r for r in range(T // RP) if rel23[r] == NCH + c]
                if r23 or c in XT:
                    x_v[pl.ds(z1 + S // 2 + HALO // 2, 8), 0:128] = pltpu.bitcast(U[0:8, c * 128:(c + 1) * 128], u32)
                for r in r23:
                    p23(r, A)
                astep('c%d' % c)
            assert len(n3p) == T // RP and len(n4p) == T // RP
            xm = jnp.concatenate(xms, axis=0)
            hB = jnp.concatenate(hBs, axis=0)
            n3 = _bf(n3b[...]) if EX3 else jnp.concatenate(n3p, axis=0)
            h1 = _gelu(_dot(n3, _bf(w1_v[...])))
            carries(xm, hB, h1, i < NT - 1)
            if static:
                if i < NT - 1:
                    attention(qbuf, kbuf, vbuf, abase, HALO, T, False, abaseh)
            elif 'noatt' not in dbg:
                if AB == 9:
                    att.steps(999)
                    att.rest()
                    if DL:
                        h1buf[0, pl.ds(z1 + T + 2 * HALO, 8), :] = att.OC[T // RB - 1, NCH - 1]
                elif AB:
                    attention2(HALO, T, AB, abase, abaseh)
                else:
                    attention(qbuf, kbuf, vbuf, abase, HALO, T, False, abaseh)
            h2 = _dot(u, _bf(w4_v[...]))
            if static:
                obuf[(i - 1) * (T // 2):i * (T // 2), :] = pltpu.bitcast((base + gb * h2).astype(bf16), u32)
            else:
                obuf[pl.ds(pl.multiple_of((i - 1) * (T // 2), T // 2), T // 2), :] = pltpu.bitcast((base + gb * h2).astype(bf16), u32)
            hsbuf[0:T, :] = _dot(g_val(), _bf(w2_v[...]))
            return carry

        if upto >= 4:
            if UB:
                for i in range(1, 1 + UB):
                    bbody(i, 0)
                    if i in BAR:
                        out_copy_i(i).start()
                if 1 + UB < NT:
                    lax.fori_loop(1 + UB, NT, bbody, 0)
            else:
                lax.fori_loop(1, NT, bbody, 0)

        def blast():
            r0 = (NT - 1) * (T // 2)
            out_copy(0, r0, 0).start()
            base, n4 = ln4(hsbuf[0:T, :])
            if BL:
                FC = F // BL
                xmid[0:T, :] = base
                n4b[...] = pltpu.bitcast(n4, u32)
                hsbuf[0:T, :] = jnp.zeros((T, D), f32)

                def body(c, carry):
                    w3c = w3_v[:, pl.ds(pl.multiple_of(c * FC, 128), FC)]
                    u = _gelu(_dot(_bf(n4b[...]), _bf(w3c))).astype(bf16)
                    w4c = w4_v[pl.ds(pl.multiple_of(c * (FC // 2), 32), FC // 2), :]
                    hsbuf[0:T, :] += _dot(u, _bf(w4c))
                    return carry

                lax.fori_loop(0, BL, body, 0)
                obuf[r0:r0 + T // 2, :] = pltpu.bitcast((xmid[0:T, :] + row(5) * hsbuf[0:T, :]).astype(bf16), u32)
            else:
                u = _gelu(_dot(n4, _bf(w3_v[...]))).astype(bf16)
                h2 = _dot(u, _bf(w4_v[...]))
                obuf[r0:r0 + T // 2, :] = pltpu.bitcast((base + row(5) * h2).astype(bf16), u32)
            out_copy(r0, T // 2, 1).start()
            out_copy(0, r0, 0).wait()
            out_copy(r0, T // 2, 1).wait()

        if upto >= 5 and 'L' not in skip:
            blast()

    @jax.jit
    def fn(A_x, A_wqkv, A_wo, B_x, B_w1, B_w2, B_w3, B_w4, c, w_mod):
        x = A_x.reshape(S, D)
        any_spec = pl.BlockSpec(memory_space=pl.ANY)
        out = pl.pallas_call(
            kernel,
            in_specs=[any_spec] * 9,
            out_specs=any_spec,
            out_shape=jax.ShapeDtypeStruct((S, D), bf16),
            scratch_shapes=[
                pltpu.VMEM((S // 2 + HALO // 2 + 8, D), u32),
                pltpu.VMEM((D // 2 + 32, 3 * D), u32),
                pltpu.VMEM((D // 2, D), u32),
                pltpu.VMEM((D // 2, D), u32),
                pltpu.VMEM((D // 2, D), u32),
                pltpu.VMEM((NCH + WS, D // 2 + 32, 128), u32),
                pltpu.VMEM((NCH + WS, D // 2, 128), u32),
                pltpu.VMEM((D // 2, D), u32),
                pltpu.VMEM((D // 2, D), u32),
                pltpu.VMEM((D // 2, F), u32),
                pltpu.VMEM((F // 2, D), u32),
                pltpu.VMEM((D // 2, 128), f32),
                pltpu.VMEM((D // 2, 128), f32),
                pltpu.VMEM((8, D // 2 + 16, 256), u32),
                pltpu.VMEM((33, D // 2 + 32, 128), u32),
                pltpu.VMEM((8, 8, 256), f32),
                pltpu.VMEM((36, 8, 128), f32),
                pltpu.VMEM((3 if MU else NCH, S + 32, 128), f32),
                pltpu.VMEM((PR // 2, 128), u32),
                pltpu.VMEM((S // 2, 128), u32),
                pltpu.VMEM((NCH, S + 32, 128), f32),
                pltpu.VMEM((NCH, S + 2 * HALO + 32 * (AB == 9), 128), f32),
                pltpu.VMEM((NCH, S + 2 * HALO + 32 * (AB == 9), 128), f32),
                pltpu.VMEM((T + HALO, D), f32),
                pltpu.VMEM((T + HALO, D), f32),
                pltpu.VMEM((NCH, T + 2 * HALO + 32 * DL, 128), f32),
                pltpu.VMEM((S // 2, D), u32),
                pltpu.VMEM((S // 2 + HALO // 2, D), u32),
                pltpu.VMEM((T + 32, D), f32),
                pltpu.VMEM((T // 2, D), u32),
                pltpu.VMEM((T // 2, D), u32),
                pltpu.VMEM((1, D), bf16),
            ] + ([pltpu.VMEM((padr, 128), f32)] if padr else []) + [
                pltpu.SMEM((8,), jnp.int32),
                pltpu.SemaphoreType.DMA((NSEM,)),
                pltpu.SemaphoreType.DMA((2,)),
            ],
            compiler_params=pltpu.CompilerParams(vmem_limit_bytes=120 * 1024 * 1024),
        )(x, A_wqkv, A_wo, B_w1, B_w2, B_w3, B_w4, c, w_mod)
        return out.reshape(1, S, D)
    return fn


_fn = make()


def pallas_adaLN_cond__sliding_local_dilated__mixer_s_mlp__prompt_kernel(A_x, A_wqkv, A_wo, B_x, B_w1, B_w2, B_w3, B_w4, c, w_mod):
    return _fn(A_x, A_wqkv, A_wo, B_x, B_w1, B_w2, B_w3, B_w4, c, w_mod)
```

```python
import functools
import jax
import jax.numpy as jnp
from jax import lax
import jax.experimental.pallas as pl
import jax.experimental.pallas.tpu as pltpu

S, D, F = 2048, 1024, 3584
H, DH, W, DIL = 32, 32, 8, 2
NCH = D // 128
EPS = 1e-5
SCALE = DH ** -0.5
f32, bf16, u32 = jnp.float32, jnp.bfloat16, jnp.uint32
HALO = 16


def _ln(x):
    m = jnp.mean(x, axis=-1, keepdims=True)
    xc = x - m
    v = jnp.mean(xc * xc, axis=-1, keepdims=True)
    return xc * lax.rsqrt(v + EPS)


def _gelu(x):
    c0 = 0.7978845608028654
    c1 = c0 * 0.044715
    t = jnp.tanh(x * (c0 + c1 * (x * x)))
    hx = 0.5 * x
    return hx + hx * t


def _dot(a, b):
    return jnp.dot(a, b, preferred_element_type=f32)


def _bf(w):
    return pltpu.bitcast(w, bf16)


def _lane_xor(x, s):
    lane = lax.broadcasted_iota(jnp.int32, x.shape, 1)
    return jnp.take_along_axis(x, lane ^ s, axis=1)


def _exchange8_multi(XS):
    XS = [list(X) for X in XS]
    lane = lax.broadcasted_iota(jnp.int32, XS[0][0].shape, 1)
    for t in range(3):
        s = 1 << (t + 2)
        m = (lane & s) != 0
        for X in XS:
            for p in range(8):
                if p & (1 << t):
                    continue
                p2 = p | (1 << t)
                tmp = _lane_xor(jnp.where(m, X[p], X[p2]), s)
                X[p], X[p2] = jnp.where(m, tmp, X[p]), jnp.where(m, X[p2], tmp)
    return XS


def _group4_sum(acc):
    lane = lax.broadcasted_iota(jnp.int32, acc.shape, 1)
    acc = acc + jnp.where((lane & 1) != 0, pltpu.roll(acc, 1, 1), pltpu.roll(acc, 127, 1))
    acc = acc + jnp.where((lane & 2) != 0, pltpu.roll(acc, 2, 1), pltpu.roll(acc, 126, 1))
    return acc


def make(T=128, PR=512, RB=8, EG=4, upto=9, AT0=0, AP=16,
         DO='c X0 Wq sa ca X1 Wk Wv X2 X3 X4 X5 X6 X7 X8 X9 X10 X12 X13 X11 X14 X15',
         PS=None, PSX=None, RL=1, D0='1234567', LP=16, BL='M', ZB=1,
         order0='T0 T1 X x00 x01 m0 T2 T3 X x10 x11 h0 T4 T5 X x20 H0 X x21 H1 H2 H3 H4 H5', NDEF=6, BA=None,
         side=None, KQ=4, KQ0=1, NM=5, NR=8, AG=1,
         rel4=(-1, -1, -1, 0, 1, 2, 3, 4), rel23=(8, 9, 10, 11, 12, 13, 14, 15),
         padr=0, dbg='', UB=0, BAR=(), GL=0, MU=1, WS=1, skip='', AB=9, WGS='1'*128, PD=0, ASCH='', DL=0, EX3=1, EX4=1, XT=(), MT=(4, 10, 16, 22), MA=0, MN=(1024,), NZ=8, NU=2, BPD=0, BQD=None, BWG=8):
    HS, HO = (2, 0) if MU else (0, S // 2)
    NT = S // T
    NP = S // PR
    order0 = order0.split()
    TL = S - PR
    if PS is None:
        PS = ('wc C wX0 L0 wWq e0 wsa S wca A h0 wX1 u0:0 L1 wWk u1:0 e1 wWv u0:1 u1:1 e2 wX2 u0:2 u1:2 L2 u2:0 '
              'wX3 wX4 u2:12 L3 u3:012 L4 u4:0 wX5 wX6 wX7 u4:12 L5 u5:012 L6 u6:012 L7 u7:0 '
              'wX8 wX9 wX10 wX12 wX13 u7:12 L8 u8:012 L9 u9:012 L10 ua:0 L12 L13 wX11 wX14 wX15 DW ua:12 L11 ub:012 L14 L15')
    if BA is None:
        BA = ('a0 a1 T0 T1 t0 a2 a3 W w0 w1 w2 w3 w4 w5 w6 w7 T2 t0 a4 a5 T3 t0 a6 a7 T4 t0 a8 a9 T5 t0 a10 o0 t0 a11 t4 a12 '
              'o1 t0 a13 t4 a14 M m0 m1 l0 l1 u0 t0 a15 t4 a16 u1')
    if WS and 'v0' not in BA:
        BA = BA.replace('W w0 w1 w2 w3 w4 w5 w6 w7', 'W v0 v1 v2 v3 v4 v5 v6 v7 w0 w1 w2 w3 w4 w5 w6 w7')
    if PSX:
        for k_, v_ in PSX.items():
            assert (' ' + k_ + ' ') in PS
            PS = PS.replace(' ' + k_ + ' ', ' ' + k_ + ' ' + v_ + ' ')
    S_C, S_X, S_SA, S_CA, S_W0, S_WQ, S_WO, S_MB, S_W = 0, 1, 17, 25, 33, 36, 44, 52, 60
    NSEM = 64
    DEF = list(range(6 - NDEF, 6))
    tags = ['T%d' % sd for sd in DEF] + ['%dH%d' % (p, sd) for p in range(NP) for sd in range(6 if p < NP - 1 else 6 - NDEF)]
    if side is None:
        side = 'W:7,9,11,13,15,17,19,21 M:4,5,6,7,8,9,10,11,12,13,14,15,16,17,18,19,20,21,22,22'
    if isinstance(side, str):
        sd_ = {}
        for grp in side.split():
            kind, lst = grp.split(':')
            for k, t in enumerate(lst.split(',')):
                sd_.setdefault(tags[int(t)], []).append(kind + str(k))
        side = sd_
    assert sum(1 for v in side.values() for j in v if j[0] in 'Aa') * AP == AT0

    def kernel(*refs):
        pl.run_scoped(functools.partial(body, *refs), pltpu.SemaphoreType.DMA((NSEM,)), pltpu.SemaphoreType.DMA((2,)))

    def body(x_hbm, wqkv_hbm, wo_hbm, w1_hbm, w2_hbm, w3_hbm, w4_hbm, c_hbm, wmod_hbm,
             o_hbm,
             x_v, wqkv_raw, wq_v, wk_v, wv_v, wo_raw, wo_v, w1_v, w2_v, w3_v, w4_v, cE, cO, wmA_v, wmB_v,
             modA, modB, xhat, hP, h0, qbuf, kbuf, vbuf, xmid, hb, h1buf, obuf, o_scr, hsbuf, n4b, n3b, baseb, c_v, *rest):
        zsm, sems, osems = rest[-3:]

        def cp(src, dst, k):
            return pltpu.make_async_copy(src, dst, sems.at[k])

        xu = x_hbm.bitcast(u32)
        wqkvu = wqkv_hbm.bitcast(u32)
        wou = wo_hbm.bitcast(u32)
        wmodu = wmod_hbm.bitcast(u32)

        def lane_ds(k, n, base=0):
            if isinstance(k, int):
                return pl.ds(base + k * n, n)
            return pl.ds(pl.multiple_of(base + k * n, 128), n)

        def row_ds(base, k, n):
            if isinstance(k, int):
                return pl.ds(base + k * n, n)
            return pl.ds(pl.multiple_of(base + k * n, 8), n)

        c_c = cp(c_hbm, c_v, S_C)

        def c_x(b):
            return cp(xu.at[b * 64:(b + 1) * 64], x_v.at[b * 64:(b + 1) * 64], S_X + b)

        def c_sa(k):
            return cp(wmodu.at[:, lane_ds(k, 128)], wmA_v.at[k, 0:D // 2, 0:128], S_SA + k)

        def c_ca(k):
            return cp(wmodu.at[:, lane_ds(k, 128, D)], wmA_v.at[k, 0:D // 2, 128:256], S_CA + k)

        def c_w0(b):
            return cp(wqkvu.at[0:64, b * D:(b + 1) * D], wqkv_raw.at[0:64, b * D:(b + 1) * D], S_W0 + b)

        def c_wq(k):
            return cp(wqkvu.at[row_ds(0, k, 64)], wqkv_raw.at[row_ds(0, k, 64)], S_WQ + k)

        def c_wo(p):
            return cp(wou.at[:, lane_ds(p, 128)], wo_raw.at[p, 8:8 + D // 2], S_WO + p)

        def c_mb(t, g):
            return cp(wmodu.at[:, lane_ds(t, 128, 2 * D)], wmB_v.at[t, 0:D // 2], S_MB + g)

        c_w = [cp(w1_hbm.bitcast(u32), w1_v, S_W), cp(w2_hbm.bitcast(u32), w2_v, S_W + 1),
               cp(w3_hbm.bitcast(u32), w3_v, S_W + 2), cp(w4_hbm.bitcast(u32), w4_v, S_W + 3)]

        def named(nm):
            if nm == 'c':
                return c_c
            if nm == 'sa':
                return c_sa(0)
            if nm == 'ca':
                return c_ca(0)
            if nm[0] == 'W':
                return c_w0('qkv'.index(nm[1]))
            return c_x(int(nm[1:]))

        for nm in DO.split():
            named(nm).start()
        def start_group(g):
            if g == 'W':
                if upto >= 3:
                    c_wo(7).start()
                    for t in range(6 * NM, 32):
                        c_mb(t, 6).start()
                    for c in c_w:
                        c.start()
            elif upto >= 2 and 'nodma2' not in dbg:
                r = int(g)
                c_sa(r).start()
                c_ca(r).start()
                c_wq(r).start()
                c_wo(r - 1).start()
                if r >= 2:
                    for i in range(NM):
                        c_mb(NM * (r - 2) + i, r - 2).start()

        for g in D0:
            start_group(g)
        assert sorted(list(D0) + [it[1] for it in PS.split() if it[0] == 'D']) == list('1234567W')

        def _zinit(i, carry):
            zsm[2 + i] = i >> 8
            return carry

        lax.fori_loop(0, 3, _zinit, 0)
        zp3 = pl.multiple_of(zsm[4] * 8, 8)
        zp1 = pl.multiple_of(zsm[2] * 8, 8)
        zp2 = pl.multiple_of(zsm[3] * 8, 8)

        x_v[S // 2:S // 2 + HALO // 2, :] = jnp.zeros((HALO // 2, D), u32)
        for j in range(NCH):
            z = jnp.zeros((HALO, 128), f32)
            qbuf[j, S:S + HALO, :] = z
            kbuf[j, HALO + S:2 * HALO + S, :] = z
            vbuf[j, HALO + S:2 * HALO + S, :] = z
            kbuf[j, 0:HALO, :] = z
            vbuf[j, 0:HALO, :] = z
            wo_raw[j, 0:8, :] = jnp.zeros((8, 128), u32)
            wo_raw[j, 8 + D // 2:16 + D // 2, :] = jnp.zeros((8, 128), u32)

        def mv_part(w, r0, acc):
            n = w.shape[0]
            lo = pltpu.bitcast(w << 16, f32)
            hi = pltpu.bitcast(w & jnp.uint32(0xFFFF0000), f32)
            pr = lo * cE[r0:r0 + n, :] + hi * cO[r0:r0 + n, :]
            for t in range(n // 8):
                acc = pr[8 * t:8 * t + 8] if acc is None else acc + pr[8 * t:8 * t + 8]
            return acc

        wparts = (wq_v, wk_v, wv_v)
        bufs = (qbuf, kbuf, vbuf)

        def exch_groups(grps):
            for g0 in range(0, len(grps), EG):
                gs = grps[g0:g0 + EG]
                XS = [[wqkv_raw[row_ds(rg * 8, k * 8, 8), b * D + a * 128:b * D + (a + 1) * 128] for a in range(NCH)]
                      for (k, b, rg) in gs]
                YS = _exchange8_multi(XS)
                for (k, b, rg), Y in zip(gs, YS):
                    wparts[b][row_ds(rg * 8, k * 8, 8), :] = jnp.concatenate(Y, axis=1)

        def subdot(lhs, row0, kc, sd, init=False, valid=None):
            b, hf = sd // 2, sd % 2
            n = lhs.shape[0]
            res = _dot(lhs, _bf(wparts[b][row_ds(0, kc, 64), hf * 512:(hf + 1) * 512]))
            o = row0 + (0 if b == 0 else HALO)
            for jj in range(4):
                j = hf * 4 + jj
                if init:
                    bufs[b][j, o:o + n, :] = res[:, jj * 128:(jj + 1) * 128]
                elif valid is not None:
                    bufs[b][j, o:o + n, :] = jnp.where(valid, bufs[b][j, o:o + n, :], 0.0) + res[:, jj * 128:(jj + 1) * 128]
                else:
                    bufs[b][j, o:o + n, :] += res[:, jj * 128:(jj + 1) * 128]
            return res

        def prologue():
            st = {}

            def crep():
                c = c_v[...].astype(f32)
                scf = (c * jax.nn.sigmoid(c)).astype(bf16).astype(f32)
                rr = lax.broadcasted_iota(jnp.int32, (128, 128), 0)
                ll = lax.broadcasted_iota(jnp.int32, (128, 128), 1)
                sel = ll == jnp.where(rr < 64, 2 * rr, 2 * rr - 127)
                for j in range(NCH):
                    dg = jnp.where(sel, jnp.broadcast_to(scf[:, j * 128:(j + 1) * 128], (128, 128)), 0.0).astype(bf16)
                    rep = _dot(dg, jnp.ones((128, 128), bf16))
                    cE[j * 64:(j + 1) * 64, :] = rep[0:64]
                    cO[j * 64:(j + 1) * 64, :] = rep[64:128]

            def h_store(r0, xh0):
                h = (xh0 * (1.0 + st['ca']) + st['sa']).astype(bf16)
                if r0 < TL:
                    xhat[HS, HO + r0 // 2:HO + (r0 + LP) // 2, :] = pltpu.bitcast(h, f32)
                else:
                    hP[(r0 - TL) // 2:(r0 - TL + LP) // 2, :] = pltpu.bitcast(h, u32)

            def h0_lhs(b0, nb, gated):
                r0 = HO + b0 * 64
                if not gated:
                    return _bf(xhat[HS, r0:r0 + nb * 64, :])
                if GL:
                    return jnp.concatenate([_bf(xhat[HS, r0:r0 + nb * 64 - 8, :]), _bf(xhat[HS, pl.ds(zp3 + r0 + nb * 64 - 8, 8), :])], axis=0)
                return jnp.concatenate([_bf(xhat[HS, pl.ds(zp3 + r0, 8), :]), _bf(xhat[HS, r0 + 8:r0 + nb * 64, :])], axis=0)

            def ln_piece(b, i):
                r0 = b * 128 + i * LP
                direct = 'ca' in st and 'sa' in st
                if MU:
                    x = _bf(x_v[pl.ds(zp1 + r0 // 2, LP // 2), :]).astype(f32)
                    m = jnp.mean(x, axis=-1, keepdims=True)
                    if RL:
                        x = _bf(x_v[pl.ds(zp2 + r0 // 2, LP // 2), :]).astype(f32)
                    xc = x - m
                    rs = lax.rsqrt(jnp.mean(xc * xc, axis=-1, keepdims=True) + EPS)
                    xhat[0, r0:r0 + LP, :] = jnp.broadcast_to(m, (LP, 128))
                    xhat[1, r0:r0 + LP, :] = jnp.broadcast_to(rs, (LP, 128))
                    if direct:
                        h_store(r0, xc[:, 0:128] * rs)
                    return
                if RL:
                    m = jnp.mean(_bf(x_v[pl.ds(zp1 + r0 // 2, LP // 2), :]).astype(f32), axis=-1, keepdims=True)
                    xc = _bf(x_v[pl.ds(zp2 + r0 // 2, LP // 2), :]).astype(f32) - m
                    v = jnp.mean(xc * xc, axis=-1, keepdims=True)
                    xh = (_bf(x_v[r0 // 2:(r0 + LP) // 2, :]).astype(f32) - m) * lax.rsqrt(v + EPS)
                else:
                    xh = _ln(_bf(x_v[pl.ds(zp1 + r0 // 2, LP // 2), :]).astype(f32))
                for j in range(1 if direct else 0, NCH):
                    xhat[j, r0:r0 + LP, :] = xh[:, j * 128:(j + 1) * 128]
                if direct:
                    h_store(r0, xh[:, 0:128])

            def ln_block(b):
                for i in range(128 // LP):
                    ln_piece(b, i)

            def hblk(b):
                for i in range(128 // LP):
                    r0 = b * 128 + i * LP
                    if MU:
                        x = _bf(x_v[r0 // 2:(r0 + LP) // 2, 0:128]).astype(f32)
                        h_store(r0, (x - xhat[0, r0:r0 + LP, :]) * xhat[1, r0:r0 + LP, :])
                    else:
                        h_store(r0, xhat[0, r0:r0 + LP, :])

            for it in PS.split():
                if it[0] == 'w':
                    named(it[1:]).wait()
                elif it[0] == 'D':
                    start_group(it[1])
                elif it == 'C':
                    crep()
                elif it[0] == 'L':
                    ln_block(int(it[1:]))
                elif it[0] == 'h':
                    hblk(int(it[1:]))
                elif it == 'S':
                    st['sa'] = jnp.sum(mv_part(wmA_v[0, 0:D // 2, 0:128], 0, None), axis=0, keepdims=True)
                elif it == 'A':
                    st['ca'] = jnp.sum(mv_part(wmA_v[0, 0:D // 2, 128:256], 0, None), axis=0, keepdims=True)
                elif it[0] == 'e':
                    exch_groups([(0, int(it[1]), rg) for rg in range(8)])
                elif it[0] == 'p':
                    b_, i_ = it[1:].split(':')
                    ln_piece(int(b_), int(i_))
                elif it[0] == 't':
                    x_v[pl.ds(zp3 + S // 2 + HALO // 2, 8), 0:128] = pltpu.bitcast(st['res'][0:8, 0:128], u32)
                elif it[0] in 'sg':
                    blks, sd = it[1:].split(':')
                    b0, nb = int(blks[0], 16), len(blks)
                    st['res'] = subdot(h0_lhs(b0, nb, it[0] == 'g'), b0 * 128, 0, int(sd), True)
                elif it[0] == 'u':
                    blks, parts = it[1:].split(':')
                    b0, nb = int(blks[0], 16), len(blks)
                    lhs = h0_lhs(b0, nb, False)
                    for p in parts:
                        subdot(lhs, b0 * 128, 0, 2 * int(p), True)
                        st['res'] = subdot(lhs, b0 * 128, 0, 2 * int(p) + 1, True)

        if 'P' not in skip:
            prologue()

        def attention(qb, kb, vb, base, off, M, mask_rows, baseh=None):
            row0 = base + off

            def kvds(r, w):
                return pl.ds(base + (off + HALO + r - DIL * w), RB)

            o_rows = []
            for r in range(0, M, RB):
                q = [qb[j, pl.ds(base + (off + r), RB), :] for j in range(NCH)]
                s = []
                for w in range(W):
                    acc = None
                    for j in range(NCH):
                        p = q[j] * kb[j, kvds(r, w), :]
                        acc = p if acc is None else acc + p
                    acc = _group4_sum(acc)
                    if mask_rows and off + r < DIL * (W - 1) and w > 0:
                        rows = row0 + r + lax.broadcasted_iota(jnp.int32, (RB, 128), 0)
                        acc = jnp.where(rows >= DIL * w, acc, -1e30)
                    s.append(acc)
                m = functools.reduce(jnp.maximum, s)
                e = [jnp.exp((sw - m) * SCALE) for sw in s]
                den = functools.reduce(lambda a, b: a + b, e)
                rinv = 1.0 / den
                oc = []
                for j in range(NCH):
                    acc = None
                    for w in range(W):
                        p = e[w] * vb[j, kvds(r, w), :]
                        acc = p if acc is None else acc + p
                    oc.append(acc * rinv)
                o_rows.append(jnp.concatenate(oc, axis=1))
            o = jnp.concatenate(o_rows, axis=0).astype(bf16)
            if isinstance(row0, int):
                o_scr[row0 // 2:(row0 + M) // 2, :] = pltpu.bitcast(o, u32)
            elif baseh is not None:
                o_scr[pl.ds(baseh + off // 2, M // 2), :] = pltpu.bitcast(o, u32)
            else:
                o_scr[pl.ds(pl.multiple_of(row0 // 2, 8), M // 2), :] = pltpu.bitcast(o, u32)


        def attention2(off, M, G, base=None, baseh=None):
            o_rows = []

            def rs_(a):
                return slice(a, a + RB) if base is None else pl.ds(base + a, RB)

            for r0 in range(0, M, RB * G):
                rs = [off + r0 + g * RB for g in range(G) if r0 + g * RB < M]
                lane = lax.broadcasted_iota(jnp.int32, (RB, 128), 1)
                S_ = {}
                for r in rs:
                    q = [qbuf[j, rs_(r), :] for j in range(NCH)]
                    for w in range(W):
                        acc = None
                        for j in range(NCH):
                            k0 = HALO + r - DIL * w
                            p = q[j] * kbuf[j, rs_(k0), :]
                            acc = p if acc is None else acc + p
                        S_[r, w] = acc
                keys = list(S_)
                for sh in (1, 2):
                    R = {k: (pltpu.roll(S_[k], sh, 1), pltpu.roll(S_[k], 128 - sh, 1)) for k in keys}
                    for k in keys:
                        S_[k] = S_[k] + jnp.where((lane & sh) != 0, R[k][0], R[k][1])
                for r in rs:
                    s = []
                    for w in range(W):
                        acc = S_[r, w]
                        if base is None and r < DIL * (W - 1) and w > 0:
                            rows = r + lax.broadcasted_iota(jnp.int32, (RB, 128), 0)
                            acc = jnp.where(rows >= DIL * w, acc, -1e30)
                        s.append(acc)
                    m = functools.reduce(jnp.maximum, s)
                    e = [jnp.exp((sw - m) * SCALE) for sw in s]
                    den = functools.reduce(lambda a, b: a + b, e)
                    rinv = 1.0 / den
                    oc = []
                    for j in range(NCH):
                        acc = None
                        for w in range(W):
                            k0 = HALO + r - DIL * w
                            p = e[w] * vbuf[j, rs_(k0), :]
                            acc = p if acc is None else acc + p
                        oc.append(acc * rinv)
                    o_rows.append(jnp.concatenate(oc, axis=1))
            o = jnp.concatenate(o_rows, axis=0).astype(bf16)
            if base is None:
                o_scr[off // 2:(off + M) // 2, :] = pltpu.bitcast(o, u32)
            else:
                o_scr[pl.ds(baseh + off // 2, M // 2), :] = pltpu.bitcast(o, u32)
            return o

        class Att:
            def __init__(self, base, baseh, off, M, wgs, PD, ztok, QD=None, mask=False):
                self.base, self.baseh, self.off, self.PD, self.ztok = base, baseh, off, PD, ztok
                self.QD, self.mask = QD, mask
                self.nrb = M // RB
                self.wgs = list(wgs)
                assert sum(self.wgs) == self.nrb * W
                self.Q, self.SS, self.E, self.OC = {}, {}, {}, {}
                self.win = 0
                self.done = 0

            def scores(self, wl):
                lane = lax.broadcasted_iota(jnp.int32, (RB, 128), 1)
                accs = []
                for (rb, w) in wl:
                    r = self.off + rb * RB
                    if rb not in self.Q:
                        if self.QD is not None and rb * W - self.QD >= 0:
                            qbuf[0, pl.ds(self.ztok + S + HALO, 8), :] = self.SS[divmod(rb * W - self.QD, W)]
                        self.Q[rb] = [qbuf[j, pl.ds(self.base + r, RB), :] for j in range(NCH)]
                    acc = None
                    for j in range(NCH):
                        p = self.Q[rb][j] * kbuf[j, pl.ds(self.base + (HALO + r - DIL * w), RB), :]
                        acc = p if acc is None else acc + p
                    accs.append(acc)
                for sh in (1, 2):
                    R = [(pltpu.roll(a, sh, 1), pltpu.roll(a, 128 - sh, 1)) for a in accs]
                    accs = [a + jnp.where((lane & sh) != 0, x, y) for a, (x, y) in zip(accs, R)]
                for k, a in zip(wl, accs):
                    r = self.off + k[0] * RB
                    if self.mask and r < DIL * (W - 1) and k[1] > 0:
                        rows = r + lax.broadcasted_iota(jnp.int32, (RB, 128), 0)
                        a = jnp.where(rows >= DIL * k[1], a, -1e30)
                    self.SS[k] = a
                    if k[1] == W - 1:
                        self.softmax(k[0])

            def softmax(self, rb):
                s = [self.SS[rb, w] for w in range(W)]
                m = functools.reduce(jnp.maximum, s)
                e = [jnp.exp((sw - m) * SCALE) for sw in s]
                den = functools.reduce(lambda a, b: a + b, e)
                self.E[rb] = (e, 1.0 / den)

            def pv(self):
                rb, j = divmod(self.done, NCH)
                self.done += 1
                r = self.off + rb * RB
                e, rinv = self.E[rb]
                acc = None
                for w in range(W):
                    p = e[w] * vbuf[j, pl.ds(self.base + (HALO + r - DIL * w), RB), :]
                    acc = p if acc is None else acc + p
                self.OC[rb, j] = acc * rinv
                if rb % 2 == 1 and j == NCH - 1:
                    o = jnp.concatenate([jnp.concatenate([self.OC[q, c] for c in range(NCH)], axis=1) for q in (rb - 1, rb)], axis=0)
                    o_scr[pl.ds(self.baseh + (self.off + (rb - 1) * RB) // 2, RB), :] = pltpu.bitcast(o.astype(bf16), u32)

            def token(self, v):
                vbuf[0, pl.ds(self.ztok + S + 2 * HALO, 8), :] = v

            def steps(self, n):
                for _ in range(n):
                    if not self.wgs:
                        return
                    g = self.wgs.pop(0)
                    wl = [divmod(self.win + t, W) for t in range(g)]
                    self.win += g
                    self.scores(wl)
                    tok = False
                    while self.done < self.nrb * NCH and self.done + W + self.PD <= self.win - 1 and self.done // NCH in self.E:
                        if not tok:
                            self.token(self.SS[wl[-1]])
                            tok = True
                        self.pv()

            def rest(self, n=999):
                while self.done < self.nrb * NCH and n > 0:
                    self.pv(); n -= 1

        sub = lax.broadcasted_iota(jnp.int32, (8, 128), 0)

        def pW(p, q, z):
            for tv in range(8 * q, 8 * q + 8):
                j = tv >> 3
                hh = (tv >> 1) & 3
                a2 = tv & 1
                parts = []
                for al in range(4):
                    a = a2 * 4 + al
                    src = a * 64 + hh * 16 + j * 2
                    st = src - 2 * al + 8
                    if isinstance(z, int):
                        parts.append(wo_raw[p, z + st:z + st + 8, :])
                    else:
                        parts.append(wo_raw[p, pl.ds(z + st, 8), :])
                v = jnp.where(sub < 2, parts[0], parts[1])
                v2 = jnp.where(sub < 6, parts[2], parts[3])
                wo_v[p, 8 * tv:8 * tv + 8, :] = jnp.where(sub < 4, v, v2)

        def pM(t, kq, z, macc, key):
            n = D // 2 // KQ
            rows = pl.ds(z + kq * n, n)
            macc[key] = mv_part(wmB_v[t, rows, :], kq * n, macc.get(key))
            if kq == KQ - 1:
                modB[t, 0:1, :] = jnp.sum(macc[key], axis=0, keepdims=True)

        def region_waits(r):
            c_sa(r).wait(); c_ca(r).wait(); c_wq(r).wait()
            if not WS:
                c_wo(r - 1).wait()

            @pl.when(r >= 2)
            def _():
                if WS:
                    c_wo(r - 2).wait()
                for i in range(NM):
                    c_mb(NM * (r - 2) + i, r - 2).wait()

        if 'prewait' in dbg:
            for r in range(1, 8):
                region_waits(r)

        def region(r, carry):
            if 'prewait' not in dbg and 'nodma2' not in dbg:
                region_waits(r)
            z1 = pl.multiple_of((r >> 8) * 8, 8)
            z2 = pl.multiple_of((r >> 9) * 8, 8)
            pm = [jnp.where(r >= 2, NM * (r - 2) + i, 32) for i in range(NM)]
            pw = jnp.where(r >= 2, r - 2, NCH) if WS else r - 1
            hp = _bf(hP[...])
            st = {'acc': [None, None], 'res': None}
            macc = {}

            def mvp(kq):
                n = D // 2 // KQ0
                for q in range(2):
                    st['acc'][q] = mv_part(wmA_v[r, pl.ds(z2 + kq * n, n), q * 128:(q + 1) * 128], kq * n, st['acc'][q])
                if kq == KQ0 - 1:
                    st['sa'] = jnp.sum(st['acc'][0], axis=0, keepdims=True)
                    st['ca'] = jnp.sum(st['acc'][1], axis=0, keepdims=True)
                    modA[r, 0:1, 0:128] = st['sa']
                    modA[r, 0:1, 128:256] = st['ca']

            def hpass(p):
                if MU:
                    x = _bf(x_v[p * PR // 2:(p + 1) * PR // 2, lane_ds(r, 128)]).astype(f32)
                    xh = (x - xhat[0, p * PR:(p + 1) * PR, :]) * xhat[1, p * PR:(p + 1) * PR, :]
                else:
                    xh = xhat[r, p * PR:(p + 1) * PR, :]
                st['h'] = (xh * (1.0 + st['ca']) + st['sa']).astype(bf16)
                st['row'] = p * PR
                if p == NP - 1:
                    hP[...] = pltpu.bitcast(st['h'], u32)

            def do_side(tag):
                jobs = side.get(tag, ())
                if not jobs:
                    return
                tk = pltpu.bitcast(st['res'][0:8, 0:128], u32)
                kinds = set(j[0] for j in jobs)
                if 'W' in kinds:
                    wo_raw[pw, pl.ds(z1 + D // 2 + 16, 8), :] = tk
                if 'M' in kinds:
                    wmB_v[32, pl.ds(z1 + D // 2, 8), :] = tk
                if 'A' in kinds:
                    qbuf[0, pl.ds(z1 + S + HALO, 8), :] = pltpu.bitcast(tk, f32)
                for j in jobs:
                    k = int(j[1:])
                    if j[0] == 'W':
                        pW(pw, k, z2)
                    elif j[0] == 'w':
                        pW(pw, k, 0)
                    elif j[0] == 'M':
                        pM(pm[k // KQ], k % KQ, z2, macc, k // KQ)
                    elif j[0] in 'Aa':
                        attention(qbuf, kbuf, vbuf, 0, k * AP, AP, True)

            for it in order0:
                if it[0] == 'T':
                    st['res'] = subdot(hp, TL, r - 1, int(it[1]), valid=r >= 2)
                    do_side(it)
                elif it[0] == 'H':
                    st['res'] = subdot(st['h'], st['row'], r, int(it[1]))
                    do_side('0' + it)
                elif it[0] == 'm':
                    mvp(int(it[1]))
                elif it[0] == 'K':
                    q = int(it[1:] or 0) * 128
                    wmA_v[r, pl.ds(z1 + D // 2, 8), 0:128] = pltpu.bitcast(st['res'][q:q + 8, 0:128], u32)
                elif it[0] == 'X':
                    q = int(it[1:] or 0) * 128
                    wqkv_raw[pl.ds(z1 + D // 2, 8), 0:128] = pltpu.bitcast(st['res'][q:q + 8, 0:128], u32)
                elif it[0] == 'h':
                    hpass(int(it[1]))
                elif it[0] == 'y':
                    b, qf = int(it[1]), int(it[2])
                    exch_groups([(r, b, rg) for rg in range(2 * qf, 2 * qf + 2)])
                elif it[0] == 'x':
                    b, hf = int(it[1]), int(it[2])
                    exch_groups([(r, b, rg) for rg in range(4 * hf, 4 * hf + 4)])
            for p in range(1, NP):
                hpass(p)
                for sd in range(6 if p < NP - 1 else 6 - NDEF):
                    st['res'] = subdot(st['h'], st['row'], r, sd)
                    do_side('%dH%d' % (p, sd))
            zsm[0] = r >> 8
            zsm[1] = r >> 9
            return carry

        if upto >= 2:
            if 'R' not in skip:
                lax.fori_loop(1, NR, region, 0)
            zero = zsm[0]
            zero2 = zsm[1]

        if WS and upto >= 2:
            c_wo(6).wait()
        if upto >= 3:
            c_wo(7).wait()
            for t in range(6 * NM, 32):
                c_mb(t, 6).wait()
            for c in c_w:
                c.wait()

        def rows_u32(ref, row0, M):
            if isinstance(row0, int):
                return _bf(ref[row0 // 2:(row0 + M) // 2, :])
            if isinstance(row0, tuple):
                return _bf(ref[pl.ds(row0[0] + row0[1] // 2, M // 2), :])
            return _bf(ref[pl.ds(pl.multiple_of(row0 // 2, 8), M // 2), :])

        def wo_dot(row0, M):
            o = rows_u32(o_scr, row0, M)
            return jnp.concatenate([_dot(o, _bf(wo_v[n])) for n in range(NCH)], axis=1)

        def row(k):
            return jnp.concatenate([modB[8 * (k - 2) + j, 0:1, :] for j in range(NCH)], axis=1)

        def ln23(row0, M, A):
            ga = row(2); sb = row(3); cb = row(4)
            x = rows_u32(x_v, row0, M).astype(f32)
            xm = x + ga * A
            hB = _ln(xm) * (1.0 + cb) + sb
            n3 = _ln(hB).astype(bf16)
            return xm, hB, n3

        shifts = [-1, -1, 1, 1, -2, -2, 2, 2]

        def g_val():
            return jnp.concatenate(
                [h1buf[j, HALO + shifts[j]:HALO + shifts[j] + T, :] for j in range(NCH)], axis=1).astype(bf16)

        def out_copy(r0, n, k, c0=0, cw=D):
            if cw == D:
                return pltpu.make_async_copy(obuf.at[pl.ds(r0, n)], o_hbm.bitcast(u32).at[pl.ds(r0, n)], osems.at[k])
            return pltpu.make_async_copy(obuf.at[pl.ds(r0, n), c0:c0 + cw], o_hbm.bitcast(u32).at[pl.ds(r0, n), c0:c0 + cw], osems.at[k])

        def ln4(hs):
            gb = row(5)
            x1 = hb[0:T, :] + hs
            base = xmid[0:T, :] + gb * x1
            n4 = _ln(x1).astype(bf16)
            return base, n4

        def bfirst():
            for j in range(NCH):
                h1buf[j, 0:HALO, :] = jnp.zeros((HALO, 128), f32)
            h7 = _bf(hP[...])
            zb = pl.multiple_of(zero * 8, 8) if ZB else 0
            h0 = (T + HALO) // 2 // 16 * 16 + (16 if T == 128 else 0)
            halves = [(0, h0), (h0, T + HALO - h0)]
            nA = (2 * T + HALO - AT0) // AP
            st = {'res': None, 'As': [], 'n3': [], 'h1': [], 'macc': {}}

            def att(k):
                if AG:
                    st['o'] = attention2(AT0 + k * AP, AP, AG)
                else:
                    attention(qbuf, kbuf, vbuf, 0, AT0 + k * AP, AP, True)

            def tok_q(cc=0):
                qbuf[0, pl.ds(zb + S + HALO, 8), :] = st['res'][0:8, cc * 128:(cc + 1) * 128]

            batt = None
            if 'A' in BA:
                batt = Att(0, 0, 0, 2 * T + HALO, [BWG] * ((2 * T + HALO) // RB * W // BWG), BPD, zb, BQD, True)
            for it in BA.split():
                k = int(it[1:]) if len(it) > 1 and it[1:].isdigit() else None
                if not ZB and it[0] in 'tWM':
                    continue
                if it[0] == 'A':
                    batt.steps(k)
                elif it[0] == 'R':
                    batt.steps(999)
                    batt.rest()
                elif it[0] == 'T':
                    st['res'] = subdot(h7, TL, 7, k)
                elif it[0] == 'a':
                    att(k)
                elif it[0] == 't':
                    tok_q(k or 0)
                elif it[0] == 'w':
                    pW(7, k, zb)
                elif it[0] == 'v':
                    pW(6, k, zb)
                elif it[0] == 'm':
                    for kq in range(KQ):
                        pM(6 * NM + k, kq, zb, st['macc'], k)
                elif it[0] == 'M':
                    wmB_v[32, pl.ds(zb + D // 2, 8), :] = pltpu.bitcast(st['res'][0:8, 0:128], u32)
                elif it[0] == 'W':
                    wo_raw[7, pl.ds(zb + D // 2 + 16, 8), :] = pltpu.bitcast(st['res'][0:8, 0:128], u32)
                elif it[0] == 'o':
                    assert batt is None or batt.done >= (halves[k][0] + halves[k][1]) // RB * NCH, batt.done
                    st['res'] = wo_dot(*halves[k])
                    st['As'].append(st['res'])
                elif it[0] == 'l':
                    r0, m = halves[k]
                    xm, hB, n3 = ln23(r0, m, st['As'][k])
                    xmid[r0:r0 + m, :] = xm
                    hb[r0:r0 + m, :] = hB
                    st['n3'].append(n3)
                elif it[0] == 'u':
                    r0, m = halves[k]
                    st['res'] = _dot(st['n3'][k], _bf(w1_v[...]))
                    h1 = _gelu(st['res'])
                    for j in range(NCH):
                        h1buf[j, HALO + r0:HALO + r0 + m, :] = h1[:, j * 128:(j + 1) * 128]
                elif it[0] == 'z':
                    if 'g' not in st:
                        st['g'] = g_val()
                    cw_ = D // NZ
                    st['res'] = _dot(st['g'], _bf(w2_v[:, k * cw_:(k + 1) * cw_]))
                    hsbuf[0:T, k * cw_:(k + 1) * cw_] = st['res']
                elif it[0] == 'U':
                    hh, pp = divmod(k, 10)
                    r0, m = halves[hh]
                    cw_ = D // NU
                    st['res'] = _dot(st['n3'][hh], _bf(w1_v[:, pp * cw_:(pp + 1) * cw_]))
                    h1 = _gelu(st['res'])
                    for j in range(cw_ // 128):
                        h1buf[pp * (cw_ // 128) + j, HALO + r0:HALO + r0 + m, :] = h1[:, j * 128:(j + 1) * 128]
            if 'g' not in st:
                hsbuf[0:T, :] = _dot(g_val(), _bf(w2_v[...]))

        if upto >= 3 and 'F' not in skip:
            bfirst()

        def carries(xm, hB, h1, notlast):
            xmid[0:HALO, :] = xmid[T:T + HALO, :]
            hb[0:HALO, :] = hb[T:T + HALO, :]
            for j in range(NCH):
                h1buf[j, 0:2 * HALO, :] = h1buf[j, T:T + 2 * HALO, :]
            xmid[HALO:HALO + T, :] = xm
            hb[HALO:HALO + T, :] = hB
            for j in range(NCH):
                h1j = h1[:, j * 128:(j + 1) * 128]
                h1buf[j, 2 * HALO:HALO + T, :] = h1j[0:T - HALO]
                h1buf[j, HALO + T:2 * HALO + T, :] = jnp.where(notlast, h1j[T - HALO:T], 0.0)

        RP = 16

        def bbody(i, carry):
            static = isinstance(i, int)
            if static:
                row0h = i * (T // 2)
                abase = (i + 1) * T
                abaseh = (i + 1) * (T // 2)
                z1 = pl.multiple_of(zero * 8, 8)
                z2 = pl.multiple_of(zero2 * 8, 8)
            else:
                row0h = pl.multiple_of(i * (T // 2), T // 2)
                nxt = jnp.minimum(i + 1, NT - 1)
                abase = pl.multiple_of(nxt * T, T)
                abaseh = pl.multiple_of(nxt * (T // 2), T // 2)
                z1 = pl.multiple_of((i >> 8) * 8, 8)
                z2 = pl.multiple_of((i >> 9) * 8, 8)
            ga = row(2); sb = row(3); cb = row(4); gb = row(5)
            bases, n4p, xms, hBs, n3p, As = [], [], [], [], [], []
            att = None
            asch = {}
            if AB == 9:
                att = Att(abase, abaseh, HALO, T, [int(t) for t in WGS], PD, z1)
                for t in ASCH.split():
                    k_, v_ = t.split(':')
                    asch[k_] = int(v_)

            def astep(tag):
                if att is not None and tag in asch:
                    att.steps(asch[tag])

            def p4(r):
                r0 = r * RP
                x1 = hb[r0:r0 + RP, :] + hsbuf[pl.ds(z2 + r0, RP), :]
                bases.append(xmid[r0:r0 + RP, :] + gb * x1)
                n4v = _ln(x1).astype(bf16)
                if EX4:
                    n4b[r0 // 2:(r0 + RP) // 2, :] = pltpu.bitcast(n4v, u32)
                n4p.append(n4v)

            def p23(r, A):
                r0 = r * RP
                x = rows_u32(x_v, (row0h, HALO + r0), RP).astype(f32)
                xm = x + ga * A[r0:r0 + RP]
                hB = _ln(xm) * (1.0 + cb) + sb
                xms.append(xm); hBs.append(hB)
                n3v = _ln(hB).astype(bf16)
                if EX3:
                    n3b[r0 // 2:(r0 + RP) // 2, :] = pltpu.bitcast(n3v, u32)
                n3p.append(n3v)

            for r in range(T // RP):
                if rel4[r] < 0:
                    p4(r)
            o = rows_u32(o_scr, (row0h, HALO), T)
            for n in range(NCH):
                An = _dot(o, _bf(wo_v[n]))
                As.append(An)
                r4 = [r for r in range(T // RP) if rel4[r] == n]
                if r4:
                    hsbuf[pl.ds(z1 + T, 8), 0:128] = An[0:8, 0:128]
                for r in r4:
                    p4(r)
                astep('o%d' % n)
            A = jnp.concatenate(As, axis=1)
            base = jnp.concatenate(bases, axis=0)
            n4 = _bf(n4b[...]) if EX4 else jnp.concatenate(n4p, axis=0)
            U = _dot(n4, _bf(w3_v[...]))
            u = _gelu(U).astype(bf16)
            for c in range(F // 128):
                r23 = [r for r in range(T // RP) if rel23[r] == NCH + c]
                if r23 or c in XT:
                    x_v[pl.ds(z1 + S // 2 + HALO // 2, 8), 0:128] = pltpu.bitcast(U[0:8, c * 128:(c + 1) * 128], u32)
                for r in r23:
                    p23(r, A)
                astep('c%d' % c)
            assert len(n3p) == T // RP and len(n4p) == T // RP
            xm = jnp.concatenate(xms, axis=0)
            hB = jnp.concatenate(hBs, axis=0)
            n3 = _bf(n3b[...]) if EX3 else jnp.concatenate(n3p, axis=0)
            h1 = _gelu(_dot(n3, _bf(w1_v[...])))
            carries(xm, hB, h1, i < NT - 1)
            if static:
                if i < NT - 1:
                    attention(qbuf, kbuf, vbuf, abase, HALO, T, False, abaseh)
            elif 'noatt' not in dbg:
                if AB == 9:
                    att.steps(999)
                    att.rest()
                    if DL:
                        h1buf[0, pl.ds(z1 + T + 2 * HALO, 8), :] = att.OC[T // RB - 1, NCH - 1]
                elif AB:
                    attention2(HALO, T, AB, abase, abaseh)
                else:
                    attention(qbuf, kbuf, vbuf, abase, HALO, T, False, abaseh)
            h2 = _dot(u, _bf(w4_v[...]))
            if static:
                obuf[(i - 1) * (T // 2):i * (T // 2), :] = pltpu.bitcast((base + gb * h2).astype(bf16), u32)
            else:
                obuf[pl.ds(pl.multiple_of((i - 1) * (T // 2), T // 2), T // 2), :] = pltpu.bitcast((base + gb * h2).astype(bf16), u32)
            hsbuf[0:T, :] = _dot(g_val(), _bf(w2_v[...]))
            return carry

        if upto >= 4 and 'B' not in skip:
            if UB:
                for i in range(1, 1 + UB):
                    bbody(i, 0)
                    if i in BAR:
                        out_copy_i(i).start()
                if 1 + UB < NT:
                    lax.fori_loop(1 + UB, NT, bbody, 0)
            else:
                lax.fori_loop(1, NT, bbody, 0)

        def blast():
            r0 = (NT - 1) * (T // 2)
            out_copy(0, r0, 0).start()
            if BL == 'M':
                HM = T // 2
                gb = row(5)

                def l4(p0, zz, dst):
                    x1 = hb[p0:p0 + RP, :] + (hsbuf[pl.ds(zz + p0, RP), :] if zz is not None else hsbuf[p0:p0 + RP, :])
                    baseb[p0:p0 + RP, :] = xmid[p0:p0 + RP, :] + gb * x1
                    q0 = (p0 % HM) // 2
                    dst[q0:q0 + RP // 2, :] = pltpu.bitcast(_ln(x1).astype(bf16), u32)

                for p0 in range(0, HM, RP):
                    l4(p0, None, n4b)

                def mbody(m, carry):
                    zz = pl.multiple_of((m >> 8) * 8, 8)
                    if MA:
                        n4 = _bf(n4b[0:HM // 2, :])
                    else:
                        n4 = _bf(n4b[pl.ds(pl.multiple_of(m * (HM // 2), HM // 2), HM // 2), :])
                    U = _dot(n4, _bf(w3_v[...]))
                    u = _gelu(U).astype(bf16)
                    for k, p0 in enumerate(range(HM, T, RP)):
                        if MT is not None and (k == 0 or MT[k] != MT[k - 1]):
                            hsbuf[pl.ds(zz + T, 8), 0:128] = U[0:8, MT[k] * 128:(MT[k] + 1) * 128]
                        l4(p0, zz if MT is not None else None, n3b if MA else n4b.at[HM // 2:T // 2])
                    if MA:
                        n4b[0:HM // 2, :] = n3b[0:HM // 2, :]
                    ro = pl.multiple_of(r0 + m * (HM // 2), HM // 2)
                    c0 = 0
                    for cw_ in MN:
                        h2 = _dot(u, _bf(w4_v[:, c0:c0 + cw_]))
                        bs = baseb[pl.ds(pl.multiple_of(m * HM, HM), HM), c0:c0 + cw_]
                        obuf[pl.ds(ro, HM // 2), c0:c0 + cw_] = pltpu.bitcast((bs + gb[:, c0:c0 + cw_] * h2).astype(bf16), u32)
                        out_copy(ro, HM // 2, 1, c0, cw_).start()
                        c0 += cw_
                    return carry

                lax.fori_loop(0, 2, mbody, 0)
                out_copy(0, r0, 0).wait()
                for hf in range(2):
                    c0 = 0
                    for cw_ in MN:
                        out_copy(r0 + hf * (HM // 2), HM // 2, 1, c0, cw_).wait()
                        c0 += cw_
                return
            base, n4 = ln4(hsbuf[0:T, :])
            if BL:
                FC = F // BL
                xmid[0:T, :] = base
                n4b[...] = pltpu.bitcast(n4, u32)
                hsbuf[0:T, :] = jnp.zeros((T, D), f32)

                def body(c, carry):
                    w3c = w3_v[:, pl.ds(pl.multiple_of(c * FC, 128), FC)]
                    u = _gelu(_dot(_bf(n4b[...]), _bf(w3c))).astype(bf16)
                    w4c = w4_v[pl.ds(pl.multiple_of(c * (FC // 2), 32), FC // 2), :]
                    hsbuf[0:T, :] += _dot(u, _bf(w4c))
                    return carry

                lax.fori_loop(0, BL, body, 0)
                obuf[r0:r0 + T // 2, :] = pltpu.bitcast((xmid[0:T, :] + row(5) * hsbuf[0:T, :]).astype(bf16), u32)
            else:
                u = _gelu(_dot(n4, _bf(w3_v[...]))).astype(bf16)
                h2 = _dot(u, _bf(w4_v[...]))
                obuf[r0:r0 + T // 2, :] = pltpu.bitcast((base + row(5) * h2).astype(bf16), u32)
            out_copy(r0, T // 2, 1).start()
            out_copy(0, r0, 0).wait()
            out_copy(r0, T // 2, 1).wait()

        if upto >= 5 and 'L' not in skip:
            blast()

    @jax.jit
    def fn(A_x, A_wqkv, A_wo, B_x, B_w1, B_w2, B_w3, B_w4, c, w_mod):
        x = A_x.reshape(S, D)
        any_spec = pl.BlockSpec(memory_space=pl.ANY)
        out = pl.pallas_call(
            kernel,
            in_specs=[any_spec] * 9,
            out_specs=any_spec,
            out_shape=jax.ShapeDtypeStruct((S, D), bf16),
            scratch_shapes=[
                pltpu.VMEM((S // 2 + HALO // 2 + 8, D), u32),
                pltpu.VMEM((D // 2 + 32, 3 * D), u32),
                pltpu.VMEM((D // 2, D), u32),
                pltpu.VMEM((D // 2, D), u32),
                pltpu.VMEM((D // 2, D), u32),
                pltpu.VMEM((NCH + WS, D // 2 + 32, 128), u32),
                pltpu.VMEM((NCH + WS, D // 2, 128), u32),
                pltpu.VMEM((D // 2, D), u32),
                pltpu.VMEM((D // 2, D), u32),
                pltpu.VMEM((D // 2, F), u32),
                pltpu.VMEM((F // 2, D), u32),
                pltpu.VMEM((D // 2, 128), f32),
                pltpu.VMEM((D // 2, 128), f32),
                pltpu.VMEM((8, D // 2 + 16, 256), u32),
                pltpu.VMEM((33, D // 2 + 32, 128), u32),
                pltpu.VMEM((8, 8, 256), f32),
                pltpu.VMEM((36, 8, 128), f32),
                pltpu.VMEM((3 if MU else NCH, S + 32, 128), f32),
                pltpu.VMEM((PR // 2, 128), u32),
                pltpu.VMEM((S // 2, 128), u32),
                pltpu.VMEM((NCH, S + 32, 128), f32),
                pltpu.VMEM((NCH, S + 2 * HALO + 32 * (AB == 9), 128), f32),
                pltpu.VMEM((NCH, S + 2 * HALO + 32 * (AB == 9), 128), f32),
                pltpu.VMEM((T + HALO, D), f32),
                pltpu.VMEM((T + HALO, D), f32),
                pltpu.VMEM((NCH, T + 2 * HALO + 32 * DL, 128), f32),
                pltpu.VMEM((S // 2, D), u32),
                pltpu.VMEM((S // 2 + HALO // 2, D), u32),
                pltpu.VMEM((T + 32, D), f32),
                pltpu.VMEM((T // 2, D), u32),
                pltpu.VMEM((T // 2, D), u32),
                pltpu.VMEM((T, D), f32),
                pltpu.VMEM((1, D), bf16),
            ] + ([pltpu.VMEM((padr, 128), f32)] if padr else []) + [
                pltpu.SMEM((8,), jnp.int32),
            ],
            compiler_params=pltpu.CompilerParams(vmem_limit_bytes=120 * 1024 * 1024),
        )(x, A_wqkv, A_wo, B_w1, B_w2, B_w3, B_w4, c, w_mod)
        return out.reshape(1, S, D)
    return fn


_fn = make()


def pallas_adaLN_cond__sliding_local_dilated__mixer_s_mlp__prompt_kernel(A_x, A_wqkv, A_wo, B_x, B_w1, B_w2, B_w3, B_w4, c, w_mod):
    return _fn(A_x, A_wqkv, A_wo, B_x, B_w1, B_w2, B_w3, B_w4, c, w_mod)
```

```python
import functools
import jax
import jax.numpy as jnp
from jax import lax
import jax.experimental.pallas as pl
import jax.experimental.pallas.tpu as pltpu

S, D, F = 2048, 1024, 3584
H, DH, W, DIL = 32, 32, 8, 2
NCH = D // 128
EPS = 1e-5
SCALE = DH ** -0.5
f32, bf16, u32 = jnp.float32, jnp.bfloat16, jnp.uint32
HALO = 16


def _ln(x):
    m = jnp.mean(x, axis=-1, keepdims=True)
    xc = x - m
    v = jnp.mean(xc * xc, axis=-1, keepdims=True)
    return xc * lax.rsqrt(v + EPS)


def _gelu(x):
    c0 = 0.7978845608028654
    c1 = c0 * 0.044715
    t = jnp.tanh(x * (c0 + c1 * (x * x)))
    hx = 0.5 * x
    return hx + hx * t


def _dot(a, b):
    return jnp.dot(a, b, preferred_element_type=f32)


def _bf(w):
    return pltpu.bitcast(w, bf16)


def _lane_xor(x, s):
    lane = lax.broadcasted_iota(jnp.int32, x.shape, 1)
    return jnp.take_along_axis(x, lane ^ s, axis=1)


def _exchange8_multi(XS):
    XS = [list(X) for X in XS]
    lane = lax.broadcasted_iota(jnp.int32, XS[0][0].shape, 1)
    for t in range(3):
        s = 1 << (t + 2)
        m = (lane & s) != 0
        for X in XS:
            for p in range(8):
                if p & (1 << t):
                    continue
                p2 = p | (1 << t)
                tmp = _lane_xor(jnp.where(m, X[p], X[p2]), s)
                X[p], X[p2] = jnp.where(m, tmp, X[p]), jnp.where(m, X[p2], tmp)
    return XS


def _group4_sum(acc):
    lane = lax.broadcasted_iota(jnp.int32, acc.shape, 1)
    acc = acc + jnp.where((lane & 1) != 0, pltpu.roll(acc, 1, 1), pltpu.roll(acc, 127, 1))
    acc = acc + jnp.where((lane & 2) != 0, pltpu.roll(acc, 2, 1), pltpu.roll(acc, 126, 1))
    return acc


def make(T=128, PR=512, RB=8, EG=4, upto=9, AT0=0, AP=16,
         DO='c X0 Wq sa ca X1 Wk Wv X2 X3 X4 X5 X6 X7 X8 X9 X10 X12 X13 X11 X14 X15',
         PS=None, PSX=None, RL=1, D0='1234567', LP=16, BL='M', ZB=1,
         order0='T0 T1 X x00 x01 m0 T2 T3 X x10 x11 h0 T4 T5 X x20 H0 X x21 H1 H2 H3 H4 H5', NDEF=6, BA=None,
         side=None, KQ=4, KQ0=1, NM=5, NR=8, AG=1,
         rel4=(-1, -1, -1, 0, 1, 2, 3, 4), rel23=(8, 9, 10, 11, 12, 13, 14, 15),
         padr=0, dbg='', UB=0, BAR=(), GL=0, MU=1, WS=1, skip='', AB=9, WGS='1'*128, PD=0, ASCH='', DL=0, EX3=1, EX4=1, XT=(), MT=(4, 10, 16, 22), MA=0, MN=(1024,), NZ=8, NU=2, BPD=0, BQD=None, BWG=8,
         ST=1, ORD4=(0, 4, 1, 5, 2, 6, 3, 7), R23=(0, 4, 8, 12, 16, 20, 24, 28), PRE='L', CW3=128, CW4=128, SB='S'):
    HS, HO = (2, 0) if MU else (0, S // 2)
    NT = S // T
    NP = S // PR
    order0 = order0.split()
    TL = S - PR
    if PS is None:
        PS = ('wc C wX0 L0 wWq e0 wsa S wca A h0 wX1 u0:0 L1 wWk u1:0 e1 wWv u0:1 u1:1 e2 wX2 u0:2 u1:2 L2 u2:0 '
              'wX3 wX4 u2:12 L3 u3:012 L4 u4:0 wX5 wX6 wX7 u4:12 L5 u5:012 L6 u6:012 L7 u7:0 '
              'wX8 wX9 wX10 wX12 wX13 u7:12 L8 u8:012 L9 u9:012 L10 ua:0 L12 L13 wX11 wX14 wX15 DW ua:12 L11 ub:012 L14 L15')
    if BA is None:
        BA = ('a0 a1 T0 T1 t0 a2 a3 W w0 w1 w2 w3 w4 w5 w6 w7 T2 t0 a4 a5 T3 t0 a6 a7 T4 t0 a8 a9 T5 t0 a10 o0 t0 a11 t4 a12 '
              'o1 t0 a13 t4 a14 M m0 m1 l0 l1 u0 t0 a15 t4 a16 u1')
    if WS and 'v0' not in BA:
        BA = BA.replace('W w0 w1 w2 w3 w4 w5 w6 w7', 'W v0 v1 v2 v3 v4 v5 v6 v7 w0 w1 w2 w3 w4 w5 w6 w7')
    if PSX:
        for k_, v_ in PSX.items():
            assert (' ' + k_ + ' ') in PS
            PS = PS.replace(' ' + k_ + ' ', ' ' + k_ + ' ' + v_ + ' ')
    S_C, S_X, S_SA, S_CA, S_W0, S_WQ, S_WO, S_MB, S_W = 0, 1, 17, 25, 33, 36, 44, 52, 60
    NSEM = 64
    DEF = list(range(6 - NDEF, 6))
    tags = ['T%d' % sd for sd in DEF] + ['%dH%d' % (p, sd) for p in range(NP) for sd in range(6 if p < NP - 1 else 6 - NDEF)]
    if side is None:
        side = 'W:7,9,11,13,15,17,19,21 M:4,5,6,7,8,9,10,11,12,13,14,15,16,17,18,19,20,21,22,22'
    if isinstance(side, str):
        sd_ = {}
        for grp in side.split():
            kind, lst = grp.split(':')
            for k, t in enumerate(lst.split(',')):
                sd_.setdefault(tags[int(t)], []).append(kind + str(k))
        side = sd_
    assert sum(1 for v in side.values() for j in v if j[0] in 'Aa') * AP == AT0

    def kernel(*refs):
        pl.run_scoped(functools.partial(body, *refs), pltpu.SemaphoreType.DMA((NSEM,)), pltpu.SemaphoreType.DMA((2,)))

    def body(x_hbm, wqkv_hbm, wo_hbm, w1_hbm, w2_hbm, w3_hbm, w4_hbm, c_hbm, wmod_hbm,
             o_hbm,
             x_v, wqkv_raw, wq_v, wk_v, wv_v, wo_raw, wo_v, w1_v, w2_v, w3_v, w4_v, cE, cO, wmA_v, wmB_v,
             modA, modB, xhat, hP, h0, qbuf, kbuf, vbuf, xmid, hb, h1buf, obuf, o_scr, hsbuf, n4b, n3b, baseb, w3s, w4s, n4f, a4, ua, macc, c_v, *rest):
        zsm, sems, osems = rest[-3:]

        def cp(src, dst, k):
            return pltpu.make_async_copy(src, dst, sems.at[k])

        xu = x_hbm.bitcast(u32)
        wqkvu = wqkv_hbm.bitcast(u32)
        wou = wo_hbm.bitcast(u32)
        wmodu = wmod_hbm.bitcast(u32)

        def lane_ds(k, n, base=0):
            if isinstance(k, int):
                return pl.ds(base + k * n, n)
            return pl.ds(pl.multiple_of(base + k * n, 128), n)

        def row_ds(base, k, n):
            if isinstance(k, int):
                return pl.ds(base + k * n, n)
            return pl.ds(pl.multiple_of(base + k * n, 8), n)

        c_c = cp(c_hbm, c_v, S_C)

        def c_x(b):
            return cp(xu.at[b * 64:(b + 1) * 64], x_v.at[b * 64:(b + 1) * 64], S_X + b)

        def c_sa(k):
            return cp(wmodu.at[:, lane_ds(k, 128)], wmA_v.at[k, 0:D // 2, 0:128], S_SA + k)

        def c_ca(k):
            return cp(wmodu.at[:, lane_ds(k, 128, D)], wmA_v.at[k, 0:D // 2, 128:256], S_CA + k)

        def c_w0(b):
            return cp(wqkvu.at[0:64, b * D:(b + 1) * D], wqkv_raw.at[0:64, b * D:(b + 1) * D], S_W0 + b)

        def c_wq(k):
            return cp(wqkvu.at[row_ds(0, k, 64)], wqkv_raw.at[row_ds(0, k, 64)], S_WQ + k)

        def c_wo(p):
            return cp(wou.at[:, lane_ds(p, 128)], wo_raw.at[p, 8:8 + D // 2], S_WO + p)

        def c_mb(t, g):
            return cp(wmodu.at[:, lane_ds(t, 128, 2 * D)], wmB_v.at[t, 0:D // 2], S_MB + g)

        c_w = [cp(w1_hbm.bitcast(u32), w1_v, S_W), cp(w2_hbm.bitcast(u32), w2_v, S_W + 1),
               cp(w3_hbm.bitcast(u32), w3_v, S_W + 2), cp(w4_hbm.bitcast(u32), w4_v, S_W + 3)]

        def named(nm):
            if nm == 'c':
                return c_c
            if nm == 'sa':
                return c_sa(0)
            if nm == 'ca':
                return c_ca(0)
            if nm[0] == 'W':
                return c_w0('qkv'.index(nm[1]))
            return c_x(int(nm[1:]))

        for nm in DO.split():
            named(nm).start()
        def start_group(g):
            if g == 'W':
                if upto >= 3:
                    c_wo(7).start()
                    for t in range(6 * NM, 32):
                        c_mb(t, 6).start()
                    for c in c_w:
                        c.start()
            elif upto >= 2 and 'nodma2' not in dbg:
                r = int(g)
                c_sa(r).start()
                c_ca(r).start()
                c_wq(r).start()
                c_wo(r - 1).start()
                if r >= 2:
                    for i in range(NM):
                        c_mb(NM * (r - 2) + i, r - 2).start()

        for g in D0:
            start_group(g)
        assert sorted(list(D0) + [it[1] for it in PS.split() if it[0] == 'D']) == list('1234567W')

        def _zinit(i, carry):
            zsm[2 + i] = i >> 8
            return carry

        lax.fori_loop(0, 3, _zinit, 0)
        zp3 = pl.multiple_of(zsm[4] * 8, 8)
        zp1 = pl.multiple_of(zsm[2] * 8, 8)
        zp2 = pl.multiple_of(zsm[3] * 8, 8)

        x_v[S // 2:S // 2 + HALO // 2, :] = jnp.zeros((HALO // 2, D), u32)
        for j in range(NCH):
            z = jnp.zeros((HALO, 128), f32)
            qbuf[j, S:S + HALO, :] = z
            kbuf[j, HALO + S:2 * HALO + S, :] = z
            vbuf[j, HALO + S:2 * HALO + S, :] = z
            kbuf[j, 0:HALO, :] = z
            vbuf[j, 0:HALO, :] = z
            wo_raw[j, 0:8, :] = jnp.zeros((8, 128), u32)
            wo_raw[j, 8 + D // 2:16 + D // 2, :] = jnp.zeros((8, 128), u32)

        def mv_part(w, r0, acc):
            n = w.shape[0]
            lo = pltpu.bitcast(w << 16, f32)
            hi = pltpu.bitcast(w & jnp.uint32(0xFFFF0000), f32)
            pr = lo * cE[r0:r0 + n, :] + hi * cO[r0:r0 + n, :]
            for t in range(n // 8):
                acc = pr[8 * t:8 * t + 8] if acc is None else acc + pr[8 * t:8 * t + 8]
            return acc

        wparts = (wq_v, wk_v, wv_v)
        bufs = (qbuf, kbuf, vbuf)

        def exch_groups(grps):
            for g0 in range(0, len(grps), EG):
                gs = grps[g0:g0 + EG]
                XS = [[wqkv_raw[row_ds(rg * 8, k * 8, 8), b * D + a * 128:b * D + (a + 1) * 128] for a in range(NCH)]
                      for (k, b, rg) in gs]
                YS = _exchange8_multi(XS)
                for (k, b, rg), Y in zip(gs, YS):
                    wparts[b][row_ds(rg * 8, k * 8, 8), :] = jnp.concatenate(Y, axis=1)

        def subdot(lhs, row0, kc, sd, init=False, valid=None):
            b, hf = sd // 2, sd % 2
            n = lhs.shape[0]
            res = _dot(lhs, _bf(wparts[b][row_ds(0, kc, 64), hf * 512:(hf + 1) * 512]))
            o = row0 + (0 if b == 0 else HALO)
            for jj in range(4):
                j = hf * 4 + jj
                if init:
                    bufs[b][j, o:o + n, :] = res[:, jj * 128:(jj + 1) * 128]
                elif valid is not None:
                    bufs[b][j, o:o + n, :] = jnp.where(valid, bufs[b][j, o:o + n, :], 0.0) + res[:, jj * 128:(jj + 1) * 128]
                else:
                    bufs[b][j, o:o + n, :] += res[:, jj * 128:(jj + 1) * 128]
            return res

        def prologue():
            st = {}

            def crep():
                c = c_v[...].astype(f32)
                scf = (c * jax.nn.sigmoid(c)).astype(bf16).astype(f32)
                rr = lax.broadcasted_iota(jnp.int32, (128, 128), 0)
                ll = lax.broadcasted_iota(jnp.int32, (128, 128), 1)
                sel = ll == jnp.where(rr < 64, 2 * rr, 2 * rr - 127)
                for j in range(NCH):
                    dg = jnp.where(sel, jnp.broadcast_to(scf[:, j * 128:(j + 1) * 128], (128, 128)), 0.0).astype(bf16)
                    rep = _dot(dg, jnp.ones((128, 128), bf16))
                    cE[j * 64:(j + 1) * 64, :] = rep[0:64]
                    cO[j * 64:(j + 1) * 64, :] = rep[64:128]

            def h_store(r0, xh0):
                h = (xh0 * (1.0 + st['ca']) + st['sa']).astype(bf16)
                if r0 < TL:
                    xhat[HS, HO + r0 // 2:HO + (r0 + LP) // 2, :] = pltpu.bitcast(h, f32)
                else:
                    hP[(r0 - TL) // 2:(r0 - TL + LP) // 2, :] = pltpu.bitcast(h, u32)

            def h0_lhs(b0, nb, gated):
                r0 = HO + b0 * 64
                if not gated:
                    return _bf(xhat[HS, r0:r0 + nb * 64, :])
                if GL:
                    return jnp.concatenate([_bf(xhat[HS, r0:r0 + nb * 64 - 8, :]), _bf(xhat[HS, pl.ds(zp3 + r0 + nb * 64 - 8, 8), :])], axis=0)
                return jnp.concatenate([_bf(xhat[HS, pl.ds(zp3 + r0, 8), :]), _bf(xhat[HS, r0 + 8:r0 + nb * 64, :])], axis=0)

            def ln_piece(b, i):
                r0 = b * 128 + i * LP
                direct = 'ca' in st and 'sa' in st
                if MU:
                    x = _bf(x_v[pl.ds(zp1 + r0 // 2, LP // 2), :]).astype(f32)
                    m = jnp.mean(x, axis=-1, keepdims=True)
                    if RL:
                        x = _bf(x_v[pl.ds(zp2 + r0 // 2, LP // 2), :]).astype(f32)
                    xc = x - m
                    rs = lax.rsqrt(jnp.mean(xc * xc, axis=-1, keepdims=True) + EPS)
                    xhat[0, r0:r0 + LP, :] = jnp.broadcast_to(m, (LP, 128))
                    xhat[1, r0:r0 + LP, :] = jnp.broadcast_to(rs, (LP, 128))
                    if direct:
                        h_store(r0, xc[:, 0:128] * rs)
                    return
                if RL:
                    m = jnp.mean(_bf(x_v[pl.ds(zp1 + r0 // 2, LP // 2), :]).astype(f32), axis=-1, keepdims=True)
                    xc = _bf(x_v[pl.ds(zp2 + r0 // 2, LP // 2), :]).astype(f32) - m
                    v = jnp.mean(xc * xc, axis=-1, keepdims=True)
                    xh = (_bf(x_v[r0 // 2:(r0 + LP) // 2, :]).astype(f32) - m) * lax.rsqrt(v + EPS)
                else:
                    xh = _ln(_bf(x_v[pl.ds(zp1 + r0 // 2, LP // 2), :]).astype(f32))
                for j in range(1 if direct else 0, NCH):
                    xhat[j, r0:r0 + LP, :] = xh[:, j * 128:(j + 1) * 128]
                if direct:
                    h_store(r0, xh[:, 0:128])

            def ln_block(b):
                for i in range(128 // LP):
                    ln_piece(b, i)

            def hblk(b):
                for i in range(128 // LP):
                    r0 = b * 128 + i * LP
                    if MU:
                        x = _bf(x_v[r0 // 2:(r0 + LP) // 2, 0:128]).astype(f32)
                        h_store(r0, (x - xhat[0, r0:r0 + LP, :]) * xhat[1, r0:r0 + LP, :])
                    else:
                        h_store(r0, xhat[0, r0:r0 + LP, :])

            for it in PS.split():
                if it[0] == 'w':
                    named(it[1:]).wait()
                elif it[0] == 'D':
                    start_group(it[1])
                elif it == 'C':
                    crep()
                elif it[0] == 'L':
                    ln_block(int(it[1:]))
                elif it[0] == 'h':
                    hblk(int(it[1:]))
                elif it == 'S':
                    st['sa'] = jnp.sum(mv_part(wmA_v[0, 0:D // 2, 0:128], 0, None), axis=0, keepdims=True)
                elif it == 'A':
                    st['ca'] = jnp.sum(mv_part(wmA_v[0, 0:D // 2, 128:256], 0, None), axis=0, keepdims=True)
                elif it[0] == 'e':
                    exch_groups([(0, int(it[1]), rg) for rg in range(8)])
                elif it[0] == 'p':
                    b_, i_ = it[1:].split(':')
                    ln_piece(int(b_), int(i_))
                elif it[0] == 't':
                    x_v[pl.ds(zp3 + S // 2 + HALO // 2, 8), 0:128] = pltpu.bitcast(st['res'][0:8, 0:128], u32)
                elif it[0] in 'sg':
                    blks, sd = it[1:].split(':')
                    b0, nb = int(blks[0], 16), len(blks)
                    st['res'] = subdot(h0_lhs(b0, nb, it[0] == 'g'), b0 * 128, 0, int(sd), True)
                elif it[0] == 'u':
                    blks, parts = it[1:].split(':')
                    b0, nb = int(blks[0], 16), len(blks)
                    lhs = h0_lhs(b0, nb, False)
                    for p in parts:
                        subdot(lhs, b0 * 128, 0, 2 * int(p), True)
                        st['res'] = subdot(lhs, b0 * 128, 0, 2 * int(p) + 1, True)

        if 'P' not in skip:
            prologue()

        def attention(qb, kb, vb, base, off, M, mask_rows, baseh=None):
            row0 = base + off

            def kvds(r, w):
                return pl.ds(base + (off + HALO + r - DIL * w), RB)

            o_rows = []
            for r in range(0, M, RB):
                q = [qb[j, pl.ds(base + (off + r), RB), :] for j in range(NCH)]
                s = []
                for w in range(W):
                    acc = None
                    for j in range(NCH):
                        p = q[j] * kb[j, kvds(r, w), :]
                        acc = p if acc is None else acc + p
                    acc = _group4_sum(acc)
                    if mask_rows and off + r < DIL * (W - 1) and w > 0:
                        rows = row0 + r + lax.broadcasted_iota(jnp.int32, (RB, 128), 0)
                        acc = jnp.where(rows >= DIL * w, acc, -1e30)
                    s.append(acc)
                m = functools.reduce(jnp.maximum, s)
                e = [jnp.exp((sw - m) * SCALE) for sw in s]
                den = functools.reduce(lambda a, b: a + b, e)
                rinv = 1.0 / den
                oc = []
                for j in range(NCH):
                    acc = None
                    for w in range(W):
                        p = e[w] * vb[j, kvds(r, w), :]
                        acc = p if acc is None else acc + p
                    oc.append(acc * rinv)
                o_rows.append(jnp.concatenate(oc, axis=1))
            o = jnp.concatenate(o_rows, axis=0).astype(bf16)
            if isinstance(row0, int):
                o_scr[row0 // 2:(row0 + M) // 2, :] = pltpu.bitcast(o, u32)
            elif baseh is not None:
                o_scr[pl.ds(baseh + off // 2, M // 2), :] = pltpu.bitcast(o, u32)
            else:
                o_scr[pl.ds(pl.multiple_of(row0 // 2, 8), M // 2), :] = pltpu.bitcast(o, u32)


        def attention2(off, M, G, base=None, baseh=None):
            o_rows = []

            def rs_(a):
                return slice(a, a + RB) if base is None else pl.ds(base + a, RB)

            for r0 in range(0, M, RB * G):
                rs = [off + r0 + g * RB for g in range(G) if r0 + g * RB < M]
                lane = lax.broadcasted_iota(jnp.int32, (RB, 128), 1)
                S_ = {}
                for r in rs:
                    q = [qbuf[j, rs_(r), :] for j in range(NCH)]
                    for w in range(W):
                        acc = None
                        for j in range(NCH):
                            k0 = HALO + r - DIL * w
                            p = q[j] * kbuf[j, rs_(k0), :]
                            acc = p if acc is None else acc + p
                        S_[r, w] = acc
                keys = list(S_)
                for sh in (1, 2):
                    R = {k: (pltpu.roll(S_[k], sh, 1), pltpu.roll(S_[k], 128 - sh, 1)) for k in keys}
                    for k in keys:
                        S_[k] = S_[k] + jnp.where((lane & sh) != 0, R[k][0], R[k][1])
                for r in rs:
                    s = []
                    for w in range(W):
                        acc = S_[r, w]
                        if base is None and r < DIL * (W - 1) and w > 0:
                            rows = r + lax.broadcasted_iota(jnp.int32, (RB, 128), 0)
                            acc = jnp.where(rows >= DIL * w, acc, -1e30)
                        s.append(acc)
                    m = functools.reduce(jnp.maximum, s)
                    e = [jnp.exp((sw - m) * SCALE) for sw in s]
                    den = functools.reduce(lambda a, b: a + b, e)
                    rinv = 1.0 / den
                    oc = []
                    for j in range(NCH):
                        acc = None
                        for w in range(W):
                            k0 = HALO + r - DIL * w
                            p = e[w] * vbuf[j, rs_(k0), :]
                            acc = p if acc is None else acc + p
                        oc.append(acc * rinv)
                    o_rows.append(jnp.concatenate(oc, axis=1))
            o = jnp.concatenate(o_rows, axis=0).astype(bf16)
            if base is None:
                o_scr[off // 2:(off + M) // 2, :] = pltpu.bitcast(o, u32)
            else:
                o_scr[pl.ds(baseh + off // 2, M // 2), :] = pltpu.bitcast(o, u32)
            return o

        class Att:
            def __init__(self, base, baseh, off, M, wgs, PD, ztok, QD=None, mask=False):
                self.base, self.baseh, self.off, self.PD, self.ztok = base, baseh, off, PD, ztok
                self.QD, self.mask = QD, mask
                self.nrb = M // RB
                self.wgs = list(wgs)
                assert sum(self.wgs) == self.nrb * W
                self.Q, self.SS, self.E, self.OC = {}, {}, {}, {}
                self.win = 0
                self.done = 0

            def scores(self, wl):
                lane = lax.broadcasted_iota(jnp.int32, (RB, 128), 1)
                accs = []
                for (rb, w) in wl:
                    r = self.off + rb * RB
                    if rb not in self.Q:
                        if self.QD is not None and rb * W - self.QD >= 0:
                            qbuf[0, pl.ds(self.ztok + S + HALO, 8), :] = self.SS[divmod(rb * W - self.QD, W)]
                        self.Q[rb] = [qbuf[j, pl.ds(self.base + r, RB), :] for j in range(NCH)]
                    acc = None
                    for j in range(NCH):
                        p = self.Q[rb][j] * kbuf[j, pl.ds(self.base + (HALO + r - DIL * w), RB), :]
                        acc = p if acc is None else acc + p
                    accs.append(acc)
                for sh in (1, 2):
                    R = [(pltpu.roll(a, sh, 1), pltpu.roll(a, 128 - sh, 1)) for a in accs]
                    accs = [a + jnp.where((lane & sh) != 0, x, y) for a, (x, y) in zip(accs, R)]
                for k, a in zip(wl, accs):
                    r = self.off + k[0] * RB
                    if self.mask and r < DIL * (W - 1) and k[1] > 0:
                        rows = r + lax.broadcasted_iota(jnp.int32, (RB, 128), 0)
                        a = jnp.where(rows >= DIL * k[1], a, -1e30)
                    self.SS[k] = a
                    if k[1] == W - 1:
                        self.softmax(k[0])

            def softmax(self, rb):
                s = [self.SS[rb, w] for w in range(W)]
                m = functools.reduce(jnp.maximum, s)
                e = [jnp.exp((sw - m) * SCALE) for sw in s]
                den = functools.reduce(lambda a, b: a + b, e)
                self.E[rb] = (e, 1.0 / den)

            def pv(self):
                rb, j = divmod(self.done, NCH)
                self.done += 1
                r = self.off + rb * RB
                e, rinv = self.E[rb]
                acc = None
                for w in range(W):
                    p = e[w] * vbuf[j, pl.ds(self.base + (HALO + r - DIL * w), RB), :]
                    acc = p if acc is None else acc + p
                self.OC[rb, j] = acc * rinv
                if rb % 2 == 1 and j == NCH - 1:
                    o = jnp.concatenate([jnp.concatenate([self.OC[q, c] for c in range(NCH)], axis=1) for q in (rb - 1, rb)], axis=0)
                    o_scr[pl.ds(self.baseh + (self.off + (rb - 1) * RB) // 2, RB), :] = pltpu.bitcast(o.astype(bf16), u32)

            def token(self, v):
                vbuf[0, pl.ds(self.ztok + S + 2 * HALO, 8), :] = v

            def steps(self, n):
                for _ in range(n):
                    if not self.wgs:
                        return
                    g = self.wgs.pop(0)
                    wl = [divmod(self.win + t, W) for t in range(g)]
                    self.win += g
                    self.scores(wl)
                    tok = False
                    while self.done < self.nrb * NCH and self.done + W + self.PD <= self.win - 1 and self.done // NCH in self.E:
                        if not tok:
                            self.token(self.SS[wl[-1]])
                            tok = True
                        self.pv()

            def rest(self, n=999):
                while self.done < self.nrb * NCH and n > 0:
                    self.pv(); n -= 1

        sub = lax.broadcasted_iota(jnp.int32, (8, 128), 0)

        def pW(p, q, z):
            for tv in range(8 * q, 8 * q + 8):
                j = tv >> 3
                hh = (tv >> 1) & 3
                a2 = tv & 1
                parts = []
                for al in range(4):
                    a = a2 * 4 + al
                    src = a * 64 + hh * 16 + j * 2
                    st = src - 2 * al + 8
                    if isinstance(z, int):
                        parts.append(wo_raw[p, z + st:z + st + 8, :])
                    else:
                        parts.append(wo_raw[p, pl.ds(z + st, 8), :])
                v = jnp.where(sub < 2, parts[0], parts[1])
                v2 = jnp.where(sub < 6, parts[2], parts[3])
                wo_v[p, 8 * tv:8 * tv + 8, :] = jnp.where(sub < 4, v, v2)

        def pM(t, kq, z, macc, key):
            n = D // 2 // KQ
            rows = pl.ds(z + kq * n, n)
            macc[key] = mv_part(wmB_v[t, rows, :], kq * n, macc.get(key))
            if kq == KQ - 1:
                modB[t, 0:1, :] = jnp.sum(macc[key], axis=0, keepdims=True)

        def region_waits(r):
            c_sa(r).wait(); c_ca(r).wait(); c_wq(r).wait()
            if not WS:
                c_wo(r - 1).wait()

            @pl.when(r >= 2)
            def _():
                if WS:
                    c_wo(r - 2).wait()
                for i in range(NM):
                    c_mb(NM * (r - 2) + i, r - 2).wait()

        if 'prewait' in dbg:
            for r in range(1, 8):
                region_waits(r)

        def region(r, carry):
            if 'prewait' not in dbg and 'nodma2' not in dbg:
                region_waits(r)
            z1 = pl.multiple_of((r >> 8) * 8, 8)
            z2 = pl.multiple_of((r >> 9) * 8, 8)
            pm = [jnp.where(r >= 2, NM * (r - 2) + i, 32) for i in range(NM)]
            pw = jnp.where(r >= 2, r - 2, NCH) if WS else r - 1
            hp = _bf(hP[...])
            st = {'acc': [None, None], 'res': None}
            macc = {}

            def mvp(kq):
                n = D // 2 // KQ0
                for q in range(2):
                    st['acc'][q] = mv_part(wmA_v[r, pl.ds(z2 + kq * n, n), q * 128:(q + 1) * 128], kq * n, st['acc'][q])
                if kq == KQ0 - 1:
                    st['sa'] = jnp.sum(st['acc'][0], axis=0, keepdims=True)
                    st['ca'] = jnp.sum(st['acc'][1], axis=0, keepdims=True)
                    modA[r, 0:1, 0:128] = st['sa']
                    modA[r, 0:1, 128:256] = st['ca']

            def hpass(p):
                if MU:
                    x = _bf(x_v[p * PR // 2:(p + 1) * PR // 2, lane_ds(r, 128)]).astype(f32)
                    xh = (x - xhat[0, p * PR:(p + 1) * PR, :]) * xhat[1, p * PR:(p + 1) * PR, :]
                else:
                    xh = xhat[r, p * PR:(p + 1) * PR, :]
                st['h'] = (xh * (1.0 + st['ca']) + st['sa']).astype(bf16)
                st['row'] = p * PR
                if p == NP - 1:
                    hP[...] = pltpu.bitcast(st['h'], u32)

            def do_side(tag):
                jobs = side.get(tag, ())
                if not jobs:
                    return
                tk = pltpu.bitcast(st['res'][0:8, 0:128], u32)
                kinds = set(j[0] for j in jobs)
                if 'W' in kinds:
                    wo_raw[pw, pl.ds(z1 + D // 2 + 16, 8), :] = tk
                if 'M' in kinds:
                    wmB_v[32, pl.ds(z1 + D // 2, 8), :] = tk
                if 'A' in kinds:
                    qbuf[0, pl.ds(z1 + S + HALO, 8), :] = pltpu.bitcast(tk, f32)
                for j in jobs:
                    k = int(j[1:])
                    if j[0] == 'W':
                        pW(pw, k, z2)
                    elif j[0] == 'w':
                        pW(pw, k, 0)
                    elif j[0] == 'M':
                        pM(pm[k // KQ], k % KQ, z2, macc, k // KQ)
                    elif j[0] in 'Aa':
                        attention(qbuf, kbuf, vbuf, 0, k * AP, AP, True)

            for it in order0:
                if it[0] == 'T':
                    st['res'] = subdot(hp, TL, r - 1, int(it[1]), valid=r >= 2)
                    do_side(it)
                elif it[0] == 'H':
                    st['res'] = subdot(st['h'], st['row'], r, int(it[1]))
                    do_side('0' + it)
                elif it[0] == 'm':
                    mvp(int(it[1]))
                elif it[0] == 'K':
                    q = int(it[1:] or 0) * 128
                    wmA_v[r, pl.ds(z1 + D // 2, 8), 0:128] = pltpu.bitcast(st['res'][q:q + 8, 0:128], u32)
                elif it[0] == 'X':
                    q = int(it[1:] or 0) * 128
                    wqkv_raw[pl.ds(z1 + D // 2, 8), 0:128] = pltpu.bitcast(st['res'][q:q + 8, 0:128], u32)
                elif it[0] == 'h':
                    hpass(int(it[1]))
                elif it[0] == 'y':
                    b, qf = int(it[1]), int(it[2])
                    exch_groups([(r, b, rg) for rg in range(2 * qf, 2 * qf + 2)])
                elif it[0] == 'x':
                    b, hf = int(it[1]), int(it[2])
                    exch_groups([(r, b, rg) for rg in range(4 * hf, 4 * hf + 4)])
            for p in range(1, NP):
                hpass(p)
                for sd in range(6 if p < NP - 1 else 6 - NDEF):
                    st['res'] = subdot(st['h'], st['row'], r, sd)
                    do_side('%dH%d' % (p, sd))
            zsm[0] = r >> 8
            zsm[1] = r >> 9
            return carry

        if upto >= 2:
            if 'R' not in skip:
                lax.fori_loop(1, NR, region, 0)
            zero = zsm[0]
            zero2 = zsm[1]

        if WS and upto >= 2:
            c_wo(6).wait()
        if upto >= 3:
            c_wo(7).wait()
            for t in range(6 * NM, 32):
                c_mb(t, 6).wait()
            for c in c_w:
                c.wait()

        def rows_u32(ref, row0, M):
            if isinstance(row0, int):
                return _bf(ref[row0 // 2:(row0 + M) // 2, :])
            if isinstance(row0, tuple):
                return _bf(ref[pl.ds(row0[0] + row0[1] // 2, M // 2), :])
            return _bf(ref[pl.ds(pl.multiple_of(row0 // 2, 8), M // 2), :])

        def wo_dot(row0, M):
            o = rows_u32(o_scr, row0, M)
            return jnp.concatenate([_dot(o, _bf(wo_v[n])) for n in range(NCH)], axis=1)

        def row(k):
            return jnp.concatenate([modB[8 * (k - 2) + j, 0:1, :] for j in range(NCH)], axis=1)

        def ln23(row0, M, A):
            ga = row(2); sb = row(3); cb = row(4)
            x = rows_u32(x_v, row0, M).astype(f32)
            xm = x + ga * A
            hB = _ln(xm) * (1.0 + cb) + sb
            n3 = _ln(hB).astype(bf16)
            return xm, hB, n3

        shifts = [-1, -1, 1, 1, -2, -2, 2, 2]

        def g_val():
            return jnp.concatenate(
                [h1buf[j, HALO + shifts[j]:HALO + shifts[j] + T, :] for j in range(NCH)], axis=1).astype(bf16)

        def out_copy(r0, n, k, c0=0, cw=D):
            if cw == D:
                return pltpu.make_async_copy(obuf.at[pl.ds(r0, n)], o_hbm.bitcast(u32).at[pl.ds(r0, n)], osems.at[k])
            return pltpu.make_async_copy(obuf.at[pl.ds(r0, n), c0:c0 + cw], o_hbm.bitcast(u32).at[pl.ds(r0, n), c0:c0 + cw], osems.at[k])

        def ln4(hs):
            gb = row(5)
            x1 = hb[0:T, :] + hs
            base = xmid[0:T, :] + gb * x1
            n4 = _ln(x1).astype(bf16)
            return base, n4

        FH, DH2, HM = F // 2, D // 2, T // 2
        SIDX = {0: 0, 2: 1, 3: 2, 5: 3, 6: 4}

        def asums(a11, a12, a21, a22):
            return [a11 + a22, a21 + a22, a11, a22, a11 + a12, a21 - a11, a12 - a22]

        def bsums(src, dst, KH, NH, r0, n, c0=0, cw=None):
            cw = NH if cw is None else cw
            ld = lambda a, b: _bf(src[pl.ds(a * (KH // 2) + r0, n), b * NH + c0:b * NH + c0 + cw]).astype(f32)
            b11, b12, b21, b22 = ld(0, 0), ld(0, 1), ld(1, 0), ld(1, 1)
            outs = [b11 + b22, b12 - b22, b21 - b11, b11 + b12, b21 + b22]
            for i, o in enumerate(outs):
                dst[i, pl.ds(r0, n), c0:c0 + cw] = pltpu.bitcast(o.astype(bf16), u32)

        def w3op(k, c0, cw):
            def sl(a):
                return pl.ds(c0 + a, cw) if not isinstance(c0, int) else slice(c0 + a, c0 + a + cw)
            if k == 1:
                return _bf(w3_v[0:D // 4, sl(0)])
            if k == 4:
                return _bf(w3_v[D // 4:D // 2, sl(FH)])
            return _bf(w3s[SIDX[k], :, sl(0)])

        def w4op(k, c0, cw, r0=0, nr=F // 4):
            def rs(a):
                return pl.ds(r0 + a, nr) if not isinstance(r0, int) else slice(r0 + a, r0 + a + nr)
            if k == 1:
                return _bf(w4_v[rs(0), c0:c0 + cw])
            if k == 4:
                return _bf(w4_v[rs(F // 4), DH2 + c0:DH2 + c0 + cw])
            return _bf(w4s[SIDX[k], rs(0), c0:c0 + cw])

        def strass(dotk, hook=None):
            M = dotk(0); c11 = M; c22 = M
            if hook: hook(0, M)
            M = dotk(1); c21 = M; c22 = c22 - M
            if hook: hook(1, M)
            M = dotk(2); c12 = M; c22 = c22 + M
            if hook: hook(2, M)
            M = dotk(3); c11 = c11 + M; c21 = c21 + M
            if hook: hook(3, M)
            M = dotk(4); c11 = c11 - M; c12 = c12 + M
            if hook: hook(4, M)
            M = dotk(5); c22 = c22 + M
            if hook: hook(5, M)
            M = dotk(6); c11 = c11 + M
            if hook: hook(6, M)
            return c11, c12, c21, c22

        def n4_sums(r, n4v):
            q = T // RP0 // 2
            if r < q:
                n4f[r * RP0:(r + 1) * RP0, :] = n4v
            else:
                top = n4f[(r - q) * RP0:(r - q + 1) * RP0, :]
                A = asums(top[:, :DH2], top[:, DH2:], n4v[:, :DH2], n4v[:, DH2:])
                for k in range(7):
                    a4[k, (r - q) * RP0 // 2:(r - q + 1) * RP0 // 2, :] = pltpu.bitcast(A[k].astype(bf16), u32)

        def stage3(c0, cw, uc0, hook=None):
            U = strass(lambda k: _dot(_bf(a4[k]), w3op(k, c0, cw)), hook)
            A = asums(*[_gelu(x) for x in U])
            for k in range(7):
                ua[k, :, uc0:uc0 + cw] = pltpu.bitcast(A[k].astype(bf16), u32)

        RP0 = 16

        def preprocess():
            def p3(i, c):
                bsums(w3_v, w3s, D // 2, FH, pl.multiple_of(i * 8, 8), 8)
                return c
            lax.fori_loop(0, D // 4 // 8, p3, 0)

            def p4_(i, c):
                bsums(w4_v, w4s, F // 2, DH2, pl.multiple_of(i * 16, 16), 16)
                return c
            lax.fori_loop(0, F // 4 // 16, p4_, 0)

        if ST and PRE == 'L' and 'S' not in skip:
            preprocess()

        def bfirst():
            for j in range(NCH):
                h1buf[j, 0:HALO, :] = jnp.zeros((HALO, 128), f32)
            h7 = _bf(hP[...])
            zb = pl.multiple_of(zero * 8, 8) if ZB else 0
            h0 = (T + HALO) // 2 // 16 * 16 + (16 if T == 128 else 0)
            halves = [(0, h0), (h0, T + HALO - h0)]
            nA = (2 * T + HALO - AT0) // AP
            st = {'res': None, 'As': [], 'n3': [], 'h1': [], 'macc': {}}

            def att(k):
                if AG:
                    st['o'] = attention2(AT0 + k * AP, AP, AG)
                else:
                    attention(qbuf, kbuf, vbuf, 0, AT0 + k * AP, AP, True)

            def tok_q(cc=0):
                qbuf[0, pl.ds(zb + S + HALO, 8), :] = st['res'][0:8, cc * 128:(cc + 1) * 128]

            batt = None
            if 'A' in BA:
                batt = Att(0, 0, 0, 2 * T + HALO, [BWG] * ((2 * T + HALO) // RB * W // BWG), BPD, zb, BQD, True)
            for it in BA.split():
                k = int(it[1:]) if len(it) > 1 and it[1:].isdigit() else None
                if not ZB and it[0] in 'tWM':
                    continue
                if it[0] == 'A':
                    batt.steps(k)
                elif it[0] == 'R':
                    batt.steps(999)
                    batt.rest()
                elif it[0] == 'T':
                    st['res'] = subdot(h7, TL, 7, k)
                elif it[0] == 'a':
                    att(k)
                elif it[0] == 't':
                    tok_q(k or 0)
                elif it[0] == 'w':
                    pW(7, k, zb)
                elif it[0] == 'v':
                    pW(6, k, zb)
                elif it[0] == 'm':
                    for kq in range(KQ):
                        pM(6 * NM + k, kq, zb, st['macc'], k)
                elif it[0] == 'M':
                    wmB_v[32, pl.ds(zb + D // 2, 8), :] = pltpu.bitcast(st['res'][0:8, 0:128], u32)
                elif it[0] == 'W':
                    wo_raw[7, pl.ds(zb + D // 2 + 16, 8), :] = pltpu.bitcast(st['res'][0:8, 0:128], u32)
                elif it[0] == 'o':
                    assert batt is None or batt.done >= (halves[k][0] + halves[k][1]) // RB * NCH, batt.done
                    st['res'] = wo_dot(*halves[k])
                    st['As'].append(st['res'])
                elif it[0] == 'l':
                    r0, m = halves[k]
                    xm, hB, n3 = ln23(r0, m, st['As'][k])
                    xmid[r0:r0 + m, :] = xm
                    hb[r0:r0 + m, :] = hB
                    st['n3'].append(n3)
                elif it[0] == 'u':
                    r0, m = halves[k]
                    st['res'] = _dot(st['n3'][k], _bf(w1_v[...]))
                    h1 = _gelu(st['res'])
                    for j in range(NCH):
                        h1buf[j, HALO + r0:HALO + r0 + m, :] = h1[:, j * 128:(j + 1) * 128]
                elif it[0] == 'z':
                    if 'g' not in st:
                        st['g'] = g_val()
                    cw_ = D // NZ
                    st['res'] = _dot(st['g'], _bf(w2_v[:, k * cw_:(k + 1) * cw_]))
                    hsbuf[0:T, k * cw_:(k + 1) * cw_] = st['res']
                elif it[0] == 'U':
                    hh, pp = divmod(k, 10)
                    r0, m = halves[hh]
                    cw_ = D // NU
                    st['res'] = _dot(st['n3'][hh], _bf(w1_v[:, pp * cw_:(pp + 1) * cw_]))
                    h1 = _gelu(st['res'])
                    for j in range(cw_ // 128):
                        h1buf[pp * (cw_ // 128) + j, HALO + r0:HALO + r0 + m, :] = h1[:, j * 128:(j + 1) * 128]
            if 'g' not in st:
                hsbuf[0:T, :] = _dot(g_val(), _bf(w2_v[...]))

        if upto >= 3 and 'F' not in skip:
            bfirst()

        def carries(xm, hB, h1, notlast):
            xmid[0:HALO, :] = xmid[T:T + HALO, :]
            hb[0:HALO, :] = hb[T:T + HALO, :]
            for j in range(NCH):
                h1buf[j, 0:2 * HALO, :] = h1buf[j, T:T + 2 * HALO, :]
            xmid[HALO:HALO + T, :] = xm
            hb[HALO:HALO + T, :] = hB
            for j in range(NCH):
                h1j = h1[:, j * 128:(j + 1) * 128]
                h1buf[j, 2 * HALO:HALO + T, :] = h1j[0:T - HALO]
                h1buf[j, HALO + T:2 * HALO + T, :] = jnp.where(notlast, h1j[T - HALO:T], 0.0)

        RP = 16

        def bbody(i, carry):
            static = isinstance(i, int)
            if static:
                row0h = i * (T // 2)
                abase = (i + 1) * T
                abaseh = (i + 1) * (T // 2)
                z1 = pl.multiple_of(zero * 8, 8)
                z2 = pl.multiple_of(zero2 * 8, 8)
            else:
                row0h = pl.multiple_of(i * (T // 2), T // 2)
                nxt = jnp.minimum(i + 1, NT - 1)
                abase = pl.multiple_of(nxt * T, T)
                abaseh = pl.multiple_of(nxt * (T // 2), T // 2)
                z1 = pl.multiple_of((i >> 8) * 8, 8)
                z2 = pl.multiple_of((i >> 9) * 8, 8)
            ga = row(2); sb = row(3); cb = row(4); gb = row(5)
            bases, n4p, xms, hBs, n3p, As = [], [], [], [], [], []
            att = None
            asch = {}
            if AB == 9:
                att = Att(abase, abaseh, HALO, T, [int(t) for t in WGS], PD, z1)
                for t in ASCH.split():
                    k_, v_ = t.split(':')
                    asch[k_] = int(v_)

            def astep(tag):
                if att is not None and tag in asch:
                    att.steps(asch[tag])

            def p4(r):
                r0 = r * RP
                x1 = hb[r0:r0 + RP, :] + hsbuf[pl.ds(z2 + r0, RP), :]
                if ST:
                    bases.append((r, xmid[r0:r0 + RP, :] + gb * x1))
                    n4_sums(r, _ln(x1))
                    n4p.append(None)
                    return
                bases.append(xmid[r0:r0 + RP, :] + gb * x1)
                n4v = _ln(x1).astype(bf16)
                if EX4:
                    n4b[r0 // 2:(r0 + RP) // 2, :] = pltpu.bitcast(n4v, u32)
                n4p.append(n4v)

            def p23(r, A):
                r0 = r * RP
                x = rows_u32(x_v, (row0h, HALO + r0), RP).astype(f32)
                xm = x + ga * A[r0:r0 + RP]
                hB = _ln(xm) * (1.0 + cb) + sb
                xms.append(xm); hBs.append(hB)
                n3v = _ln(hB).astype(bf16)
                if EX3:
                    n3b[r0 // 2:(r0 + RP) // 2, :] = pltpu.bitcast(n3v, u32)
                n3p.append(n3v)

            ord4 = list(ORD4) if ST else list(range(T // RP))
            for r in range(T // RP):
                if rel4[r] < 0:
                    p4(ord4[r])
            o = rows_u32(o_scr, (row0h, HALO), T)
            for n in range(NCH):
                An = _dot(o, _bf(wo_v[n]))
                As.append(An)
                r4 = [r for r in range(T // RP) if rel4[r] == n]
                if r4:
                    hsbuf[pl.ds(z1 + T, 8), 0:128] = An[0:8, 0:128]
                for r in r4:
                    p4(ord4[r])
                astep('o%d' % n)
            A = jnp.concatenate(As, axis=1)
            if ST:
                base = jnp.concatenate([b for _, b in sorted(bases, key=lambda t: t[0])], axis=0)
                for c in range(FH // CW3):
                    def hook(k, M, c=c):
                        r23 = [r for r in range(T // RP) if R23[r] == 7 * c + k]
                        if r23:
                            x_v[pl.ds(z1 + S // 2 + HALO // 2, 8), 0:128] = pltpu.bitcast(M[0:8, 0:128], u32)
                        for r in r23:
                            p23(r, A)
                    stage3(c * CW3, CW3, c * CW3, hook)
            else:
                base = jnp.concatenate(bases, axis=0)
                n4 = _bf(n4b[...]) if EX4 else jnp.concatenate(n4p, axis=0)
                U = _dot(n4, _bf(w3_v[...]))
                u = _gelu(U).astype(bf16)
            for c in range(0 if ST else F // 128):
                r23 = [r for r in range(T // RP) if rel23[r] == NCH + c]
                if r23 or c in XT:
                    x_v[pl.ds(z1 + S // 2 + HALO // 2, 8), 0:128] = pltpu.bitcast(U[0:8, c * 128:(c + 1) * 128], u32)
                for r in r23:
                    p23(r, A)
                astep('c%d' % c)
            assert len(n3p) == T // RP and len(n4p) == T // RP
            xm = jnp.concatenate(xms, axis=0)
            hB = jnp.concatenate(hBs, axis=0)
            n3 = _bf(n3b[...]) if EX3 else jnp.concatenate(n3p, axis=0)
            h1 = _gelu(_dot(n3, _bf(w1_v[...])))
            carries(xm, hB, h1, i < NT - 1)
            if static:
                if i < NT - 1:
                    attention(qbuf, kbuf, vbuf, abase, HALO, T, False, abaseh)
            elif 'noatt' not in dbg:
                if AB == 9:
                    att.steps(999)
                    att.rest()
                    if DL:
                        h1buf[0, pl.ds(z1 + T + 2 * HALO, 8), :] = att.OC[T // RB - 1, NCH - 1]
                elif AB:
                    attention2(HALO, T, AB, abase, abaseh)
                else:
                    attention(qbuf, kbuf, vbuf, abase, HALO, T, False, abaseh)
            if ST:
                ro = pl.multiple_of((i - 1) * (T // 2), T // 2)
                for c in range(DH2 // CW4):
                    c0 = c * CW4
                    Hs = strass(lambda k: _dot(_bf(ua[k]), w4op(k, c0, CW4)))
                    for q, Hq in enumerate(Hs):
                        rr, cc = (q // 2) * HM, (q % 2) * DH2 + c0
                        o_ = base[rr:rr + HM, cc:cc + CW4] + gb[:, cc:cc + CW4] * Hq
                        obuf[pl.ds(ro + rr // 2, HM // 2), cc:cc + CW4] = pltpu.bitcast(o_.astype(bf16), u32)
                hsbuf[0:T, :] = _dot(g_val(), _bf(w2_v[...]))
                return carry
            h2 = _dot(u, _bf(w4_v[...]))
            if static:
                obuf[(i - 1) * (T // 2):i * (T // 2), :] = pltpu.bitcast((base + gb * h2).astype(bf16), u32)
            else:
                obuf[pl.ds(pl.multiple_of((i - 1) * (T // 2), T // 2), T // 2), :] = pltpu.bitcast((base + gb * h2).astype(bf16), u32)
            hsbuf[0:T, :] = _dot(g_val(), _bf(w2_v[...]))
            return carry

        if upto >= 4 and 'B' not in skip:
            if UB:
                for i in range(1, 1 + UB):
                    bbody(i, 0)
                    if i in BAR:
                        out_copy_i(i).start()
                if 1 + UB < NT:
                    lax.fori_loop(1 + UB, NT, bbody, 0)
            else:
                lax.fori_loop(1, NT, bbody, 0)

        def blast():
            r0 = (NT - 1) * (T // 2)
            out_copy(0, r0, 0).start()
            if ST:
                gb = row(5)
                for r in ORD4:
                    p0 = r * RP
                    x1 = hb[p0:p0 + RP, :] + hsbuf[p0:p0 + RP, :]
                    baseb[p0:p0 + RP, :] = xmid[p0:p0 + RP, :] + gb * x1
                    n4_sums(r, _ln(x1))

                def fin(q, Hq, c0, cw):
                    rr, cc = (q // 2) * HM, (q % 2) * DH2 + c0
                    o_ = baseb[rr:rr + HM, cc:cc + cw] + gb[:, cc:cc + cw] * Hq
                    obuf[r0 + rr // 2:r0 + rr // 2 + HM // 2, cc:cc + cw] = pltpu.bitcast(o_.astype(bf16), u32)

                if SB == 'F':
                    for c in range(FH // CW3):
                        stage3(c * CW3, CW3, c * CW3)
                    for c in range(DH2 // CW4):
                        Hs = strass(lambda k: _dot(_bf(ua[k]), w4op(k, c * CW4, CW4)))
                        for q, Hq in enumerate(Hs):
                            fin(q, Hq, c * CW4, CW4)
                else:
                    QF = FH // 2

                    def sbody(m, carry):
                        cb_ = pl.multiple_of(m * QF, 128)
                        for c in range(QF // 128):
                            stage3(cb_ + c * 128, 128, c * 128)
                        rb_ = pl.multiple_of(m * (QF // 2), 32)
                        for c in range(DH2 // CW4):
                            for k in range(7):
                                Mk = _dot(_bf(ua[k, :, 0:QF]), w4op(k, c * CW4, CW4, rb_, QF // 2))
                                macc[k, :, c * CW4:(c + 1) * CW4] = jnp.where(m > 0, macc[k, :, c * CW4:(c + 1) * CW4], 0.0) + Mk
                        return carry

                    lax.fori_loop(0, 2, sbody, 0)
                    for c in range(DH2 // 128):
                        Hs = strass(lambda k: macc[k, :, c * 128:(c + 1) * 128])
                        for q, Hq in enumerate(Hs):
                            fin(q, Hq, c * 128, 128)
                out_copy(r0, T // 2, 1).start()
                out_copy(0, r0, 0).wait()
                out_copy(r0, T // 2, 1).wait()
                return
            if BL == 'M':
                gb = row(5)

                def l4(p0, zz, dst):
                    x1 = hb[p0:p0 + RP, :] + (hsbuf[pl.ds(zz + p0, RP), :] if zz is not None else hsbuf[p0:p0 + RP, :])
                    baseb[p0:p0 + RP, :] = xmid[p0:p0 + RP, :] + gb * x1
                    q0 = (p0 % HM) // 2
                    dst[q0:q0 + RP // 2, :] = pltpu.bitcast(_ln(x1).astype(bf16), u32)

                for p0 in range(0, HM, RP):
                    l4(p0, None, n4b)

                def mbody(m, carry):
                    zz = pl.multiple_of((m >> 8) * 8, 8)
                    if MA:
                        n4 = _bf(n4b[0:HM // 2, :])
                    else:
                        n4 = _bf(n4b[pl.ds(pl.multiple_of(m * (HM // 2), HM // 2), HM // 2), :])
                    U = _dot(n4, _bf(w3_v[...]))
                    u = _gelu(U).astype(bf16)
                    for k, p0 in enumerate(range(HM, T, RP)):
                        if MT is not None and (k == 0 or MT[k] != MT[k - 1]):
                            hsbuf[pl.ds(zz + T, 8), 0:128] = U[0:8, MT[k] * 128:(MT[k] + 1) * 128]
                        l4(p0, zz if MT is not None else None, n3b if MA else n4b.at[HM // 2:T // 2])
                    if MA:
                        n4b[0:HM // 2, :] = n3b[0:HM // 2, :]
                    ro = pl.multiple_of(r0 + m * (HM // 2), HM // 2)
                    c0 = 0
                    for cw_ in MN:
                        h2 = _dot(u, _bf(w4_v[:, c0:c0 + cw_]))
                        bs = baseb[pl.ds(pl.multiple_of(m * HM, HM), HM), c0:c0 + cw_]
                        obuf[pl.ds(ro, HM // 2), c0:c0 + cw_] = pltpu.bitcast((bs + gb[:, c0:c0 + cw_] * h2).astype(bf16), u32)
                        out_copy(ro, HM // 2, 1, c0, cw_).start()
                        c0 += cw_
                    return carry

                lax.fori_loop(0, 2, mbody, 0)
                out_copy(0, r0, 0).wait()
                for hf in range(2):
                    c0 = 0
                    for cw_ in MN:
                        out_copy(r0 + hf * (HM // 2), HM // 2, 1, c0, cw_).wait()
                        c0 += cw_
                return
            base, n4 = ln4(hsbuf[0:T, :])
            if BL:
                FC = F // BL
                xmid[0:T, :] = base
                n4b[...] = pltpu.bitcast(n4, u32)
                hsbuf[0:T, :] = jnp.zeros((T, D), f32)

                def body(c, carry):
                    w3c = w3_v[:, pl.ds(pl.multiple_of(c * FC, 128), FC)]
                    u = _gelu(_dot(_bf(n4b[...]), _bf(w3c))).astype(bf16)
                    w4c = w4_v[pl.ds(pl.multiple_of(c * (FC // 2), 32), FC // 2), :]
                    hsbuf[0:T, :] += _dot(u, _bf(w4c))
                    return carry

                lax.fori_loop(0, BL, body, 0)
                obuf[r0:r0 + T // 2, :] = pltpu.bitcast((xmid[0:T, :] + row(5) * hsbuf[0:T, :]).astype(bf16), u32)
            else:
                u = _gelu(_dot(n4, _bf(w3_v[...]))).astype(bf16)
                h2 = _dot(u, _bf(w4_v[...]))
                obuf[r0:r0 + T // 2, :] = pltpu.bitcast((base + row(5) * h2).astype(bf16), u32)
            out_copy(r0, T // 2, 1).start()
            out_copy(0, r0, 0).wait()
            out_copy(r0, T // 2, 1).wait()

        if upto >= 5 and 'L' not in skip:
            blast()

    @jax.jit
    def fn(A_x, A_wqkv, A_wo, B_x, B_w1, B_w2, B_w3, B_w4, c, w_mod):
        x = A_x.reshape(S, D)
        any_spec = pl.BlockSpec(memory_space=pl.ANY)
        out = pl.pallas_call(
            kernel,
            in_specs=[any_spec] * 9,
            out_specs=any_spec,
            out_shape=jax.ShapeDtypeStruct((S, D), bf16),
            scratch_shapes=[
                pltpu.VMEM((S // 2 + HALO // 2 + 8, D), u32),
                pltpu.VMEM((D // 2 + 32, 3 * D), u32),
                pltpu.VMEM((D // 2, D), u32),
                pltpu.VMEM((D // 2, D), u32),
                pltpu.VMEM((D // 2, D), u32),
                pltpu.VMEM((NCH + WS, D // 2 + 32, 128), u32),
                pltpu.VMEM((NCH + WS, D // 2, 128), u32),
                pltpu.VMEM((D // 2, D), u32),
                pltpu.VMEM((D // 2, D), u32),
                pltpu.VMEM((D // 2, F), u32),
                pltpu.VMEM((F // 2, D), u32),
                pltpu.VMEM((D // 2, 128), f32),
                pltpu.VMEM((D // 2, 128), f32),
                pltpu.VMEM((8, D // 2 + 16, 256), u32),
                pltpu.VMEM((33, D // 2 + 32, 128), u32),
                pltpu.VMEM((8, 8, 256), f32),
                pltpu.VMEM((36, 8, 128), f32),
                pltpu.VMEM((3 if MU else NCH, S + 32, 128), f32),
                pltpu.VMEM((PR // 2, 128), u32),
                pltpu.VMEM((S // 2, 128), u32),
                pltpu.VMEM((NCH, S + 32, 128), f32),
                pltpu.VMEM((NCH, S + 2 * HALO + 32 * (AB == 9), 128), f32),
                pltpu.VMEM((NCH, S + 2 * HALO + 32 * (AB == 9), 128), f32),
                pltpu.VMEM((T + HALO, D), f32),
                pltpu.VMEM((T + HALO, D), f32),
                pltpu.VMEM((NCH, T + 2 * HALO + 32 * DL, 128), f32),
                pltpu.VMEM((S // 2, D), u32),
                pltpu.VMEM((S // 2 + HALO // 2, D), u32),
                pltpu.VMEM((T + 32, D), f32),
                pltpu.VMEM((T // 2, D), u32),
                pltpu.VMEM((T // 2, D), u32),
                pltpu.VMEM((T, D), f32),
                pltpu.VMEM((5, D // 4, F // 2), u32),
                pltpu.VMEM((5, F // 4, D // 2), u32),
                pltpu.VMEM((T, D), f32),
                pltpu.VMEM((7, T // 4, D // 2), u32),
                pltpu.VMEM((7, T // 4, F // 2), u32),
                pltpu.VMEM((7, T // 2, D // 2), f32),
                pltpu.VMEM((1, D), bf16),
            ] + ([pltpu.VMEM((padr, 128), f32)] if padr else []) + [
                pltpu.SMEM((8,), jnp.int32),
            ],
            compiler_params=pltpu.CompilerParams(vmem_limit_bytes=126 * 1024 * 1024),
        )(x, A_wqkv, A_wo, B_w1, B_w2, B_w3, B_w4, c, w_mod)
        return out.reshape(1, S, D)
    return fn


_fn = make()


def pallas_adaLN_cond__sliding_local_dilated__mixer_s_mlp__prompt_kernel(A_x, A_wqkv, A_wo, B_x, B_w1, B_w2, B_w3, B_w4, c, w_mod):
    return _fn(A_x, A_wqkv, A_wo, B_x, B_w1, B_w2, B_w3, B_w4, c, w_mod)
```

```python
import functools
import jax
import jax.numpy as jnp
from jax import lax
import jax.experimental.pallas as pl
import jax.experimental.pallas.tpu as pltpu

S, D, F = 2048, 1024, 3584
H, DH, W, DIL = 32, 32, 8, 2
NCH = D // 128
EPS = 1e-5
SCALE = DH ** -0.5
f32, bf16, u32 = jnp.float32, jnp.bfloat16, jnp.uint32
HALO = 16


def _ln(x):
    m = jnp.mean(x, axis=-1, keepdims=True)
    xc = x - m
    v = jnp.mean(xc * xc, axis=-1, keepdims=True)
    return xc * lax.rsqrt(v + EPS)


def _gelu(x):
    c0 = 0.7978845608028654
    c1 = c0 * 0.044715
    t = jnp.tanh(x * (c0 + c1 * (x * x)))
    hx = 0.5 * x
    return hx + hx * t


def _dot(a, b):
    return jnp.dot(a, b, preferred_element_type=f32)


def _bf(w):
    return pltpu.bitcast(w, bf16)


def _lane_xor(x, s):
    lane = lax.broadcasted_iota(jnp.int32, x.shape, 1)
    return jnp.take_along_axis(x, lane ^ s, axis=1)


def _exchange8_multi(XS):
    XS = [list(X) for X in XS]
    lane = lax.broadcasted_iota(jnp.int32, XS[0][0].shape, 1)
    for t in range(3):
        s = 1 << (t + 2)
        m = (lane & s) != 0
        for X in XS:
            for p in range(8):
                if p & (1 << t):
                    continue
                p2 = p | (1 << t)
                tmp = _lane_xor(jnp.where(m, X[p], X[p2]), s)
                X[p], X[p2] = jnp.where(m, tmp, X[p]), jnp.where(m, X[p2], tmp)
    return XS


def _group4_sum(acc):
    lane = lax.broadcasted_iota(jnp.int32, acc.shape, 1)
    acc = acc + jnp.where((lane & 1) != 0, pltpu.roll(acc, 1, 1), pltpu.roll(acc, 127, 1))
    acc = acc + jnp.where((lane & 2) != 0, pltpu.roll(acc, 2, 1), pltpu.roll(acc, 126, 1))
    return acc


def make(T=128, PR=512, RB=8, EG=4, upto=9, AT0=0, AP=16,
         DO='c X0 Wq sa ca X1 Wk Wv X2 X3 X4 X5 X6 X7 X8 X9 X10 X12 X13 X11 X14 X15',
         PS=None, PSX=None, RL=1, D0='1234', LP=16, BL='M', ZB=1,
         order0='T0 T1 X x00 x01 m0 T2 T3 X x10 x11 h0 T4 T5 X x20 H0 X x21 H1 H2 H3 H4 H5', NDEF=6, BA=None,
         side=None, KQ=4, KQ0=1, NM=5, NR=8, AG=1,
         rel4=(-1, -1, -1, 0, 1, 2, 3, 4), rel23=(8, 9, 10, 11, 12, 13, 14, 15),
         padr=0, dbg='', UB=0, BAR=(), GL=0, MU=1, WS=1, skip='', AB=9, WGS='1'*128, PD=0, ASCH='', DL=0, EX3=1, EX4=1, XT=(), MT=(4, 10, 16, 22), MA=0, MN=(1024,), NZ=8, NU=2, BPD=0, BQD=None, BWG=8,
         ST=1, ORD4=(0, 4, 1, 5, 2, 6, 3, 7), R23=(0, 4, 8, 12, 16, 20, 24, 28), PRE='R', CW3=128, CW4=128, SB='S', SJ='8,9,10,11,12,13,14,15,16,17,18,19,20,21,22', P0R=4, LK3=1, LK4=1, TKS=0, TKW=0, TKM=0, SW=1, SK=None, SL=1, TG=1, TD=480, NC=1):
    HS, HO = (2, 0) if MU else (0, S // 2)
    NT = S // T
    NP = S // PR
    order0 = order0.split()
    TL = S - PR
    if PS is None:
        PS = ('wc C wX0 L0 wWq e0 wsa S wca A h0 wX1 u0:0 L1 wWk u1:0 e1 wWv u0:1 u1:1 e2 wX2 u0:2 u1:2 L2 u2:0 '
              'wX3 wX4 u2:12 L3 u3:012 L4 u4:0 wX5 wX6 wX7 u4:12 L5 u5:012 L6 u6:012 L7 u7:0 '
              'wX8 wX9 wX10 wX12 wX13 u7:12 L8 u8:012 L9 u9:012 L10 ua:0 L12 L13 wX11 wX14 wX15 Da D5 Db D6 Dc D7 Dd DW ua:12 L11 ub:012 L14 L15')
    if BA is None:
        BA = ('a0 a1 T0 T1 t0 a2 a3 W w0 w1 w2 w3 w4 w5 w6 w7 T2 t0 a4 a5 T3 t0 a6 a7 T4 t0 a8 a9 T5 t0 a10 o0 t0 a11 t4 a12 '
              'o1 t0 a13 t4 a14 M m0 m1 l0 l1 u0 t0 a15 t4 a16 u1')
    if WS and 'v0' not in BA:
        BA = BA.replace('W w0 w1 w2 w3 w4 w5 w6 w7', 'W v0 v1 v2 v3 v4 v5 v6 v7 w0 w1 w2 w3 w4 w5 w6 w7')
    if PSX:
        for k_, v_ in PSX.items():
            assert (' ' + k_ + ' ') in PS
            PS = PS.replace(' ' + k_ + ' ', ' ' + k_ + ' ' + v_ + ' ')
    S_C, S_X, S_SA, S_CA, S_W0, S_WQ, S_WO, S_MB, S_W = 0, 1, 17, 25, 33, 36, 44, 52, 60
    S_P = 64
    NSEM = 68
    DEF = list(range(6 - NDEF, 6))
    tags = ['T%d' % sd for sd in DEF] + ['%dH%d' % (p, sd) for p in range(NP) for sd in range(6 if p < NP - 1 else 6 - NDEF)]
    if side is None:
        side = 'W:7,9,11,13,15,17,19,21 M:4,5,6,7,8,9,10,11,12,13,14,15,16,17,18,19,20,21,22,22'
        if PRE == 'R':
            side += ' S:' + SJ
    if isinstance(side, str):
        sd_ = {}
        for grp in side.split():
            kind, lst = grp.split(':')
            for k, t in enumerate(lst.split(',')):
                sd_.setdefault(tags[int(t)], []).append(kind + str(k))
        side = sd_
    assert sum(1 for v in side.values() for j in v if j[0] in 'Aa') * AP == AT0

    def kernel(*refs):
        pl.run_scoped(functools.partial(body, *refs), pltpu.SemaphoreType.DMA((NSEM,)), pltpu.SemaphoreType.DMA((2,)))

    def body(x_hbm, wqkv_hbm, wo_hbm, w1_hbm, w2_hbm, w3_hbm, w4_hbm, c_hbm, wmod_hbm,
             o_hbm,
             x_v, wqkv_raw, wq_v, wk_v, wv_v, wo_raw, wo_v, w1_v, w2_v, w3_v, w4_v, cE, cO, wmA_v, wmB_v,
             modA, modB, xhat, hP, h0, qbuf, kbuf, vbuf, xmid, hb, h1buf, obuf, o_scr, hsbuf, n4b, n3b, baseb, n4f, a4, ua, macc, c_v, *rest):
        zsm, sems, osems = rest[-3:]

        def cp(src, dst, k):
            return pltpu.make_async_copy(src, dst, sems.at[k])

        xu = x_hbm.bitcast(u32)
        wqkvu = wqkv_hbm.bitcast(u32)
        wou = wo_hbm.bitcast(u32)
        wmodu = wmod_hbm.bitcast(u32)

        def lane_ds(k, n, base=0):
            if isinstance(k, int):
                return pl.ds(base + k * n, n)
            return pl.ds(pl.multiple_of(base + k * n, 128), n)

        def row_ds(base, k, n):
            if isinstance(k, int):
                return pl.ds(base + k * n, n)
            return pl.ds(pl.multiple_of(base + k * n, 8), n)

        c_c = cp(c_hbm, c_v, S_C)

        def c_x(b):
            return cp(xu.at[b * 64:(b + 1) * 64], x_v.at[b * 64:(b + 1) * 64], S_X + b)

        def c_sa(k):
            return cp(wmodu.at[:, lane_ds(k, 128)], wmA_v.at[k, 0:D // 2, 0:128], S_SA + k)

        def c_ca(k):
            return cp(wmodu.at[:, lane_ds(k, 128, D)], wmA_v.at[k, 0:D // 2, 128:256], S_CA + k)

        def c_w0(b):
            return cp(wqkvu.at[0:64, b * D:(b + 1) * D], wqkv_raw.at[0:64, b * D:(b + 1) * D], S_W0 + b)

        def c_wq(k):
            return cp(wqkvu.at[row_ds(0, k, 64)], wqkv_raw.at[row_ds(0, k, 64)], S_WQ + k)

        def c_wo(p):
            return cp(wou.at[:, lane_ds(p, 128)], wo_raw.at[p, 8:8 + D // 2], S_WO + p)

        def c_mb(t, g):
            return cp(wmodu.at[:, lane_ds(t, 128, 2 * D)], wmB_v.at[t, 0:D // 2], S_MB + g)

        c_w = [cp(w1_hbm.bitcast(u32), w1_v, S_W), cp(w2_hbm.bitcast(u32), w2_v, S_W + 1)]
        w3u, w4u = w3_hbm.bitcast(u32), w4_hbm.bitcast(u32)
        N3, N4 = D // 4 // 4, F // 4 // 4

        def c_p(p):
            def rows(base, n):
                if isinstance(p, int):
                    return pl.ds(base + p * n, n)
                return pl.ds(pl.multiple_of(base + p * n, 8), n)
            return ([cp(w3u.at[rows(a * (D // 4), N3)], w3_v.at[a, rows(0, N3)], S_P + p) for a in range(2)]
                    + [cp(w4u.at[rows(a * (F // 4), N4)], w4_v.at[a, rows(0, N4)], S_P + p) for a in range(2)])

        def named(nm):
            if nm == 'c':
                return c_c
            if nm == 'sa':
                return c_sa(0)
            if nm == 'ca':
                return c_ca(0)
            if nm[0] == 'W':
                return c_w0('qkv'.index(nm[1]))
            return c_x(int(nm[1:]))

        for nm in DO.split():
            named(nm).start()
        def start_group(g):
            if g == 'W':
                if upto >= 3:
                    c_wo(7).start()
                    for t in range(6 * NM, 32):
                        c_mb(t, 6).start()
                    for c in c_w:
                        c.start()
            elif g in 'abcd':
                for c in c_p('abcd'.index(g)):
                    c.start()
            elif upto >= 2 and 'nodma2' not in dbg:
                r = int(g)
                c_sa(r).start()
                c_ca(r).start()
                c_wq(r).start()
                c_wo(r - 1).start()
                if r >= 2:
                    for i in range(NM):
                        c_mb(NM * (r - 2) + i, r - 2).start()

        for g in D0:
            start_group(g)
        assert sorted(list(D0) + [it[1] for it in PS.split() if it[0] == 'D']) == sorted('1234567Wabcd')

        def _zinit(i, carry):
            zsm[2 + i] = i >> 8
            return carry

        lax.fori_loop(0, 3, _zinit, 0)
        zp3 = pl.multiple_of(zsm[4] * 8, 8)
        zp1 = pl.multiple_of(zsm[2] * 8, 8)
        zp2 = pl.multiple_of(zsm[3] * 8, 8)

        x_v[S // 2:S // 2 + HALO // 2, :] = jnp.zeros((HALO // 2, D), u32)
        for j in range(NCH):
            z = jnp.zeros((HALO, 128), f32)
            qbuf[j, S:S + HALO, :] = z
            kbuf[j, HALO + S:2 * HALO + S, :] = z
            vbuf[j, HALO + S:2 * HALO + S, :] = z
            kbuf[j, 0:HALO, :] = z
            vbuf[j, 0:HALO, :] = z
            wo_raw[j, 0:8, :] = jnp.zeros((8, 128), u32)
            wo_raw[j, 8 + D // 2:16 + D // 2, :] = jnp.zeros((8, 128), u32)

        def mv_part(w, r0, acc):
            n = w.shape[0]
            lo = pltpu.bitcast(w << 16, f32)
            hi = pltpu.bitcast(w & jnp.uint32(0xFFFF0000), f32)
            pr = lo * cE[r0:r0 + n, :] + hi * cO[r0:r0 + n, :]
            for t in range(n // 8):
                acc = pr[8 * t:8 * t + 8] if acc is None else acc + pr[8 * t:8 * t + 8]
            return acc

        wparts = (wq_v, wk_v, wv_v)
        bufs = (qbuf, kbuf, vbuf)

        def exch_groups(grps):
            for g0 in range(0, len(grps), EG):
                gs = grps[g0:g0 + EG]
                XS = [[wqkv_raw[row_ds(rg * 8, k * 8, 8), b * D + a * 128:b * D + (a + 1) * 128] for a in range(NCH)]
                      for (k, b, rg) in gs]
                YS = _exchange8_multi(XS)
                for (k, b, rg), Y in zip(gs, YS):
                    wparts[b][row_ds(rg * 8, 0 if SW else k * 8, 8), :] = jnp.concatenate(Y, axis=1)

        def subdot(lhs, row0, kc, sd, init=False, valid=None):
            b, hf = sd // 2, sd % 2
            n = lhs.shape[0]
            res = _dot(lhs, _bf(wparts[b][row_ds(0, 0 if SW else kc, 64), hf * 512:(hf + 1) * 512]))
            o = row0 + (0 if b == 0 else HALO)
            for jj in range(4):
                j = hf * 4 + jj
                if init:
                    bufs[b][j, o:o + n, :] = res[:, jj * 128:(jj + 1) * 128]
                elif valid is not None:
                    bufs[b][j, o:o + n, :] = jnp.where(valid, bufs[b][j, o:o + n, :], 0.0) + res[:, jj * 128:(jj + 1) * 128]
                else:
                    bufs[b][j, o:o + n, :] += res[:, jj * 128:(jj + 1) * 128]
            return res

        def prologue():
            st = {}

            def crep():
                c = c_v[...].astype(f32)
                scf = (c * jax.nn.sigmoid(c)).astype(bf16).astype(f32)
                rr = lax.broadcasted_iota(jnp.int32, (128, 128), 0)
                ll = lax.broadcasted_iota(jnp.int32, (128, 128), 1)
                sel = ll == jnp.where(rr < 64, 2 * rr, 2 * rr - 127)
                for j in range(NCH):
                    dg = jnp.where(sel, jnp.broadcast_to(scf[:, j * 128:(j + 1) * 128], (128, 128)), 0.0).astype(bf16)
                    rep = _dot(dg, jnp.ones((128, 128), bf16))
                    cE[j * 64:(j + 1) * 64, :] = rep[0:64]
                    cO[j * 64:(j + 1) * 64, :] = rep[64:128]

            def h_store(r0, xh0):
                h = (xh0 * (1.0 + st['ca']) + st['sa']).astype(bf16)
                if r0 < TL:
                    xhat[HS, HO + r0 // 2:HO + (r0 + LP) // 2, :] = pltpu.bitcast(h, f32)
                else:
                    hP[(r0 - TL) // 2:(r0 - TL + LP) // 2, :] = pltpu.bitcast(h, u32)

            def h0_lhs(b0, nb, gated):
                r0 = HO + b0 * 64
                if not gated:
                    return _bf(xhat[HS, r0:r0 + nb * 64, :])
                if GL:
                    return jnp.concatenate([_bf(xhat[HS, r0:r0 + nb * 64 - 8, :]), _bf(xhat[HS, pl.ds(zp3 + r0 + nb * 64 - 8, 8), :])], axis=0)
                return jnp.concatenate([_bf(xhat[HS, pl.ds(zp3 + r0, 8), :]), _bf(xhat[HS, r0 + 8:r0 + nb * 64, :])], axis=0)

            def ln_piece(b, i):
                r0 = b * 128 + i * LP
                direct = 'ca' in st and 'sa' in st
                if MU:
                    x = _bf(x_v[pl.ds(zp1 + r0 // 2, LP // 2), :]).astype(f32)
                    m = jnp.mean(x, axis=-1, keepdims=True)
                    if RL:
                        x = _bf(x_v[pl.ds(zp2 + r0 // 2, LP // 2), :]).astype(f32)
                    xc = x - m
                    rs = lax.rsqrt(jnp.mean(xc * xc, axis=-1, keepdims=True) + EPS)
                    xhat[0, r0:r0 + LP, :] = jnp.broadcast_to(m, (LP, 128))
                    xhat[1, r0:r0 + LP, :] = jnp.broadcast_to(rs, (LP, 128))
                    if direct:
                        h_store(r0, xc[:, 0:128] * rs)
                    return
                if RL:
                    m = jnp.mean(_bf(x_v[pl.ds(zp1 + r0 // 2, LP // 2), :]).astype(f32), axis=-1, keepdims=True)
                    xc = _bf(x_v[pl.ds(zp2 + r0 // 2, LP // 2), :]).astype(f32) - m
                    v = jnp.mean(xc * xc, axis=-1, keepdims=True)
                    xh = (_bf(x_v[r0 // 2:(r0 + LP) // 2, :]).astype(f32) - m) * lax.rsqrt(v + EPS)
                else:
                    xh = _ln(_bf(x_v[pl.ds(zp1 + r0 // 2, LP // 2), :]).astype(f32))
                for j in range(1 if direct else 0, NCH):
                    xhat[j, r0:r0 + LP, :] = xh[:, j * 128:(j + 1) * 128]
                if direct:
                    h_store(r0, xh[:, 0:128])

            def ln_block(b):
                for i in range(128 // LP):
                    ln_piece(b, i)

            def hblk(b):
                for i in range(128 // LP):
                    r0 = b * 128 + i * LP
                    if MU:
                        x = _bf(x_v[r0 // 2:(r0 + LP) // 2, 0:128]).astype(f32)
                        h_store(r0, (x - xhat[0, r0:r0 + LP, :]) * xhat[1, r0:r0 + LP, :])
                    else:
                        h_store(r0, xhat[0, r0:r0 + LP, :])

            for it in PS.split():
                if it[0] == 'w':
                    named(it[1:]).wait()
                elif it[0] == 'D':
                    start_group(it[1])
                elif it == 'C':
                    crep()
                elif it[0] == 'L':
                    ln_block(int(it[1:]))
                elif it[0] == 'h':
                    hblk(int(it[1:]))
                elif it == 'S':
                    st['sa'] = jnp.sum(mv_part(wmA_v[0, 0:D // 2, 0:128], 0, None), axis=0, keepdims=True)
                elif it == 'A':
                    st['ca'] = jnp.sum(mv_part(wmA_v[0, 0:D // 2, 128:256], 0, None), axis=0, keepdims=True)
                elif it[0] == 'e':
                    exch_groups([(0, int(it[1]), rg) for rg in range(8)])
                elif it[0] == 'p':
                    b_, i_ = it[1:].split(':')
                    ln_piece(int(b_), int(i_))
                elif it[0] == 't':
                    x_v[pl.ds(zp3 + S // 2 + HALO // 2, 8), 0:128] = pltpu.bitcast(st['res'][0:8, 0:128], u32)
                elif it[0] in 'sg':
                    blks, sd = it[1:].split(':')
                    b0, nb = int(blks[0], 16), len(blks)
                    st['res'] = subdot(h0_lhs(b0, nb, it[0] == 'g'), b0 * 128, 0, int(sd), True)
                elif it[0] == 'u':
                    blks, parts = it[1:].split(':')
                    b0, nb = int(blks[0], 16), len(blks)
                    lhs = h0_lhs(b0, nb, False)
                    for p in parts:
                        subdot(lhs, b0 * 128, 0, 2 * int(p), True)
                        st['res'] = subdot(lhs, b0 * 128, 0, 2 * int(p) + 1, True)

        if 'P' not in skip:
            prologue()

        def attention(qb, kb, vb, base, off, M, mask_rows, baseh=None):
            row0 = base + off

            def kvds(r, w):
                return pl.ds(base + (off + HALO + r - DIL * w), RB)

            o_rows = []
            for r in range(0, M, RB):
                q = [qb[j, pl.ds(base + (off + r), RB), :] for j in range(NCH)]
                s = []
                for w in range(W):
                    acc = None
                    for j in range(NCH):
                        p = q[j] * kb[j, kvds(r, w), :]
                        acc = p if acc is None else acc + p
                    acc = _group4_sum(acc)
                    if mask_rows and off + r < DIL * (W - 1) and w > 0:
                        rows = row0 + r + lax.broadcasted_iota(jnp.int32, (RB, 128), 0)
                        acc = jnp.where(rows >= DIL * w, acc, -1e30)
                    s.append(acc)
                m = functools.reduce(jnp.maximum, s)
                e = [jnp.exp((sw - m) * SCALE) for sw in s]
                den = functools.reduce(lambda a, b: a + b, e)
                rinv = 1.0 / den
                oc = []
                for j in range(NCH):
                    acc = None
                    for w in range(W):
                        p = e[w] * vb[j, kvds(r, w), :]
                        acc = p if acc is None else acc + p
                    oc.append(acc * rinv)
                o_rows.append(jnp.concatenate(oc, axis=1))
            o = jnp.concatenate(o_rows, axis=0).astype(bf16)
            if isinstance(row0, int):
                o_scr[row0 // 2:(row0 + M) // 2, :] = pltpu.bitcast(o, u32)
            elif baseh is not None:
                o_scr[pl.ds(baseh + off // 2, M // 2), :] = pltpu.bitcast(o, u32)
            else:
                o_scr[pl.ds(pl.multiple_of(row0 // 2, 8), M // 2), :] = pltpu.bitcast(o, u32)


        def attention2(off, M, G, base=None, baseh=None):
            o_rows = []

            def rs_(a):
                return slice(a, a + RB) if base is None else pl.ds(base + a, RB)

            for r0 in range(0, M, RB * G):
                rs = [off + r0 + g * RB for g in range(G) if r0 + g * RB < M]
                lane = lax.broadcasted_iota(jnp.int32, (RB, 128), 1)
                S_ = {}
                for r in rs:
                    q = [qbuf[j, rs_(r), :] for j in range(NCH)]
                    for w in range(W):
                        acc = None
                        for j in range(NCH):
                            k0 = HALO + r - DIL * w
                            p = q[j] * kbuf[j, rs_(k0), :]
                            acc = p if acc is None else acc + p
                        S_[r, w] = acc
                keys = list(S_)
                for sh in (1, 2):
                    R = {k: (pltpu.roll(S_[k], sh, 1), pltpu.roll(S_[k], 128 - sh, 1)) for k in keys}
                    for k in keys:
                        S_[k] = S_[k] + jnp.where((lane & sh) != 0, R[k][0], R[k][1])
                for r in rs:
                    s = []
                    for w in range(W):
                        acc = S_[r, w]
                        if base is None and r < DIL * (W - 1) and w > 0:
                            rows = r + lax.broadcasted_iota(jnp.int32, (RB, 128), 0)
                            acc = jnp.where(rows >= DIL * w, acc, -1e30)
                        s.append(acc)
                    m = functools.reduce(jnp.maximum, s)
                    e = [jnp.exp((sw - m) * SCALE) for sw in s]
                    den = functools.reduce(lambda a, b: a + b, e)
                    rinv = 1.0 / den
                    oc = []
                    for j in range(NCH):
                        acc = None
                        for w in range(W):
                            k0 = HALO + r - DIL * w
                            p = e[w] * vbuf[j, rs_(k0), :]
                            acc = p if acc is None else acc + p
                        oc.append(acc * rinv)
                    o_rows.append(jnp.concatenate(oc, axis=1))
            o = jnp.concatenate(o_rows, axis=0).astype(bf16)
            if base is None:
                o_scr[off // 2:(off + M) // 2, :] = pltpu.bitcast(o, u32)
            else:
                o_scr[pl.ds(baseh + off // 2, M // 2), :] = pltpu.bitcast(o, u32)
            return o

        class Att:
            def __init__(self, base, baseh, off, M, wgs, PD, ztok, QD=None, mask=False):
                self.base, self.baseh, self.off, self.PD, self.ztok = base, baseh, off, PD, ztok
                self.QD, self.mask = QD, mask
                self.nrb = M // RB
                self.wgs = list(wgs)
                assert sum(self.wgs) == self.nrb * W
                self.Q, self.SS, self.E, self.OC = {}, {}, {}, {}
                self.win = 0
                self.done = 0

            def scores(self, wl):
                lane = lax.broadcasted_iota(jnp.int32, (RB, 128), 1)
                accs = []
                for (rb, w) in wl:
                    r = self.off + rb * RB
                    if rb not in self.Q:
                        if self.QD is not None and rb * W - self.QD >= 0:
                            qbuf[0, pl.ds(self.ztok + S + HALO, 8), :] = self.SS[divmod(rb * W - self.QD, W)]
                        self.Q[rb] = [qbuf[j, pl.ds(self.base + r, RB), :] for j in range(NCH)]
                    acc = None
                    for j in range(NCH):
                        p = self.Q[rb][j] * kbuf[j, pl.ds(self.base + (HALO + r - DIL * w), RB), :]
                        acc = p if acc is None else acc + p
                    accs.append(acc)
                for sh in (1, 2):
                    R = [(pltpu.roll(a, sh, 1), pltpu.roll(a, 128 - sh, 1)) for a in accs]
                    accs = [a + jnp.where((lane & sh) != 0, x, y) for a, (x, y) in zip(accs, R)]
                for k, a in zip(wl, accs):
                    r = self.off + k[0] * RB
                    if self.mask and r < DIL * (W - 1) and k[1] > 0:
                        rows = r + lax.broadcasted_iota(jnp.int32, (RB, 128), 0)
                        a = jnp.where(rows >= DIL * k[1], a, -1e30)
                    self.SS[k] = a
                    if k[1] == W - 1:
                        self.softmax(k[0])

            def softmax(self, rb):
                s = [self.SS[rb, w] for w in range(W)]
                m = functools.reduce(jnp.maximum, s)
                e = [jnp.exp((sw - m) * SCALE) for sw in s]
                den = functools.reduce(lambda a, b: a + b, e)
                self.E[rb] = (e, 1.0 / den)

            def pv(self):
                rb, j = divmod(self.done, NCH)
                self.done += 1
                r = self.off + rb * RB
                e, rinv = self.E[rb]
                acc = None
                for w in range(W):
                    p = e[w] * vbuf[j, pl.ds(self.base + (HALO + r - DIL * w), RB), :]
                    acc = p if acc is None else acc + p
                self.OC[rb, j] = acc * rinv
                if rb % 2 == 1 and j == NCH - 1:
                    o = jnp.concatenate([jnp.concatenate([self.OC[q, c] for c in range(NCH)], axis=1) for q in (rb - 1, rb)], axis=0)
                    o_scr[pl.ds(self.baseh + (self.off + (rb - 1) * RB) // 2, RB), :] = pltpu.bitcast(o.astype(bf16), u32)

            def token(self, v):
                vbuf[0, pl.ds(self.ztok + S + 2 * HALO, 8), :] = v

            def steps(self, n):
                for _ in range(n):
                    if not self.wgs:
                        return
                    g = self.wgs.pop(0)
                    wl = [divmod(self.win + t, W) for t in range(g)]
                    self.win += g
                    self.scores(wl)
                    tok = False
                    while self.done < self.nrb * NCH and self.done + W + self.PD <= self.win - 1 and self.done // NCH in self.E:
                        if not tok:
                            self.token(self.SS[wl[-1]])
                            tok = True
                        self.pv()

            def rest(self, n=999):
                while self.done < self.nrb * NCH and n > 0:
                    self.pv(); n -= 1

        sub = lax.broadcasted_iota(jnp.int32, (8, 128), 0)

        def pW(p, q, z):
            for tv in range(8 * q, 8 * q + 8):
                j = tv >> 3
                hh = (tv >> 1) & 3
                a2 = tv & 1
                parts = []
                for al in range(4):
                    a = a2 * 4 + al
                    src = a * 64 + hh * 16 + j * 2
                    st = src - 2 * al + 8
                    if isinstance(z, int):
                        parts.append(wo_raw[p, z + st:z + st + 8, :])
                    else:
                        parts.append(wo_raw[p, pl.ds(z + st, 8), :])
                v = jnp.where(sub < 2, parts[0], parts[1])
                v2 = jnp.where(sub < 6, parts[2], parts[3])
                wo_v[p, 8 * tv:8 * tv + 8, :] = jnp.where(sub < 4, v, v2)

        def pM(t, kq, z, macc, key):
            n = D // 2 // KQ
            rows = pl.ds(z + kq * n, n)
            macc[key] = mv_part(wmB_v[t, rows, :], kq * n, macc.get(key))
            if kq == KQ - 1:
                modB[t, 0:1, :] = jnp.sum(macc[key], axis=0, keepdims=True)

        FH, DH2, HM = F // 2, D // 2, T // 2

        def bsums(W, NH, rl, rs_, n, c0, cw):
            w = {(a, b): W[a, pl.ds(rl, n), b * NH + c0:b * NH + c0 + cw] for a in range(2) for b in range(2)}
            res = {}
            for h in range(2):
                e = {k: pltpu.unpack_elementwise(v, index=h, packed_dtype=bf16, unpacked_dtype=f32) for k, v in w.items()}
                b11, b12, b21, b22 = e[0, 0], e[0, 1], e[1, 0], e[1, 1]
                for k, o in (((2, 0), b11 + b22), ((0, 1), b12 - b22), ((1, 0), b21 - b11), ((2, 1), b11 + b12), ((3, 0), b21 + b22)):
                    res.setdefault(k, []).append(o)
            for (a, b), o in res.items():
                W[a, pl.ds(rs_, n), b * NH + c0:b * NH + c0 + cw] = pltpu.bitcast(pltpu.pack_elementwise(o, packed_dtype=bf16), u32)

        def pS(k, r, za, zb_, tok=None):
            links = []
            if k < N3 // 8:
                r0 = jnp.where(r >= P0R, (r - P0R) * N3 + 8 * k, D // 4)
                for c in range(0, FH // 128, LK3):
                    links.append(functools.partial(bsums, w3_v, FH, pl.multiple_of(r0 + za, 8), pl.multiple_of(r0 + zb_, 8), 8, c * 128, LK3 * 128))
            else:
                k -= N3 // 8
                r0 = jnp.where(r >= P0R, (r - P0R) * N4 + 32 * k, F // 4)
                for t in range(4):
                    for c in range(0, DH2 // 128, LK4):
                        links.append(functools.partial(bsums, w4_v, DH2, pl.multiple_of(r0 + 8 * t + za, 8), pl.multiple_of(r0 + 8 * t + zb_, 8), 8, c * 128, LK4 * 128))
            for n, l in enumerate(links):
                if tok is not None:
                    tok(n, len(links))
                l()

        def region_waits(r):
            c_sa(r).wait(); c_ca(r).wait(); c_wq(r).wait()
            if not WS:
                c_wo(r - 1).wait()

            @pl.when(r >= 2)
            def _():
                if WS:
                    c_wo(r - 2).wait()
                for i in range(NM):
                    c_mb(NM * (r - 2) + i, r - 2).wait()

            @pl.when(r >= P0R)
            def _():
                for c in c_p(r - P0R):
                    c.wait()

        if 'prewait' in dbg:
            for r in range(1, 8):
                region_waits(r)

        def region(r, carry):
            if 'prewait' not in dbg and 'nodma2' not in dbg:
                region_waits(r)
            z1 = pl.multiple_of((r >> 8) * 8, 8)
            z2 = pl.multiple_of((r >> 9) * 8, 8)
            pm = [jnp.where(r >= 2, NM * (r - 2) + i, 32) for i in range(NM)]
            pw = jnp.where(r >= 2, r - 2, NCH) if WS else r - 1
            hp = _bf(hP[...])
            st = {'acc': [None, None], 'res': None}
            macc_ = {}

            def mvp(kq):
                n = D // 2 // KQ0
                for q in range(2):
                    st['acc'][q] = mv_part(wmA_v[r, pl.ds(z2 + kq * n, n), q * 128:(q + 1) * 128], kq * n, st['acc'][q])
                if kq == KQ0 - 1:
                    st['sa'] = jnp.sum(st['acc'][0], axis=0, keepdims=True)
                    st['ca'] = jnp.sum(st['acc'][1], axis=0, keepdims=True)
                    modA[r, 0:1, 0:128] = st['sa']
                    modA[r, 0:1, 128:256] = st['ca']

            def hpass(p):
                if MU:
                    x = _bf(x_v[p * PR // 2:(p + 1) * PR // 2, lane_ds(r, 128)]).astype(f32)
                    xh = (x - xhat[0, p * PR:(p + 1) * PR, :]) * xhat[1, p * PR:(p + 1) * PR, :]
                else:
                    xh = xhat[r, p * PR:(p + 1) * PR, :]
                st['h'] = (xh * (1.0 + st['ca']) + st['sa']).astype(bf16)
                st['row'] = p * PR
                if p == NP - 1:
                    hP[...] = pltpu.bitcast(st['h'], u32)

            def do_side(tag):
                prev, st['prev'] = st.get('prev'), st['res']
                jobs = side.get(tag, ())
                if not jobs:
                    return
                tkr = lambda row: pltpu.bitcast(st['res'][row:row + 8, 0:128], u32)
                sj = [int(j[1:]) for j in jobs if j[0] == 'S']
                def sjobs():
                    if TKS >= 0 and (SK is None or any(k in SK for k in sj)):
                        tks = pltpu.bitcast((st['res'] if SL else prev)[TKS:TKS + 8, 0:128], u32)
                        if any(k < N3 // 8 for k in sj):
                            w3_v[0, pl.ds(z1 + D // 4, 8), 0:128] = tks
                        if any(k >= N3 // 8 for k in sj):
                            w4_v[0, pl.ds(z1 + F // 4, 8), 0:128] = tks
                    def tok(k, n, nl):
                        if n == 0 or n % TG:
                            return
                        row = min(TKS + (n * TD // nl) // 8 * 8, PR - 8)
                        src = (st['res'] if SL else prev)
                        if row >= PR - 8 or (TKS + n * TD // nl) >= PR:
                            src = st['res']; row = ((TKS + n * TD // nl) - PR) // 8 * 8 if (TKS + n * TD // nl) >= PR else row
                        tv = pltpu.bitcast(src[row:row + 8, 0:128], u32)
                        if k < N3 // 8:
                            w3_v[0, pl.ds(z1 + D // 4, 8), 0:128] = tv
                        else:
                            w4_v[0, pl.ds(z1 + F // 4, 8), 0:128] = tv
                    for k in sj:
                        pS(k, r, z1, z1 if NC else z2, functools.partial(tok, k) if TG else None)
                if sj and not SL:
                    sjobs()
                tk = tkr(0)
                kinds = set(j[0] for j in jobs)
                if 'W' in kinds:
                    wo_raw[pw, pl.ds(z1 + D // 2 + 16, 8), :] = tkr(TKW)
                if 'M' in kinds:
                    wmB_v[32, pl.ds(z1 + D // 2, 8), :] = tkr(TKM)
                if 'A' in kinds:
                    qbuf[0, pl.ds(z1 + S + HALO, 8), :] = pltpu.bitcast(tk, f32)
                for j in jobs:
                    k = int(j[1:])
                    if j[0] == 'W':
                        pW(pw, k, z2)
                    elif j[0] == 'w':
                        pW(pw, k, 0)
                    elif j[0] == 'M':
                        pM(pm[k // KQ], k % KQ, z2, macc_, k // KQ)
                    elif j[0] in 'Aa':
                        attention(qbuf, kbuf, vbuf, 0, k * AP, AP, True)
                if sj and SL:
                    sjobs()

            for it in order0:
                if it[0] == 'T':
                    st['res'] = subdot(hp, TL, r - 1, int(it[1]), valid=r >= 2)
                    do_side(it)
                elif it[0] == 'H':
                    st['res'] = subdot(st['h'], st['row'], r, int(it[1]))
                    do_side('0' + it)
                elif it[0] == 'm':
                    mvp(int(it[1]))
                elif it[0] == 'K':
                    q = int(it[1:] or 0) * 128
                    wmA_v[r, pl.ds(z1 + D // 2, 8), 0:128] = pltpu.bitcast(st['res'][q:q + 8, 0:128], u32)
                elif it[0] == 'X':
                    q = int(it[1:] or 0) * 128
                    wqkv_raw[pl.ds(z1 + D // 2, 8), 0:128] = pltpu.bitcast(st['res'][q:q + 8, 0:128], u32)
                elif it[0] == 'h':
                    hpass(int(it[1]))
                elif it[0] == 'y':
                    b, qf = int(it[1]), int(it[2])
                    exch_groups([(r, b, rg) for rg in range(2 * qf, 2 * qf + 2)])
                elif it[0] == 'x':
                    b, hf = int(it[1]), int(it[2])
                    exch_groups([(r, b, rg) for rg in range(4 * hf, 4 * hf + 4)])
            for p in range(1, NP):
                hpass(p)
                for sd in range(6 if p < NP - 1 else 6 - NDEF):
                    st['res'] = subdot(st['h'], st['row'], r, sd)
                    do_side('%dH%d' % (p, sd))
            zsm[0] = r >> 8
            zsm[1] = r >> 9
            return carry

        if upto >= 2:
            if 'R' not in skip:
                lax.fori_loop(1, NR, region, 0)
            zero = zsm[0]
            zero2 = zsm[1]

        if WS and upto >= 2:
            c_wo(6).wait()
        if upto >= 3:
            c_wo(7).wait()
            for t in range(6 * NM, 32):
                c_mb(t, 6).wait()
            for c in c_w:
                c.wait()

        def rows_u32(ref, row0, M):
            if isinstance(row0, int):
                return _bf(ref[row0 // 2:(row0 + M) // 2, :])
            if isinstance(row0, tuple):
                return _bf(ref[pl.ds(row0[0] + row0[1] // 2, M // 2), :])
            return _bf(ref[pl.ds(pl.multiple_of(row0 // 2, 8), M // 2), :])

        def wo_dot(row0, M):
            o = rows_u32(o_scr, row0, M)
            return jnp.concatenate([_dot(o, _bf(wo_v[n])) for n in range(NCH)], axis=1)

        def row(k):
            return jnp.concatenate([modB[8 * (k - 2) + j, 0:1, :] for j in range(NCH)], axis=1)

        def ln23(row0, M, A):
            ga = row(2); sb = row(3); cb = row(4)
            x = rows_u32(x_v, row0, M).astype(f32)
            xm = x + ga * A
            hB = _ln(xm) * (1.0 + cb) + sb
            n3 = _ln(hB).astype(bf16)
            return xm, hB, n3

        shifts = [-1, -1, 1, 1, -2, -2, 2, 2]

        def g_val():
            return jnp.concatenate(
                [h1buf[j, HALO + shifts[j]:HALO + shifts[j] + T, :] for j in range(NCH)], axis=1).astype(bf16)

        def out_copy(r0, n, k, c0=0, cw=D):
            if cw == D:
                return pltpu.make_async_copy(obuf.at[pl.ds(r0, n)], o_hbm.bitcast(u32).at[pl.ds(r0, n)], osems.at[k])
            return pltpu.make_async_copy(obuf.at[pl.ds(r0, n), c0:c0 + cw], o_hbm.bitcast(u32).at[pl.ds(r0, n), c0:c0 + cw], osems.at[k])

        def ln4(hs):
            gb = row(5)
            x1 = hb[0:T, :] + hs
            base = xmid[0:T, :] + gb * x1
            n4 = _ln(x1).astype(bf16)
            return base, n4

        def asums(a11, a12, a21, a22):
            return [a11 + a22, a21 + a22, a11, a22, a11 + a12, a21 - a11, a12 - a22]

        SLOT = {0: (2, 0), 1: (0, 0), 2: (0, 1), 3: (1, 0), 4: (1, 1), 5: (2, 1), 6: (3, 0)}

        def w3op(k, c0, cw):
            a, b = SLOT[k]
            c0 = c0 + b * FH
            return _bf(w3_v[a, 0:D // 4, pl.ds(c0, cw) if not isinstance(c0, int) else slice(c0, c0 + cw)])

        def w4op(k, c0, cw, r0=0, nr=F // 4):
            a, b = SLOT[k]
            return _bf(w4_v[a, pl.ds(r0, nr) if not isinstance(r0, int) else slice(r0, r0 + nr), b * DH2 + c0:b * DH2 + c0 + cw])

        def strass(dotk, hook=None):
            M = dotk(0); c11 = M; c22 = M
            if hook: hook(0, M)
            M = dotk(1); c21 = M; c22 = c22 - M
            if hook: hook(1, M)
            M = dotk(2); c12 = M; c22 = c22 + M
            if hook: hook(2, M)
            M = dotk(3); c11 = c11 + M; c21 = c21 + M
            if hook: hook(3, M)
            M = dotk(4); c11 = c11 - M; c12 = c12 + M
            if hook: hook(4, M)
            M = dotk(5); c22 = c22 + M
            if hook: hook(5, M)
            M = dotk(6); c11 = c11 + M
            if hook: hook(6, M)
            return c11, c12, c21, c22

        def n4_sums(r, n4v):
            q = T // RP0 // 2
            if r < q:
                n4f[r * RP0:(r + 1) * RP0, :] = n4v
            else:
                top = n4f[(r - q) * RP0:(r - q + 1) * RP0, :]
                A = asums(top[:, :DH2], top[:, DH2:], n4v[:, :DH2], n4v[:, DH2:])
                for k in range(7):
                    a4[k, (r - q) * RP0:(r - q + 1) * RP0, :] = A[k].astype(bf16)

        def stage3(c0, cw, uc0, hook=None):
            U = strass(lambda k: _dot(a4[k], w3op(k, c0, cw)), hook)
            A = asums(*[_gelu(x) for x in U])
            for k in range(7):
                ua[k, :, uc0:uc0 + cw] = A[k].astype(bf16)

        RP0 = 16

        def bfirst():
            for j in range(NCH):
                h1buf[j, 0:HALO, :] = jnp.zeros((HALO, 128), f32)
            h7 = _bf(hP[...])
            zb = pl.multiple_of(zero * 8, 8) if ZB else 0
            h0 = (T + HALO) // 2 // 16 * 16 + (16 if T == 128 else 0)
            halves = [(0, h0), (h0, T + HALO - h0)]
            nA = (2 * T + HALO - AT0) // AP
            st = {'res': None, 'As': [], 'n3': [], 'h1': [], 'macc': {}}

            def att(k):
                if AG:
                    st['o'] = attention2(AT0 + k * AP, AP, AG)
                else:
                    attention(qbuf, kbuf, vbuf, 0, AT0 + k * AP, AP, True)

            def tok_q(cc=0):
                qbuf[0, pl.ds(zb + S + HALO, 8), :] = st['res'][0:8, cc * 128:(cc + 1) * 128]

            batt = None
            if 'A' in BA:
                batt = Att(0, 0, 0, 2 * T + HALO, [BWG] * ((2 * T + HALO) // RB * W // BWG), BPD, zb, BQD, True)
            for it in BA.split():
                k = int(it[1:]) if len(it) > 1 and it[1:].isdigit() else None
                if not ZB and it[0] in 'tWM':
                    continue
                if it[0] == 'A':
                    batt.steps(k)
                elif it[0] == 'R':
                    batt.steps(999)
                    batt.rest()
                elif it[0] == 'T':
                    st['res'] = subdot(h7, TL, 7, k)
                elif it[0] == 'a':
                    att(k)
                elif it[0] == 't':
                    tok_q(k or 0)
                elif it[0] == 'w':
                    pW(7, k, zb)
                elif it[0] == 'v':
                    pW(6, k, zb)
                elif it[0] == 'm':
                    for kq in range(KQ):
                        pM(6 * NM + k, kq, zb, st['macc'], k)
                elif it[0] == 'M':
                    wmB_v[32, pl.ds(zb + D // 2, 8), :] = pltpu.bitcast(st['res'][0:8, 0:128], u32)
                elif it[0] == 'W':
                    wo_raw[7, pl.ds(zb + D // 2 + 16, 8), :] = pltpu.bitcast(st['res'][0:8, 0:128], u32)
                elif it[0] == 'o':
                    assert batt is None or batt.done >= (halves[k][0] + halves[k][1]) // RB * NCH, batt.done
                    st['res'] = wo_dot(*halves[k])
                    st['As'].append(st['res'])
                elif it[0] == 'l':
                    r0, m = halves[k]
                    xm, hB, n3 = ln23(r0, m, st['As'][k])
                    xmid[r0:r0 + m, :] = xm
                    hb[r0:r0 + m, :] = hB
                    st['n3'].append(n3)
                elif it[0] == 'u':
                    r0, m = halves[k]
                    st['res'] = _dot(st['n3'][k], _bf(w1_v[...]))
                    h1 = _gelu(st['res'])
                    for j in range(NCH):
                        h1buf[j, HALO + r0:HALO + r0 + m, :] = h1[:, j * 128:(j + 1) * 128]
                elif it[0] == 'z':
                    if 'g' not in st:
                        st['g'] = g_val()
                    cw_ = D // NZ
                    st['res'] = _dot(st['g'], _bf(w2_v[:, k * cw_:(k + 1) * cw_]))
                    hsbuf[0:T, k * cw_:(k + 1) * cw_] = st['res']
                elif it[0] == 'U':
                    hh, pp = divmod(k, 10)
                    r0, m = halves[hh]
                    cw_ = D // NU
                    st['res'] = _dot(st['n3'][hh], _bf(w1_v[:, pp * cw_:(pp + 1) * cw_]))
                    h1 = _gelu(st['res'])
                    for j in range(cw_ // 128):
                        h1buf[pp * (cw_ // 128) + j, HALO + r0:HALO + r0 + m, :] = h1[:, j * 128:(j + 1) * 128]
            if 'g' not in st:
                hsbuf[0:T, :] = _dot(g_val(), _bf(w2_v[...]))

        if upto >= 3 and 'F' not in skip:
            bfirst()

        def carries(xm, hB, h1, notlast):
            xmid[0:HALO, :] = xmid[T:T + HALO, :]
            hb[0:HALO, :] = hb[T:T + HALO, :]
            for j in range(NCH):
                h1buf[j, 0:2 * HALO, :] = h1buf[j, T:T + 2 * HALO, :]
            xmid[HALO:HALO + T, :] = xm
            hb[HALO:HALO + T, :] = hB
            for j in range(NCH):
                h1j = h1[:, j * 128:(j + 1) * 128]
                h1buf[j, 2 * HALO:HALO + T, :] = h1j[0:T - HALO]
                h1buf[j, HALO + T:2 * HALO + T, :] = jnp.where(notlast, h1j[T - HALO:T], 0.0)

        RP = 16

        def bbody(i, carry):
            static = isinstance(i, int)
            if static:
                row0h = i * (T // 2)
                abase = (i + 1) * T
                abaseh = (i + 1) * (T // 2)
                z1 = pl.multiple_of(zero * 8, 8)
                z2 = pl.multiple_of(zero2 * 8, 8)
            else:
                row0h = pl.multiple_of(i * (T // 2), T // 2)
                nxt = jnp.minimum(i + 1, NT - 1)
                abase = pl.multiple_of(nxt * T, T)
                abaseh = pl.multiple_of(nxt * (T // 2), T // 2)
                z1 = pl.multiple_of((i >> 8) * 8, 8)
                z2 = pl.multiple_of((i >> 9) * 8, 8)
            ga = row(2); sb = row(3); cb = row(4); gb = row(5)
            bases, n4p, xms, hBs, n3p, As = [], [], [], [], [], []
            att = None
            asch = {}
            if AB == 9:
                att = Att(abase, abaseh, HALO, T, [int(t) for t in WGS], PD, z1)
                for t in ASCH.split():
                    k_, v_ = t.split(':')
                    asch[k_] = int(v_)

            def astep(tag):
                if att is not None and tag in asch:
                    att.steps(asch[tag])

            def p4(r):
                r0 = r * RP
                x1 = hb[r0:r0 + RP, :] + hsbuf[pl.ds(z2 + r0, RP), :]
                if ST:
                    bases.append((r, xmid[r0:r0 + RP, :] + gb * x1))
                    n4_sums(r, _ln(x1))
                    n4p.append(None)
                    return
                bases.append(xmid[r0:r0 + RP, :] + gb * x1)
                n4v = _ln(x1).astype(bf16)
                if EX4:
                    n4b[r0 // 2:(r0 + RP) // 2, :] = pltpu.bitcast(n4v, u32)
                n4p.append(n4v)

            def p23(r, A):
                r0 = r * RP
                x = rows_u32(x_v, (row0h, HALO + r0), RP).astype(f32)
                xm = x + ga * A[r0:r0 + RP]
                hB = _ln(xm) * (1.0 + cb) + sb
                xms.append(xm); hBs.append(hB)
                n3v = _ln(hB).astype(bf16)
                if EX3:
                    n3b[r0 // 2:(r0 + RP) // 2, :] = pltpu.bitcast(n3v, u32)
                n3p.append(n3v)

            ord4 = list(ORD4) if ST else list(range(T // RP))
            for r in range(T // RP):
                if rel4[r] < 0:
                    p4(ord4[r])
            o = rows_u32(o_scr, (row0h, HALO), T)
            for n in range(NCH):
                An = _dot(o, _bf(wo_v[n]))
                As.append(An)
                r4 = [r for r in range(T // RP) if rel4[r] == n]
                if r4:
                    hsbuf[pl.ds(z1 + T, 8), 0:128] = An[0:8, 0:128]
                for r in r4:
                    p4(ord4[r])
                astep('o%d' % n)
            A = jnp.concatenate(As, axis=1)
            if ST:
                base = jnp.concatenate([b for _, b in sorted(bases, key=lambda t: t[0])], axis=0)
                for c in range(FH // CW3):
                    def hook(k, M, c=c):
                        r23 = [r for r in range(T // RP) if R23[r] == 7 * c + k]
                        if r23:
                            x_v[pl.ds(z1 + S // 2 + HALO // 2, 8), 0:128] = pltpu.bitcast(M[0:8, 0:128], u32)
                        for r in r23:
                            p23(r, A)
                    stage3(c * CW3, CW3, c * CW3, hook)
            else:
                base = jnp.concatenate(bases, axis=0)
                n4 = _bf(n4b[...]) if EX4 else jnp.concatenate(n4p, axis=0)
                U = _dot(n4, _bf(w3_v[...]))
                u = _gelu(U).astype(bf16)
            for c in range(0 if ST else F // 128):
                r23 = [r for r in range(T // RP) if rel23[r] == NCH + c]
                if r23 or c in XT:
                    x_v[pl.ds(z1 + S // 2 + HALO // 2, 8), 0:128] = pltpu.bitcast(U[0:8, c * 128:(c + 1) * 128], u32)
                for r in r23:
                    p23(r, A)
                astep('c%d' % c)
            assert len(n3p) == T // RP and len(n4p) == T // RP
            xm = jnp.concatenate(xms, axis=0)
            hB = jnp.concatenate(hBs, axis=0)
            n3 = _bf(n3b[...]) if EX3 else jnp.concatenate(n3p, axis=0)
            h1 = _gelu(_dot(n3, _bf(w1_v[...])))
            carries(xm, hB, h1, i < NT - 1)
            if static:
                if i < NT - 1:
                    attention(qbuf, kbuf, vbuf, abase, HALO, T, False, abaseh)
            elif 'noatt' not in dbg:
                if AB == 9:
                    att.steps(999)
                    att.rest()
                    if DL:
                        h1buf[0, pl.ds(z1 + T + 2 * HALO, 8), :] = att.OC[T // RB - 1, NCH - 1]
                elif AB:
                    attention2(HALO, T, AB, abase, abaseh)
                else:
                    attention(qbuf, kbuf, vbuf, abase, HALO, T, False, abaseh)
            if ST:
                ro = pl.multiple_of((i - 1) * (T // 2), T // 2)
                for c in range(DH2 // CW4):
                    c0 = c * CW4
                    Hs = strass(lambda k: _dot(ua[k], w4op(k, c0, CW4)))
                    for q, Hq in enumerate(Hs):
                        rr, cc = (q // 2) * HM, (q % 2) * DH2 + c0
                        o_ = base[rr:rr + HM, cc:cc + CW4] + gb[:, cc:cc + CW4] * Hq
                        obuf[pl.ds(ro + rr // 2, HM // 2), cc:cc + CW4] = pltpu.bitcast(o_.astype(bf16), u32)
                hsbuf[0:T, :] = _dot(g_val(), _bf(w2_v[...]))
                return carry
            h2 = _dot(u, _bf(w4_v[...]))
            if static:
                obuf[(i - 1) * (T // 2):i * (T // 2), :] = pltpu.bitcast((base + gb * h2).astype(bf16), u32)
            else:
                obuf[pl.ds(pl.multiple_of((i - 1) * (T // 2), T // 2), T // 2), :] = pltpu.bitcast((base + gb * h2).astype(bf16), u32)
            hsbuf[0:T, :] = _dot(g_val(), _bf(w2_v[...]))
            return carry

        if upto >= 4 and 'B' not in skip:
            if UB:
                for i in range(1, 1 + UB):
                    bbody(i, 0)
                    if i in BAR:
                        out_copy_i(i).start()
                if 1 + UB < NT:
                    lax.fori_loop(1 + UB, NT, bbody, 0)
            else:
                lax.fori_loop(1, NT, bbody, 0)

        def blast():
            r0 = (NT - 1) * (T // 2)
            out_copy(0, r0, 0).start()
            if ST:
                gb = row(5)
                for r in ORD4:
                    p0 = r * RP
                    x1 = hb[p0:p0 + RP, :] + hsbuf[p0:p0 + RP, :]
                    baseb[p0:p0 + RP, :] = xmid[p0:p0 + RP, :] + gb * x1
                    n4_sums(r, _ln(x1))

                def fin(q, Hq, c0, cw):
                    rr, cc = (q // 2) * HM, (q % 2) * DH2 + c0
                    o_ = baseb[rr:rr + HM, cc:cc + cw] + gb[:, cc:cc + cw] * Hq
                    obuf[r0 + rr // 2:r0 + rr // 2 + HM // 2, cc:cc + cw] = pltpu.bitcast(o_.astype(bf16), u32)

                if SB == 'F':
                    for c in range(FH // CW3):
                        stage3(c * CW3, CW3, c * CW3)
                    for c in range(DH2 // CW4):
                        Hs = strass(lambda k: _dot(ua[k], w4op(k, c * CW4, CW4)))
                        for q, Hq in enumerate(Hs):
                            fin(q, Hq, c * CW4, CW4)
                else:
                    QF = FH // 2

                    def sbody(m, carry):
                        cb_ = pl.multiple_of(m * QF, 128)
                        for c in range(QF // 128):
                            stage3(cb_ + c * 128, 128, c * 128)
                        rb_ = pl.multiple_of(m * (QF // 2), 32)
                        for c in range(DH2 // CW4):
                            for k in range(7):
                                Mk = _dot(ua[k, :, 0:QF], w4op(k, c * CW4, CW4, rb_, QF // 2))
                                macc[k, :, c * CW4:(c + 1) * CW4] = jnp.where(m > 0, macc[k, :, c * CW4:(c + 1) * CW4], 0.0) + Mk
                        return carry

                    lax.fori_loop(0, 2, sbody, 0)
                    for c in range(DH2 // 128):
                        Hs = strass(lambda k: macc[k, :, c * 128:(c + 1) * 128])
                        for q, Hq in enumerate(Hs):
                            fin(q, Hq, c * 128, 128)
                out_copy(r0, T // 2, 1).start()
                out_copy(0, r0, 0).wait()
                out_copy(r0, T // 2, 1).wait()
                return
            if BL == 'M':
                gb = row(5)

                def l4(p0, zz, dst):
                    x1 = hb[p0:p0 + RP, :] + (hsbuf[pl.ds(zz + p0, RP), :] if zz is not None else hsbuf[p0:p0 + RP, :])
                    baseb[p0:p0 + RP, :] = xmid[p0:p0 + RP, :] + gb * x1
                    q0 = (p0 % HM) // 2
                    dst[q0:q0 + RP // 2, :] = pltpu.bitcast(_ln(x1).astype(bf16), u32)

                for p0 in range(0, HM, RP):
                    l4(p0, None, n4b)

                def mbody(m, carry):
                    zz = pl.multiple_of((m >> 8) * 8, 8)
                    if MA:
                        n4 = _bf(n4b[0:HM // 2, :])
                    else:
                        n4 = _bf(n4b[pl.ds(pl.multiple_of(m * (HM // 2), HM // 2), HM // 2), :])
                    U = _dot(n4, _bf(w3_v[...]))
                    u = _gelu(U).astype(bf16)
                    for k, p0 in enumerate(range(HM, T, RP)):
                        if MT is not None and (k == 0 or MT[k] != MT[k - 1]):
                            hsbuf[pl.ds(zz + T, 8), 0:128] = U[0:8, MT[k] * 128:(MT[k] + 1) * 128]
                        l4(p0, zz if MT is not None else None, n3b if MA else n4b.at[HM // 2:T // 2])
                    if MA:
                        n4b[0:HM // 2, :] = n3b[0:HM // 2, :]
                    ro = pl.multiple_of(r0 + m * (HM // 2), HM // 2)
                    c0 = 0
                    for cw_ in MN:
                        h2 = _dot(u, _bf(w4_v[:, c0:c0 + cw_]))
                        bs = baseb[pl.ds(pl.multiple_of(m * HM, HM), HM), c0:c0 + cw_]
                        obuf[pl.ds(ro, HM // 2), c0:c0 + cw_] = pltpu.bitcast((bs + gb[:, c0:c0 + cw_] * h2).astype(bf16), u32)
                        out_copy(ro, HM // 2, 1, c0, cw_).start()
                        c0 += cw_
                    return carry

                lax.fori_loop(0, 2, mbody, 0)
                out_copy(0, r0, 0).wait()
                for hf in range(2):
                    c0 = 0
                    for cw_ in MN:
                        out_copy(r0 + hf * (HM // 2), HM // 2, 1, c0, cw_).wait()
                        c0 += cw_
                return
            base, n4 = ln4(hsbuf[0:T, :])
            if BL:
                FC = F // BL
                xmid[0:T, :] = base
                n4b[...] = pltpu.bitcast(n4, u32)
                hsbuf[0:T, :] = jnp.zeros((T, D), f32)

                def body(c, carry):
                    w3c = w3_v[:, pl.ds(pl.multiple_of(c * FC, 128), FC)]
                    u = _gelu(_dot(_bf(n4b[...]), _bf(w3c))).astype(bf16)
                    w4c = w4_v[pl.ds(pl.multiple_of(c * (FC // 2), 32), FC // 2), :]
                    hsbuf[0:T, :] += _dot(u, _bf(w4c))
                    return carry

                lax.fori_loop(0, BL, body, 0)
                obuf[r0:r0 + T // 2, :] = pltpu.bitcast((xmid[0:T, :] + row(5) * hsbuf[0:T, :]).astype(bf16), u32)
            else:
                u = _gelu(_dot(n4, _bf(w3_v[...]))).astype(bf16)
                h2 = _dot(u, _bf(w4_v[...]))
                obuf[r0:r0 + T // 2, :] = pltpu.bitcast((base + row(5) * h2).astype(bf16), u32)
            out_copy(r0, T // 2, 1).start()
            out_copy(0, r0, 0).wait()
            out_copy(r0, T // 2, 1).wait()

        if upto >= 5 and 'L' not in skip:
            blast()

    @jax.jit
    def fn(A_x, A_wqkv, A_wo, B_x, B_w1, B_w2, B_w3, B_w4, c, w_mod):
        x = A_x.reshape(S, D)
        any_spec = pl.BlockSpec(memory_space=pl.ANY)
        out = pl.pallas_call(
            kernel,
            in_specs=[any_spec] * 9,
            out_specs=any_spec,
            out_shape=jax.ShapeDtypeStruct((S, D), bf16),
            scratch_shapes=[
                pltpu.VMEM((S // 2 + HALO // 2 + 8, D), u32),
                pltpu.VMEM((D // 2 + 32, 3 * D), u32),
                pltpu.VMEM((64 if SW else D // 2, D), u32),
                pltpu.VMEM((64 if SW else D // 2, D), u32),
                pltpu.VMEM((64 if SW else D // 2, D), u32),
                pltpu.VMEM((NCH + WS, D // 2 + 32, 128), u32),
                pltpu.VMEM((NCH + WS, D // 2, 128), u32),
                pltpu.VMEM((D // 2, D), u32),
                pltpu.VMEM((D // 2, D), u32),
                pltpu.VMEM((4, D // 4 + 8, F), u32),
                pltpu.VMEM((4, F // 4 + 32, D), u32),
                pltpu.VMEM((D // 2, 128), f32),
                pltpu.VMEM((D // 2, 128), f32),
                pltpu.VMEM((8, D // 2 + 16, 256), u32),
                pltpu.VMEM((33, D // 2 + 32, 128), u32),
                pltpu.VMEM((8, 8, 256), f32),
                pltpu.VMEM((36, 8, 128), f32),
                pltpu.VMEM((3 if MU else NCH, S + 32, 128), f32),
                pltpu.VMEM((PR // 2, 128), u32),
                pltpu.VMEM((S // 2, 128), u32),
                pltpu.VMEM((NCH, S + 32, 128), f32),
                pltpu.VMEM((NCH, S + 2 * HALO + 32 * (AB == 9), 128), f32),
                pltpu.VMEM((NCH, S + 2 * HALO + 32 * (AB == 9), 128), f32),
                pltpu.VMEM((T + HALO, D), f32),
                pltpu.VMEM((T + HALO, D), f32),
                pltpu.VMEM((NCH, T + 2 * HALO + 32 * DL, 128), f32),
                pltpu.VMEM((S // 2, D), u32),
                pltpu.VMEM((S // 2 + HALO // 2, D), u32),
                pltpu.VMEM((T + 32, D), f32),
                pltpu.VMEM((T // 2, D), u32),
                pltpu.VMEM((T // 2, D), u32),
                pltpu.VMEM((T, D), f32),
                pltpu.VMEM((T, D), f32),
                pltpu.VMEM((7, T // 2, D // 2), bf16),
                pltpu.VMEM((7, T // 2, F // 2), bf16),
                pltpu.VMEM((7, T // 2, D // 2), f32),
                pltpu.VMEM((1, D), bf16),
            ] + ([pltpu.VMEM((padr, 128), f32)] if padr else []) + [
                pltpu.SMEM((8,), jnp.int32),
            ],
            compiler_params=pltpu.CompilerParams(vmem_limit_bytes=126 * 1024 * 1024),
        )(x, A_wqkv, A_wo, B_w1, B_w2, B_w3, B_w4, c, w_mod)
        return out.reshape(1, S, D)
    return fn


_fn = make()


def pallas_adaLN_cond__sliding_local_dilated__mixer_s_mlp__prompt_kernel(A_x, A_wqkv, A_wo, B_x, B_w1, B_w2, B_w3, B_w4, c, w_mod):
    return _fn(A_x, A_wqkv, A_wo, B_x, B_w1, B_w2, B_w3, B_w4, c, w_mod)
```

```python
import functools
import jax
import jax.numpy as jnp
from jax import lax
import jax.experimental.pallas as pl
import jax.experimental.pallas.tpu as pltpu

S, D, F = 2048, 1024, 3584
H, DH, W, DIL = 32, 32, 8, 2
NCH = D // 128
EPS = 1e-5
SCALE = DH ** -0.5
f32, bf16, u32 = jnp.float32, jnp.bfloat16, jnp.uint32
HALO = 16


def _ln(x):
    m = jnp.mean(x, axis=-1, keepdims=True)
    xc = x - m
    v = jnp.mean(xc * xc, axis=-1, keepdims=True)
    return xc * lax.rsqrt(v + EPS)


def _gelu(x):
    c0 = 0.7978845608028654
    c1 = c0 * 0.044715
    t = jnp.tanh(x * (c0 + c1 * (x * x)))
    hx = 0.5 * x
    return hx + hx * t


def _dot(a, b):
    return jnp.dot(a, b, preferred_element_type=f32)


def _bf(w):
    return pltpu.bitcast(w, bf16)


def _lane_xor(x, s):
    lane = lax.broadcasted_iota(jnp.int32, x.shape, 1)
    return jnp.take_along_axis(x, lane ^ s, axis=1)


def _exchange8_multi(XS):
    XS = [list(X) for X in XS]
    lane = lax.broadcasted_iota(jnp.int32, XS[0][0].shape, 1)
    for t in range(3):
        s = 1 << (t + 2)
        m = (lane & s) != 0
        for X in XS:
            for p in range(8):
                if p & (1 << t):
                    continue
                p2 = p | (1 << t)
                tmp = _lane_xor(jnp.where(m, X[p], X[p2]), s)
                X[p], X[p2] = jnp.where(m, tmp, X[p]), jnp.where(m, X[p2], tmp)
    return XS


def _group4_sum(acc):
    lane = lax.broadcasted_iota(jnp.int32, acc.shape, 1)
    acc = acc + jnp.where((lane & 1) != 0, pltpu.roll(acc, 1, 1), pltpu.roll(acc, 127, 1))
    acc = acc + jnp.where((lane & 2) != 0, pltpu.roll(acc, 2, 1), pltpu.roll(acc, 126, 1))
    return acc


def make(T=128, PR=512, RB=8, EG=4, upto=9, AT0=0, AP=16,
         DO='c X0 Wq sa ca X1 Wk Wv X2 X3 X4 X5 X6 X7 X8 X9 X10 X12 X13 X11 X14 X15',
         PS=None, PSX=None, RL=1, D0='1234', LP=16, BL='M', ZB=1,
         order0='T0 T1 X x00 x01 m0 T2 T3 X x10 x11 h0 T4 T5 X x20 H0 X x21 H1 H2 H3 H4 H5', NDEF=6, BA=None,
         side=None, KQ=4, KQ0=1, NM=5, NR=8, AG=1,
         rel4=(-1, -1, -1, 0, 1, 2, 3, 4), rel23=(8, 9, 10, 11, 12, 13, 14, 15),
         padr=0, dbg='', UB=0, BAR=(), GL=0, MU=1, WS=1, skip='', AB=9, WGS='112'*32, PD=0, ASCH='', DL=0, EX3=1, EX4=1, XT=(), MT=(4, 10, 16, 22), MA=0, MN=(1024,), NZ=8, NU=2, BPD=0, BQD=None, BWG=8,
         ST=1, ORD4=(0, 4, 1, 5, 2, 6, 3, 7), R23=(0, 3, 6, 9, 12, 15, 18, 21), PRE='R', CW3=128, CW4=128, SB='S', SJ=None, P0R=4, S1=1, R3O=(0, 4, 1, 5, 2, 6, 3, 7), GT=None, KD=None, LC=0, SP3=0, AP1=0, AP4=0, AP2=0, TW4=90, TW1=80, TW2=20, AP3=0, AO3=0, AWO=0, EA=1, RL3=1, RL4=0, LK3=1, LK4=1, TKS=0, TKW=0, TKM=0, SW=1, SK=None, SL=1, TG=1, TD=480, NC=1, DR=None):
    HS, HO = (2, 0) if MU else (0, S // 2)
    NT = S // T
    NP = S // PR
    order0 = order0.split()
    TL = S - PR
    if PS is None:
        PS = ('wc C wX0 L0 wWq e0 wsa S wca A h0 wX1 u0:0 L1 wWk u1:0 e1 wWv u0:1 u1:1 e2 wX2 u0:2 u1:2 L2 u2:0 '
              'wX3 wX4 u2:12 L3 u3:012 L4 u4:0 wX5 wX6 wX7 u4:12 L5 u5:012 L6 u6:012 L7 u7:0 '
              'wX8 wX9 wX10 wX12 wX13 u7:12 L8 u8:012 L9 u9:012 L10 ua:0 L12 L13 wX11 wX14 wX15 Da D5 Db D6 Dc D7 Dd DW ua:12 L11 ub:012 L14 L15')
    DR = {2: 'c7dW'} if DR is None else DR
    for v_ in DR.values():
        for g_ in v_:
            assert (' D' + g_ + ' ') in PS
            PS = PS.replace(' D' + g_ + ' ', ' ')
    if BA is None:
        BA = ('a0 a1 T0 T1 t0 a2 a3 W w0 w1 w2 w3 w4 w5 w6 w7 T2 t0 a4 a5 T3 t0 a6 a7 T4 t0 a8 a9 T5 t0 a10 o0 t0 a11 t4 a12 '
              'o1 t0 a13 t4 a14 M m0 m1 l0 l1 u0 t0 a15 t4 a16 u1')
    if WS and 'v0' not in BA:
        BA = BA.replace('W w0 w1 w2 w3 w4 w5 w6 w7', 'W v0 v1 v2 v3 v4 v5 v6 v7 w0 w1 w2 w3 w4 w5 w6 w7')
    if PSX:
        for k_, v_ in PSX.items():
            assert (' ' + k_ + ' ') in PS
            PS = PS.replace(' ' + k_ + ' ', ' ' + k_ + ' ' + v_ + ' ')
    S_C, S_X, S_SA, S_CA, S_W0, S_WQ, S_WO, S_MB, S_W = 0, 1, 17, 25, 33, 36, 44, 52, 60
    S_P = 64
    NSEM = 68
    DEF = list(range(6 - NDEF, 6))
    tags = ['T%d' % sd for sd in DEF] + ['%dH%d' % (p, sd) for p in range(NP) for sd in range(6 if p < NP - 1 else 6 - NDEF)]
    if side is None:
        side = 'W:7,9,11,13,15,17,19,21 M:4,5,6,7,8,9,10,11,12,13,14,15,16,17,18,19,20,21,22,22'
        if PRE == 'R':
            if SJ is None:
                SJ = ','.join(str(t) for t in (range(4, 23) if S1 else range(8, 23)))
            side += ' S:' + SJ
    if isinstance(side, str):
        sd_ = {}
        for grp in side.split():
            kind, lst = grp.split(':')
            for k, t in enumerate(lst.split(',')):
                sd_.setdefault(tags[int(t)], []).append(kind + str(k))
        side = sd_
    assert sum(1 for v in side.values() for j in v if j[0] in 'Aa') * AP == AT0

    def kernel(*refs):
        pl.run_scoped(functools.partial(body, *refs), pltpu.SemaphoreType.DMA((NSEM,)), pltpu.SemaphoreType.DMA((2,)))

    def body(x_hbm, wqkv_hbm, wo_hbm, w1_hbm, w2_hbm, w3_hbm, w4_hbm, c_hbm, wmod_hbm,
             o_hbm,
             x_v, wqkv_raw, wq_v, wk_v, wv_v, wo_raw, wo_v, w1_v, w2_v, w3_v, w4_v, cE, cO, wmA_v, wmB_v,
             modA, modB, xhat, hP, h0, qbuf, kbuf, vbuf, xmid, hb, h1buf, obuf, o_scr, hsbuf, n4b, n3b, baseb, n4f, a4, ua, macc, n3f, a3, a2, abuf, x1buf, c_v, *rest):
        zsm, sems, osems = rest[-3:]

        def cp(src, dst, k):
            return pltpu.make_async_copy(src, dst, sems.at[k])

        xu = x_hbm.bitcast(u32)
        wqkvu = wqkv_hbm.bitcast(u32)
        wou = wo_hbm.bitcast(u32)
        wmodu = wmod_hbm.bitcast(u32)

        def lane_ds(k, n, base=0):
            if isinstance(k, int):
                return pl.ds(base + k * n, n)
            return pl.ds(pl.multiple_of(base + k * n, 128), n)

        def row_ds(base, k, n):
            if isinstance(k, int):
                return pl.ds(base + k * n, n)
            return pl.ds(pl.multiple_of(base + k * n, 8), n)

        c_c = cp(c_hbm, c_v, S_C)

        def c_x(b):
            return cp(xu.at[b * 64:(b + 1) * 64], x_v.at[b * 64:(b + 1) * 64], S_X + b)

        def c_sa(k):
            return cp(wmodu.at[:, lane_ds(k, 128)], wmA_v.at[k, 0:D // 2, 0:128], S_SA + k)

        def c_ca(k):
            return cp(wmodu.at[:, lane_ds(k, 128, D)], wmA_v.at[k, 0:D // 2, 128:256], S_CA + k)

        def c_w0(b):
            return cp(wqkvu.at[0:64, b * D:(b + 1) * D], wqkv_raw.at[0:64, b * D:(b + 1) * D], S_W0 + b)

        def c_wq(k):
            return cp(wqkvu.at[row_ds(0, k, 64)], wqkv_raw.at[row_ds(0, k, 64)], S_WQ + k)

        def c_wo(p):
            return cp(wou.at[:, lane_ds(p, 128)], wo_raw.at[p, 8:8 + D // 2], S_WO + p)

        def c_mb(t, g):
            return cp(wmodu.at[:, lane_ds(t, 128, 2 * D)], wmB_v.at[t, 0:D // 2], S_MB + g)

        w1u, w2u = w1_hbm.bitcast(u32), w2_hbm.bitcast(u32)
        w3u, w4u = w3_hbm.bitcast(u32), w4_hbm.bitcast(u32)
        N3, N4 = D // 4 // 4, F // 4 // 4
        c_w = []

        def c_p(p):
            def rows(base, n):
                if isinstance(p, int):
                    return pl.ds(base + p * n, n)
                return pl.ds(pl.multiple_of(base + p * n, 8), n)
            return ([cp(w3u.at[rows(a * (D // 4), N3)], w3_v.at[a, rows(0, N3)], S_P + p) for a in range(2)]
                    + [cp(w4u.at[rows(a * (F // 4), N4)], w4_v.at[a, rows(0, N4)], S_P + p) for a in range(2)]
                    + [cp(w1u.at[rows(a * (D // 4), N3)], w1_v.at[a, rows(0, N3)], S_P + p) for a in range(2)]
                    + [cp(w2u.at[rows(a * (D // 4), N3)], w2_v.at[a, rows(0, N3)], S_P + p) for a in range(2)])

        def named(nm):
            if nm == 'c':
                return c_c
            if nm == 'sa':
                return c_sa(0)
            if nm == 'ca':
                return c_ca(0)
            if nm[0] == 'W':
                return c_w0('qkv'.index(nm[1]))
            return c_x(int(nm[1:]))

        for nm in DO.split():
            named(nm).start()
        def start_group(g):
            if g == 'W':
                if upto >= 3:
                    c_wo(7).start()
                    for t in range(6 * NM, 32):
                        c_mb(t, 6).start()
                    for c in c_w:
                        c.start()
            elif g in 'abcd':
                for c in c_p('abcd'.index(g)):
                    c.start()
            elif upto >= 2 and 'nodma2' not in dbg:
                r = int(g)
                c_sa(r).start()
                c_ca(r).start()
                c_wq(r).start()
                c_wo(r - 1).start()
                if r >= 2:
                    for i in range(NM):
                        c_mb(NM * (r - 2) + i, r - 2).start()

        for g in D0:
            start_group(g)
        assert sorted(list(D0) + [it[1] for it in PS.split() if it[0] == 'D'] + list(''.join(DR.values()))) == sorted('1234567Wabcd')

        def _zinit(i, carry):
            zsm[2 + i] = i >> 8
            return carry

        lax.fori_loop(0, 3, _zinit, 0)
        zp3 = pl.multiple_of(zsm[4] * 8, 8)
        zp1 = pl.multiple_of(zsm[2] * 8, 8)
        zp2 = pl.multiple_of(zsm[3] * 8, 8)

        x_v[S // 2:S // 2 + HALO // 2, :] = jnp.zeros((HALO // 2, D), u32)
        for j in range(NCH):
            z = jnp.zeros((HALO, 128), f32)
            qbuf[j, S:S + HALO, :] = z
            kbuf[j, HALO + S:2 * HALO + S, :] = z
            vbuf[j, HALO + S:2 * HALO + S, :] = z
            kbuf[j, 0:HALO, :] = z
            vbuf[j, 0:HALO, :] = z
            wo_raw[j, 0:8, :] = jnp.zeros((8, 128), u32)
            wo_raw[j, 8 + D // 2:16 + D // 2, :] = jnp.zeros((8, 128), u32)

        def mv_part(w, r0, acc):
            n = w.shape[0]
            lo = pltpu.bitcast(w << 16, f32)
            hi = pltpu.bitcast(w & jnp.uint32(0xFFFF0000), f32)
            pr = lo * cE[r0:r0 + n, :] + hi * cO[r0:r0 + n, :]
            for t in range(n // 8):
                acc = pr[8 * t:8 * t + 8] if acc is None else acc + pr[8 * t:8 * t + 8]
            return acc

        wparts = (wq_v, wk_v, wv_v)
        bufs = (qbuf, kbuf, vbuf)

        def exch_groups(grps):
            for g0 in range(0, len(grps), EG):
                gs = grps[g0:g0 + EG]
                XS = [[wqkv_raw[row_ds(rg * 8, k * 8, 8), b * D + a * 128:b * D + (a + 1) * 128] for a in range(NCH)]
                      for (k, b, rg) in gs]
                YS = _exchange8_multi(XS)
                for (k, b, rg), Y in zip(gs, YS):
                    wparts[b][row_ds(rg * 8, 0 if SW else k * 8, 8), :] = jnp.concatenate(Y, axis=1)

        def subdot(lhs, row0, kc, sd, init=False, valid=None):
            b, hf = sd // 2, sd % 2
            n = lhs.shape[0]
            res = _dot(lhs, _bf(wparts[b][row_ds(0, 0 if SW else kc, 64), hf * 512:(hf + 1) * 512]))
            o = row0 + (0 if b == 0 else HALO)
            for jj in range(4):
                j = hf * 4 + jj
                if init:
                    bufs[b][j, o:o + n, :] = res[:, jj * 128:(jj + 1) * 128]
                elif valid is not None:
                    bufs[b][j, o:o + n, :] = jnp.where(valid, bufs[b][j, o:o + n, :], 0.0) + res[:, jj * 128:(jj + 1) * 128]
                else:
                    bufs[b][j, o:o + n, :] += res[:, jj * 128:(jj + 1) * 128]
            return res

        def prologue():
            st = {}

            def crep():
                c = c_v[...].astype(f32)
                scf = (c * jax.nn.sigmoid(c)).astype(bf16).astype(f32)
                rr = lax.broadcasted_iota(jnp.int32, (128, 128), 0)
                ll = lax.broadcasted_iota(jnp.int32, (128, 128), 1)
                sel = ll == jnp.where(rr < 64, 2 * rr, 2 * rr - 127)
                for j in range(NCH):
                    dg = jnp.where(sel, jnp.broadcast_to(scf[:, j * 128:(j + 1) * 128], (128, 128)), 0.0).astype(bf16)
                    rep = _dot(dg, jnp.ones((128, 128), bf16))
                    cE[j * 64:(j + 1) * 64, :] = rep[0:64]
                    cO[j * 64:(j + 1) * 64, :] = rep[64:128]

            def h_store(r0, xh0):
                h = (xh0 * (1.0 + st['ca']) + st['sa']).astype(bf16)
                if r0 < TL:
                    xhat[HS, HO + r0 // 2:HO + (r0 + LP) // 2, :] = pltpu.bitcast(h, f32)
                else:
                    hP[(r0 - TL) // 2:(r0 - TL + LP) // 2, :] = pltpu.bitcast(h, u32)

            def h0_lhs(b0, nb, gated):
                r0 = HO + b0 * 64
                if not gated:
                    return _bf(xhat[HS, r0:r0 + nb * 64, :])
                if GL:
                    return jnp.concatenate([_bf(xhat[HS, r0:r0 + nb * 64 - 8, :]), _bf(xhat[HS, pl.ds(zp3 + r0 + nb * 64 - 8, 8), :])], axis=0)
                return jnp.concatenate([_bf(xhat[HS, pl.ds(zp3 + r0, 8), :]), _bf(xhat[HS, r0 + 8:r0 + nb * 64, :])], axis=0)

            def ln_piece(b, i):
                r0 = b * 128 + i * LP
                direct = 'ca' in st and 'sa' in st
                if MU:
                    x = _bf(x_v[pl.ds(zp1 + r0 // 2, LP // 2), :]).astype(f32)
                    m = jnp.mean(x, axis=-1, keepdims=True)
                    if RL:
                        x = _bf(x_v[pl.ds(zp2 + r0 // 2, LP // 2), :]).astype(f32)
                    xc = x - m
                    rs = lax.rsqrt(jnp.mean(xc * xc, axis=-1, keepdims=True) + EPS)
                    xhat[0, r0:r0 + LP, :] = jnp.broadcast_to(m, (LP, 128))
                    xhat[1, r0:r0 + LP, :] = jnp.broadcast_to(rs, (LP, 128))
                    if direct:
                        h_store(r0, xc[:, 0:128] * rs)
                    return
                if RL:
                    m = jnp.mean(_bf(x_v[pl.ds(zp1 + r0 // 2, LP // 2), :]).astype(f32), axis=-1, keepdims=True)
                    xc = _bf(x_v[pl.ds(zp2 + r0 // 2, LP // 2), :]).astype(f32) - m
                    v = jnp.mean(xc * xc, axis=-1, keepdims=True)
                    xh = (_bf(x_v[r0 // 2:(r0 + LP) // 2, :]).astype(f32) - m) * lax.rsqrt(v + EPS)
                else:
                    xh = _ln(_bf(x_v[pl.ds(zp1 + r0 // 2, LP // 2), :]).astype(f32))
                for j in range(1 if direct else 0, NCH):
                    xhat[j, r0:r0 + LP, :] = xh[:, j * 128:(j + 1) * 128]
                if direct:
                    h_store(r0, xh[:, 0:128])

            def ln_block(b):
                for i in range(128 // LP):
                    ln_piece(b, i)

            def hblk(b):
                for i in range(128 // LP):
                    r0 = b * 128 + i * LP
                    if MU:
                        x = _bf(x_v[r0 // 2:(r0 + LP) // 2, 0:128]).astype(f32)
                        h_store(r0, (x - xhat[0, r0:r0 + LP, :]) * xhat[1, r0:r0 + LP, :])
                    else:
                        h_store(r0, xhat[0, r0:r0 + LP, :])

            for it in PS.split():
                if it[0] == 'w':
                    named(it[1:]).wait()
                elif it[0] == 'D':
                    start_group(it[1])
                elif it == 'C':
                    crep()
                elif it[0] == 'L':
                    ln_block(int(it[1:]))
                elif it[0] == 'h':
                    hblk(int(it[1:]))
                elif it == 'S':
                    st['sa'] = jnp.sum(mv_part(wmA_v[0, 0:D // 2, 0:128], 0, None), axis=0, keepdims=True)
                elif it == 'A':
                    st['ca'] = jnp.sum(mv_part(wmA_v[0, 0:D // 2, 128:256], 0, None), axis=0, keepdims=True)
                elif it[0] == 'e':
                    exch_groups([(0, int(it[1]), rg) for rg in range(8)])
                elif it[0] == 'p':
                    b_, i_ = it[1:].split(':')
                    ln_piece(int(b_), int(i_))
                elif it[0] == 't':
                    x_v[pl.ds(zp3 + S // 2 + HALO // 2, 8), 0:128] = pltpu.bitcast(st['res'][0:8, 0:128], u32)
                elif it[0] in 'sg':
                    blks, sd = it[1:].split(':')
                    b0, nb = int(blks[0], 16), len(blks)
                    st['res'] = subdot(h0_lhs(b0, nb, it[0] == 'g'), b0 * 128, 0, int(sd), True)
                elif it[0] == 'u':
                    blks, parts = it[1:].split(':')
                    b0, nb = int(blks[0], 16), len(blks)
                    lhs = h0_lhs(b0, nb, False)
                    for p in parts:
                        subdot(lhs, b0 * 128, 0, 2 * int(p), True)
                        st['res'] = subdot(lhs, b0 * 128, 0, 2 * int(p) + 1, True)

        if 'P' not in skip:
            prologue()

        def attention(qb, kb, vb, base, off, M, mask_rows, baseh=None):
            row0 = base + off

            def kvds(r, w):
                return pl.ds(base + (off + HALO + r - DIL * w), RB)

            o_rows = []
            for r in range(0, M, RB):
                q = [qb[j, pl.ds(base + (off + r), RB), :] for j in range(NCH)]
                s = []
                for w in range(W):
                    acc = None
                    for j in range(NCH):
                        p = q[j] * kb[j, kvds(r, w), :]
                        acc = p if acc is None else acc + p
                    acc = _group4_sum(acc)
                    if mask_rows and off + r < DIL * (W - 1) and w > 0:
                        rows = row0 + r + lax.broadcasted_iota(jnp.int32, (RB, 128), 0)
                        acc = jnp.where(rows >= DIL * w, acc, -1e30)
                    s.append(acc)
                m = functools.reduce(jnp.maximum, s)
                e = [jnp.exp((sw - m) * SCALE) for sw in s]
                den = functools.reduce(lambda a, b: a + b, e)
                rinv = 1.0 / den
                oc = []
                for j in range(NCH):
                    acc = None
                    for w in range(W):
                        p = e[w] * vb[j, kvds(r, w), :]
                        acc = p if acc is None else acc + p
                    oc.append(acc * rinv)
                o_rows.append(jnp.concatenate(oc, axis=1))
            o = jnp.concatenate(o_rows, axis=0).astype(bf16)
            if isinstance(row0, int):
                o_scr[row0 // 2:(row0 + M) // 2, :] = pltpu.bitcast(o, u32)
            elif baseh is not None:
                o_scr[pl.ds(baseh + off // 2, M // 2), :] = pltpu.bitcast(o, u32)
            else:
                o_scr[pl.ds(pl.multiple_of(row0 // 2, 8), M // 2), :] = pltpu.bitcast(o, u32)


        def attention2(off, M, G, base=None, baseh=None):
            o_rows = []

            def rs_(a):
                return slice(a, a + RB) if base is None else pl.ds(base + a, RB)

            for r0 in range(0, M, RB * G):
                rs = [off + r0 + g * RB for g in range(G) if r0 + g * RB < M]
                lane = lax.broadcasted_iota(jnp.int32, (RB, 128), 1)
                S_ = {}
                for r in rs:
                    q = [qbuf[j, rs_(r), :] for j in range(NCH)]
                    for w in range(W):
                        acc = None
                        for j in range(NCH):
                            k0 = HALO + r - DIL * w
                            p = q[j] * kbuf[j, rs_(k0), :]
                            acc = p if acc is None else acc + p
                        S_[r, w] = acc
                keys = list(S_)
                for sh in (1, 2):
                    R = {k: (pltpu.roll(S_[k], sh, 1), pltpu.roll(S_[k], 128 - sh, 1)) for k in keys}
                    for k in keys:
                        S_[k] = S_[k] + jnp.where((lane & sh) != 0, R[k][0], R[k][1])
                for r in rs:
                    s = []
                    for w in range(W):
                        acc = S_[r, w]
                        if base is None and r < DIL * (W - 1) and w > 0:
                            rows = r + lax.broadcasted_iota(jnp.int32, (RB, 128), 0)
                            acc = jnp.where(rows >= DIL * w, acc, -1e30)
                        s.append(acc)
                    m = functools.reduce(jnp.maximum, s)
                    e = [jnp.exp((sw - m) * SCALE) for sw in s]
                    den = functools.reduce(lambda a, b: a + b, e)
                    rinv = 1.0 / den
                    oc = []
                    for j in range(NCH):
                        acc = None
                        for w in range(W):
                            k0 = HALO + r - DIL * w
                            p = e[w] * vbuf[j, rs_(k0), :]
                            acc = p if acc is None else acc + p
                        oc.append(acc * rinv)
                    o_rows.append(jnp.concatenate(oc, axis=1))
            o = jnp.concatenate(o_rows, axis=0).astype(bf16)
            if base is None:
                o_scr[off // 2:(off + M) // 2, :] = pltpu.bitcast(o, u32)
            else:
                o_scr[pl.ds(baseh + off // 2, M // 2), :] = pltpu.bitcast(o, u32)
            return o

        class Att:
            def __init__(self, base, baseh, off, M, wgs, PD, ztok, QD=None, mask=False, KD=None):
                self.base, self.baseh, self.off, self.PD, self.ztok = base, baseh, off, PD, ztok
                self.KD, self.PP = KD, {}
                self.QD, self.mask = QD, mask
                self.nrb = M // RB
                self.wgs = list(wgs)
                assert sum(self.wgs) == self.nrb * W
                self.Q, self.SS, self.E, self.OC = {}, {}, {}, {}
                self.win = 0
                self.done = 0

            def scores(self, wl):
                lane = lax.broadcasted_iota(jnp.int32, (RB, 128), 1)
                accs = []
                if self.KD is not None:
                    n0 = wl[0][0] * W + wl[0][1] - self.KD[1]
                    if n0 >= 0:
                        kbuf[0, pl.ds(self.ztok + S + 2 * HALO, 8), :] = (self.PP if self.KD[0] == 0 else self.SS)[divmod(n0, W)]
                for (rb, w) in wl:
                    r = self.off + rb * RB
                    if rb not in self.Q:
                        if self.QD is not None and rb * W - self.QD >= 0:
                            qbuf[0, pl.ds(self.ztok + S + HALO, 8), :] = self.SS[divmod(rb * W - self.QD, W)]
                        self.Q[rb] = [qbuf[j, pl.ds(self.base + r, RB), :] for j in range(NCH)]
                    acc = None
                    for j in range(NCH):
                        p = self.Q[rb][j] * kbuf[j, pl.ds(self.base + (HALO + r - DIL * w), RB), :]
                        acc = p if acc is None else acc + p
                    accs.append(acc)
                for sh in (1, 2):
                    R = [(pltpu.roll(a, sh, 1), pltpu.roll(a, 128 - sh, 1)) for a in accs]
                    accs = [a + jnp.where((lane & sh) != 0, x, y) for a, (x, y) in zip(accs, R)]
                    if sh == 1:
                        for k, a in zip(wl, accs):
                            self.PP[k] = a
                for k, a in zip(wl, accs):
                    r = self.off + k[0] * RB
                    if self.mask and r < DIL * (W - 1) and k[1] > 0:
                        rows = r + lax.broadcasted_iota(jnp.int32, (RB, 128), 0)
                        a = jnp.where(rows >= DIL * k[1], a, -1e30)
                    self.SS[k] = a
                    if k[1] == W - 1:
                        self.softmax(k[0])

            def softmax(self, rb):
                s = [self.SS[rb, w] for w in range(W)]
                m = functools.reduce(jnp.maximum, s)
                e = [jnp.exp((sw - m) * SCALE) for sw in s]
                den = functools.reduce(lambda a, b: a + b, e)
                self.E[rb] = (e, 1.0 / den)

            def pv(self):
                rb, j = divmod(self.done, NCH)
                self.done += 1
                r = self.off + rb * RB
                e, rinv = self.E[rb]
                acc = None
                for w in range(W):
                    p = e[w] * vbuf[j, pl.ds(self.base + (HALO + r - DIL * w), RB), :]
                    acc = p if acc is None else acc + p
                self.OC[rb, j] = acc * rinv
                if rb % 2 == 1 and j == NCH - 1:
                    o = jnp.concatenate([jnp.concatenate([self.OC[q, c] for c in range(NCH)], axis=1) for q in (rb - 1, rb)], axis=0)
                    o_scr[pl.ds(self.baseh + (self.off + (rb - 1) * RB) // 2, RB), :] = pltpu.bitcast(o.astype(bf16), u32)

            def token(self, v):
                vbuf[0, pl.ds(self.ztok + S + 2 * HALO, 8), :] = v

            def steps(self, n):
                for _ in range(n):
                    if not self.wgs:
                        return
                    g = self.wgs.pop(0)
                    wl = [divmod(self.win + t, W) for t in range(g)]
                    self.win += g
                    self.scores(wl)
                    tok = False
                    while self.done < self.nrb * NCH and self.done + W + self.PD <= self.win - 1 and self.done // NCH in self.E:
                        if not tok:
                            self.token(self.SS[wl[-1]])
                            tok = True
                        self.pv()

            def rest(self, n=999):
                while self.done < self.nrb * NCH and n > 0:
                    self.pv(); n -= 1

        sub = lax.broadcasted_iota(jnp.int32, (8, 128), 0)

        def pW(p, q, z):
            for tv in range(8 * q, 8 * q + 8):
                j = tv >> 3
                hh = (tv >> 1) & 3
                a2 = tv & 1
                parts = []
                for al in range(4):
                    a = a2 * 4 + al
                    src = a * 64 + hh * 16 + j * 2
                    st = src - 2 * al + 8
                    if isinstance(z, int):
                        parts.append(wo_raw[p, z + st:z + st + 8, :])
                    else:
                        parts.append(wo_raw[p, pl.ds(z + st, 8), :])
                v = jnp.where(sub < 2, parts[0], parts[1])
                v2 = jnp.where(sub < 6, parts[2], parts[3])
                wo_v[p, 8 * tv:8 * tv + 8, :] = jnp.where(sub < 4, v, v2)

        def pM(t, kq, z, macc, key):
            n = D // 2 // KQ
            rows = pl.ds(z + kq * n, n)
            macc[key] = mv_part(wmB_v[t, rows, :], kq * n, macc.get(key))
            if kq == KQ - 1:
                modB[t, 0:1, :] = jnp.sum(macc[key], axis=0, keepdims=True)

        FH, DH2, HM = F // 2, D // 2, T // 2
        SLOT = {0: (2, 0), 1: (0, 0), 2: (0, 1), 3: (1, 0), 4: (1, 1), 5: (2, 1), 6: (3, 0)}
        SLOT5 = {0: (2, 0), 1: (0, 0), 2: (3, 1), 3: (4, 0), 4: (1, 1), 5: (2, 1), 6: (3, 0)}

        def bsums(W, NH, rl, rs_, n, c0, cw, five=False):
            w = {(a, b): W[a, pl.ds(rl, n), b * NH + c0:b * NH + c0 + cw] for a in range(2) for b in range(2)}
            res = {}
            for h in range(2):
                e = {k: pltpu.unpack_elementwise(v, index=h, packed_dtype=bf16, unpacked_dtype=f32) for k, v in w.items()}
                b11, b12, b21, b22 = e[0, 0], e[0, 1], e[1, 0], e[1, 1]
                sl = SLOT5 if five else SLOT
                for k, o in ((0, b11 + b22), (2, b12 - b22), (3, b21 - b11), (5, b11 + b12), (6, b21 + b22)):
                    res.setdefault(sl[k], []).append(o)
            for (a, b), o in res.items():
                W[a, pl.ds(rs_, n), b * NH + c0:b * NH + c0 + cw] = pltpu.bitcast(pltpu.pack_elementwise(o, packed_dtype=bf16), u32)

        NS3, NS4 = N3 // 8, N4 // 32

        def s_ref(k):
            return w3_v if k < NS3 else w4_v if k < NS3 + NS4 else w1_v if k < NS3 + NS4 + 2 else w2_v

        def s_links(k, r, z):
            links = []
            W = s_ref(k)
            if k < NS3:
                r0 = jnp.where(r >= P0R, (r - P0R) * N3 + 8 * k, D // 4) + z
                for c in range(FH // 128):
                    links.append(functools.partial(bsums, W, FH, pl.multiple_of(r0, 8), pl.multiple_of(r0, 8), 8, c * 128, 128))
            elif k < NS3 + NS4:
                k -= NS3
                r0 = jnp.where(r >= P0R, (r - P0R) * N4 + 32 * k, F // 4) + z
                for t in range(4):
                    for c in range(DH2 // 128):
                        links.append(functools.partial(bsums, W, DH2, pl.multiple_of(r0 + 8 * t, 8), pl.multiple_of(r0 + 8 * t, 8), 8, c * 128, 128))
            else:
                k = (k - NS3 - NS4) % 2
                r0 = jnp.where(r >= P0R, (r - P0R) * N3 + 32 * k, D // 4) + z
                for t in range(4):
                    for c in range(DH2 // 128):
                        links.append(functools.partial(bsums, W, DH2, pl.multiple_of(r0 + 8 * t, 8), pl.multiple_of(r0 + 8 * t, 8), 8, c * 128, 128, True))
            return links

        def region_waits(r):
            c_sa(r).wait(); c_ca(r).wait(); c_wq(r).wait()
            if not WS:
                c_wo(r - 1).wait()

            @pl.when(r >= 2)
            def _():
                if WS:
                    c_wo(r - 2).wait()
                for i in range(NM):
                    c_mb(NM * (r - 2) + i, r - 2).wait()

            @pl.when(r >= P0R)
            def _():
                for c in c_p(r - P0R):
                    c.wait()

            for r_, gs_ in DR.items():
                @pl.when(r == r_)
                def _(gs_=gs_):
                    for g_ in gs_:
                        start_group(g_)

        if 'prewait' in dbg:
            for r in range(1, 8):
                region_waits(r)

        def region(r, carry):
            if 'prewait' not in dbg and 'nodma2' not in dbg:
                region_waits(r)
            z1 = pl.multiple_of((r >> 8) * 8, 8)
            z2 = pl.multiple_of((r >> 9) * 8, 8)
            pm = [jnp.where(r >= 2, NM * (r - 2) + i, 32) for i in range(NM)]
            pw = jnp.where(r >= 2, r - 2, NCH) if WS else r - 1
            hp = _bf(hP[...])
            st = {'acc': [None, None], 'res': None}
            macc_ = {}

            def mvp(kq):
                n = D // 2 // KQ0
                for q in range(2):
                    st['acc'][q] = mv_part(wmA_v[r, pl.ds(z2 + kq * n, n), q * 128:(q + 1) * 128], kq * n, st['acc'][q])
                if kq == KQ0 - 1:
                    st['sa'] = jnp.sum(st['acc'][0], axis=0, keepdims=True)
                    st['ca'] = jnp.sum(st['acc'][1], axis=0, keepdims=True)
                    modA[r, 0:1, 0:128] = st['sa']
                    modA[r, 0:1, 128:256] = st['ca']

            def hpass(p):
                if MU:
                    x = _bf(x_v[p * PR // 2:(p + 1) * PR // 2, lane_ds(r, 128)]).astype(f32)
                    xh = (x - xhat[0, p * PR:(p + 1) * PR, :]) * xhat[1, p * PR:(p + 1) * PR, :]
                else:
                    xh = xhat[r, p * PR:(p + 1) * PR, :]
                st['h'] = (xh * (1.0 + st['ca']) + st['sa']).astype(bf16)
                st['row'] = p * PR
                if p == NP - 1:
                    hP[...] = pltpu.bitcast(st['h'], u32)

            def do_side(tag):
                prev, st['prev'] = st.get('prev'), st['res']
                jobs = side.get(tag, ())
                if not jobs:
                    return
                tkr = lambda row: pltpu.bitcast(st['res'][row:row + 8, 0:128], u32)
                sj = [int(j[1:]) for j in jobs if j[0] == 'S']
                def sjobs():
                    links = [(k, l) for k in sj for l in s_links(k, r, z1)]
                    for n, (k, l) in enumerate(links):
                        row = (TKS + n * TD // len(links)) // 8 * 8
                        W = s_ref(k)
                        W[0, pl.ds(z1 + (F // 4 if W is w4_v else D // 4), 8), 0:128] = tkr(row)
                        l()
                tk = tkr(0)
                kinds = set(j[0] for j in jobs)
                if 'W' in kinds:
                    wo_raw[pw, pl.ds(z1 + D // 2 + 16, 8), :] = tkr(TKW)
                if 'M' in kinds:
                    wmB_v[32, pl.ds(z1 + D // 2, 8), :] = tkr(TKM)
                if 'A' in kinds:
                    qbuf[0, pl.ds(z1 + S + HALO, 8), :] = pltpu.bitcast(tk, f32)
                for j in jobs:
                    k = int(j[1:])
                    if j[0] == 'W':
                        pW(pw, k, z2)
                    elif j[0] == 'w':
                        pW(pw, k, 0)
                    elif j[0] == 'M':
                        pM(pm[k // KQ], k % KQ, z2, macc_, k // KQ)
                    elif j[0] in 'Aa':
                        attention(qbuf, kbuf, vbuf, 0, k * AP, AP, True)
                if sj:
                    sjobs()

            for it in order0:
                if it[0] == 'T':
                    st['res'] = subdot(hp, TL, r - 1, int(it[1]), valid=r >= 2)
                    do_side(it)
                elif it[0] == 'H':
                    st['res'] = subdot(st['h'], st['row'], r, int(it[1]))
                    do_side('0' + it)
                elif it[0] == 'm':
                    mvp(int(it[1]))
                elif it[0] == 'K':
                    q = int(it[1:] or 0) * 128
                    wmA_v[r, pl.ds(z1 + D // 2, 8), 0:128] = pltpu.bitcast(st['res'][q:q + 8, 0:128], u32)
                elif it[0] == 'X':
                    q = int(it[1:] or 0) * 128
                    wqkv_raw[pl.ds(z1 + D // 2, 8), 0:128] = pltpu.bitcast(st['res'][q:q + 8, 0:128], u32)
                elif it[0] == 'h':
                    hpass(int(it[1]))
                elif it[0] == 'y':
                    b, qf = int(it[1]), int(it[2])
                    exch_groups([(r, b, rg) for rg in range(2 * qf, 2 * qf + 2)])
                elif it[0] == 'x':
                    b, hf = int(it[1]), int(it[2])
                    exch_groups([(r, b, rg) for rg in range(4 * hf, 4 * hf + 4)])
            for p in range(1, NP):
                hpass(p)
                for sd in range(6 if p < NP - 1 else 6 - NDEF):
                    st['res'] = subdot(st['h'], st['row'], r, sd)
                    do_side('%dH%d' % (p, sd))
            zsm[0] = r >> 8
            zsm[1] = r >> 9
            return carry

        if upto >= 2:
            if 'R' not in skip:
                lax.fori_loop(1, NR, region, 0)
            zero = zsm[0]
            zero2 = zsm[1]

        if WS and upto >= 2:
            c_wo(6).wait()
        if upto >= 3:
            c_wo(7).wait()
            for t in range(6 * NM, 32):
                c_mb(t, 6).wait()
            for c in c_w:
                c.wait()

        def rows_u32(ref, row0, M):
            if isinstance(row0, int):
                return _bf(ref[row0 // 2:(row0 + M) // 2, :])
            if isinstance(row0, tuple):
                return _bf(ref[pl.ds(row0[0] + row0[1] // 2, M // 2), :])
            return _bf(ref[pl.ds(pl.multiple_of(row0 // 2, 8), M // 2), :])

        def wo_dot(row0, M):
            o = rows_u32(o_scr, row0, M)
            return jnp.concatenate([_dot(o, _bf(wo_v[n])) for n in range(NCH)], axis=1)

        def row(k):
            return jnp.concatenate([modB[8 * (k - 2) + j, 0:1, :] for j in range(NCH)], axis=1)

        def ln23(row0, M, A):
            ga = row(2); sb = row(3); cb = row(4)
            x = rows_u32(x_v, row0, M).astype(f32)
            xm = x + ga * A
            hB = _ln(xm) * (1.0 + cb) + sb
            n3 = _ln(hB).astype(bf16)
            return xm, hB, n3

        shifts = [-1, -1, 1, 1, -2, -2, 2, 2]

        def g_val():
            return jnp.concatenate(
                [h1buf[j, HALO + shifts[j]:HALO + shifts[j] + T, :] for j in range(NCH)], axis=1).astype(bf16)

        def out_copy(r0, n, k, c0=0, cw=D):
            if cw == D:
                return pltpu.make_async_copy(obuf.at[pl.ds(r0, n)], o_hbm.bitcast(u32).at[pl.ds(r0, n)], osems.at[k])
            return pltpu.make_async_copy(obuf.at[pl.ds(r0, n), c0:c0 + cw], o_hbm.bitcast(u32).at[pl.ds(r0, n), c0:c0 + cw], osems.at[k])

        def ln4(hs):
            gb = row(5)
            x1 = hb[0:T, :] + hs
            base = xmid[0:T, :] + gb * x1
            n4 = _ln(x1).astype(bf16)
            return base, n4

        def asums(a11, a12, a21, a22):
            return [a11 + a22, a21 + a22, a11, a22, a11 + a12, a21 - a11, a12 - a22]

        def w3op(k, c0, cw):
            a, b = SLOT[k]
            c0 = c0 + b * FH
            return _bf(w3_v[a, 0:D // 4, pl.ds(c0, cw) if not isinstance(c0, int) else slice(c0, c0 + cw)])

        def w4op(k, c0, cw, r0=0, nr=F // 4, z=None):
            a, b = SLOT[k]
            if z is not None:
                r0 = z + r0
            return _bf(w4_v[a, pl.ds(r0, nr) if not isinstance(r0, int) else slice(r0, r0 + nr), b * DH2 + c0:b * DH2 + c0 + cw])

        def strass(dotk, hook=None):
            M = dotk(0); c11 = M; c22 = M
            if hook: hook(0, M)
            M = dotk(1); c21 = M; c22 = c22 - M
            if hook: hook(1, M)
            M = dotk(2); c12 = M; c22 = c22 + M
            if hook: hook(2, M)
            M = dotk(3); c11 = c11 + M; c21 = c21 + M
            if hook: hook(3, M)
            M = dotk(4); c11 = c11 - M; c12 = c12 + M
            if hook: hook(4, M)
            M = dotk(5); c22 = c22 + M
            if hook: hook(5, M)
            M = dotk(6); c11 = c11 + M
            if hook: hook(6, M)
            return c11, c12, c21, c22

        def n_sums(r, nv, stg, dst):
            q = T // RP0 // 2
            if r < q:
                stg[r * RP0:(r + 1) * RP0, :] = nv
            else:
                top = stg[(r - q) * RP0:(r - q + 1) * RP0, :]
                A = asums(top[:, :DH2], top[:, DH2:], nv[:, :DH2], nv[:, DH2:])
                for k in range(7):
                    dst[k, (r - q) * RP0:(r - q + 1) * RP0, :] = A[k].astype(bf16)

        def n4_sums(r, n4v):
            n_sums(r, n4v, n4f, a4)

        def w12op(W, k, c0, cw, z=None):
            a, b = SLOT5[k]
            if z is not None:
                return _bf(W[a, pl.ds(z, D // 4), b * DH2 + c0:b * DH2 + c0 + cw])
            return _bf(W[a, 0:D // 4, b * DH2 + c0:b * DH2 + c0 + cw])

        def raw_dot(x, W):
            return _dot(x[:, :DH2], _bf(W[0, 0:D // 4, :])) + _dot(x[:, DH2:], _bf(W[1, 0:D // 4, :]))

        def g_sums(j, q, z):
            def ld(jj, r0):
                r0 = HALO + shifts[jj] + r0
                return h1buf[jj, r0:r0 + RP0, :] if z is None else h1buf[jj, pl.ds(z + r0, RP0), :]
            A = asums(ld(j, q * RP0), ld(j + 4, q * RP0), ld(j, HM + q * RP0), ld(j + 4, HM + q * RP0))
            for k in range(7):
                a2[k, q * RP0:(q + 1) * RP0, j * 128:(j + 1) * 128] = A[k].astype(bf16)

        def stage3(c0, cw, uc0, hook=None):
            U = strass(lambda k: _dot(a4[k], w3op(k, c0, cw)), hook)
            A = asums(*[_gelu(x) for x in U])
            for k in range(7):
                ua[k, :, uc0:uc0 + cw] = A[k].astype(bf16)

        RP0 = 16

        def bfirst():
            for j in range(NCH):
                h1buf[j, 0:HALO, :] = jnp.zeros((HALO, 128), f32)
            h7 = _bf(hP[...])
            zb = pl.multiple_of(zero * 8, 8) if ZB else 0
            h0 = (T + HALO) // 2 // 16 * 16 + (16 if T == 128 else 0)
            halves = [(0, h0), (h0, T + HALO - h0)]
            nA = (2 * T + HALO - AT0) // AP
            st = {'res': None, 'As': [], 'n3': [], 'h1': [], 'macc': {}}

            def att(k):
                if AG:
                    st['o'] = attention2(AT0 + k * AP, AP, AG)
                else:
                    attention(qbuf, kbuf, vbuf, 0, AT0 + k * AP, AP, True)

            def tok_q(cc=0):
                qbuf[0, pl.ds(zb + S + HALO, 8), :] = st['res'][0:8, cc * 128:(cc + 1) * 128]

            batt = None
            if 'A' in BA:
                batt = Att(0, 0, 0, 2 * T + HALO, [BWG] * ((2 * T + HALO) // RB * W // BWG), BPD, zb, BQD, True)
            for it in BA.split():
                k = int(it[1:]) if len(it) > 1 and it[1:].isdigit() else None
                if not ZB and it[0] in 'tWM':
                    continue
                if it[0] == 'A':
                    batt.steps(k)
                elif it[0] == 'R':
                    batt.steps(999)
                    batt.rest()
                elif it[0] == 'T':
                    st['res'] = subdot(h7, TL, 7, k)
                elif it[0] == 'a':
                    att(k)
                elif it[0] == 't':
                    tok_q(k or 0)
                elif it[0] == 'w':
                    pW(7, k, zb)
                elif it[0] == 'v':
                    pW(6, k, zb)
                elif it[0] == 'm':
                    for kq in range(KQ):
                        pM(6 * NM + k, kq, zb, st['macc'], k)
                elif it[0] == 'M':
                    wmB_v[32, pl.ds(zb + D // 2, 8), :] = pltpu.bitcast(st['res'][0:8, 0:128], u32)
                elif it[0] == 'W':
                    wo_raw[7, pl.ds(zb + D // 2 + 16, 8), :] = pltpu.bitcast(st['res'][0:8, 0:128], u32)
                elif it[0] == 'o':
                    assert batt is None or batt.done >= (halves[k][0] + halves[k][1]) // RB * NCH, batt.done
                    st['res'] = wo_dot(*halves[k])
                    st['As'].append(st['res'])
                elif it[0] == 'l':
                    r0, m = halves[k]
                    xm, hB, n3 = ln23(r0, m, st['As'][k])
                    xmid[r0:r0 + m, :] = xm
                    hb[r0:r0 + m, :] = hB
                    st['n3'].append(n3)
                elif it[0] == 'u':
                    r0, m = halves[k]
                    st['res'] = raw_dot(st['n3'][k], w1_v)
                    h1 = _gelu(st['res'])
                    for j in range(NCH):
                        h1buf[j, HALO + r0:HALO + r0 + m, :] = h1[:, j * 128:(j + 1) * 128]
                elif it[0] == 'z':
                    if 'g' not in st:
                        st['g'] = g_val()
                    cw_ = D // NZ
                    st['res'] = _dot(st['g'], _bf(w2_v[:, k * cw_:(k + 1) * cw_]))
                    hsbuf[0:T, k * cw_:(k + 1) * cw_] = st['res']
                elif it[0] == 'U':
                    hh, pp = divmod(k, 10)
                    r0, m = halves[hh]
                    cw_ = D // NU
                    st['res'] = _dot(st['n3'][hh], _bf(w1_v[:, pp * cw_:(pp + 1) * cw_]))
                    h1 = _gelu(st['res'])
                    for j in range(cw_ // 128):
                        h1buf[pp * (cw_ // 128) + j, HALO + r0:HALO + r0 + m, :] = h1[:, j * 128:(j + 1) * 128]
            if 'g' not in st:
                hsbuf[0:T, :] = raw_dot(g_val(), w2_v)

        if upto >= 3 and 'F' not in skip:
            bfirst()

        def carries(xm, hB, h1, notlast):
            xmid[0:HALO, :] = xmid[T:T + HALO, :]
            hb[0:HALO, :] = hb[T:T + HALO, :]
            for j in range(NCH):
                h1buf[j, 0:2 * HALO, :] = h1buf[j, T:T + 2 * HALO, :]
            xmid[HALO:HALO + T, :] = xm
            hb[HALO:HALO + T, :] = hB
            for j in range(NCH if h1 is not None else 0):
                h1j = h1[:, j * 128:(j + 1) * 128]
                h1buf[j, 2 * HALO:HALO + T, :] = h1j[0:T - HALO]
                h1buf[j, HALO + T:2 * HALO + T, :] = jnp.where(notlast, h1j[T - HALO:T], 0.0)

        RP = 16

        def bbody(i, carry):
            static = isinstance(i, int)
            if static:
                row0h = i * (T // 2)
                abase = (i + 1) * T
                abaseh = (i + 1) * (T // 2)
                z1 = pl.multiple_of(zero * 8, 8)
                z2 = pl.multiple_of(zero2 * 8, 8)
            else:
                row0h = pl.multiple_of(i * (T // 2), T // 2)
                nxt = jnp.minimum(i + 1, NT - 1)
                abase = pl.multiple_of(nxt * T, T)
                abaseh = pl.multiple_of(nxt * (T // 2), T // 2)
                z1 = pl.multiple_of((i >> 8) * 8, 8)
                z2 = pl.multiple_of((i >> 9) * 8, 8)
            ga = row(2); sb = row(3); cb = row(4); gb = row(5)
            bases, n4p, xms, hBs, n3p, As = [], [], {}, {}, [], []
            att = None
            asch = {}
            if AB == 9:
                att = Att(abase, abaseh, HALO, T, [int(t) for t in WGS], PD, z1, KD=KD)
                for t in ASCH.split():
                    k_, v_ = t.split(':')
                    asch[k_] = int(v_)

            def astep(tag):
                if att is not None and tag in asch:
                    att.steps(asch[tag])

            def p4(r):
                r0 = r * RP
                x1 = hb[r0:r0 + RP, :] + hsbuf[pl.ds(z2 + r0, RP), :]
                if ST and RL4:
                    bases.append((r, xmid[r0:r0 + RP, :] + gb * x1))
                    m = jnp.mean(x1, axis=-1, keepdims=True)
                    x1buf[r0:r0 + RP, :] = x1
                    rd = lambda z: x1buf[r0:r0 + RP, :] if RL4 == 1 else x1buf[pl.ds(z + r0, RP), :]
                    xc = rd(z1) - m
                    rs = lax.rsqrt(jnp.mean(xc * xc, axis=-1, keepdims=True) + EPS)
                    n4_sums(r, (rd(z2) - m) * rs)
                    n4p.append(None)
                    return
                if ST:
                    bases.append((r, xmid[r0:r0 + RP, :] + gb * x1))
                    n4_sums(r, _ln(x1))
                    n4p.append(None)
                    return
                bases.append(xmid[r0:r0 + RP, :] + gb * x1)
                n4v = _ln(x1).astype(bf16)
                if EX4:
                    n4b[r0 // 2:(r0 + RP) // 2, :] = pltpu.bitcast(n4v, u32)
                n4p.append(n4v)

            chain = []

            def p23(r, A):
                r0 = r * RP
                if LC and len(chain) >= LC:
                    abuf[pl.ds(z1 + T, 8), 0:128] = chain[len(chain) - LC]
                    x_v[pl.ds(z1 + S // 2 + HALO // 2, 8), 0:128] = pltpu.bitcast(chain[len(chain) - LC], u32)
                x = rows_u32(x_v, (row0h, HALO + r0), RP).astype(f32)
                xm = x + ga * (abuf[pl.ds(z2 + r0, RP), :] if EA else A[r0:r0 + RP])
                if RL3:
                    def rd(ref, z):
                        return ref[HALO + r0:HALO + r0 + RP, :] if RL3 == 1 else ref[pl.ds(z + HALO + r0, RP), :]
                    xmid[HALO + r0:HALO + r0 + RP, :] = xm
                    m = jnp.mean(xm, axis=-1, keepdims=True)
                    xc = rd(xmid, z1) - m
                    rs = lax.rsqrt(jnp.mean(xc * xc, axis=-1, keepdims=True) + EPS)
                    hB = (rd(xmid, z2) - m) * rs * (1.0 + cb) + sb
                    hb[HALO + r0:HALO + r0 + RP, :] = hB
                    m = jnp.mean(hB, axis=-1, keepdims=True)
                    xc = rd(hb, z1) - m
                    rs = lax.rsqrt(jnp.mean(xc * xc, axis=-1, keepdims=True) + EPS)
                    n3v = (rd(hb, z2) - m) * rs
                    n_sums(r, n3v, n3f, a3)
                    n3p.append(None)
                    chain.append(n3v[0:8, 0:128])
                    return
                hB = _ln(xm) * (1.0 + cb) + sb
                xms[r] = xm; hBs[r] = hB
                if S1:
                    n_sums(r, _ln(hB), n3f, a3)
                    n3p.append(None)
                    return
                n3v = _ln(hB).astype(bf16)
                n3b[r0 // 2:(r0 + RP) // 2, :] = pltpu.bitcast(n3v, u32)
                n3p.append(n3v)

            def p23_stages(r):
                r0 = r * RP
                rows = slice(HALO + r0, HALO + r0 + RP)
                v = {}

                def sa():
                    x = rows_u32(x_v, (row0h, HALO + r0), RP).astype(f32)
                    xm = x + ga * abuf[pl.ds(z2 + r0, RP), :]
                    xmid[rows, :] = xm
                    v['m'] = jnp.mean(xm, axis=-1, keepdims=True)

                def sb_():
                    xc = xmid[rows, :] - v['m']
                    v['rs'] = lax.rsqrt(jnp.mean(xc * xc, axis=-1, keepdims=True) + EPS)

                def sc():
                    hB = (xmid[rows, :] - v['m']) * v['rs'] * (1.0 + cb) + sb
                    hb[rows, :] = hB
                    v['m2'] = jnp.mean(hB, axis=-1, keepdims=True)

                def sd():
                    xc = hb[rows, :] - v['m2']
                    v['rs2'] = lax.rsqrt(jnp.mean(xc * xc, axis=-1, keepdims=True) + EPS)

                def se():
                    n_sums(r, (hb[rows, :] - v['m2']) * v['rs2'], n3f, a3)
                    n3p.append(None)
                return [sa, sb_, sc, sd, se]

            ord4 = list(ORD4) if ST else list(range(T // RP))
            for r in range(T // RP):
                if rel4[r] < 0:
                    p4(ord4[r])
            o = rows_u32(o_scr, (row0h, HALO), T)
            for n in range(NCH):
                An = _dot(o, _bf(wo_v[n]))
                As.append(An)
                if EA:
                    abuf[0:T, n * 128:(n + 1) * 128] = An
                r4 = [r for r in range(T // RP) if rel4[r] == n]
                if r4:
                    hsbuf[pl.ds(z1 + T, 8), 0:128] = An[0:8, 0:128]
                for r in r4:
                    p4(ord4[r])
                astep('o%d' % n)
                if AWO and att is not None:
                    att.steps(AWO)
            A = jnp.concatenate(As, axis=1)
            if RL3:
                xmid[0:HALO, :] = xmid[T:T + HALO, :]
                hb[0:HALO, :] = hb[T:T + HALO, :]
            if ST:
                stg = {}
                base = jnp.concatenate([b for _, b in sorted(bases, key=lambda t: t[0])], axis=0)
                for c in range(FH // CW3):
                    def hook(k, M, c=c):
                        r23 = [r for r in range(T // RP) if R23[r] == 7 * c + k]
                        if r23:
                            x_v[pl.ds(z1 + S // 2 + HALO // 2, 8), 0:128] = pltpu.bitcast(M[0:8, 0:128], u32)
                            if EA:
                                abuf[pl.ds(z1 + T, 8), 0:128] = M[0:8, 0:128]
                        if SP3:
                            for r in range(T // RP):
                                d_ = 7 * c + k - R23[r]
                                if d_ == 0:
                                    stg[r] = p23_stages(R3O[r])
                                if d_ >= 0 and d_ % SP3 == 0 and d_ // SP3 < 5:
                                    stg[r][d_ // SP3]()
                        for r in r23:
                            if not SP3:
                                p23(R3O[r] if S1 else r, A)
                        t = 7 * c + k
                        if t == TW4:
                            w4_v[0, pl.ds(z1 + F // 4, 8), 0:128] = pltpu.bitcast(M[0:8, 0:128], u32)
                        if t == TW1:
                            w1_v[0, pl.ds(z1 + D // 4, 8), 0:128] = pltpu.bitcast(M[0:8, 0:128], u32)
                        if AP3 and att is not None and t >= AO3 and (t - AO3) % AP3 == 0:
                            att.steps(1)
                    stage3(c * CW3, CW3, c * CW3, hook)
            else:
                base = jnp.concatenate(bases, axis=0)
                n4 = _bf(n4b[...]) if EX4 else jnp.concatenate(n4p, axis=0)
                U = _dot(n4, _bf(w3_v[...]))
                u = _gelu(U).astype(bf16)
            for c in range(0 if ST else F // 128):
                r23 = [r for r in range(T // RP) if rel23[r] == NCH + c]
                if r23 or c in XT:
                    x_v[pl.ds(z1 + S // 2 + HALO // 2, 8), 0:128] = pltpu.bitcast(U[0:8, c * 128:(c + 1) * 128], u32)
                for r in r23:
                    p23(r, A)
                astep('c%d' % c)
            assert len(n3p) == T // RP and len(n4p) == T // RP
            if S1:
                if not RL3:
                    xm = jnp.concatenate([xms[r] for r in range(T // RP)], axis=0)
                    hB = jnp.concatenate([hBs[r] for r in range(T // RP)], axis=0)
                    carries(xm, hB, None, None)
                else:
                    for j in range(NCH):
                        h1buf[j, 0:2 * HALO, :] = h1buf[j, T:T + 2 * HALO, :]
                for c in range(DH2 // 128):
                    def hook1(k, M, c=c):
                        if AP1 and att is not None and (7 * c + k) % AP1 == 0:
                            att.steps(1)
                    U = strass(lambda k: _dot(a3[k], w12op(w1_v, k, c * 128, 128, None if TW1 is None else z2)), hook1)
                    for q, Uq in enumerate(U):
                        j, r0 = (q % 2) * 4 + c, 2 * HALO + (q // 2) * HM
                        hq = _gelu(Uq)
                        if q // 2:
                            h1buf[j, r0:r0 + HM - HALO, :] = hq[0:HM - HALO]
                            h1buf[j, r0 + HM - HALO:r0 + HM, :] = jnp.where(i < NT - 1, hq[HM - HALO:HM], 0.0)
                        else:
                            h1buf[j, r0:r0 + HM, :] = hq
            else:
                xm = jnp.concatenate([xms[r] for r in range(T // RP)], axis=0)
                hB = jnp.concatenate([hBs[r] for r in range(T // RP)], axis=0)
                h1 = _gelu(raw_dot(_bf(n3b[...]), w1_v))
                carries(xm, hB, h1, i < NT - 1)
            if static:
                if i < NT - 1:
                    attention(qbuf, kbuf, vbuf, abase, HALO, T, False, abaseh)
            elif 'noatt' not in dbg and not AP4:
                if AB == 9:
                    att.steps(999)
                    att.rest()
                    if DL:
                        h1buf[0, pl.ds(z1 + T + 2 * HALO, 8), :] = att.OC[T // RB - 1, NCH - 1]
                elif AB:
                    attention2(HALO, T, AB, abase, abaseh)
                else:
                    attention(qbuf, kbuf, vbuf, abase, HALO, T, False, abaseh)
            if ST:
                ro = pl.multiple_of((i - 1) * (T // 2), T // 2)
                gdone = []
                for c in range(DH2 // CW4):
                    c0 = c * CW4

                    def hook4(k, M, c=c):
                        if AP4 and att is not None:
                            att.steps(AP4)
                        if 7 * c + k == TW2:
                            w2_v[0, pl.ds(z1 + D // 4, 8), 0:128] = pltpu.bitcast(M[0:8, 0:128], u32)
                        if not S1 or GT is None:
                            return
                        for n, t in enumerate(GT):
                            if t == 7 * c + k:
                                h1buf[0, pl.ds(z1 + T + 2 * HALO, 8), :] = M[0:8, 0:128]
                                g_sums(n // 4, n % 4, z2)
                                gdone.append(n)
                    Hs = strass(lambda k: _dot(ua[k], w4op(k, c0, CW4, z=None if TW4 is None else z2)), hook4)
                    for q, Hq in enumerate(Hs):
                        rr, cc = (q // 2) * HM, (q % 2) * DH2 + c0
                        o_ = base[rr:rr + HM, cc:cc + CW4] + gb[:, cc:cc + CW4] * Hq
                        obuf[pl.ds(ro + rr // 2, HM // 2), cc:cc + CW4] = pltpu.bitcast(o_.astype(bf16), u32)
                if S1:
                    for n in range(16):
                        if n not in gdone:
                            g_sums(n // 4, n % 4, None)
                    for c in range(DH2 // 128):
                        def hook2(k, M, c=c):
                            if AP2 and att is not None and (7 * c + k) % AP2 == 0:
                                att.steps(1)
                        Hs = strass(lambda k: _dot(a2[k], w12op(w2_v, k, c * 128, 128, None if TW2 is None else z2)), hook2)
                        for q, Hq in enumerate(Hs):
                            rr, cc = (q // 2) * HM, (q % 2) * DH2 + c * 128
                            hsbuf[rr:rr + HM, cc:cc + 128] = Hq
                else:
                    hsbuf[0:T, :] = raw_dot(g_val(), w2_v)
                if AP4:
                    att.steps(999)
                    att.rest()
                return carry
            h2 = _dot(u, _bf(w4_v[...]))
            if static:
                obuf[(i - 1) * (T // 2):i * (T // 2), :] = pltpu.bitcast((base + gb * h2).astype(bf16), u32)
            else:
                obuf[pl.ds(pl.multiple_of((i - 1) * (T // 2), T // 2), T // 2), :] = pltpu.bitcast((base + gb * h2).astype(bf16), u32)
            hsbuf[0:T, :] = _dot(g_val(), _bf(w2_v[...]))
            return carry

        if upto >= 4 and 'B' not in skip:
            if UB:
                for i in range(1, 1 + UB):
                    bbody(i, 0)
                    if i in BAR:
                        out_copy_i(i).start()
                if 1 + UB < NT:
                    lax.fori_loop(1 + UB, NT, bbody, 0)
            else:
                lax.fori_loop(1, NT, bbody, 0)

        def blast():
            r0 = (NT - 1) * (T // 2)
            out_copy(0, r0, 0).start()
            if ST:
                gb = row(5)
                for r in ORD4:
                    p0 = r * RP
                    x1 = hb[p0:p0 + RP, :] + hsbuf[p0:p0 + RP, :]
                    baseb[p0:p0 + RP, :] = xmid[p0:p0 + RP, :] + gb * x1
                    n4_sums(r, _ln(x1))

                def fin(q, Hq, c0, cw):
                    rr, cc = (q // 2) * HM, (q % 2) * DH2 + c0
                    o_ = baseb[rr:rr + HM, cc:cc + cw] + gb[:, cc:cc + cw] * Hq
                    obuf[r0 + rr // 2:r0 + rr // 2 + HM // 2, cc:cc + cw] = pltpu.bitcast(o_.astype(bf16), u32)

                if SB == 'F':
                    for c in range(FH // CW3):
                        stage3(c * CW3, CW3, c * CW3)
                    for c in range(DH2 // CW4):
                        Hs = strass(lambda k: _dot(ua[k], w4op(k, c * CW4, CW4)))
                        for q, Hq in enumerate(Hs):
                            fin(q, Hq, c * CW4, CW4)
                else:
                    QF = FH // 2

                    def sbody(m, carry):
                        cb_ = pl.multiple_of(m * QF, 128)
                        for c in range(QF // 128):
                            stage3(cb_ + c * 128, 128, c * 128)
                        rb_ = pl.multiple_of(m * (QF // 2), 32)
                        for c in range(DH2 // CW4):
                            for k in range(7):
                                Mk = _dot(ua[k, :, 0:QF], w4op(k, c * CW4, CW4, rb_, QF // 2))
                                macc[k, :, c * CW4:(c + 1) * CW4] = jnp.where(m > 0, macc[k, :, c * CW4:(c + 1) * CW4], 0.0) + Mk
                        return carry

                    lax.fori_loop(0, 2, sbody, 0)
                    for c in range(DH2 // 128):
                        Hs = strass(lambda k: macc[k, :, c * 128:(c + 1) * 128])
                        for q, Hq in enumerate(Hs):
                            fin(q, Hq, c * 128, 128)
                out_copy(r0, T // 2, 1).start()
                out_copy(0, r0, 0).wait()
                out_copy(r0, T // 2, 1).wait()
                return
            if BL == 'M':
                gb = row(5)

                def l4(p0, zz, dst):
                    x1 = hb[p0:p0 + RP, :] + (hsbuf[pl.ds(zz + p0, RP), :] if zz is not None else hsbuf[p0:p0 + RP, :])
                    baseb[p0:p0 + RP, :] = xmid[p0:p0 + RP, :] + gb * x1
                    q0 = (p0 % HM) // 2
                    dst[q0:q0 + RP // 2, :] = pltpu.bitcast(_ln(x1).astype(bf16), u32)

                for p0 in range(0, HM, RP):
                    l4(p0, None, n4b)

                def mbody(m, carry):
                    zz = pl.multiple_of((m >> 8) * 8, 8)
                    if MA:
                        n4 = _bf(n4b[0:HM // 2, :])
                    else:
                        n4 = _bf(n4b[pl.ds(pl.multiple_of(m * (HM // 2), HM // 2), HM // 2), :])
                    U = _dot(n4, _bf(w3_v[...]))
                    u = _gelu(U).astype(bf16)
                    for k, p0 in enumerate(range(HM, T, RP)):
                        if MT is not None and (k == 0 or MT[k] != MT[k - 1]):
                            hsbuf[pl.ds(zz + T, 8), 0:128] = U[0:8, MT[k] * 128:(MT[k] + 1) * 128]
                        l4(p0, zz if MT is not None else None, n3b if MA else n4b.at[HM // 2:T // 2])
                    if MA:
                        n4b[0:HM // 2, :] = n3b[0:HM // 2, :]
                    ro = pl.multiple_of(r0 + m * (HM // 2), HM // 2)
                    c0 = 0
                    for cw_ in MN:
                        h2 = _dot(u, _bf(w4_v[:, c0:c0 + cw_]))
                        bs = baseb[pl.ds(pl.multiple_of(m * HM, HM), HM), c0:c0 + cw_]
                        obuf[pl.ds(ro, HM // 2), c0:c0 + cw_] = pltpu.bitcast((bs + gb[:, c0:c0 + cw_] * h2).astype(bf16), u32)
                        out_copy(ro, HM // 2, 1, c0, cw_).start()
                        c0 += cw_
                    return carry

                lax.fori_loop(0, 2, mbody, 0)
                out_copy(0, r0, 0).wait()
                for hf in range(2):
                    c0 = 0
                    for cw_ in MN:
                        out_copy(r0 + hf * (HM // 2), HM // 2, 1, c0, cw_).wait()
                        c0 += cw_
                return
            base, n4 = ln4(hsbuf[0:T, :])
            if BL:
                FC = F // BL
                xmid[0:T, :] = base
                n4b[...] = pltpu.bitcast(n4, u32)
                hsbuf[0:T, :] = jnp.zeros((T, D), f32)

                def body(c, carry):
                    w3c = w3_v[:, pl.ds(pl.multiple_of(c * FC, 128), FC)]
                    u = _gelu(_dot(_bf(n4b[...]), _bf(w3c))).astype(bf16)
                    w4c = w4_v[pl.ds(pl.multiple_of(c * (FC // 2), 32), FC // 2), :]
                    hsbuf[0:T, :] += _dot(u, _bf(w4c))
                    return carry

                lax.fori_loop(0, BL, body, 0)
                obuf[r0:r0 + T // 2, :] = pltpu.bitcast((xmid[0:T, :] + row(5) * hsbuf[0:T, :]).astype(bf16), u32)
            else:
                u = _gelu(_dot(n4, _bf(w3_v[...]))).astype(bf16)
                h2 = _dot(u, _bf(w4_v[...]))
                obuf[r0:r0 + T // 2, :] = pltpu.bitcast((base + row(5) * h2).astype(bf16), u32)
            out_copy(r0, T // 2, 1).start()
            out_copy(0, r0, 0).wait()
            out_copy(r0, T // 2, 1).wait()

        if upto >= 5 and 'L' not in skip:
            blast()

    @jax.jit
    def fn(A_x, A_wqkv, A_wo, B_x, B_w1, B_w2, B_w3, B_w4, c, w_mod):
        x = A_x.reshape(S, D)
        any_spec = pl.BlockSpec(memory_space=pl.ANY)
        out = pl.pallas_call(
            kernel,
            in_specs=[any_spec] * 9,
            out_specs=any_spec,
            out_shape=jax.ShapeDtypeStruct((S, D), bf16),
            scratch_shapes=[
                pltpu.VMEM((S // 2 + HALO // 2 + 8, D), u32),
                pltpu.VMEM((D // 2 + 32, 3 * D), u32),
                pltpu.VMEM((64 if SW else D // 2, D), u32),
                pltpu.VMEM((64 if SW else D // 2, D), u32),
                pltpu.VMEM((64 if SW else D // 2, D), u32),
                pltpu.VMEM((NCH + WS, D // 2 + 32, 128), u32),
                pltpu.VMEM((NCH + WS, D // 2, 128), u32),
                pltpu.VMEM((5, D // 4 + 32, D), u32),
                pltpu.VMEM((5, D // 4 + 32, D), u32),
                pltpu.VMEM((4, D // 4 + 8, F), u32),
                pltpu.VMEM((4, F // 4 + 32, D), u32),
                pltpu.VMEM((D // 2, 128), f32),
                pltpu.VMEM((D // 2, 128), f32),
                pltpu.VMEM((8, D // 2 + 16, 256), u32),
                pltpu.VMEM((33, D // 2 + 32, 128), u32),
                pltpu.VMEM((8, 8, 256), f32),
                pltpu.VMEM((36, 8, 128), f32),
                pltpu.VMEM((3 if MU else NCH, S + 32, 128), f32),
                pltpu.VMEM((PR // 2, 128), u32),
                pltpu.VMEM((S // 2, 128), u32),
                pltpu.VMEM((NCH, S + 32, 128), f32),
                pltpu.VMEM((NCH, S + 2 * HALO + 32 * (AB == 9), 128), f32),
                pltpu.VMEM((NCH, S + 2 * HALO + 32 * (AB == 9), 128), f32),
                pltpu.VMEM((T + HALO, D), f32),
                pltpu.VMEM((T + HALO, D), f32),
                pltpu.VMEM((NCH, T + 2 * HALO + 32, 128), f32),
                pltpu.VMEM((S // 2, D), u32),
                pltpu.VMEM((S // 2 + HALO // 2, D), u32),
                pltpu.VMEM((T + 32, D), f32),
                pltpu.VMEM((T // 2, D), u32),
                pltpu.VMEM((T // 2, D), u32),
                pltpu.VMEM((T, D), f32),
                pltpu.VMEM((T, D), f32),
                pltpu.VMEM((7, T // 2, D // 2), bf16),
                pltpu.VMEM((7, T // 2, F // 2), bf16),
                pltpu.VMEM((7, T // 2, D // 2), f32),
                pltpu.VMEM((T // 2, D), f32),
                pltpu.VMEM((7, T // 2, D // 2), bf16),
                pltpu.VMEM((7, T // 2, D // 2), bf16),
                pltpu.VMEM((T + 32, D), f32),
                pltpu.VMEM((T, D), f32),
                pltpu.VMEM((1, D), bf16),
            ] + ([pltpu.VMEM((padr, 128), f32)] if padr else []) + [
                pltpu.SMEM((8,), jnp.int32),
            ],
            compiler_params=pltpu.CompilerParams(vmem_limit_bytes=126 * 1024 * 1024),
        )(x, A_wqkv, A_wo, B_w1, B_w2, B_w3, B_w4, c, w_mod)
        return out.reshape(1, S, D)
    return fn


_fn = make()


def pallas_adaLN_cond__sliding_local_dilated__mixer_s_mlp__prompt_kernel(A_x, A_wqkv, A_wo, B_x, B_w1, B_w2, B_w3, B_w4, c, w_mod):
    return _fn(A_x, A_wqkv, A_wo, B_x, B_w1, B_w2, B_w3, B_w4, c, w_mod)
```

```python
import functools
import jax
import jax.numpy as jnp
from jax import lax
import jax.experimental.pallas as pl
import jax.experimental.pallas.tpu as pltpu

S, D, F = 2048, 1024, 3584
H, DH, W, DIL = 32, 32, 8, 2
NCH = D // 128
EPS = 1e-5
SCALE = DH ** -0.5
f32, bf16, u32 = jnp.float32, jnp.bfloat16, jnp.uint32
HALO = 16


def _ln(x):
    m = jnp.mean(x, axis=-1, keepdims=True)
    xc = x - m
    v = jnp.mean(xc * xc, axis=-1, keepdims=True)
    return xc * lax.rsqrt(v + EPS)


def _gelu(x):
    c0 = 0.7978845608028654
    c1 = c0 * 0.044715
    t = jnp.tanh(x * (c0 + c1 * (x * x)))
    hx = 0.5 * x
    return hx + hx * t


def _dot(a, b):
    return jnp.dot(a, b, preferred_element_type=f32)


def _bf(w):
    return pltpu.bitcast(w, bf16)


def _lane_xor(x, s):
    lane = lax.broadcasted_iota(jnp.int32, x.shape, 1)
    return jnp.take_along_axis(x, lane ^ s, axis=1)


def _exchange8_multi(XS):
    XS = [list(X) for X in XS]
    lane = lax.broadcasted_iota(jnp.int32, XS[0][0].shape, 1)
    for t in range(3):
        s = 1 << (t + 2)
        m = (lane & s) != 0
        for X in XS:
            for p in range(8):
                if p & (1 << t):
                    continue
                p2 = p | (1 << t)
                tmp = _lane_xor(jnp.where(m, X[p], X[p2]), s)
                X[p], X[p2] = jnp.where(m, tmp, X[p]), jnp.where(m, X[p2], tmp)
    return XS


def _group4_sum(acc):
    lane = lax.broadcasted_iota(jnp.int32, acc.shape, 1)
    acc = acc + jnp.where((lane & 1) != 0, pltpu.roll(acc, 1, 1), pltpu.roll(acc, 127, 1))
    acc = acc + jnp.where((lane & 2) != 0, pltpu.roll(acc, 2, 1), pltpu.roll(acc, 126, 1))
    return acc


def make(T=128, PR=512, RB=8, EG=4, upto=9, AT0=0, AP=16,
         DO='c X0 Wq sa ca X1 Wk Wv X2 X3 X4 X5 X6 X7 X8 X9 X10 X12 X13 X11 X14 X15',
         PS=None, PSX=None, RL=1, D0='1234', LP=16, BL='M', ZB=1,
         order0='T0 T1 X x00 x01 m0 T2 T3 X x10 x11 h0 T4 T5 X x20 H0 X x21 H1 H2 H3 H4 H5', NDEF=6, BA=None,
         side=None, KQ=4, KQ0=1, NM=5, NR=8, AG=1,
         rel4=(-1, -1, -1, 0, 1, 2, 3, 4), rel23=(8, 9, 10, 11, 12, 13, 14, 15),
         padr=0, dbg='', UB=0, BAR=(), GL=0, MU=1, WS=1, skip='', AB=9, WGS='12'*42+'2', PD=0, ASCH='', DL=0, EX3=1, EX4=1, XT=(), MT=(4, 10, 16, 22), MA=0, MN=(1024,), NZ=8, NU=2, BPD=0, BQD=None, BWG=8,
         ST=1, ORD4=(0, 4, 1, 5, 2, 6, 3, 7), R23=(0, 6, 12, 18, 24, 30, 36, 42), PRE='R', CW3=128, CW4=128, SB='S', SJ=None, P0R=4, S1=1, R3O=(0, 4, 1, 5, 2, 6, 3, 7), GT=None, KD=None, LC=0, SP3=0, AP1=0, AP4=0, AP2=0, TW4=None, TW1=None, TW2=None, AP3=0, AO3=0, AWO=0, EA=1, RL3=1, RL4=0, LK3=1, LK4=1, TKS=64, TKW=0, TKM=0, SW=1, SK=None, SL=1, TG=1, TD=400, NC=1, DR=None, GA=(0, 4, 4, 4, 4, 4, 4, 4), PVG=None, PVM=None):
    HS, HO = (2, 0) if MU else (0, S // 2)
    NT = S // T
    NP = S // PR
    order0 = order0.split()
    TL = S - PR
    if PS is None:
        PS = ('wc C wX0 L0 wWq e0 wsa S wca A h0 wX1 u0:0 L1 wWk u1:0 e1 wWv u0:1 u1:1 e2 wX2 u0:2 u1:2 L2 u2:0 '
              'wX3 wX4 u2:12 L3 u3:012 L4 u4:0 wX5 wX6 wX7 u4:12 L5 u5:012 L6 u6:012 L7 u7:0 '
              'wX8 wX9 wX10 wX12 wX13 u7:12 L8 u8:012 L9 u9:012 L10 ua:0 L12 L13 wX11 wX14 wX15 Da D5 Db D6 Dc D7 Dd DW ua:12 L11 ub:012 L14 L15')
    DR = {2: 'c7dW'} if DR is None else DR
    for v_ in DR.values():
        for g_ in v_:
            assert (' D' + g_ + ' ') in PS
            PS = PS.replace(' D' + g_ + ' ', ' ')
    if BA is None:
        BA = ('a0 a1 T0 T1 t0 a2 a3 W w0 w1 w2 w3 w4 w5 w6 w7 T2 t0 a4 a5 T3 t0 a6 a7 T4 t0 a8 a9 T5 t0 a10 o0 t0 a11 t4 a12 '
              'o1 t0 a13 t4 a14 M m0 m1 l0 l1 u0 t0 a15 t4 a16 u1')
    if WS and 'v0' not in BA:
        BA = BA.replace('W w0 w1 w2 w3 w4 w5 w6 w7', 'W v0 v1 v2 v3 v4 v5 v6 v7 w0 w1 w2 w3 w4 w5 w6 w7')
    if PSX:
        for k_, v_ in PSX.items():
            assert (' ' + k_ + ' ') in PS
            PS = PS.replace(' ' + k_ + ' ', ' ' + k_ + ' ' + v_ + ' ')
    S_C, S_X, S_SA, S_CA, S_W0, S_WQ, S_WO, S_MB, S_W = 0, 1, 17, 25, 33, 36, 44, 52, 60
    S_P = 64
    NSEM = 68
    DEF = list(range(6 - NDEF, 6))
    tags = ['T%d' % sd for sd in DEF] + ['%dH%d' % (p, sd) for p in range(NP) for sd in range(6 if p < NP - 1 else 6 - NDEF)]
    if side is None:
        side = 'W:7,9,11,13,15,17,19,21 M:4,5,6,7,8,9,10,11,12,13,14,15,16,17,18,19,20,21,22,22'
        if PRE == 'R':
            if SJ is None:
                SJ = ','.join(str(t) for t in (range(4, 23) if S1 else range(8, 23)))
            side += ' S:' + SJ
    if isinstance(side, str):
        sd_ = {}
        for grp in side.split():
            kind, lst = grp.split(':')
            for k, t in enumerate(lst.split(',')):
                sd_.setdefault(tags[int(t)], []).append(kind + str(k))
        side = sd_
    assert sum(1 for v in side.values() for j in v if j[0] in 'Aa') * AP == AT0

    def kernel(*refs):
        pl.run_scoped(functools.partial(body, *refs), pltpu.SemaphoreType.DMA((NSEM,)), pltpu.SemaphoreType.DMA((2,)))

    def body(x_hbm, wqkv_hbm, wo_hbm, w1_hbm, w2_hbm, w3_hbm, w4_hbm, c_hbm, wmod_hbm,
             o_hbm,
             x_v, wqkv_raw, wq_v, wk_v, wv_v, wo_raw, wo_v, w1_v, w2_v, w3_v, w4_v, cE, cO, wmA_v, wmB_v,
             modA, modB, xhat, hP, h0, qbuf, kbuf, vbuf, xmid, hb, h1buf, obuf, o_scr, hsbuf, n4b, n3b, baseb, n4f, a4, ua, macc, n3f, a3, a2, abuf, x1buf, c_v, *rest):
        zsm, sems, osems = rest[-3:]

        def cp(src, dst, k):
            return pltpu.make_async_copy(src, dst, sems.at[k])

        xu = x_hbm.bitcast(u32)
        wqkvu = wqkv_hbm.bitcast(u32)
        wou = wo_hbm.bitcast(u32)
        wmodu = wmod_hbm.bitcast(u32)

        def lane_ds(k, n, base=0):
            if isinstance(k, int):
                return pl.ds(base + k * n, n)
            return pl.ds(pl.multiple_of(base + k * n, 128), n)

        def row_ds(base, k, n):
            if isinstance(k, int):
                return pl.ds(base + k * n, n)
            return pl.ds(pl.multiple_of(base + k * n, 8), n)

        c_c = cp(c_hbm, c_v, S_C)

        def c_x(b):
            return cp(xu.at[b * 64:(b + 1) * 64], x_v.at[b * 64:(b + 1) * 64], S_X + b)

        def c_sa(k):
            return cp(wmodu.at[:, lane_ds(k, 128)], wmA_v.at[k, 0:D // 2, 0:128], S_SA + k)

        def c_ca(k):
            return cp(wmodu.at[:, lane_ds(k, 128, D)], wmA_v.at[k, 0:D // 2, 128:256], S_CA + k)

        def c_w0(b):
            return cp(wqkvu.at[0:64, b * D:(b + 1) * D], wqkv_raw.at[0:64, b * D:(b + 1) * D], S_W0 + b)

        def c_wq(k):
            return cp(wqkvu.at[row_ds(0, k, 64)], wqkv_raw.at[row_ds(0, k, 64)], S_WQ + k)

        def c_wo(p):
            return cp(wou.at[:, lane_ds(p, 128)], wo_raw.at[p, 8:8 + D // 2], S_WO + p)

        def c_mb(t, g):
            return cp(wmodu.at[:, lane_ds(t, 128, 2 * D)], wmB_v.at[t, 0:D // 2], S_MB + g)

        w1u, w2u = w1_hbm.bitcast(u32), w2_hbm.bitcast(u32)
        w3u, w4u = w3_hbm.bitcast(u32), w4_hbm.bitcast(u32)
        N3, N4 = D // 4 // 4, F // 4 // 4
        c_w = []

        def c_p(p):
            def rows(base, n):
                if isinstance(p, int):
                    return pl.ds(base + p * n, n)
                return pl.ds(pl.multiple_of(base + p * n, 8), n)
            return ([cp(w3u.at[rows(a * (D // 4), N3)], w3_v.at[a, rows(0, N3)], S_P + p) for a in range(2)]
                    + [cp(w4u.at[rows(a * (F // 4), N4)], w4_v.at[a, rows(0, N4)], S_P + p) for a in range(2)]
                    + [cp(w1u.at[rows(a * (D // 4), N3)], w1_v.at[a, rows(0, N3)], S_P + p) for a in range(2)]
                    + [cp(w2u.at[rows(a * (D // 4), N3)], w2_v.at[a, rows(0, N3)], S_P + p) for a in range(2)])

        def named(nm):
            if nm == 'c':
                return c_c
            if nm == 'sa':
                return c_sa(0)
            if nm == 'ca':
                return c_ca(0)
            if nm[0] == 'W':
                return c_w0('qkv'.index(nm[1]))
            return c_x(int(nm[1:]))

        for nm in DO.split():
            named(nm).start()
        def start_group(g):
            if g == 'W':
                if upto >= 3:
                    c_wo(7).start()
                    for t in range(6 * NM, 32):
                        c_mb(t, 6).start()
                    for c in c_w:
                        c.start()
            elif g in 'abcd':
                for c in c_p('abcd'.index(g)):
                    c.start()
            elif upto >= 2 and 'nodma2' not in dbg:
                r = int(g)
                c_sa(r).start()
                c_ca(r).start()
                c_wq(r).start()
                c_wo(r - 1).start()
                if r >= 2:
                    for i in range(NM):
                        c_mb(NM * (r - 2) + i, r - 2).start()

        for g in D0:
            start_group(g)
        assert sorted(list(D0) + [it[1] for it in PS.split() if it[0] == 'D'] + list(''.join(DR.values()))) == sorted('1234567Wabcd')

        def _zinit(i, carry):
            zsm[2 + i] = i >> 8
            return carry

        lax.fori_loop(0, 3, _zinit, 0)
        zp3 = pl.multiple_of(zsm[4] * 8, 8)
        zp1 = pl.multiple_of(zsm[2] * 8, 8)
        zp2 = pl.multiple_of(zsm[3] * 8, 8)

        x_v[S // 2:S // 2 + HALO // 2, :] = jnp.zeros((HALO // 2, D), u32)
        for j in range(NCH):
            z = jnp.zeros((HALO, 128), f32)
            qbuf[j, S:S + HALO, :] = z
            kbuf[j, HALO + S:2 * HALO + S, :] = z
            vbuf[j, HALO + S:2 * HALO + S, :] = z
            kbuf[j, 0:HALO, :] = z
            vbuf[j, 0:HALO, :] = z
            wo_raw[j, 0:8, :] = jnp.zeros((8, 128), u32)
            wo_raw[j, 8 + D // 2:16 + D // 2, :] = jnp.zeros((8, 128), u32)

        def mv_part(w, r0, acc):
            n = w.shape[0]
            lo = pltpu.bitcast(w << 16, f32)
            hi = pltpu.bitcast(w & jnp.uint32(0xFFFF0000), f32)
            pr = lo * cE[r0:r0 + n, :] + hi * cO[r0:r0 + n, :]
            for t in range(n // 8):
                acc = pr[8 * t:8 * t + 8] if acc is None else acc + pr[8 * t:8 * t + 8]
            return acc

        wparts = (wq_v, wk_v, wv_v)
        bufs = (qbuf, kbuf, vbuf)

        def exch_groups(grps):
            for g0 in range(0, len(grps), EG):
                gs = grps[g0:g0 + EG]
                XS = [[wqkv_raw[row_ds(rg * 8, k * 8, 8), b * D + a * 128:b * D + (a + 1) * 128] for a in range(NCH)]
                      for (k, b, rg) in gs]
                YS = _exchange8_multi(XS)
                for (k, b, rg), Y in zip(gs, YS):
                    wparts[b][row_ds(rg * 8, 0 if SW else k * 8, 8), :] = jnp.concatenate(Y, axis=1)

        def subdot(lhs, row0, kc, sd, init=False, valid=None):
            b, hf = sd // 2, sd % 2
            n = lhs.shape[0]
            res = _dot(lhs, _bf(wparts[b][row_ds(0, 0 if SW else kc, 64), hf * 512:(hf + 1) * 512]))
            o = row0 + (0 if b == 0 else HALO)
            for jj in range(4):
                j = hf * 4 + jj
                if init:
                    bufs[b][j, o:o + n, :] = res[:, jj * 128:(jj + 1) * 128]
                elif valid is not None:
                    bufs[b][j, o:o + n, :] = jnp.where(valid, bufs[b][j, o:o + n, :], 0.0) + res[:, jj * 128:(jj + 1) * 128]
                else:
                    bufs[b][j, o:o + n, :] += res[:, jj * 128:(jj + 1) * 128]
            return res

        def prologue():
            st = {}

            def crep():
                c = c_v[...].astype(f32)
                scf = (c * jax.nn.sigmoid(c)).astype(bf16).astype(f32)
                rr = lax.broadcasted_iota(jnp.int32, (128, 128), 0)
                ll = lax.broadcasted_iota(jnp.int32, (128, 128), 1)
                sel = ll == jnp.where(rr < 64, 2 * rr, 2 * rr - 127)
                for j in range(NCH):
                    dg = jnp.where(sel, jnp.broadcast_to(scf[:, j * 128:(j + 1) * 128], (128, 128)), 0.0).astype(bf16)
                    rep = _dot(dg, jnp.ones((128, 128), bf16))
                    cE[j * 64:(j + 1) * 64, :] = rep[0:64]
                    cO[j * 64:(j + 1) * 64, :] = rep[64:128]

            def h_store(r0, xh0):
                h = (xh0 * (1.0 + st['ca']) + st['sa']).astype(bf16)
                if r0 < TL:
                    xhat[HS, HO + r0 // 2:HO + (r0 + LP) // 2, :] = pltpu.bitcast(h, f32)
                else:
                    hP[(r0 - TL) // 2:(r0 - TL + LP) // 2, :] = pltpu.bitcast(h, u32)

            def h0_lhs(b0, nb, gated):
                r0 = HO + b0 * 64
                if not gated:
                    return _bf(xhat[HS, r0:r0 + nb * 64, :])
                if GL:
                    return jnp.concatenate([_bf(xhat[HS, r0:r0 + nb * 64 - 8, :]), _bf(xhat[HS, pl.ds(zp3 + r0 + nb * 64 - 8, 8), :])], axis=0)
                return jnp.concatenate([_bf(xhat[HS, pl.ds(zp3 + r0, 8), :]), _bf(xhat[HS, r0 + 8:r0 + nb * 64, :])], axis=0)

            def ln_piece(b, i):
                r0 = b * 128 + i * LP
                direct = 'ca' in st and 'sa' in st
                if MU:
                    x = _bf(x_v[pl.ds(zp1 + r0 // 2, LP // 2), :]).astype(f32)
                    m = jnp.mean(x, axis=-1, keepdims=True)
                    if RL:
                        x = _bf(x_v[pl.ds(zp2 + r0 // 2, LP // 2), :]).astype(f32)
                    xc = x - m
                    rs = lax.rsqrt(jnp.mean(xc * xc, axis=-1, keepdims=True) + EPS)
                    xhat[0, r0:r0 + LP, :] = jnp.broadcast_to(m, (LP, 128))
                    xhat[1, r0:r0 + LP, :] = jnp.broadcast_to(rs, (LP, 128))
                    if direct:
                        h_store(r0, xc[:, 0:128] * rs)
                    return
                if RL:
                    m = jnp.mean(_bf(x_v[pl.ds(zp1 + r0 // 2, LP // 2), :]).astype(f32), axis=-1, keepdims=True)
                    xc = _bf(x_v[pl.ds(zp2 + r0 // 2, LP // 2), :]).astype(f32) - m
                    v = jnp.mean(xc * xc, axis=-1, keepdims=True)
                    xh = (_bf(x_v[r0 // 2:(r0 + LP) // 2, :]).astype(f32) - m) * lax.rsqrt(v + EPS)
                else:
                    xh = _ln(_bf(x_v[pl.ds(zp1 + r0 // 2, LP // 2), :]).astype(f32))
                for j in range(1 if direct else 0, NCH):
                    xhat[j, r0:r0 + LP, :] = xh[:, j * 128:(j + 1) * 128]
                if direct:
                    h_store(r0, xh[:, 0:128])

            def ln_block(b):
                for i in range(128 // LP):
                    ln_piece(b, i)

            def hblk(b):
                for i in range(128 // LP):
                    r0 = b * 128 + i * LP
                    if MU:
                        x = _bf(x_v[r0 // 2:(r0 + LP) // 2, 0:128]).astype(f32)
                        h_store(r0, (x - xhat[0, r0:r0 + LP, :]) * xhat[1, r0:r0 + LP, :])
                    else:
                        h_store(r0, xhat[0, r0:r0 + LP, :])

            for it in PS.split():
                if it[0] == 'w':
                    named(it[1:]).wait()
                elif it[0] == 'D':
                    start_group(it[1])
                elif it == 'C':
                    crep()
                elif it[0] == 'L':
                    ln_block(int(it[1:]))
                elif it[0] == 'h':
                    hblk(int(it[1:]))
                elif it == 'S':
                    st['sa'] = jnp.sum(mv_part(wmA_v[0, 0:D // 2, 0:128], 0, None), axis=0, keepdims=True)
                elif it == 'A':
                    st['ca'] = jnp.sum(mv_part(wmA_v[0, 0:D // 2, 128:256], 0, None), axis=0, keepdims=True)
                elif it[0] == 'e':
                    exch_groups([(0, int(it[1]), rg) for rg in range(8)])
                elif it[0] == 'p':
                    b_, i_ = it[1:].split(':')
                    ln_piece(int(b_), int(i_))
                elif it[0] == 't':
                    x_v[pl.ds(zp3 + S // 2 + HALO // 2, 8), 0:128] = pltpu.bitcast(st['res'][0:8, 0:128], u32)
                elif it[0] in 'sg':
                    blks, sd = it[1:].split(':')
                    b0, nb = int(blks[0], 16), len(blks)
                    st['res'] = subdot(h0_lhs(b0, nb, it[0] == 'g'), b0 * 128, 0, int(sd), True)
                elif it[0] == 'u':
                    blks, parts = it[1:].split(':')
                    b0, nb = int(blks[0], 16), len(blks)
                    lhs = h0_lhs(b0, nb, False)
                    for p in parts:
                        subdot(lhs, b0 * 128, 0, 2 * int(p), True)
                        st['res'] = subdot(lhs, b0 * 128, 0, 2 * int(p) + 1, True)

        if 'P' not in skip:
            prologue()

        def attention(qb, kb, vb, base, off, M, mask_rows, baseh=None):
            row0 = base + off

            def kvds(r, w):
                return pl.ds(base + (off + HALO + r - DIL * w), RB)

            o_rows = []
            for r in range(0, M, RB):
                q = [qb[j, pl.ds(base + (off + r), RB), :] for j in range(NCH)]
                s = []
                for w in range(W):
                    acc = None
                    for j in range(NCH):
                        p = q[j] * kb[j, kvds(r, w), :]
                        acc = p if acc is None else acc + p
                    acc = _group4_sum(acc)
                    if mask_rows and off + r < DIL * (W - 1) and w > 0:
                        rows = row0 + r + lax.broadcasted_iota(jnp.int32, (RB, 128), 0)
                        acc = jnp.where(rows >= DIL * w, acc, -1e30)
                    s.append(acc)
                m = functools.reduce(jnp.maximum, s)
                e = [jnp.exp((sw - m) * SCALE) for sw in s]
                den = functools.reduce(lambda a, b: a + b, e)
                rinv = 1.0 / den
                oc = []
                for j in range(NCH):
                    acc = None
                    for w in range(W):
                        p = e[w] * vb[j, kvds(r, w), :]
                        acc = p if acc is None else acc + p
                    oc.append(acc * rinv)
                o_rows.append(jnp.concatenate(oc, axis=1))
            o = jnp.concatenate(o_rows, axis=0).astype(bf16)
            if isinstance(row0, int):
                o_scr[row0 // 2:(row0 + M) // 2, :] = pltpu.bitcast(o, u32)
            elif baseh is not None:
                o_scr[pl.ds(baseh + off // 2, M // 2), :] = pltpu.bitcast(o, u32)
            else:
                o_scr[pl.ds(pl.multiple_of(row0 // 2, 8), M // 2), :] = pltpu.bitcast(o, u32)


        def attention2(off, M, G, base=None, baseh=None):
            o_rows = []

            def rs_(a):
                return slice(a, a + RB) if base is None else pl.ds(base + a, RB)

            for r0 in range(0, M, RB * G):
                rs = [off + r0 + g * RB for g in range(G) if r0 + g * RB < M]
                lane = lax.broadcasted_iota(jnp.int32, (RB, 128), 1)
                S_ = {}
                for r in rs:
                    q = [qbuf[j, rs_(r), :] for j in range(NCH)]
                    for w in range(W):
                        acc = None
                        for j in range(NCH):
                            k0 = HALO + r - DIL * w
                            p = q[j] * kbuf[j, rs_(k0), :]
                            acc = p if acc is None else acc + p
                        S_[r, w] = acc
                keys = list(S_)
                for sh in (1, 2):
                    R = {k: (pltpu.roll(S_[k], sh, 1), pltpu.roll(S_[k], 128 - sh, 1)) for k in keys}
                    for k in keys:
                        S_[k] = S_[k] + jnp.where((lane & sh) != 0, R[k][0], R[k][1])
                for r in rs:
                    s = []
                    for w in range(W):
                        acc = S_[r, w]
                        if base is None and r < DIL * (W - 1) and w > 0:
                            rows = r + lax.broadcasted_iota(jnp.int32, (RB, 128), 0)
                            acc = jnp.where(rows >= DIL * w, acc, -1e30)
                        s.append(acc)
                    m = functools.reduce(jnp.maximum, s)
                    e = [jnp.exp((sw - m) * SCALE) for sw in s]
                    den = functools.reduce(lambda a, b: a + b, e)
                    rinv = 1.0 / den
                    oc = []
                    for j in range(NCH):
                        acc = None
                        for w in range(W):
                            k0 = HALO + r - DIL * w
                            p = e[w] * vbuf[j, rs_(k0), :]
                            acc = p if acc is None else acc + p
                        oc.append(acc * rinv)
                    o_rows.append(jnp.concatenate(oc, axis=1))
            o = jnp.concatenate(o_rows, axis=0).astype(bf16)
            if base is None:
                o_scr[off // 2:(off + M) // 2, :] = pltpu.bitcast(o, u32)
            else:
                o_scr[pl.ds(baseh + off // 2, M // 2), :] = pltpu.bitcast(o, u32)
            return o

        class Att:
            def __init__(self, base, baseh, off, M, wgs, PD, ztok, QD=None, mask=False, KD=None):
                self.base, self.baseh, self.off, self.PD, self.ztok = base, baseh, off, PD, ztok
                self.KD, self.PP = KD, {}
                self.QD, self.mask = QD, mask
                self.nrb = M // RB
                self.wgs = list(wgs)
                assert sum(self.wgs) == self.nrb * W
                self.Q, self.SS, self.E, self.OC = {}, {}, {}, {}
                self.win = 0
                self.done = 0

            def scores(self, wl):
                lane = lax.broadcasted_iota(jnp.int32, (RB, 128), 1)
                accs = []
                if self.KD is not None:
                    n0 = wl[0][0] * W + wl[0][1] - self.KD[1]
                    if n0 >= 0:
                        kbuf[0, pl.ds(self.ztok + S + 2 * HALO, 8), :] = (self.PP if self.KD[0] == 0 else self.SS)[divmod(n0, W)]
                for (rb, w) in wl:
                    r = self.off + rb * RB
                    if rb not in self.Q:
                        if self.QD is not None and rb * W - self.QD >= 0:
                            qbuf[0, pl.ds(self.ztok + S + HALO, 8), :] = self.SS[divmod(rb * W - self.QD, W)]
                        self.Q[rb] = [qbuf[j, pl.ds(self.base + r, RB), :] for j in range(NCH)]
                    acc = None
                    for j in range(NCH):
                        p = self.Q[rb][j] * kbuf[j, pl.ds(self.base + (HALO + r - DIL * w), RB), :]
                        acc = p if acc is None else acc + p
                    accs.append(acc)
                for sh in (1, 2):
                    R = [(pltpu.roll(a, sh, 1), pltpu.roll(a, 128 - sh, 1)) for a in accs]
                    accs = [a + jnp.where((lane & sh) != 0, x, y) for a, (x, y) in zip(accs, R)]
                    if sh == 1:
                        for k, a in zip(wl, accs):
                            self.PP[k] = a
                for k, a in zip(wl, accs):
                    r = self.off + k[0] * RB
                    if self.mask and r < DIL * (W - 1) and k[1] > 0:
                        rows = r + lax.broadcasted_iota(jnp.int32, (RB, 128), 0)
                        a = jnp.where(rows >= DIL * k[1], a, -1e30)
                    self.SS[k] = a
                    if k[1] == W - 1:
                        self.softmax(k[0])

            def softmax(self, rb):
                s = [self.SS[rb, w] for w in range(W)]
                m = functools.reduce(jnp.maximum, s)
                e = [jnp.exp((sw - m) * SCALE) for sw in s]
                den = functools.reduce(lambda a, b: a + b, e)
                self.E[rb] = (e, 1.0 / den)

            def pv(self):
                rb, j = divmod(self.done, NCH)
                self.done += 1
                r = self.off + rb * RB
                e, rinv = self.E[rb]
                acc = None
                for w in range(W):
                    p = e[w] * vbuf[j, pl.ds(self.base + (HALO + r - DIL * w), RB), :]
                    acc = p if acc is None else acc + p
                self.OC[rb, j] = acc * rinv
                if rb % 2 == 1 and j == NCH - 1:
                    o = jnp.concatenate([jnp.concatenate([self.OC[q, c] for c in range(NCH)], axis=1) for q in (rb - 1, rb)], axis=0)
                    o_scr[pl.ds(self.baseh + (self.off + (rb - 1) * RB) // 2, RB), :] = pltpu.bitcast(o.astype(bf16), u32)

            def token(self, v):
                vbuf[0, pl.ds(self.ztok + S + 2 * HALO, 8), :] = v

            def steps(self, n, pvmax=None):
                for _ in range(n):
                    if not self.wgs:
                        return
                    g = self.wgs.pop(0)
                    wl = [divmod(self.win + t, W) for t in range(g)]
                    self.win += g
                    self.scores(wl)
                    tok = False
                    npv = 0
                    while self.done < self.nrb * NCH and self.done + W + self.PD <= self.win - 1 and self.done // NCH in self.E:
                        if pvmax is not None and npv >= pvmax:
                            break
                        npv += 1
                        if not tok:
                            self.token(self.SS[wl[-1]])
                            tok = True
                        self.pv()

            def rest(self, n=999):
                while self.done < self.nrb * NCH and n > 0:
                    self.pv(); n -= 1

        sub = lax.broadcasted_iota(jnp.int32, (8, 128), 0)

        def pW(p, q, z):
            for tv in range(8 * q, 8 * q + 8):
                j = tv >> 3
                hh = (tv >> 1) & 3
                a2 = tv & 1
                parts = []
                for al in range(4):
                    a = a2 * 4 + al
                    src = a * 64 + hh * 16 + j * 2
                    st = src - 2 * al + 8
                    if isinstance(z, int):
                        parts.append(wo_raw[p, z + st:z + st + 8, :])
                    else:
                        parts.append(wo_raw[p, pl.ds(z + st, 8), :])
                v = jnp.where(sub < 2, parts[0], parts[1])
                v2 = jnp.where(sub < 6, parts[2], parts[3])
                wo_v[p, 8 * tv:8 * tv + 8, :] = jnp.where(sub < 4, v, v2)

        def pM(t, kq, z, macc, key):
            n = D // 2 // KQ
            rows = pl.ds(z + kq * n, n)
            macc[key] = mv_part(wmB_v[t, rows, :], kq * n, macc.get(key))
            if kq == KQ - 1:
                modB[t, 0:1, :] = jnp.sum(macc[key], axis=0, keepdims=True)

        FH, DH2, HM = F // 2, D // 2, T // 2
        SLOT = {0: (2, 0), 1: (0, 0), 2: (0, 1), 3: (1, 0), 4: (1, 1), 5: (2, 1), 6: (3, 0)}
        SLOT5 = {0: (2, 0), 1: (0, 0), 2: (3, 1), 3: (4, 0), 4: (1, 1), 5: (2, 1), 6: (3, 0)}

        def bsums(W, NH, rl, rs_, n, c0, cw, five=False):
            w = {(a, b): W[a, pl.ds(rl, n), b * NH + c0:b * NH + c0 + cw] for a in range(2) for b in range(2)}
            res = {}
            for h in range(2):
                e = {k: pltpu.unpack_elementwise(v, index=h, packed_dtype=bf16, unpacked_dtype=f32) for k, v in w.items()}
                b11, b12, b21, b22 = e[0, 0], e[0, 1], e[1, 0], e[1, 1]
                sl = SLOT5 if five else SLOT
                for k, o in ((0, b11 + b22), (2, b12 - b22), (3, b21 - b11), (5, b11 + b12), (6, b21 + b22)):
                    res.setdefault(sl[k], []).append(o)
            for (a, b), o in res.items():
                W[a, pl.ds(rs_, n), b * NH + c0:b * NH + c0 + cw] = pltpu.bitcast(pltpu.pack_elementwise(o, packed_dtype=bf16), u32)

        NS3, NS4 = N3 // 8, N4 // 32

        def s_ref(k):
            return w3_v if k < NS3 else w4_v if k < NS3 + NS4 else w1_v if k < NS3 + NS4 + 2 else w2_v

        def s_links(k, r, z):
            links = []
            W = s_ref(k)
            if k < NS3:
                r0 = jnp.where(r >= P0R, (r - P0R) * N3 + 8 * k, D // 4) + z
                for c in range(FH // 128):
                    links.append(functools.partial(bsums, W, FH, pl.multiple_of(r0, 8), pl.multiple_of(r0, 8), 8, c * 128, 128))
            elif k < NS3 + NS4:
                k -= NS3
                r0 = jnp.where(r >= P0R, (r - P0R) * N4 + 32 * k, F // 4) + z
                for t in range(4):
                    for c in range(DH2 // 128):
                        links.append(functools.partial(bsums, W, DH2, pl.multiple_of(r0 + 8 * t, 8), pl.multiple_of(r0 + 8 * t, 8), 8, c * 128, 128))
            else:
                k = (k - NS3 - NS4) % 2
                r0 = jnp.where(r >= P0R, (r - P0R) * N3 + 32 * k, D // 4) + z
                for t in range(4):
                    for c in range(DH2 // 128):
                        links.append(functools.partial(bsums, W, DH2, pl.multiple_of(r0 + 8 * t, 8), pl.multiple_of(r0 + 8 * t, 8), 8, c * 128, 128, True))
            return links

        def region_waits(r):
            c_sa(r).wait(); c_ca(r).wait(); c_wq(r).wait()
            if not WS:
                c_wo(r - 1).wait()

            @pl.when(r >= 2)
            def _():
                if WS:
                    c_wo(r - 2).wait()
                for i in range(NM):
                    c_mb(NM * (r - 2) + i, r - 2).wait()

            @pl.when(r >= P0R)
            def _():
                for c in c_p(r - P0R):
                    c.wait()

            for r_, gs_ in DR.items():
                @pl.when(r == r_)
                def _(gs_=gs_):
                    for g_ in gs_:
                        start_group(g_)

        if 'prewait' in dbg:
            for r in range(1, 8):
                region_waits(r)

        def region(r, carry):
            if 'prewait' not in dbg and 'nodma2' not in dbg:
                region_waits(r)
            z1 = pl.multiple_of((r >> 8) * 8, 8)
            z2 = pl.multiple_of((r >> 9) * 8, 8)
            pm = [jnp.where(r >= 2, NM * (r - 2) + i, 32) for i in range(NM)]
            pw = jnp.where(r >= 2, r - 2, NCH) if WS else r - 1
            hp = _bf(hP[...])
            st = {'acc': [None, None], 'res': None}
            macc_ = {}

            def mvp(kq):
                n = D // 2 // KQ0
                for q in range(2):
                    st['acc'][q] = mv_part(wmA_v[r, pl.ds(z2 + kq * n, n), q * 128:(q + 1) * 128], kq * n, st['acc'][q])
                if kq == KQ0 - 1:
                    st['sa'] = jnp.sum(st['acc'][0], axis=0, keepdims=True)
                    st['ca'] = jnp.sum(st['acc'][1], axis=0, keepdims=True)
                    modA[r, 0:1, 0:128] = st['sa']
                    modA[r, 0:1, 128:256] = st['ca']

            def hpass(p):
                if MU:
                    x = _bf(x_v[p * PR // 2:(p + 1) * PR // 2, lane_ds(r, 128)]).astype(f32)
                    xh = (x - xhat[0, p * PR:(p + 1) * PR, :]) * xhat[1, p * PR:(p + 1) * PR, :]
                else:
                    xh = xhat[r, p * PR:(p + 1) * PR, :]
                st['h'] = (xh * (1.0 + st['ca']) + st['sa']).astype(bf16)
                st['row'] = p * PR
                if p == NP - 1:
                    hP[...] = pltpu.bitcast(st['h'], u32)

            def do_side(tag):
                prev, st['prev'] = st.get('prev'), st['res']
                jobs = side.get(tag, ())
                if not jobs:
                    return
                tkr = lambda row: pltpu.bitcast(st['res'][row:row + 8, 0:128], u32)
                sj = [int(j[1:]) for j in jobs if j[0] == 'S']
                def sjobs():
                    links = [(k, l) for k in sj for l in s_links(k, r, z1)]
                    for n, (k, l) in enumerate(links):
                        row = (TKS + n * TD // len(links)) // 8 * 8
                        W = s_ref(k)
                        W[0, pl.ds(z1 + (F // 4 if W is w4_v else D // 4), 8), 0:128] = tkr(row)
                        l()
                tk = tkr(0)
                kinds = set(j[0] for j in jobs)
                if 'W' in kinds:
                    wo_raw[pw, pl.ds(z1 + D // 2 + 16, 8), :] = tkr(TKW)
                if 'M' in kinds:
                    wmB_v[32, pl.ds(z1 + D // 2, 8), :] = tkr(TKM)
                if 'A' in kinds:
                    qbuf[0, pl.ds(z1 + S + HALO, 8), :] = pltpu.bitcast(tk, f32)
                for j in jobs:
                    k = int(j[1:])
                    if j[0] == 'W':
                        pW(pw, k, z2)
                    elif j[0] == 'w':
                        pW(pw, k, 0)
                    elif j[0] == 'M':
                        pM(pm[k // KQ], k % KQ, z2, macc_, k // KQ)
                    elif j[0] in 'Aa':
                        attention(qbuf, kbuf, vbuf, 0, k * AP, AP, True)
                if sj:
                    sjobs()

            for it in order0:
                if it[0] == 'T':
                    st['res'] = subdot(hp, TL, r - 1, int(it[1]), valid=r >= 2)
                    do_side(it)
                elif it[0] == 'H':
                    st['res'] = subdot(st['h'], st['row'], r, int(it[1]))
                    do_side('0' + it)
                elif it[0] == 'm':
                    mvp(int(it[1]))
                elif it[0] == 'K':
                    q = int(it[1:] or 0) * 128
                    wmA_v[r, pl.ds(z1 + D // 2, 8), 0:128] = pltpu.bitcast(st['res'][q:q + 8, 0:128], u32)
                elif it[0] == 'X':
                    q = int(it[1:] or 0) * 128
                    wqkv_raw[pl.ds(z1 + D // 2, 8), 0:128] = pltpu.bitcast(st['res'][q:q + 8, 0:128], u32)
                elif it[0] == 'h':
                    hpass(int(it[1]))
                elif it[0] == 'y':
                    b, qf = int(it[1]), int(it[2])
                    exch_groups([(r, b, rg) for rg in range(2 * qf, 2 * qf + 2)])
                elif it[0] == 'x':
                    b, hf = int(it[1]), int(it[2])
                    exch_groups([(r, b, rg) for rg in range(4 * hf, 4 * hf + 4)])
            for p in range(1, NP):
                hpass(p)
                for sd in range(6 if p < NP - 1 else 6 - NDEF):
                    st['res'] = subdot(st['h'], st['row'], r, sd)
                    do_side('%dH%d' % (p, sd))
            zsm[0] = r >> 8
            zsm[1] = r >> 9
            return carry

        if upto >= 2:
            if 'R' not in skip:
                lax.fori_loop(1, NR, region, 0)
            zero = zsm[0]
            zero2 = zsm[1]

        if WS and upto >= 2:
            c_wo(6).wait()
        if upto >= 3:
            c_wo(7).wait()
            for t in range(6 * NM, 32):
                c_mb(t, 6).wait()
            for c in c_w:
                c.wait()

        def rows_u32(ref, row0, M):
            if isinstance(row0, int):
                return _bf(ref[row0 // 2:(row0 + M) // 2, :])
            if isinstance(row0, tuple):
                return _bf(ref[pl.ds(row0[0] + row0[1] // 2, M // 2), :])
            return _bf(ref[pl.ds(pl.multiple_of(row0 // 2, 8), M // 2), :])

        def wo_dot(row0, M):
            o = rows_u32(o_scr, row0, M)
            return jnp.concatenate([_dot(o, _bf(wo_v[n])) for n in range(NCH)], axis=1)

        def row(k):
            return jnp.concatenate([modB[8 * (k - 2) + j, 0:1, :] for j in range(NCH)], axis=1)

        def ln23(row0, M, A):
            ga = row(2); sb = row(3); cb = row(4)
            x = rows_u32(x_v, row0, M).astype(f32)
            xm = x + ga * A
            hB = _ln(xm) * (1.0 + cb) + sb
            n3 = _ln(hB).astype(bf16)
            return xm, hB, n3

        shifts = [-1, -1, 1, 1, -2, -2, 2, 2]

        def g_val():
            return jnp.concatenate(
                [h1buf[j, HALO + shifts[j]:HALO + shifts[j] + T, :] for j in range(NCH)], axis=1).astype(bf16)

        def out_copy(r0, n, k, c0=0, cw=D):
            if cw == D:
                return pltpu.make_async_copy(obuf.at[pl.ds(r0, n)], o_hbm.bitcast(u32).at[pl.ds(r0, n)], osems.at[k])
            return pltpu.make_async_copy(obuf.at[pl.ds(r0, n), c0:c0 + cw], o_hbm.bitcast(u32).at[pl.ds(r0, n), c0:c0 + cw], osems.at[k])

        def ln4(hs):
            gb = row(5)
            x1 = hb[0:T, :] + hs
            base = xmid[0:T, :] + gb * x1
            n4 = _ln(x1).astype(bf16)
            return base, n4

        def asums(a11, a12, a21, a22):
            return [a11 + a22, a21 + a22, a11, a22, a11 + a12, a21 - a11, a12 - a22]

        def w3op(k, c0, cw):
            a, b = SLOT[k]
            c0 = c0 + b * FH
            return _bf(w3_v[a, 0:D // 4, pl.ds(c0, cw) if not isinstance(c0, int) else slice(c0, c0 + cw)])

        def w4op(k, c0, cw, r0=0, nr=F // 4, z=None):
            a, b = SLOT[k]
            if z is not None:
                r0 = z + r0
            return _bf(w4_v[a, pl.ds(r0, nr) if not isinstance(r0, int) else slice(r0, r0 + nr), b * DH2 + c0:b * DH2 + c0 + cw])

        def strass(dotk, hook=None):
            M = dotk(0); c11 = M; c22 = M
            if hook: hook(0, M)
            M = dotk(1); c21 = M; c22 = c22 - M
            if hook: hook(1, M)
            M = dotk(2); c12 = M; c22 = c22 + M
            if hook: hook(2, M)
            M = dotk(3); c11 = c11 + M; c21 = c21 + M
            if hook: hook(3, M)
            M = dotk(4); c11 = c11 - M; c12 = c12 + M
            if hook: hook(4, M)
            M = dotk(5); c22 = c22 + M
            if hook: hook(5, M)
            M = dotk(6); c11 = c11 + M
            if hook: hook(6, M)
            return c11, c12, c21, c22

        def n_sums(r, nv, stg, dst):
            q = T // RP0 // 2
            if r < q:
                stg[r * RP0:(r + 1) * RP0, :] = nv
            else:
                top = stg[(r - q) * RP0:(r - q + 1) * RP0, :]
                A = asums(top[:, :DH2], top[:, DH2:], nv[:, :DH2], nv[:, DH2:])
                for k in range(7):
                    dst[k, (r - q) * RP0:(r - q + 1) * RP0, :] = A[k].astype(bf16)

        def n4_sums(r, n4v):
            n_sums(r, n4v, n4f, a4)

        def w12op(W, k, c0, cw, z=None):
            a, b = SLOT5[k]
            if z is not None:
                return _bf(W[a, pl.ds(z, D // 4), b * DH2 + c0:b * DH2 + c0 + cw])
            return _bf(W[a, 0:D // 4, b * DH2 + c0:b * DH2 + c0 + cw])

        def raw_dot(x, W):
            return _dot(x[:, :DH2], _bf(W[0, 0:D // 4, :])) + _dot(x[:, DH2:], _bf(W[1, 0:D // 4, :]))

        def g_sums(j, q, z):
            def ld(jj, r0):
                r0 = HALO + shifts[jj] + r0
                return h1buf[jj, r0:r0 + RP0, :] if z is None else h1buf[jj, pl.ds(z + r0, RP0), :]
            A = asums(ld(j, q * RP0), ld(j + 4, q * RP0), ld(j, HM + q * RP0), ld(j + 4, HM + q * RP0))
            for k in range(7):
                a2[k, q * RP0:(q + 1) * RP0, j * 128:(j + 1) * 128] = A[k].astype(bf16)

        def stage3(c0, cw, uc0, hook=None):
            U = strass(lambda k: _dot(a4[k], w3op(k, c0, cw)), hook)
            A = asums(*[_gelu(x) for x in U])
            for k in range(7):
                ua[k, :, uc0:uc0 + cw] = A[k].astype(bf16)

        RP0 = 16

        def bfirst():
            for j in range(NCH):
                h1buf[j, 0:HALO, :] = jnp.zeros((HALO, 128), f32)
            h7 = _bf(hP[...])
            zb = pl.multiple_of(zero * 8, 8) if ZB else 0
            h0 = (T + HALO) // 2 // 16 * 16 + (16 if T == 128 else 0)
            halves = [(0, h0), (h0, T + HALO - h0)]
            nA = (2 * T + HALO - AT0) // AP
            st = {'res': None, 'As': [], 'n3': [], 'h1': [], 'macc': {}}

            def att(k):
                if AG:
                    st['o'] = attention2(AT0 + k * AP, AP, AG)
                else:
                    attention(qbuf, kbuf, vbuf, 0, AT0 + k * AP, AP, True)

            def tok_q(cc=0):
                qbuf[0, pl.ds(zb + S + HALO, 8), :] = st['res'][0:8, cc * 128:(cc + 1) * 128]

            batt = None
            if 'A' in BA:
                batt = Att(0, 0, 0, 2 * T + HALO, [BWG] * ((2 * T + HALO) // RB * W // BWG), BPD, zb, BQD, True)
            for it in BA.split():
                k = int(it[1:]) if len(it) > 1 and it[1:].isdigit() else None
                if not ZB and it[0] in 'tWM':
                    continue
                if it[0] == 'A':
                    batt.steps(k)
                elif it[0] == 'R':
                    batt.steps(999)
                    batt.rest()
                elif it[0] == 'T':
                    st['res'] = subdot(h7, TL, 7, k)
                elif it[0] == 'a':
                    att(k)
                elif it[0] == 't':
                    tok_q(k or 0)
                elif it[0] == 'w':
                    pW(7, k, zb)
                elif it[0] == 'v':
                    pW(6, k, zb)
                elif it[0] == 'm':
                    for kq in range(KQ):
                        pM(6 * NM + k, kq, zb, st['macc'], k)
                elif it[0] == 'M':
                    wmB_v[32, pl.ds(zb + D // 2, 8), :] = pltpu.bitcast(st['res'][0:8, 0:128], u32)
                elif it[0] == 'W':
                    wo_raw[7, pl.ds(zb + D // 2 + 16, 8), :] = pltpu.bitcast(st['res'][0:8, 0:128], u32)
                elif it[0] == 'o':
                    assert batt is None or batt.done >= (halves[k][0] + halves[k][1]) // RB * NCH, batt.done
                    st['res'] = wo_dot(*halves[k])
                    st['As'].append(st['res'])
                elif it[0] == 'l':
                    r0, m = halves[k]
                    xm, hB, n3 = ln23(r0, m, st['As'][k])
                    xmid[r0:r0 + m, :] = xm
                    hb[r0:r0 + m, :] = hB
                    st['n3'].append(n3)
                elif it[0] == 'u':
                    r0, m = halves[k]
                    st['res'] = raw_dot(st['n3'][k], w1_v)
                    h1 = _gelu(st['res'])
                    for j in range(NCH):
                        h1buf[j, HALO + r0:HALO + r0 + m, :] = h1[:, j * 128:(j + 1) * 128]
                elif it[0] == 'z':
                    if 'g' not in st:
                        st['g'] = g_val()
                    cw_ = D // NZ
                    st['res'] = _dot(st['g'], _bf(w2_v[:, k * cw_:(k + 1) * cw_]))
                    hsbuf[0:T, k * cw_:(k + 1) * cw_] = st['res']
                elif it[0] == 'U':
                    hh, pp = divmod(k, 10)
                    r0, m = halves[hh]
                    cw_ = D // NU
                    st['res'] = _dot(st['n3'][hh], _bf(w1_v[:, pp * cw_:(pp + 1) * cw_]))
                    h1 = _gelu(st['res'])
                    for j in range(cw_ // 128):
                        h1buf[pp * (cw_ // 128) + j, HALO + r0:HALO + r0 + m, :] = h1[:, j * 128:(j + 1) * 128]
            if 'g' not in st:
                hsbuf[0:T, :] = raw_dot(g_val(), w2_v)

        if upto >= 3 and 'F' not in skip:
            bfirst()

        def carries(xm, hB, h1, notlast):
            xmid[0:HALO, :] = xmid[T:T + HALO, :]
            hb[0:HALO, :] = hb[T:T + HALO, :]
            for j in range(NCH):
                h1buf[j, 0:2 * HALO, :] = h1buf[j, T:T + 2 * HALO, :]
            xmid[HALO:HALO + T, :] = xm
            hb[HALO:HALO + T, :] = hB
            for j in range(NCH if h1 is not None else 0):
                h1j = h1[:, j * 128:(j + 1) * 128]
                h1buf[j, 2 * HALO:HALO + T, :] = h1j[0:T - HALO]
                h1buf[j, HALO + T:2 * HALO + T, :] = jnp.where(notlast, h1j[T - HALO:T], 0.0)

        RP = 16

        def bbody(i, carry):
            static = isinstance(i, int)
            if static:
                row0h = i * (T // 2)
                abase = (i + 1) * T
                abaseh = (i + 1) * (T // 2)
                z1 = pl.multiple_of(zero * 8, 8)
                z2 = pl.multiple_of(zero2 * 8, 8)
            else:
                row0h = pl.multiple_of(i * (T // 2), T // 2)
                nxt = jnp.minimum(i + 1, NT - 1)
                abase = pl.multiple_of(nxt * T, T)
                abaseh = pl.multiple_of(nxt * (T // 2), T // 2)
                z1 = pl.multiple_of((i >> 8) * 8, 8)
                z2 = pl.multiple_of((i >> 9) * 8, 8)
            ga = row(2); sb = row(3); cb = row(4); gb = row(5)
            bases, n4p, xms, hBs, n3p, As = [], [], {}, {}, [], []
            att = None
            asch = {}
            if AB == 9:
                att = Att(abase, abaseh, HALO, T, [int(t) for t in WGS], PD, z1, KD=KD)
                for t in ASCH.split():
                    k_, v_ = t.split(':')
                    asch[k_] = int(v_)

            def astep(tag):
                if att is not None and tag in asch:
                    att.steps(asch[tag])

            def p4(r):
                r0 = r * RP
                x1 = hb[r0:r0 + RP, :] + hsbuf[pl.ds(z2 + r0, RP), :]
                if ST and RL4:
                    bases.append((r, xmid[r0:r0 + RP, :] + gb * x1))
                    m = jnp.mean(x1, axis=-1, keepdims=True)
                    x1buf[r0:r0 + RP, :] = x1
                    rd = lambda z: x1buf[r0:r0 + RP, :] if RL4 == 1 else x1buf[pl.ds(z + r0, RP), :]
                    xc = rd(z1) - m
                    rs = lax.rsqrt(jnp.mean(xc * xc, axis=-1, keepdims=True) + EPS)
                    n4_sums(r, (rd(z2) - m) * rs)
                    n4p.append(None)
                    return
                if ST:
                    bases.append((r, xmid[r0:r0 + RP, :] + gb * x1))
                    n4_sums(r, _ln(x1))
                    n4p.append(None)
                    return
                bases.append(xmid[r0:r0 + RP, :] + gb * x1)
                n4v = _ln(x1).astype(bf16)
                if EX4:
                    n4b[r0 // 2:(r0 + RP) // 2, :] = pltpu.bitcast(n4v, u32)
                n4p.append(n4v)

            chain = []

            def p23(r, A):
                r0 = r * RP
                if LC and len(chain) >= LC:
                    abuf[pl.ds(z1 + T, 8), 0:128] = chain[len(chain) - LC]
                    x_v[pl.ds(z1 + S // 2 + HALO // 2, 8), 0:128] = pltpu.bitcast(chain[len(chain) - LC], u32)
                x = rows_u32(x_v, (row0h, HALO + r0), RP).astype(f32)
                xm = x + ga * (abuf[pl.ds(z2 + r0, RP), :] if EA else A[r0:r0 + RP])
                if RL3:
                    def rd(ref, z):
                        return ref[HALO + r0:HALO + r0 + RP, :] if RL3 == 1 else ref[pl.ds(z + HALO + r0, RP), :]
                    xmid[HALO + r0:HALO + r0 + RP, :] = xm
                    m = jnp.mean(xm, axis=-1, keepdims=True)
                    xc = rd(xmid, z1) - m
                    rs = lax.rsqrt(jnp.mean(xc * xc, axis=-1, keepdims=True) + EPS)
                    hB = (rd(xmid, z2) - m) * rs * (1.0 + cb) + sb
                    hb[HALO + r0:HALO + r0 + RP, :] = hB
                    m = jnp.mean(hB, axis=-1, keepdims=True)
                    xc = rd(hb, z1) - m
                    rs = lax.rsqrt(jnp.mean(xc * xc, axis=-1, keepdims=True) + EPS)
                    n3v = (rd(hb, z2) - m) * rs
                    n_sums(r, n3v, n3f, a3)
                    n3p.append(None)
                    chain.append(n3v[0:8, 0:128])
                    return
                hB = _ln(xm) * (1.0 + cb) + sb
                xms[r] = xm; hBs[r] = hB
                if S1:
                    n_sums(r, _ln(hB), n3f, a3)
                    n3p.append(None)
                    return
                n3v = _ln(hB).astype(bf16)
                n3b[r0 // 2:(r0 + RP) // 2, :] = pltpu.bitcast(n3v, u32)
                n3p.append(n3v)

            def p23_stages(r):
                r0 = r * RP
                rows = slice(HALO + r0, HALO + r0 + RP)
                v = {}

                def sa():
                    x = rows_u32(x_v, (row0h, HALO + r0), RP).astype(f32)
                    xm = x + ga * abuf[pl.ds(z2 + r0, RP), :]
                    xmid[rows, :] = xm
                    v['m'] = jnp.mean(xm, axis=-1, keepdims=True)

                def sb_():
                    xc = xmid[rows, :] - v['m']
                    v['rs'] = lax.rsqrt(jnp.mean(xc * xc, axis=-1, keepdims=True) + EPS)

                def sc():
                    hB = (xmid[rows, :] - v['m']) * v['rs'] * (1.0 + cb) + sb
                    hb[rows, :] = hB
                    v['m2'] = jnp.mean(hB, axis=-1, keepdims=True)

                def sd():
                    xc = hb[rows, :] - v['m2']
                    v['rs2'] = lax.rsqrt(jnp.mean(xc * xc, axis=-1, keepdims=True) + EPS)

                def se():
                    n_sums(r, (hb[rows, :] - v['m2']) * v['rs2'], n3f, a3)
                    n3p.append(None)
                return [sa, sb_, sc, sd, se]

            ord4 = list(ORD4) if ST else list(range(T // RP))
            for r in range(T // RP):
                if rel4[r] < 0:
                    p4(ord4[r])
            o = rows_u32(o_scr, (row0h, HALO), T)
            for n in range(NCH):
                An = _dot(o, _bf(wo_v[n]))
                As.append(An)
                if EA:
                    abuf[0:T, n * 128:(n + 1) * 128] = An
                r4 = [r for r in range(T // RP) if rel4[r] == n]
                if r4:
                    hsbuf[pl.ds(z1 + T, 8), 0:128] = An[0:8, 0:128]
                for r in r4:
                    p4(ord4[r])
                astep('o%d' % n)
                if AWO and att is not None:
                    att.steps(AWO)
            A = jnp.concatenate(As, axis=1)
            if RL3:
                xmid[0:HALO, :] = xmid[T:T + HALO, :]
                hb[0:HALO, :] = hb[T:T + HALO, :]
            if ST:
                stg = {}
                base = jnp.concatenate([b for _, b in sorted(bases, key=lambda t: t[0])], axis=0)
                for c in range(FH // CW3):
                    def hook(k, M, c=c):
                        r23 = [r for r in range(T // RP) if R23[r] == 7 * c + k]
                        if r23:
                            x_v[pl.ds(z1 + S // 2 + HALO // 2, 8), 0:128] = pltpu.bitcast(M[0:8, 0:128], u32)
                            if EA:
                                abuf[pl.ds(z1 + T, 8), 0:128] = M[0:8, 0:128]
                        if SP3:
                            for r in range(T // RP):
                                d_ = 7 * c + k - R23[r]
                                if d_ == 0:
                                    stg[r] = p23_stages(R3O[r])
                                if d_ >= 0 and d_ % SP3 == 0 and d_ // SP3 < 5:
                                    stg[r][d_ // SP3]()
                        for r in r23:
                            if GA and GA[r] and att is not None:
                                w0_ = att.win
                                att.steps(GA[r], PVG)
                                tv_ = functools.reduce(lambda a_, b_: a_ + b_, [att.SS[divmod(w_, W)] for w_ in range(w0_, att.win)])
                                x_v[pl.ds(z1 + S // 2 + HALO // 2, 8), 0:128] = pltpu.bitcast(tv_, u32)
                                if EA:
                                    abuf[pl.ds(z1 + T, 8), 0:128] = tv_
                            if not SP3:
                                p23(R3O[r] if S1 else r, A)
                        t = 7 * c + k
                        if t == TW4:
                            w4_v[0, pl.ds(z1 + F // 4, 8), 0:128] = pltpu.bitcast(M[0:8, 0:128], u32)
                        if t == TW1:
                            w1_v[0, pl.ds(z1 + D // 4, 8), 0:128] = pltpu.bitcast(M[0:8, 0:128], u32)
                        if AP3 and att is not None and t >= AO3 and (t - AO3) % AP3 == 0:
                            att.steps(1)
                    stage3(c * CW3, CW3, c * CW3, hook)
            else:
                base = jnp.concatenate(bases, axis=0)
                n4 = _bf(n4b[...]) if EX4 else jnp.concatenate(n4p, axis=0)
                U = _dot(n4, _bf(w3_v[...]))
                u = _gelu(U).astype(bf16)
            for c in range(0 if ST else F // 128):
                r23 = [r for r in range(T // RP) if rel23[r] == NCH + c]
                if r23 or c in XT:
                    x_v[pl.ds(z1 + S // 2 + HALO // 2, 8), 0:128] = pltpu.bitcast(U[0:8, c * 128:(c + 1) * 128], u32)
                for r in r23:
                    p23(r, A)
                astep('c%d' % c)
            assert len(n3p) == T // RP and len(n4p) == T // RP
            if S1:
                if not RL3:
                    xm = jnp.concatenate([xms[r] for r in range(T // RP)], axis=0)
                    hB = jnp.concatenate([hBs[r] for r in range(T // RP)], axis=0)
                    carries(xm, hB, None, None)
                else:
                    for j in range(NCH):
                        h1buf[j, 0:2 * HALO, :] = h1buf[j, T:T + 2 * HALO, :]
                for c in range(DH2 // 128):
                    def hook1(k, M, c=c):
                        if AP1 and att is not None and (7 * c + k) % AP1 == 0:
                            att.steps(1)
                    U = strass(lambda k: _dot(a3[k], w12op(w1_v, k, c * 128, 128, None if TW1 is None else z2)), hook1)
                    for q, Uq in enumerate(U):
                        j, r0 = (q % 2) * 4 + c, 2 * HALO + (q // 2) * HM
                        hq = _gelu(Uq)
                        if q // 2:
                            h1buf[j, r0:r0 + HM - HALO, :] = hq[0:HM - HALO]
                            h1buf[j, r0 + HM - HALO:r0 + HM, :] = jnp.where(i < NT - 1, hq[HM - HALO:HM], 0.0)
                        else:
                            h1buf[j, r0:r0 + HM, :] = hq
            else:
                xm = jnp.concatenate([xms[r] for r in range(T // RP)], axis=0)
                hB = jnp.concatenate([hBs[r] for r in range(T // RP)], axis=0)
                h1 = _gelu(raw_dot(_bf(n3b[...]), w1_v))
                carries(xm, hB, h1, i < NT - 1)
            if static:
                if i < NT - 1:
                    attention(qbuf, kbuf, vbuf, abase, HALO, T, False, abaseh)
            elif 'noatt' not in dbg and not AP4:
                if AB == 9:
                    att.steps(999, PVM)
                    att.rest()
                    if DL:
                        h1buf[0, pl.ds(z1 + T + 2 * HALO, 8), :] = att.OC[T // RB - 1, NCH - 1]
                elif AB:
                    attention2(HALO, T, AB, abase, abaseh)
                else:
                    attention(qbuf, kbuf, vbuf, abase, HALO, T, False, abaseh)
            if ST:
                ro = pl.multiple_of((i - 1) * (T // 2), T // 2)
                gdone = []
                for c in range(DH2 // CW4):
                    c0 = c * CW4

                    def hook4(k, M, c=c):
                        if AP4 and att is not None:
                            att.steps(AP4)
                        if 7 * c + k == TW2:
                            w2_v[0, pl.ds(z1 + D // 4, 8), 0:128] = pltpu.bitcast(M[0:8, 0:128], u32)
                        if not S1 or GT is None:
                            return
                        for n, t in enumerate(GT):
                            if t == 7 * c + k:
                                h1buf[0, pl.ds(z1 + T + 2 * HALO, 8), :] = M[0:8, 0:128]
                                g_sums(n // 4, n % 4, z2)
                                gdone.append(n)
                    Hs = strass(lambda k: _dot(ua[k], w4op(k, c0, CW4, z=None if TW4 is None else z2)), hook4)
                    for q, Hq in enumerate(Hs):
                        rr, cc = (q // 2) * HM, (q % 2) * DH2 + c0
                        o_ = base[rr:rr + HM, cc:cc + CW4] + gb[:, cc:cc + CW4] * Hq
                        obuf[pl.ds(ro + rr // 2, HM // 2), cc:cc + CW4] = pltpu.bitcast(o_.astype(bf16), u32)
                if S1:
                    for n in range(16):
                        if n not in gdone:
                            g_sums(n // 4, n % 4, None)
                    for c in range(DH2 // 128):
                        def hook2(k, M, c=c):
                            if AP2 and att is not None and (7 * c + k) % AP2 == 0:
                                att.steps(1)
                        Hs = strass(lambda k: _dot(a2[k], w12op(w2_v, k, c * 128, 128, None if TW2 is None else z2)), hook2)
                        for q, Hq in enumerate(Hs):
                            rr, cc = (q // 2) * HM, (q % 2) * DH2 + c * 128
                            hsbuf[rr:rr + HM, cc:cc + 128] = Hq
                else:
                    hsbuf[0:T, :] = raw_dot(g_val(), w2_v)
                if AP4:
                    att.steps(999, PVM)
                    att.rest()
                return carry
            h2 = _dot(u, _bf(w4_v[...]))
            if static:
                obuf[(i - 1) * (T // 2):i * (T // 2), :] = pltpu.bitcast((base + gb * h2).astype(bf16), u32)
            else:
                obuf[pl.ds(pl.multiple_of((i - 1) * (T // 2), T // 2), T // 2), :] = pltpu.bitcast((base + gb * h2).astype(bf16), u32)
            hsbuf[0:T, :] = _dot(g_val(), _bf(w2_v[...]))
            return carry

        if upto >= 4 and 'B' not in skip:
            if UB:
                for i in range(1, 1 + UB):
                    bbody(i, 0)
                    if i in BAR:
                        out_copy_i(i).start()
                if 1 + UB < NT:
                    lax.fori_loop(1 + UB, NT, bbody, 0)
            else:
                lax.fori_loop(1, NT, bbody, 0)

        def blast():
            r0 = (NT - 1) * (T // 2)
            out_copy(0, r0, 0).start()
            if ST:
                gb = row(5)
                for r in ORD4:
                    p0 = r * RP
                    x1 = hb[p0:p0 + RP, :] + hsbuf[p0:p0 + RP, :]
                    baseb[p0:p0 + RP, :] = xmid[p0:p0 + RP, :] + gb * x1
                    n4_sums(r, _ln(x1))

                def fin(q, Hq, c0, cw):
                    rr, cc = (q // 2) * HM, (q % 2) * DH2 + c0
                    o_ = baseb[rr:rr + HM, cc:cc + cw] + gb[:, cc:cc + cw] * Hq
                    obuf[r0 + rr // 2:r0 + rr // 2 + HM // 2, cc:cc + cw] = pltpu.bitcast(o_.astype(bf16), u32)

                if SB == 'F':
                    for c in range(FH // CW3):
                        stage3(c * CW3, CW3, c * CW3)
                    for c in range(DH2 // CW4):
                        Hs = strass(lambda k: _dot(ua[k], w4op(k, c * CW4, CW4)))
                        for q, Hq in enumerate(Hs):
                            fin(q, Hq, c * CW4, CW4)
                else:
                    QF = FH // 2

                    def sbody(m, carry):
                        cb_ = pl.multiple_of(m * QF, 128)
                        for c in range(QF // 128):
                            stage3(cb_ + c * 128, 128, c * 128)
                        rb_ = pl.multiple_of(m * (QF // 2), 32)
                        for c in range(DH2 // CW4):
                            for k in range(7):
                                Mk = _dot(ua[k, :, 0:QF], w4op(k, c * CW4, CW4, rb_, QF // 2))
                                macc[k, :, c * CW4:(c + 1) * CW4] = jnp.where(m > 0, macc[k, :, c * CW4:(c + 1) * CW4], 0.0) + Mk
                        return carry

                    lax.fori_loop(0, 2, sbody, 0)
                    for c in range(DH2 // 128):
                        Hs = strass(lambda k: macc[k, :, c * 128:(c + 1) * 128])
                        for q, Hq in enumerate(Hs):
                            fin(q, Hq, c * 128, 128)
                out_copy(r0, T // 2, 1).start()
                out_copy(0, r0, 0).wait()
                out_copy(r0, T // 2, 1).wait()
                return
            if BL == 'M':
                gb = row(5)

                def l4(p0, zz, dst):
                    x1 = hb[p0:p0 + RP, :] + (hsbuf[pl.ds(zz + p0, RP), :] if zz is not None else hsbuf[p0:p0 + RP, :])
                    baseb[p0:p0 + RP, :] = xmid[p0:p0 + RP, :] + gb * x1
                    q0 = (p0 % HM) // 2
                    dst[q0:q0 + RP // 2, :] = pltpu.bitcast(_ln(x1).astype(bf16), u32)

                for p0 in range(0, HM, RP):
                    l4(p0, None, n4b)

                def mbody(m, carry):
                    zz = pl.multiple_of((m >> 8) * 8, 8)
                    if MA:
                        n4 = _bf(n4b[0:HM // 2, :])
                    else:
                        n4 = _bf(n4b[pl.ds(pl.multiple_of(m * (HM // 2), HM // 2), HM // 2), :])
                    U = _dot(n4, _bf(w3_v[...]))
                    u = _gelu(U).astype(bf16)
                    for k, p0 in enumerate(range(HM, T, RP)):
                        if MT is not None and (k == 0 or MT[k] != MT[k - 1]):
                            hsbuf[pl.ds(zz + T, 8), 0:128] = U[0:8, MT[k] * 128:(MT[k] + 1) * 128]
                        l4(p0, zz if MT is not None else None, n3b if MA else n4b.at[HM // 2:T // 2])
                    if MA:
                        n4b[0:HM // 2, :] = n3b[0:HM // 2, :]
                    ro = pl.multiple_of(r0 + m * (HM // 2), HM // 2)
                    c0 = 0
                    for cw_ in MN:
                        h2 = _dot(u, _bf(w4_v[:, c0:c0 + cw_]))
                        bs = baseb[pl.ds(pl.multiple_of(m * HM, HM), HM), c0:c0 + cw_]
                        obuf[pl.ds(ro, HM // 2), c0:c0 + cw_] = pltpu.bitcast((bs + gb[:, c0:c0 + cw_] * h2).astype(bf16), u32)
                        out_copy(ro, HM // 2, 1, c0, cw_).start()
                        c0 += cw_
                    return carry

                lax.fori_loop(0, 2, mbody, 0)
                out_copy(0, r0, 0).wait()
                for hf in range(2):
                    c0 = 0
                    for cw_ in MN:
                        out_copy(r0 + hf * (HM // 2), HM // 2, 1, c0, cw_).wait()
                        c0 += cw_
                return
            base, n4 = ln4(hsbuf[0:T, :])
            if BL:
                FC = F // BL
                xmid[0:T, :] = base
                n4b[...] = pltpu.bitcast(n4, u32)
                hsbuf[0:T, :] = jnp.zeros((T, D), f32)

                def body(c, carry):
                    w3c = w3_v[:, pl.ds(pl.multiple_of(c * FC, 128), FC)]
                    u = _gelu(_dot(_bf(n4b[...]), _bf(w3c))).astype(bf16)
                    w4c = w4_v[pl.ds(pl.multiple_of(c * (FC // 2), 32), FC // 2), :]
                    hsbuf[0:T, :] += _dot(u, _bf(w4c))
                    return carry

                lax.fori_loop(0, BL, body, 0)
                obuf[r0:r0 + T // 2, :] = pltpu.bitcast((xmid[0:T, :] + row(5) * hsbuf[0:T, :]).astype(bf16), u32)
            else:
                u = _gelu(_dot(n4, _bf(w3_v[...]))).astype(bf16)
                h2 = _dot(u, _bf(w4_v[...]))
                obuf[r0:r0 + T // 2, :] = pltpu.bitcast((base + row(5) * h2).astype(bf16), u32)
            out_copy(r0, T // 2, 1).start()
            out_copy(0, r0, 0).wait()
            out_copy(r0, T // 2, 1).wait()

        if upto >= 5 and 'L' not in skip:
            blast()

    @jax.jit
    def fn(A_x, A_wqkv, A_wo, B_x, B_w1, B_w2, B_w3, B_w4, c, w_mod):
        x = A_x.reshape(S, D)
        any_spec = pl.BlockSpec(memory_space=pl.ANY)
        out = pl.pallas_call(
            kernel,
            in_specs=[any_spec] * 9,
            out_specs=any_spec,
            out_shape=jax.ShapeDtypeStruct((S, D), bf16),
            scratch_shapes=[
                pltpu.VMEM((S // 2 + HALO // 2 + 8, D), u32),
                pltpu.VMEM((D // 2 + 32, 3 * D), u32),
                pltpu.VMEM((64 if SW else D // 2, D), u32),
                pltpu.VMEM((64 if SW else D // 2, D), u32),
                pltpu.VMEM((64 if SW else D // 2, D), u32),
                pltpu.VMEM((NCH + WS, D // 2 + 32, 128), u32),
                pltpu.VMEM((NCH + WS, D // 2, 128), u32),
                pltpu.VMEM((5, D // 4 + 32, D), u32),
                pltpu.VMEM((5, D // 4 + 32, D), u32),
                pltpu.VMEM((4, D // 4 + 8, F), u32),
                pltpu.VMEM((4, F // 4 + 32, D), u32),
                pltpu.VMEM((D // 2, 128), f32),
                pltpu.VMEM((D // 2, 128), f32),
                pltpu.VMEM((8, D // 2 + 16, 256), u32),
                pltpu.VMEM((33, D // 2 + 32, 128), u32),
                pltpu.VMEM((8, 8, 256), f32),
                pltpu.VMEM((36, 8, 128), f32),
                pltpu.VMEM((3 if MU else NCH, S + 32, 128), f32),
                pltpu.VMEM((PR // 2, 128), u32),
                pltpu.VMEM((S // 2, 128), u32),
                pltpu.VMEM((NCH, S + 32, 128), f32),
                pltpu.VMEM((NCH, S + 2 * HALO + 32 * (AB == 9), 128), f32),
                pltpu.VMEM((NCH, S + 2 * HALO + 32 * (AB == 9), 128), f32),
                pltpu.VMEM((T + HALO, D), f32),
                pltpu.VMEM((T + HALO, D), f32),
                pltpu.VMEM((NCH, T + 2 * HALO + 32, 128), f32),
                pltpu.VMEM((S // 2, D), u32),
                pltpu.VMEM((S // 2 + HALO // 2, D), u32),
                pltpu.VMEM((T + 32, D), f32),
                pltpu.VMEM((T // 2, D), u32),
                pltpu.VMEM((T // 2, D), u32),
                pltpu.VMEM((T, D), f32),
                pltpu.VMEM((T, D), f32),
                pltpu.VMEM((7, T // 2, D // 2), bf16),
                pltpu.VMEM((7, T // 2, F // 2), bf16),
                pltpu.VMEM((7, T // 2, D // 2), f32),
                pltpu.VMEM((T // 2, D), f32),
                pltpu.VMEM((7, T // 2, D // 2), bf16),
                pltpu.VMEM((7, T // 2, D // 2), bf16),
                pltpu.VMEM((T + 32, D), f32),
                pltpu.VMEM((T, D), f32),
                pltpu.VMEM((1, D), bf16),
            ] + ([pltpu.VMEM((padr, 128), f32)] if padr else []) + [
                pltpu.SMEM((8,), jnp.int32),
            ],
            compiler_params=pltpu.CompilerParams(vmem_limit_bytes=126 * 1024 * 1024),
        )(x, A_wqkv, A_wo, B_w1, B_w2, B_w3, B_w4, c, w_mod)
        return out.reshape(1, S, D)
    return fn


_fn = make()


def pallas_adaLN_cond__sliding_local_dilated__mixer_s_mlp__prompt_kernel(A_x, A_wqkv, A_wo, B_x, B_w1, B_w2, B_w3, B_w4, c, w_mod):
    return _fn(A_x, A_wqkv, A_wo, B_x, B_w1, B_w2, B_w3, B_w4, c, w_mod)
```

```python
import functools
import jax
import jax.numpy as jnp
from jax import lax
import jax.experimental.pallas as pl
import jax.experimental.pallas.tpu as pltpu

S, D, F = 2048, 1024, 3584
H, DH, W, DIL = 32, 32, 8, 2
NCH = D // 128
EPS = 1e-5
SCALE = DH ** -0.5
f32, bf16, u32 = jnp.float32, jnp.bfloat16, jnp.uint32
HALO = 16


def _ln(x):
    m = jnp.mean(x, axis=-1, keepdims=True)
    xc = x - m
    v = jnp.mean(xc * xc, axis=-1, keepdims=True)
    return xc * lax.rsqrt(v + EPS)


def _gelu(x):
    c0 = 0.7978845608028654
    c1 = c0 * 0.044715
    t = jnp.tanh(x * (c0 + c1 * (x * x)))
    hx = 0.5 * x
    return hx + hx * t


def _dot(a, b):
    return jnp.dot(a, b, preferred_element_type=f32)


def _bf(w):
    return pltpu.bitcast(w, bf16)


def _lane_xor(x, s):
    lane = lax.broadcasted_iota(jnp.int32, x.shape, 1)
    return jnp.take_along_axis(x, lane ^ s, axis=1)


def _exchange8_multi(XS):
    XS = [list(X) for X in XS]
    lane = lax.broadcasted_iota(jnp.int32, XS[0][0].shape, 1)
    for t in range(3):
        s = 1 << (t + 2)
        m = (lane & s) != 0
        for X in XS:
            for p in range(8):
                if p & (1 << t):
                    continue
                p2 = p | (1 << t)
                tmp = _lane_xor(jnp.where(m, X[p], X[p2]), s)
                X[p], X[p2] = jnp.where(m, tmp, X[p]), jnp.where(m, X[p2], tmp)
    return XS


def _group4_sum(acc):
    lane = lax.broadcasted_iota(jnp.int32, acc.shape, 1)
    acc = acc + jnp.where((lane & 1) != 0, pltpu.roll(acc, 1, 1), pltpu.roll(acc, 127, 1))
    acc = acc + jnp.where((lane & 2) != 0, pltpu.roll(acc, 2, 1), pltpu.roll(acc, 126, 1))
    return acc


def make(T=128, PR=512, RB=8, EG=4, upto=9, AT0=0, AP=16,
         DO='c X0 Wq sa ca X1 Wk Wv X2 X3 X4 X5 X6 X7 X8 X9 X10 X12 X13 X11 X14 X15',
         PS=None, PSX=None, RL=1, D0='1234', LP=16, BL='M', ZB=1,
         order0='T0 T1 X x00 x01 m0 T2 T3 X x10 x11 h0 T4 T5 X x20 H0 X x21 H1 H2 H3 H4 H5', NDEF=6, BA=None,
         side=None, KQ=4, KQ0=1, NM=5, NR=8, AG=1,
         rel4=(-1, -1, -1, 0, 1, 2, 3, 4), rel23=(8, 9, 10, 11, 12, 13, 14, 15),
         padr=0, dbg='', UB=0, BAR=(), GL=0, MU=1, WS=1, skip='', AB=9, WGS='12'*42+'2', PD=0, ASCH='', DL=0, EX3=1, EX4=1, XT=(), MT=(4, 10, 16, 22), MA=0, MN=(1024,), NZ=8, NU=2, BPD=0, BQD=None, BWG=8,
         ST=1, ORD4=(0, 4, 1, 5, 2, 6, 3, 7), R23=(0, 8, 16, 24, 32, 40, 48, 56), OX=1, OPRE=0, PRE='R', CW3=128, CW4=128, SB='S', SJ=None, P0R=4, S1=1, R3O=(0, 4, 1, 5, 2, 6, 3, 7), GT=None, KD=None, LC=0, SP3=0, AP1=0, AP4=0, AP2=0, TW4=None, TW1=None, TW2=None, AP3=0, AO3=0, AWO=0, EA=1, RL3=1, RL4=0, LK3=1, LK4=1, TKS=32, TKW=0, TKM=0, SW=1, SK=None, SL=1, TG=1, TD=440, NC=1, DR=None, GA=(0, 2, 2, 2, 2, 2, 2, 2), PVG=None, PVM=None, WOS=2, REL4=(-1, -1, -1, 2, 5, 8, 11, 14), TDW=96, AT3=None, AT1=None, AK4=0, AS4=None, OSC=0, DAO=0, AL=0, PCH=None, OORD=(2, 3, 0, 1, 4, 5, 6), OOR2=(0, 1, 2, 3, 4, 5, 6)):
    HS, HO = (2, 0) if MU else (0, S // 2)
    NT = S // T
    NP = S // PR
    order0 = order0.split()
    TL = S - PR
    if PS is None:
        PS = ('wc C wX0 L0 wWq e0 wsa S wca A h0 wX1 u0:0 L1 wWk u1:0 e1 wWv u0:1 u1:1 e2 wX2 u0:2 u1:2 L2 u2:0 '
              'wX3 wX4 u2:12 L3 u3:012 L4 u4:0 wX5 wX6 wX7 u4:12 L5 u5:012 L6 u6:012 L7 u7:0 '
              'wX8 wX9 wX10 wX12 wX13 u7:12 L8 u8:012 L9 u9:012 L10 ua:0 L12 L13 wX11 wX14 wX15 Da D5 Db D6 Dc D7 Dd DW ua:12 L11 ub:012 L14 L15')
    DR = {2: 'c7dW'} if DR is None else DR
    for v_ in DR.values():
        for g_ in v_:
            assert (' D' + g_ + ' ') in PS
            PS = PS.replace(' D' + g_ + ' ', ' ')
    if BA is None:
        BA = ('a0 a1 T0 T1 t0 a2 a3 W w0 w1 w2 w3 w4 w5 w6 w7 T2 t0 a4 a5 T3 t0 a6 a7 T4 t0 a8 a9 T5 t0 a10 o0 t0 a11 t4 a12 '
              'o1 t0 a13 t4 a14 M m0 m1 l0 l1 u0 t0 a15 t4 a16 u1')
    if WOS == 2 and BA.startswith('a0 a1 T0 T1 t0 a2 a3 W w0'):
        BA = ('a0 a1 T0 T1 M m0 m1 t0 a2 a3 T2 t0 a4 a5 T3 t0 a6 a7 T4 t0 a8 a9 T5 t0 a10 o0 t0 a11 t4 a12 '
              'l0 o1 t0 a13 t4 a14 l1 u0 t0 a15 t4 a16 u1')
    if WOS == 1 and BA.startswith('a0 a1 T0 T1 t0 a2 a3 W w0'):
        BA = ('a0 a1 T0 T1 t0 a2 a3 T2 t0 a4 a5 T3 t0 a6 a7 T4 t0 a8 b0 T5 t0 b1 o0 t0 b2 t4 b3 '
              'o1 t0 b4 t4 b5 M m0 m1 l0 l1 u0 t0 b6 t4 b7 u1')
    if WS and not WOS and 'v0' not in BA:
        BA = BA.replace('W w0 w1 w2 w3 w4 w5 w6 w7', 'W v0 v1 v2 v3 v4 v5 v6 v7 w0 w1 w2 w3 w4 w5 w6 w7')
    if PSX:
        for k_, v_ in PSX.items():
            assert (' ' + k_ + ' ') in PS
            PS = PS.replace(' ' + k_ + ' ', ' ' + k_ + ' ' + v_ + ' ')
    S_C, S_X, S_SA, S_CA, S_W0, S_WQ, S_WO, S_MB, S_W = 0, 1, 17, 25, 33, 36, 44, 52, 60
    S_P = 64
    NSEM = 68
    DEF = list(range(6 - NDEF, 6))
    tags = ['T%d' % sd for sd in DEF] + ['%dH%d' % (p, sd) for p in range(NP) for sd in range(6 if p < NP - 1 else 6 - NDEF)]
    if side is None:
        side = 'W:7,9,11,13,15,17,19,21 M:4,5,6,7,8,9,10,11,12,13,14,15,16,17,18,19,20,21,22,22'
        if PRE == 'R':
            if SJ is None:
                SJ = ','.join(str(t) for t in (range(4, 23) if S1 else range(8, 23)))
            side += ' S:' + SJ
    if isinstance(side, str):
        sd_ = {}
        for grp in side.split():
            kind, lst = grp.split(':')
            for k, t in enumerate(lst.split(',')):
                sd_.setdefault(tags[int(t)], []).append(kind + str(k))
        side = sd_
    assert sum(1 for v in side.values() for j in v if j[0] in 'Aa') * AP == AT0

    def kernel(*refs):
        pl.run_scoped(functools.partial(body, *refs), pltpu.SemaphoreType.DMA((NSEM,)), pltpu.SemaphoreType.DMA((2,)))

    def body(x_hbm, wqkv_hbm, wo_hbm, w1_hbm, w2_hbm, w3_hbm, w4_hbm, c_hbm, wmod_hbm,
             o_hbm,
             x_v, wqkv_raw, wq_v, wk_v, wv_v, wo_raw, wo_v, w1_v, w2_v, w3_v, w4_v, cE, cO, wmA_v, wmB_v,
             modA, modB, xhat, hP, h0, qbuf, kbuf, vbuf, xmid, hb, h1buf, obuf, o_scr, hsbuf, n4b, n3b, baseb, n4f, a4, ua, macc, n3f, a3, a2, abuf, x1buf, wos, aof, ao, c_v, *rest):
        if OX:
            obuf = x_v
        zsm, sems, osems = rest[-3:]

        def cp(src, dst, k):
            return pltpu.make_async_copy(src, dst, sems.at[k])

        xu = x_hbm.bitcast(u32)
        wqkvu = wqkv_hbm.bitcast(u32)
        wou = wo_hbm.bitcast(u32)
        wmodu = wmod_hbm.bitcast(u32)

        def lane_ds(k, n, base=0):
            if isinstance(k, int):
                return pl.ds(base + k * n, n)
            return pl.ds(pl.multiple_of(base + k * n, 128), n)

        def row_ds(base, k, n):
            if isinstance(k, int):
                return pl.ds(base + k * n, n)
            return pl.ds(pl.multiple_of(base + k * n, 8), n)

        c_c = cp(c_hbm, c_v, S_C)

        def c_x(b):
            return cp(xu.at[b * 64:(b + 1) * 64], x_v.at[b * 64:(b + 1) * 64], S_X + b)

        def c_sa(k):
            return cp(wmodu.at[:, lane_ds(k, 128)], wmA_v.at[k, 0:D // 2, 0:128], S_SA + k)

        def c_ca(k):
            return cp(wmodu.at[:, lane_ds(k, 128, D)], wmA_v.at[k, 0:D // 2, 128:256], S_CA + k)

        def c_w0(b):
            return cp(wqkvu.at[0:64, b * D:(b + 1) * D], wqkv_raw.at[0:64, b * D:(b + 1) * D], S_W0 + b)

        def c_wq(k):
            return cp(wqkvu.at[row_ds(0, k, 64)], wqkv_raw.at[row_ds(0, k, 64)], S_WQ + k)

        def c_wo(p):
            return cp(wou.at[:, lane_ds(p, 128)], wo_raw.at[p, 8:8 + D // 2], S_WO + p)

        def c_mb(t, g):
            return cp(wmodu.at[:, lane_ds(t, 128, 2 * D)], wmB_v.at[t, 0:D // 2], S_MB + g)

        w1u, w2u = w1_hbm.bitcast(u32), w2_hbm.bitcast(u32)
        w3u, w4u = w3_hbm.bitcast(u32), w4_hbm.bitcast(u32)
        N3, N4 = D // 4 // 4, F // 4 // 4
        c_w = []

        def c_p(p):
            def rows(base, n):
                if isinstance(p, int):
                    return pl.ds(base + p * n, n)
                return pl.ds(pl.multiple_of(base + p * n, 8), n)
            return ([cp(w3u.at[rows(a * (D // 4), N3)], w3_v.at[a, rows(0, N3)], S_P + p) for a in range(2)]
                    + [cp(w4u.at[rows(a * (F // 4), N4)], w4_v.at[a, rows(0, N4)], S_P + p) for a in range(2)]
                    + [cp(w1u.at[rows(a * (D // 4), N3)], w1_v.at[a, rows(0, N3)], S_P + p) for a in range(2)]
                    + [cp(w2u.at[rows(a * (D // 4), N3)], w2_v.at[a, rows(0, N3)], S_P + p) for a in range(2)])

        def named(nm):
            if nm == 'c':
                return c_c
            if nm == 'sa':
                return c_sa(0)
            if nm == 'ca':
                return c_ca(0)
            if nm[0] == 'W':
                return c_w0('qkv'.index(nm[1]))
            return c_x(int(nm[1:]))

        for nm in DO.split():
            named(nm).start()
        def start_group(g):
            if g == 'W':
                if upto >= 3:
                    if not WOS:
                        c_wo(7).start()
                    for t in range(6 * NM, 32):
                        c_mb(t, 6).start()
                    for c in c_w:
                        c.start()
            elif g in 'abcd':
                for c in c_p('abcd'.index(g)):
                    c.start()
            elif upto >= 2 and 'nodma2' not in dbg:
                r = int(g)
                c_sa(r).start()
                c_ca(r).start()
                c_wq(r).start()
                if not WOS:
                    c_wo(r - 1).start()
                elif 2 <= r <= 5:
                    c_wo(2 * r - 4).start()
                    c_wo(2 * r - 3).start()
                if r >= 2:
                    for i in range(NM):
                        c_mb(NM * (r - 2) + i, r - 2).start()

        for g in D0:
            start_group(g)
        assert sorted(list(D0) + [it[1] for it in PS.split() if it[0] == 'D'] + list(''.join(DR.values()))) == sorted('1234567Wabcd')

        def _zinit(i, carry):
            zsm[2 + i] = i >> 8
            return carry

        lax.fori_loop(0, 3, _zinit, 0)
        zp3 = pl.multiple_of(zsm[4] * 8, 8)
        zp1 = pl.multiple_of(zsm[2] * 8, 8)
        zp2 = pl.multiple_of(zsm[3] * 8, 8)

        x_v[S // 2:S // 2 + HALO // 2, :] = jnp.zeros((HALO // 2, D), u32)
        for j in range(NCH):
            z = jnp.zeros((HALO, 128), f32)
            qbuf[j, S:S + HALO, :] = z
            kbuf[j, HALO + S:2 * HALO + S, :] = z
            vbuf[j, HALO + S:2 * HALO + S, :] = z
            kbuf[j, 0:HALO, :] = z
            vbuf[j, 0:HALO, :] = z
            wo_raw[j, 0:8, :] = jnp.zeros((8, 128), u32)
            wo_raw[j, 8 + D // 2:16 + D // 2, :] = jnp.zeros((8, 128), u32)

        def mv_part(w, r0, acc):
            n = w.shape[0]
            lo = pltpu.bitcast(w << 16, f32)
            hi = pltpu.bitcast(w & jnp.uint32(0xFFFF0000), f32)
            pr = lo * cE[r0:r0 + n, :] + hi * cO[r0:r0 + n, :]
            for t in range(n // 8):
                acc = pr[8 * t:8 * t + 8] if acc is None else acc + pr[8 * t:8 * t + 8]
            return acc

        wparts = (wq_v, wk_v, wv_v)
        bufs = (qbuf, kbuf, vbuf)

        def exch_groups(grps):
            for g0 in range(0, len(grps), EG):
                gs = grps[g0:g0 + EG]
                XS = [[wqkv_raw[row_ds(rg * 8, k * 8, 8), b * D + a * 128:b * D + (a + 1) * 128] for a in range(NCH)]
                      for (k, b, rg) in gs]
                YS = _exchange8_multi(XS)
                for (k, b, rg), Y in zip(gs, YS):
                    wparts[b][row_ds(rg * 8, 0 if SW else k * 8, 8), :] = jnp.concatenate(Y, axis=1)

        def subdot(lhs, row0, kc, sd, init=False, valid=None):
            b, hf = sd // 2, sd % 2
            n = lhs.shape[0]
            res = _dot(lhs, _bf(wparts[b][row_ds(0, 0 if SW else kc, 64), hf * 512:(hf + 1) * 512]))
            o = row0 + (0 if b == 0 else HALO)
            for jj in range(4):
                j = hf * 4 + jj
                if init:
                    bufs[b][j, o:o + n, :] = res[:, jj * 128:(jj + 1) * 128]
                elif valid is not None:
                    bufs[b][j, o:o + n, :] = jnp.where(valid, bufs[b][j, o:o + n, :], 0.0) + res[:, jj * 128:(jj + 1) * 128]
                else:
                    bufs[b][j, o:o + n, :] += res[:, jj * 128:(jj + 1) * 128]
            return res

        def prologue():
            st = {}

            def crep():
                c = c_v[...].astype(f32)
                scf = (c * jax.nn.sigmoid(c)).astype(bf16).astype(f32)
                rr = lax.broadcasted_iota(jnp.int32, (128, 128), 0)
                ll = lax.broadcasted_iota(jnp.int32, (128, 128), 1)
                sel = ll == jnp.where(rr < 64, 2 * rr, 2 * rr - 127)
                for j in range(NCH):
                    dg = jnp.where(sel, jnp.broadcast_to(scf[:, j * 128:(j + 1) * 128], (128, 128)), 0.0).astype(bf16)
                    rep = _dot(dg, jnp.ones((128, 128), bf16))
                    cE[j * 64:(j + 1) * 64, :] = rep[0:64]
                    cO[j * 64:(j + 1) * 64, :] = rep[64:128]

            def h_store(r0, xh0):
                h = (xh0 * (1.0 + st['ca']) + st['sa']).astype(bf16)
                if r0 < TL:
                    xhat[HS, HO + r0 // 2:HO + (r0 + LP) // 2, :] = pltpu.bitcast(h, f32)
                else:
                    hP[(r0 - TL) // 2:(r0 - TL + LP) // 2, :] = pltpu.bitcast(h, u32)

            def h0_lhs(b0, nb, gated):
                r0 = HO + b0 * 64
                if not gated:
                    return _bf(xhat[HS, r0:r0 + nb * 64, :])
                if GL:
                    return jnp.concatenate([_bf(xhat[HS, r0:r0 + nb * 64 - 8, :]), _bf(xhat[HS, pl.ds(zp3 + r0 + nb * 64 - 8, 8), :])], axis=0)
                return jnp.concatenate([_bf(xhat[HS, pl.ds(zp3 + r0, 8), :]), _bf(xhat[HS, r0 + 8:r0 + nb * 64, :])], axis=0)

            def ln_piece(b, i):
                r0 = b * 128 + i * LP
                direct = 'ca' in st and 'sa' in st
                if MU:
                    x = _bf(x_v[pl.ds(zp1 + r0 // 2, LP // 2), :]).astype(f32)
                    m = jnp.mean(x, axis=-1, keepdims=True)
                    if RL:
                        x = _bf(x_v[pl.ds(zp2 + r0 // 2, LP // 2), :]).astype(f32)
                    xc = x - m
                    rs = lax.rsqrt(jnp.mean(xc * xc, axis=-1, keepdims=True) + EPS)
                    xhat[0, r0:r0 + LP, :] = jnp.broadcast_to(m, (LP, 128))
                    xhat[1, r0:r0 + LP, :] = jnp.broadcast_to(rs, (LP, 128))
                    if direct:
                        h_store(r0, xc[:, 0:128] * rs)
                    return
                if RL:
                    m = jnp.mean(_bf(x_v[pl.ds(zp1 + r0 // 2, LP // 2), :]).astype(f32), axis=-1, keepdims=True)
                    xc = _bf(x_v[pl.ds(zp2 + r0 // 2, LP // 2), :]).astype(f32) - m
                    v = jnp.mean(xc * xc, axis=-1, keepdims=True)
                    xh = (_bf(x_v[r0 // 2:(r0 + LP) // 2, :]).astype(f32) - m) * lax.rsqrt(v + EPS)
                else:
                    xh = _ln(_bf(x_v[pl.ds(zp1 + r0 // 2, LP // 2), :]).astype(f32))
                for j in range(1 if direct else 0, NCH):
                    xhat[j, r0:r0 + LP, :] = xh[:, j * 128:(j + 1) * 128]
                if direct:
                    h_store(r0, xh[:, 0:128])

            def ln_block(b):
                for i in range(128 // LP):
                    ln_piece(b, i)

            def hblk(b):
                for i in range(128 // LP):
                    r0 = b * 128 + i * LP
                    if MU:
                        x = _bf(x_v[r0 // 2:(r0 + LP) // 2, 0:128]).astype(f32)
                        h_store(r0, (x - xhat[0, r0:r0 + LP, :]) * xhat[1, r0:r0 + LP, :])
                    else:
                        h_store(r0, xhat[0, r0:r0 + LP, :])

            for it in PS.split():
                if it[0] == 'w':
                    named(it[1:]).wait()
                elif it[0] == 'D':
                    start_group(it[1])
                elif it == 'C':
                    crep()
                elif it[0] == 'L':
                    ln_block(int(it[1:]))
                elif it[0] == 'h':
                    hblk(int(it[1:]))
                elif it == 'S':
                    st['sa'] = jnp.sum(mv_part(wmA_v[0, 0:D // 2, 0:128], 0, None), axis=0, keepdims=True)
                elif it == 'A':
                    st['ca'] = jnp.sum(mv_part(wmA_v[0, 0:D // 2, 128:256], 0, None), axis=0, keepdims=True)
                elif it[0] == 'e':
                    exch_groups([(0, int(it[1]), rg) for rg in range(8)])
                elif it[0] == 'p':
                    b_, i_ = it[1:].split(':')
                    ln_piece(int(b_), int(i_))
                elif it[0] == 't':
                    x_v[pl.ds(zp3 + S // 2 + HALO // 2, 8), 0:128] = pltpu.bitcast(st['res'][0:8, 0:128], u32)
                elif it[0] in 'sg':
                    blks, sd = it[1:].split(':')
                    b0, nb = int(blks[0], 16), len(blks)
                    st['res'] = subdot(h0_lhs(b0, nb, it[0] == 'g'), b0 * 128, 0, int(sd), True)
                elif it[0] == 'u':
                    blks, parts = it[1:].split(':')
                    b0, nb = int(blks[0], 16), len(blks)
                    lhs = h0_lhs(b0, nb, False)
                    for p in parts:
                        subdot(lhs, b0 * 128, 0, 2 * int(p), True)
                        st['res'] = subdot(lhs, b0 * 128, 0, 2 * int(p) + 1, True)

        if 'P' not in skip:
            prologue()

        def attention(qb, kb, vb, base, off, M, mask_rows, baseh=None):
            row0 = base + off

            def kvds(r, w):
                return pl.ds(base + (off + HALO + r - DIL * w), RB)

            o_rows = []
            for r in range(0, M, RB):
                q = [qb[j, pl.ds(base + (off + r), RB), :] for j in range(NCH)]
                s = []
                for w in range(W):
                    acc = None
                    for j in range(NCH):
                        p = q[j] * kb[j, kvds(r, w), :]
                        acc = p if acc is None else acc + p
                    acc = _group4_sum(acc)
                    if mask_rows and off + r < DIL * (W - 1) and w > 0:
                        rows = row0 + r + lax.broadcasted_iota(jnp.int32, (RB, 128), 0)
                        acc = jnp.where(rows >= DIL * w, acc, -1e30)
                    s.append(acc)
                m = functools.reduce(jnp.maximum, s)
                e = [jnp.exp((sw - m) * SCALE) for sw in s]
                den = functools.reduce(lambda a, b: a + b, e)
                rinv = 1.0 / den
                oc = []
                for j in range(NCH):
                    acc = None
                    for w in range(W):
                        p = e[w] * vb[j, kvds(r, w), :]
                        acc = p if acc is None else acc + p
                    oc.append(acc * rinv)
                o_rows.append(jnp.concatenate(oc, axis=1))
            o = jnp.concatenate(o_rows, axis=0).astype(bf16)
            if isinstance(row0, int):
                o_scr[row0 // 2:(row0 + M) // 2, :] = pltpu.bitcast(o, u32)
            elif baseh is not None:
                o_scr[pl.ds(baseh + off // 2, M // 2), :] = pltpu.bitcast(o, u32)
            else:
                o_scr[pl.ds(pl.multiple_of(row0 // 2, 8), M // 2), :] = pltpu.bitcast(o, u32)


        def attention2(off, M, G, base=None, baseh=None, sums=None):
            o_rows = []

            def rs_(a):
                return slice(a, a + RB) if base is None else pl.ds(base + a, RB)

            for r0 in range(0, M, RB * G):
                rs = [off + r0 + g * RB for g in range(G) if r0 + g * RB < M]
                lane = lax.broadcasted_iota(jnp.int32, (RB, 128), 1)
                S_ = {}
                for r in rs:
                    q = [qbuf[j, rs_(r), :] for j in range(NCH)]
                    for w in range(W):
                        acc = None
                        for j in range(NCH):
                            k0 = HALO + r - DIL * w
                            p = q[j] * kbuf[j, rs_(k0), :]
                            acc = p if acc is None else acc + p
                        S_[r, w] = acc
                keys = list(S_)
                for sh in (1, 2):
                    R = {k: (pltpu.roll(S_[k], sh, 1), pltpu.roll(S_[k], 128 - sh, 1)) for k in keys}
                    for k in keys:
                        S_[k] = S_[k] + jnp.where((lane & sh) != 0, R[k][0], R[k][1])
                for r in rs:
                    s = []
                    for w in range(W):
                        acc = S_[r, w]
                        if base is None and r < DIL * (W - 1) and w > 0:
                            rows = r + lax.broadcasted_iota(jnp.int32, (RB, 128), 0)
                            acc = jnp.where(rows >= DIL * w, acc, -1e30)
                        s.append(acc)
                    m = functools.reduce(jnp.maximum, s)
                    e = [jnp.exp((sw - m) * SCALE) for sw in s]
                    den = functools.reduce(lambda a, b: a + b, e)
                    rinv = 1.0 / den
                    oc = []
                    for j in range(NCH):
                        acc = None
                        for w in range(W):
                            k0 = HALO + r - DIL * w
                            p = e[w] * vbuf[j, rs_(k0), :]
                            acc = p if acc is None else acc + p
                        oc.append(acc * rinv)
                    o_rows.append(jnp.concatenate(oc, axis=1))
            if sums is not None:
                n_sums(sums, jnp.concatenate(o_rows, axis=0), aof, ao)
                return o_rows[0]
            o = jnp.concatenate(o_rows, axis=0).astype(bf16)
            if base is None:
                o_scr[off // 2:(off + M) // 2, :] = pltpu.bitcast(o, u32)
            else:
                o_scr[pl.ds(baseh + off // 2, M // 2), :] = pltpu.bitcast(o, u32)
            return o

        class Att:
            def __init__(self, base, baseh, off, M, wgs, PD, ztok, QD=None, mask=False, KD=None, sums=False):
                self.sums = sums
                self.base, self.baseh, self.off, self.PD, self.ztok = base, baseh, off, PD, ztok
                self.KD, self.PP = KD, {}
                self.QD, self.mask = QD, mask
                self.nrb = M // RB
                self.wgs = list(wgs)
                assert sum(self.wgs) == self.nrb * W
                self.Q, self.SS, self.E, self.OC = {}, {}, {}, {}
                self.win = 0
                self.done = 0

            def scores(self, wl):
                lane = lax.broadcasted_iota(jnp.int32, (RB, 128), 1)
                accs = []
                if self.KD is not None:
                    n0 = wl[0][0] * W + wl[0][1] - self.KD[1]
                    if n0 >= 0:
                        kbuf[0, pl.ds(self.ztok + S + 2 * HALO, 8), :] = (self.PP if self.KD[0] == 0 else self.SS)[divmod(n0, W)]
                for (rb, w) in wl:
                    r = self.off + rb * RB
                    if rb not in self.Q:
                        if self.QD is not None and rb * W - self.QD >= 0:
                            qbuf[0, pl.ds(self.ztok + S + HALO, 8), :] = self.SS[divmod(rb * W - self.QD, W)]
                        self.Q[rb] = [qbuf[j, pl.ds(self.base + r, RB), :] for j in range(NCH)]
                    acc = None
                    for j in range(NCH):
                        p = self.Q[rb][j] * kbuf[j, pl.ds(self.base + (HALO + r - DIL * w), RB), :]
                        acc = p if acc is None else acc + p
                    accs.append(acc)
                for sh in (1, 2):
                    R = [(pltpu.roll(a, sh, 1), pltpu.roll(a, 128 - sh, 1)) for a in accs]
                    accs = [a + jnp.where((lane & sh) != 0, x, y) for a, (x, y) in zip(accs, R)]
                    if sh == 1:
                        for k, a in zip(wl, accs):
                            self.PP[k] = a
                for k, a in zip(wl, accs):
                    r = self.off + k[0] * RB
                    if self.mask and r < DIL * (W - 1) and k[1] > 0:
                        rows = r + lax.broadcasted_iota(jnp.int32, (RB, 128), 0)
                        a = jnp.where(rows >= DIL * k[1], a, -1e30)
                    self.SS[k] = a
                    if k[1] == W - 1:
                        self.softmax(k[0])

            def softmax(self, rb):
                s = [self.SS[rb, w] for w in range(W)]
                m = functools.reduce(jnp.maximum, s)
                e = [jnp.exp((sw - m) * SCALE) for sw in s]
                den = functools.reduce(lambda a, b: a + b, e)
                self.E[rb] = (e, 1.0 / den)

            def pv(self):
                rb, j = divmod(self.done, NCH)
                self.done += 1
                r = self.off + rb * RB
                e, rinv = self.E[rb]
                acc = None
                for w in range(W):
                    p = e[w] * vbuf[j, pl.ds(self.base + (HALO + r - DIL * w), RB), :]
                    acc = p if acc is None else acc + p
                self.OC[rb, j] = acc * rinv
                if self.sums and PCH and rb >= PCH[0] and (rb * NCH + j + 1) % PCH[1] == 0:
                    kbuf[0, pl.ds(self.ztok + S + 2 * HALO, 8), :] = self.OC[rb, j]
                if rb % 2 == 1 and j == NCH - 1:
                    o = jnp.concatenate([jnp.concatenate([self.OC[q, c] for c in range(NCH)], axis=1) for q in (rb - 1, rb)], axis=0)
                    if self.sums:
                        n_sums(rb // 2, o, aof, ao, pl.multiple_of(self.ztok * 2, 16) if DAO else None)
                        if OSC == 2:
                            o_scr[pl.ds(self.baseh + (self.off + (rb - 1) * RB) // 2, RB), 0:128] = pltpu.bitcast(o[8:16, D - 128:D], u32)
                        if OSC != 1:
                            return
                    o_scr[pl.ds(self.baseh + (self.off + (rb - 1) * RB) // 2, RB), :] = pltpu.bitcast(o.astype(bf16), u32)

            def token(self, v):
                vbuf[0, pl.ds(self.ztok + S + 2 * HALO, 8), :] = v

            def steps(self, n, pvmax=None):
                for _ in range(n):
                    if not self.wgs:
                        return
                    g = self.wgs.pop(0)
                    wl = [divmod(self.win + t, W) for t in range(g)]
                    self.win += g
                    self.scores(wl)
                    tok = False
                    npv = 0
                    while self.done < self.nrb * NCH and self.done + W + self.PD <= self.win - 1 and self.done // NCH in self.E:
                        if pvmax is not None and npv >= pvmax:
                            break
                        npv += 1
                        if not tok:
                            self.token(self.SS[wl[-1]])
                            tok = True
                        self.pv()

            def rest(self, n=999):
                while self.done < self.nrb * NCH and n > 0:
                    self.pv(); n -= 1

        sub = lax.broadcasted_iota(jnp.int32, (8, 128), 0)

        def pW(p, q, z):
            for tv in range(8 * q, 8 * q + 8):
                j = tv >> 3
                hh = (tv >> 1) & 3
                a2 = tv & 1
                parts = []
                for al in range(4):
                    a = a2 * 4 + al
                    src = a * 64 + hh * 16 + j * 2
                    st = src - 2 * al + 8
                    if isinstance(z, int):
                        parts.append(wo_raw[p, z + st:z + st + 8, :])
                    else:
                        parts.append(wo_raw[p, pl.ds(z + st, 8), :])
                v = jnp.where(sub < 2, parts[0], parts[1])
                v2 = jnp.where(sub < 6, parts[2], parts[3])
                wo_v[p, 8 * tv:8 * tv + 8, :] = jnp.where(sub < 4, v, v2)

        def wo_vreg(p, tv, z):
            j = tv >> 3
            hh = (tv >> 1) & 3
            a2 = tv & 1
            parts = []
            for al in range(4):
                st = (a2 * 4 + al) * 64 + hh * 16 + j * 2 - 2 * al + 8
                parts.append(wo_raw[p, pl.ds(z + st, 8), :])
            v = jnp.where(sub < 2, parts[0], parts[1])
            v2 = jnp.where(sub < 6, parts[2], parts[3])
            return jnp.where(sub < 4, v, v2)

        def wo_link(pa, pb, da, db, ds_, tv, z):
            h = D // 32
            w = {(0, 0): wo_vreg(pa, tv, z), (0, 1): wo_vreg(pb, tv, z), (1, 0): wo_vreg(pa, tv + h, z), (1, 1): wo_vreg(pb, tv + h, z)}
            for (a, b), v in w.items():
                wo_v[db if b else da, 8 * (tv + a * h):8 * (tv + a * h) + 8, :] = v
            res = [[] for _ in range(5)]
            for hf in range(2):
                e = {k: pltpu.unpack_elementwise(v, index=hf, packed_dtype=bf16, unpacked_dtype=f32) for k, v in w.items()}
                b11, b12, b21, b22 = e[0, 0], e[0, 1], e[1, 0], e[1, 1]
                for n, o in enumerate((b11 + b22, b12 - b22, b21 - b11, b11 + b12, b21 + b22)):
                    res[n].append(o)
            for n in range(5):
                wos[ds_[n], 8 * tv:8 * tv + 8, :] = pltpu.bitcast(pltpu.pack_elementwise(res[n], packed_dtype=bf16), u32)

        def woop(k, q):
            if k == 1:
                return _bf(wo_v[2 * q, 0:D // 4, :])
            if k == 4:
                return _bf(wo_v[2 * q + 1, D // 4:D // 2, :])
            return _bf(wos[5 * q + {0: 0, 2: 1, 3: 2, 5: 3, 6: 4}[k]])

        def pM(t, kq, z, macc, key):
            n = D // 2 // KQ
            rows = pl.ds(z + kq * n, n)
            macc[key] = mv_part(wmB_v[t, rows, :], kq * n, macc.get(key))
            if kq == KQ - 1:
                modB[t, 0:1, :] = jnp.sum(macc[key], axis=0, keepdims=True)

        FH, DH2, HM = F // 2, D // 2, T // 2
        SLOT = {0: (2, 0), 1: (0, 0), 2: (0, 1), 3: (1, 0), 4: (1, 1), 5: (2, 1), 6: (3, 0)}
        SLOT5 = {0: (2, 0), 1: (0, 0), 2: (3, 1), 3: (4, 0), 4: (1, 1), 5: (2, 1), 6: (3, 0)}

        def bsums(W, NH, rl, rs_, n, c0, cw, five=False):
            w = {(a, b): W[a, pl.ds(rl, n), b * NH + c0:b * NH + c0 + cw] for a in range(2) for b in range(2)}
            res = {}
            for h in range(2):
                e = {k: pltpu.unpack_elementwise(v, index=h, packed_dtype=bf16, unpacked_dtype=f32) for k, v in w.items()}
                b11, b12, b21, b22 = e[0, 0], e[0, 1], e[1, 0], e[1, 1]
                sl = SLOT5 if five else SLOT
                for k, o in ((0, b11 + b22), (2, b12 - b22), (3, b21 - b11), (5, b11 + b12), (6, b21 + b22)):
                    res.setdefault(sl[k], []).append(o)
            for (a, b), o in res.items():
                W[a, pl.ds(rs_, n), b * NH + c0:b * NH + c0 + cw] = pltpu.bitcast(pltpu.pack_elementwise(o, packed_dtype=bf16), u32)

        NS3, NS4 = N3 // 8, N4 // 32

        def s_ref(k):
            return w3_v if k < NS3 else w4_v if k < NS3 + NS4 else w1_v if k < NS3 + NS4 + 2 else w2_v

        def s_links(k, r, z):
            links = []
            W = s_ref(k)
            if k < NS3:
                r0 = jnp.where(r >= P0R, (r - P0R) * N3 + 8 * k, D // 4) + z
                for c in range(FH // 128):
                    links.append(functools.partial(bsums, W, FH, pl.multiple_of(r0, 8), pl.multiple_of(r0, 8), 8, c * 128, 128))
            elif k < NS3 + NS4:
                k -= NS3
                r0 = jnp.where(r >= P0R, (r - P0R) * N4 + 32 * k, F // 4) + z
                for t in range(4):
                    for c in range(DH2 // 128):
                        links.append(functools.partial(bsums, W, DH2, pl.multiple_of(r0 + 8 * t, 8), pl.multiple_of(r0 + 8 * t, 8), 8, c * 128, 128))
            else:
                k = (k - NS3 - NS4) % 2
                r0 = jnp.where(r >= P0R, (r - P0R) * N3 + 32 * k, D // 4) + z
                for t in range(4):
                    for c in range(DH2 // 128):
                        links.append(functools.partial(bsums, W, DH2, pl.multiple_of(r0 + 8 * t, 8), pl.multiple_of(r0 + 8 * t, 8), 8, c * 128, 128, True))
            return links

        def region_waits(r):
            c_sa(r).wait(); c_ca(r).wait(); c_wq(r).wait()
            if not WS:
                c_wo(r - 1).wait()

            if WOS:
                @pl.when((r >= 2) & (r <= 5))
                def _():
                    c_wo(2 * r - 4).wait()
                    c_wo(2 * r - 3).wait()

            @pl.when(r >= 2)
            def _():
                if WS and not WOS:
                    c_wo(r - 2).wait()
                for i in range(NM):
                    c_mb(NM * (r - 2) + i, r - 2).wait()

            @pl.when(r >= P0R)
            def _():
                for c in c_p(r - P0R):
                    c.wait()

            for r_, gs_ in DR.items():
                @pl.when(r == r_)
                def _(gs_=gs_):
                    for g_ in gs_:
                        start_group(g_)

        if 'prewait' in dbg:
            for r in range(1, 8):
                region_waits(r)

        def region(r, carry):
            if 'prewait' not in dbg and 'nodma2' not in dbg:
                region_waits(r)
            z1 = pl.multiple_of((r >> 8) * 8, 8)
            z2 = pl.multiple_of((r >> 9) * 8, 8)
            pm = [jnp.where(r >= 2, NM * (r - 2) + i, 32) for i in range(NM)]
            pw = jnp.where(r >= 2, r - 2, NCH) if WS else r - 1
            hp = _bf(hP[...])
            st = {'acc': [None, None], 'res': None}
            macc_ = {}

            def mvp(kq):
                n = D // 2 // KQ0
                for q in range(2):
                    st['acc'][q] = mv_part(wmA_v[r, pl.ds(z2 + kq * n, n), q * 128:(q + 1) * 128], kq * n, st['acc'][q])
                if kq == KQ0 - 1:
                    st['sa'] = jnp.sum(st['acc'][0], axis=0, keepdims=True)
                    st['ca'] = jnp.sum(st['acc'][1], axis=0, keepdims=True)
                    modA[r, 0:1, 0:128] = st['sa']
                    modA[r, 0:1, 128:256] = st['ca']

            def hpass(p):
                if MU:
                    x = _bf(x_v[p * PR // 2:(p + 1) * PR // 2, lane_ds(r, 128)]).astype(f32)
                    xh = (x - xhat[0, p * PR:(p + 1) * PR, :]) * xhat[1, p * PR:(p + 1) * PR, :]
                else:
                    xh = xhat[r, p * PR:(p + 1) * PR, :]
                st['h'] = (xh * (1.0 + st['ca']) + st['sa']).astype(bf16)
                st['row'] = p * PR
                if p == NP - 1:
                    hP[...] = pltpu.bitcast(st['h'], u32)

            def do_side(tag):
                prev, st['prev'] = st.get('prev'), st['res']
                jobs = side.get(tag, ())
                if not jobs:
                    return
                tkr = lambda row: pltpu.bitcast(st['res'][row:row + 8, 0:128], u32)
                sj = [int(j[1:]) for j in jobs if j[0] == 'S']
                def sjobs():
                    links = [(k, l) for k in sj for l in s_links(k, r, z1)]
                    for n, (k, l) in enumerate(links):
                        row = (TKS + n * TD // len(links)) // 8 * 8
                        W = s_ref(k)
                        W[0, pl.ds(z1 + (F // 4 if W is w4_v else D // 4), 8), 0:128] = tkr(row)
                        l()
                tk = tkr(0)
                kinds = set(j[0] for j in jobs)
                if 'W' in kinds and WOS:
                    ok = (r >= 2) & (r <= 5)
                    pa = jnp.where(ok, 2 * r - 4, NCH); pb = jnp.where(ok, 2 * r - 3, NCH)
                    ds_ = [jnp.where(ok, 5 * (r - 2) + n_, 20) for n_ in range(5)]
                    for j in jobs:
                        if j[0] == 'W':
                            for n in range(4):
                                wo_raw[pa, pl.ds(z1 + D // 2 + 16, 8), :] = tkr((TKW + n * TDW) // 8 * 8)
                                wo_link(pa, pb, pa, pb, ds_, 4 * int(j[1:]) + n, z2)
                elif 'W' in kinds:
                    wo_raw[pw, pl.ds(z1 + D // 2 + 16, 8), :] = tkr(TKW)
                if 'M' in kinds:
                    wmB_v[32, pl.ds(z1 + D // 2, 8), :] = tkr(TKM)
                if 'A' in kinds:
                    qbuf[0, pl.ds(z1 + S + HALO, 8), :] = pltpu.bitcast(tk, f32)
                for j in jobs:
                    k = int(j[1:])
                    if j[0] == 'W':
                        if not WOS:
                            pW(pw, k, z2)
                    elif j[0] == 'w':
                        pW(pw, k, 0)
                    elif j[0] == 'M':
                        pM(pm[k // KQ], k % KQ, z2, macc_, k // KQ)
                    elif j[0] in 'Aa':
                        attention(qbuf, kbuf, vbuf, 0, k * AP, AP, True)
                if sj:
                    sjobs()

            for it in order0:
                if it[0] == 'T':
                    st['res'] = subdot(hp, TL, r - 1, int(it[1]), valid=r >= 2)
                    do_side(it)
                elif it[0] == 'H':
                    st['res'] = subdot(st['h'], st['row'], r, int(it[1]))
                    do_side('0' + it)
                elif it[0] == 'm':
                    mvp(int(it[1]))
                elif it[0] == 'K':
                    q = int(it[1:] or 0) * 128
                    wmA_v[r, pl.ds(z1 + D // 2, 8), 0:128] = pltpu.bitcast(st['res'][q:q + 8, 0:128], u32)
                elif it[0] == 'X':
                    q = int(it[1:] or 0) * 128
                    wqkv_raw[pl.ds(z1 + D // 2, 8), 0:128] = pltpu.bitcast(st['res'][q:q + 8, 0:128], u32)
                elif it[0] == 'h':
                    hpass(int(it[1]))
                elif it[0] == 'y':
                    b, qf = int(it[1]), int(it[2])
                    exch_groups([(r, b, rg) for rg in range(2 * qf, 2 * qf + 2)])
                elif it[0] == 'x':
                    b, hf = int(it[1]), int(it[2])
                    exch_groups([(r, b, rg) for rg in range(4 * hf, 4 * hf + 4)])
            for p in range(1, NP):
                hpass(p)
                for sd in range(6 if p < NP - 1 else 6 - NDEF):
                    st['res'] = subdot(st['h'], st['row'], r, sd)
                    do_side('%dH%d' % (p, sd))
            zsm[0] = r >> 8
            zsm[1] = r >> 9
            return carry

        if upto >= 2:
            if 'R' not in skip:
                lax.fori_loop(1, NR, region, 0)
            zero = zsm[0]
            zero2 = zsm[1]

        if WS and upto >= 2 and not WOS:
            c_wo(6).wait()
        if upto >= 3:
            if not WOS:
                c_wo(7).wait()
            for t in range(6 * NM, 32):
                c_mb(t, 6).wait()
            for c in c_w:
                c.wait()

        def rows_u32(ref, row0, M):
            if isinstance(row0, int):
                return _bf(ref[row0 // 2:(row0 + M) // 2, :])
            if isinstance(row0, tuple):
                return _bf(ref[pl.ds(row0[0] + row0[1] // 2, M // 2), :])
            return _bf(ref[pl.ds(pl.multiple_of(row0 // 2, 8), M // 2), :])

        def wo_dot(row0, M):
            o = rows_u32(o_scr, row0, M)
            return jnp.concatenate([_dot(o, _bf(wo_v[n])) for n in range(NCH)], axis=1)

        def row(k):
            return jnp.concatenate([modB[8 * (k - 2) + j, 0:1, :] for j in range(NCH)], axis=1)

        def ln23(row0, M, A):
            ga = row(2); sb = row(3); cb = row(4)
            x = rows_u32(x_v, row0, M).astype(f32)
            xm = x + ga * A
            hB = _ln(xm) * (1.0 + cb) + sb
            n3 = _ln(hB).astype(bf16)
            return xm, hB, n3

        shifts = [-1, -1, 1, 1, -2, -2, 2, 2]

        def g_val():
            return jnp.concatenate(
                [h1buf[j, HALO + shifts[j]:HALO + shifts[j] + T, :] for j in range(NCH)], axis=1).astype(bf16)

        def out_copy(r0, n, k, c0=0, cw=D):
            if cw == D:
                return pltpu.make_async_copy(obuf.at[pl.ds(r0, n)], o_hbm.bitcast(u32).at[pl.ds(r0, n)], osems.at[k])
            return pltpu.make_async_copy(obuf.at[pl.ds(r0, n), c0:c0 + cw], o_hbm.bitcast(u32).at[pl.ds(r0, n), c0:c0 + cw], osems.at[k])

        def ln4(hs):
            gb = row(5)
            x1 = hb[0:T, :] + hs
            base = xmid[0:T, :] + gb * x1
            n4 = _ln(x1).astype(bf16)
            return base, n4

        def asums(a11, a12, a21, a22):
            return [a11 + a22, a21 + a22, a11, a22, a11 + a12, a21 - a11, a12 - a22]

        def w3op(k, c0, cw):
            a, b = SLOT[k]
            c0 = c0 + b * FH
            return _bf(w3_v[a, 0:D // 4, pl.ds(c0, cw) if not isinstance(c0, int) else slice(c0, c0 + cw)])

        def w4op(k, c0, cw, r0=0, nr=F // 4, z=None):
            a, b = SLOT[k]
            if z is not None:
                r0 = z + r0
            return _bf(w4_v[a, pl.ds(r0, nr) if not isinstance(r0, int) else slice(r0, r0 + nr), b * DH2 + c0:b * DH2 + c0 + cw])

        def strass(dotk, hook=None):
            M = dotk(0); c11 = M; c22 = M
            if hook: hook(0, M)
            M = dotk(1); c21 = M; c22 = c22 - M
            if hook: hook(1, M)
            M = dotk(2); c12 = M; c22 = c22 + M
            if hook: hook(2, M)
            M = dotk(3); c11 = c11 + M; c21 = c21 + M
            if hook: hook(3, M)
            M = dotk(4); c11 = c11 - M; c12 = c12 + M
            if hook: hook(4, M)
            M = dotk(5); c22 = c22 + M
            if hook: hook(5, M)
            M = dotk(6); c11 = c11 + M
            if hook: hook(6, M)
            return c11, c12, c21, c22

        def n_sums(r, nv, stg, dst, z=None):
            q = T // RP0 // 2
            if r < q:
                stg[r * RP0:(r + 1) * RP0, :] = nv
            else:
                top = stg[(r - q) * RP0:(r - q + 1) * RP0, :]
                A = asums(top[:, :DH2], top[:, DH2:], nv[:, :DH2], nv[:, DH2:])
                for k in range(7):
                    if z is None:
                        dst[k, (r - q) * RP0:(r - q + 1) * RP0, :] = A[k].astype(bf16)
                    else:
                        dst[k, pl.ds(pl.multiple_of(z + (r - q) * RP0, 16), RP0), :] = A[k].astype(bf16)

        def n4_sums(r, n4v):
            n_sums(r, n4v, n4f, a4)

        def w12op(W, k, c0, cw, z=None):
            a, b = SLOT5[k]
            if z is not None:
                return _bf(W[a, pl.ds(z, D // 4), b * DH2 + c0:b * DH2 + c0 + cw])
            return _bf(W[a, 0:D // 4, b * DH2 + c0:b * DH2 + c0 + cw])

        def raw_dot(x, W):
            return _dot(x[:, :DH2], _bf(W[0, 0:D // 4, :])) + _dot(x[:, DH2:], _bf(W[1, 0:D // 4, :]))

        def g_sums(j, q, z):
            def ld(jj, r0):
                r0 = HALO + shifts[jj] + r0
                return h1buf[jj, r0:r0 + RP0, :] if z is None else h1buf[jj, pl.ds(z + r0, RP0), :]
            A = asums(ld(j, q * RP0), ld(j + 4, q * RP0), ld(j, HM + q * RP0), ld(j + 4, HM + q * RP0))
            for k in range(7):
                a2[k, q * RP0:(q + 1) * RP0, j * 128:(j + 1) * 128] = A[k].astype(bf16)

        def stage3(c0, cw, uc0, hook=None):
            U = strass(lambda k: _dot(a4[k], w3op(k, c0, cw)), hook)
            A = asums(*[_gelu(x) for x in U])
            for k in range(7):
                ua[k, :, uc0:uc0 + cw] = A[k].astype(bf16)

        RP0 = 16

        def bfirst():
            for j in range(NCH):
                h1buf[j, 0:HALO, :] = jnp.zeros((HALO, 128), f32)
            h7 = _bf(hP[...])
            zb = pl.multiple_of(zero * 8, 8) if ZB else 0
            h0 = (T + HALO) // 2 // 16 * 16 + (16 if T == 128 else 0)
            halves = [(0, h0), (h0, T + HALO - h0)]
            nA = (2 * T + HALO - AT0) // AP
            st = {'res': None, 'As': [], 'n3': [], 'h1': [], 'macc': {}}

            def att(k):
                if AG:
                    st['o'] = attention2(AT0 + k * AP, AP, AG)
                else:
                    attention(qbuf, kbuf, vbuf, 0, AT0 + k * AP, AP, True)

            def tok_q(cc=0):
                qbuf[0, pl.ds(zb + S + HALO, 8), :] = st['res'][0:8, cc * 128:(cc + 1) * 128]

            batt = None
            if 'A' in BA:
                batt = Att(0, 0, 0, 2 * T + HALO, [BWG] * ((2 * T + HALO) // RB * W // BWG), BPD, zb, BQD, True)
            for it in BA.split():
                k = int(it[1:]) if len(it) > 1 and it[1:].isdigit() else None
                if not ZB and it[0] in 'tWM':
                    continue
                if it[0] == 'A':
                    batt.steps(k)
                elif it[0] == 'R':
                    batt.steps(999)
                    batt.rest()
                elif it[0] == 'T':
                    st['res'] = subdot(h7, TL, 7, k)
                elif it[0] == 'a':
                    att(k)
                elif it[0] == 'b':
                    attention2(T + HALO + k * AP, AP, AG, sums=k)
                elif it[0] == 't':
                    tok_q(k or 0)
                elif it[0] == 'w':
                    pW(7, k, zb)
                elif it[0] == 'v':
                    pW(6, k, zb)
                elif it[0] == 'm':
                    for kq in range(KQ):
                        pM(6 * NM + k, kq, zb, st['macc'], k)
                elif it[0] == 'M':
                    wmB_v[32, pl.ds(zb + D // 2, 8), :] = pltpu.bitcast(st['res'][0:8, 0:128], u32)
                elif it[0] == 'W':
                    wo_raw[7, pl.ds(zb + D // 2 + 16, 8), :] = pltpu.bitcast(st['res'][0:8, 0:128], u32)
                elif it[0] == 'o':
                    assert batt is None or batt.done >= (halves[k][0] + halves[k][1]) // RB * NCH, batt.done
                    st['res'] = wo_dot(*halves[k])
                    st['As'].append(st['res'])
                elif it[0] == 'l':
                    r0, m = halves[k]
                    xm, hB, n3 = ln23(r0, m, st['As'][k])
                    xmid[r0:r0 + m, :] = xm
                    hb[r0:r0 + m, :] = hB
                    st['n3'].append(n3)
                elif it[0] == 'u':
                    r0, m = halves[k]
                    st['res'] = raw_dot(st['n3'][k], w1_v)
                    h1 = _gelu(st['res'])
                    for j in range(NCH):
                        h1buf[j, HALO + r0:HALO + r0 + m, :] = h1[:, j * 128:(j + 1) * 128]
                elif it[0] == 'z':
                    if 'g' not in st:
                        st['g'] = g_val()
                    cw_ = D // NZ
                    st['res'] = _dot(st['g'], _bf(w2_v[:, k * cw_:(k + 1) * cw_]))
                    hsbuf[0:T, k * cw_:(k + 1) * cw_] = st['res']
                elif it[0] == 'U':
                    hh, pp = divmod(k, 10)
                    r0, m = halves[hh]
                    cw_ = D // NU
                    st['res'] = _dot(st['n3'][hh], _bf(w1_v[:, pp * cw_:(pp + 1) * cw_]))
                    h1 = _gelu(st['res'])
                    for j in range(cw_ // 128):
                        h1buf[pp * (cw_ // 128) + j, HALO + r0:HALO + r0 + m, :] = h1[:, j * 128:(j + 1) * 128]
            if 'g' not in st:
                hsbuf[0:T, :] = raw_dot(g_val(), w2_v)

        if upto >= 3 and 'F' not in skip:
            bfirst()

        def carries(xm, hB, h1, notlast):
            xmid[0:HALO, :] = xmid[T:T + HALO, :]
            hb[0:HALO, :] = hb[T:T + HALO, :]
            for j in range(NCH):
                h1buf[j, 0:2 * HALO, :] = h1buf[j, T:T + 2 * HALO, :]
            xmid[HALO:HALO + T, :] = xm
            hb[HALO:HALO + T, :] = hB
            for j in range(NCH if h1 is not None else 0):
                h1j = h1[:, j * 128:(j + 1) * 128]
                h1buf[j, 2 * HALO:HALO + T, :] = h1j[0:T - HALO]
                h1buf[j, HALO + T:2 * HALO + T, :] = jnp.where(notlast, h1j[T - HALO:T], 0.0)

        RP = 16

        def bbody(i, carry):
            static = isinstance(i, int)
            if static:
                row0h = i * (T // 2)
                abase = (i + 1) * T
                abaseh = (i + 1) * (T // 2)
                z1 = pl.multiple_of(zero * 8, 8)
                z2 = pl.multiple_of(zero2 * 8, 8)
            else:
                row0h = pl.multiple_of(i * (T // 2), T // 2)
                nxt = jnp.minimum(i + 1, NT - 1)
                abase = pl.multiple_of(nxt * T, T)
                abaseh = pl.multiple_of(nxt * (T // 2), T // 2)
                z1 = pl.multiple_of((i >> 8) * 8, 8)
                z2 = pl.multiple_of((i >> 9) * 8, 8)
            ga = row(2); sb = row(3); cb = row(4); gb = row(5)
            bases, n4p, xms, hBs, n3p, As = [], [], {}, {}, [], []
            att = None
            asch = {}
            if AB == 9:
                att = Att(abase, abaseh, HALO, T, [int(t) for t in WGS], PD, z1, KD=KD, sums=WOS == 1)
                for t in ASCH.split():
                    k_, v_ = t.split(':')
                    asch[k_] = int(v_)

            def astep(tag):
                if att is not None and tag in asch:
                    att.steps(asch[tag])

            def p4(r):
                r0 = r * RP
                x1 = hb[r0:r0 + RP, :] + hsbuf[pl.ds(z2 + r0, RP), :]
                if ST and RL4:
                    bases.append((r, xmid[r0:r0 + RP, :] + gb * x1))
                    m = jnp.mean(x1, axis=-1, keepdims=True)
                    x1buf[r0:r0 + RP, :] = x1
                    rd = lambda z: x1buf[r0:r0 + RP, :] if RL4 == 1 else x1buf[pl.ds(z + r0, RP), :]
                    xc = rd(z1) - m
                    rs = lax.rsqrt(jnp.mean(xc * xc, axis=-1, keepdims=True) + EPS)
                    n4_sums(r, (rd(z2) - m) * rs)
                    n4p.append(None)
                    return
                if ST:
                    bases.append((r, xmid[r0:r0 + RP, :] + gb * x1))
                    n4_sums(r, _ln(x1))
                    n4p.append(None)
                    return
                bases.append(xmid[r0:r0 + RP, :] + gb * x1)
                n4v = _ln(x1).astype(bf16)
                if EX4:
                    n4b[r0 // 2:(r0 + RP) // 2, :] = pltpu.bitcast(n4v, u32)
                n4p.append(n4v)

            chain = []

            def p23(r, A):
                r0 = r * RP
                if LC and len(chain) >= LC:
                    abuf[pl.ds(z1 + T, 8), 0:128] = chain[len(chain) - LC]
                    x_v[pl.ds(z1 + S // 2 + HALO // 2, 8), 0:128] = pltpu.bitcast(chain[len(chain) - LC], u32)
                x = rows_u32(x_v, (row0h, HALO + r0), RP).astype(f32)
                xm = x + ga * (abuf[pl.ds(z2 + r0, RP), :] if EA else A[r0:r0 + RP])
                if RL3:
                    def rd(ref, z):
                        return ref[HALO + r0:HALO + r0 + RP, :] if RL3 == 1 else ref[pl.ds(z + HALO + r0, RP), :]
                    xmid[HALO + r0:HALO + r0 + RP, :] = xm
                    m = jnp.mean(xm, axis=-1, keepdims=True)
                    xc = rd(xmid, z1) - m
                    rs = lax.rsqrt(jnp.mean(xc * xc, axis=-1, keepdims=True) + EPS)
                    hB = (rd(xmid, z2) - m) * rs * (1.0 + cb) + sb
                    hb[HALO + r0:HALO + r0 + RP, :] = hB
                    m = jnp.mean(hB, axis=-1, keepdims=True)
                    xc = rd(hb, z1) - m
                    rs = lax.rsqrt(jnp.mean(xc * xc, axis=-1, keepdims=True) + EPS)
                    n3v = (rd(hb, z2) - m) * rs
                    n_sums(r, n3v, n3f, a3)
                    n3p.append(None)
                    chain.append(n3v[0:8, 0:128])
                    return
                hB = _ln(xm) * (1.0 + cb) + sb
                xms[r] = xm; hBs[r] = hB
                if S1:
                    n_sums(r, _ln(hB), n3f, a3)
                    n3p.append(None)
                    return
                n3v = _ln(hB).astype(bf16)
                n3b[r0 // 2:(r0 + RP) // 2, :] = pltpu.bitcast(n3v, u32)
                n3p.append(n3v)

            def p23_stages(r):
                r0 = r * RP
                rows = slice(HALO + r0, HALO + r0 + RP)
                v = {}

                def sa():
                    x = rows_u32(x_v, (row0h, HALO + r0), RP).astype(f32)
                    xm = x + ga * abuf[pl.ds(z2 + r0, RP), :]
                    xmid[rows, :] = xm
                    v['m'] = jnp.mean(xm, axis=-1, keepdims=True)

                def sb_():
                    xc = xmid[rows, :] - v['m']
                    v['rs'] = lax.rsqrt(jnp.mean(xc * xc, axis=-1, keepdims=True) + EPS)

                def sc():
                    hB = (xmid[rows, :] - v['m']) * v['rs'] * (1.0 + cb) + sb
                    hb[rows, :] = hB
                    v['m2'] = jnp.mean(hB, axis=-1, keepdims=True)

                def sd():
                    xc = hb[rows, :] - v['m2']
                    v['rs2'] = lax.rsqrt(jnp.mean(xc * xc, axis=-1, keepdims=True) + EPS)

                def se():
                    n_sums(r, (hb[rows, :] - v['m2']) * v['rs2'], n3f, a3)
                    n3p.append(None)
                return [sa, sb_, sc, sd, se]

            ord4 = list(ORD4) if ST else list(range(T // RP))
            for r in range(T // RP):
                if (REL4 if WOS else rel4)[r] < 0:
                    p4(ord4[r])
            for q in range(4 if WOS else 0):
                def hook0(k, M, q=q):
                    r4 = [r for r in range(T // RP) if REL4[r] == 7 * q + k]
                    if r4:
                        hsbuf[pl.ds(z1 + T, 8), 0:128] = M[0:8, 0:128]
                    for r in r4:
                        p4(ord4[r])
                if WOS == 2:
                    if q == 0:
                        o = rows_u32(o_scr, (row0h, HALO), T)
                        oq = [o[0:HM, 0:DH2], o[0:HM, DH2:], o[HM:, 0:DH2], o[HM:, DH2:]]
                        pre = {(qq, k): _dot(oq[0] if k == 2 else oq[3], woop(k, qq)) for qq in range(OPRE) for k in (2, 3)}
                        osum = asums(*[v.astype(f32) for v in oq])
                        for k in (0, 1, 4, 5, 6):
                            ao[k] = osum[k].astype(bf16)
                    Cs = [None] * 4
                    use = {0: ((0, 1), (3, 1)), 1: ((2, 1), (3, -1)), 2: ((1, 1), (3, 1)), 3: ((0, 1), (2, 1)),
                           4: ((0, -1), (1, 1)), 5: ((3, 1),), 6: ((0, 1),)}
                    neg = [False] * 4
                    for n_, k in enumerate(OORD if q == 0 else OOR2):
                        Mk = pre[q, k] if (q, k) in pre else _dot(oq[0] if k == 2 else oq[3] if k == 3 else ao[k], woop(k, q))
                        for c_, sg in use[k]:
                            if Cs[c_] is None:
                                assert sg > 0
                                Cs[c_] = Mk
                            else:
                                Cs[c_] = Cs[c_] + Mk if sg > 0 else Cs[c_] - Mk
                        hook0(n_, Mk)
                else:
                    Cs = strass(lambda k: _dot(ao[k], woop(k, q)), hook0)
                for qq, Cq in enumerate(Cs):
                    rr, cc = (qq // 2) * HM, (2 * q + qq % 2) * 128
                    abuf[rr:rr + HM, cc:cc + 128] = Cq
            o = None if WOS else rows_u32(o_scr, (row0h, HALO), T)
            for n in range(0 if WOS else NCH):
                An = _dot(o, _bf(wo_v[n]))
                As.append(An)
                if EA:
                    abuf[0:T, n * 128:(n + 1) * 128] = An
                r4 = [r for r in range(T // RP) if rel4[r] == n]
                if r4:
                    hsbuf[pl.ds(z1 + T, 8), 0:128] = An[0:8, 0:128]
                for r in r4:
                    p4(ord4[r])
                astep('o%d' % n)
                if AWO and att is not None:
                    att.steps(AWO)
            A = None if WOS else jnp.concatenate(As, axis=1)
            if RL3:
                xmid[0:HALO, :] = xmid[T:T + HALO, :]
                hb[0:HALO, :] = hb[T:T + HALO, :]
            if ST:
                stg = {}
                base = jnp.concatenate([b for _, b in sorted(bases, key=lambda t: t[0])], axis=0)
                for c in range(FH // CW3):
                    def hook(k, M, c=c):
                        r23 = [r for r in range(T // RP) if R23[r] == 7 * c + k]
                        if r23:
                            x_v[pl.ds(z1 + S // 2 + HALO // 2, 8), 0:128] = pltpu.bitcast(M[0:8, 0:128], u32)
                            if EA:
                                abuf[pl.ds(z1 + T, 8), 0:128] = M[0:8, 0:128]
                        if SP3:
                            for r in range(T // RP):
                                d_ = 7 * c + k - R23[r]
                                if d_ == 0:
                                    stg[r] = p23_stages(R3O[r])
                                if d_ >= 0 and d_ % SP3 == 0 and d_ // SP3 < 5:
                                    stg[r][d_ // SP3]()
                        for r in r23:
                            if GA and GA[r] and att is not None:
                                w0_ = att.win
                                att.steps(GA[r], PVG)
                                tv_ = functools.reduce(lambda a_, b_: a_ + b_, [att.SS[divmod(w_, W)] for w_ in range(w0_, att.win)])
                                x_v[pl.ds(z1 + S // 2 + HALO // 2, 8), 0:128] = pltpu.bitcast(tv_, u32)
                                if EA:
                                    abuf[pl.ds(z1 + T, 8), 0:128] = tv_
                            if not SP3:
                                p23(R3O[r] if S1 else r, A)
                        t = 7 * c + k
                        if t == AT3:
                            kbuf[0, pl.ds(z1 + S + 2 * HALO, 8), :] = M[0:8, 0:128]
                        if t == TW4:
                            w4_v[0, pl.ds(z1 + F // 4, 8), 0:128] = pltpu.bitcast(M[0:8, 0:128], u32)
                        if t == TW1:
                            w1_v[0, pl.ds(z1 + D // 4, 8), 0:128] = pltpu.bitcast(M[0:8, 0:128], u32)
                        if AP3 and att is not None and t >= AO3 and (t - AO3) % AP3 == 0:
                            att.steps(1)
                    stage3(c * CW3, CW3, c * CW3, hook)
            else:
                base = jnp.concatenate(bases, axis=0)
                n4 = _bf(n4b[...]) if EX4 else jnp.concatenate(n4p, axis=0)
                U = _dot(n4, _bf(w3_v[...]))
                u = _gelu(U).astype(bf16)
            for c in range(0 if ST else F // 128):
                r23 = [r for r in range(T // RP) if rel23[r] == NCH + c]
                if r23 or c in XT:
                    x_v[pl.ds(z1 + S // 2 + HALO // 2, 8), 0:128] = pltpu.bitcast(U[0:8, c * 128:(c + 1) * 128], u32)
                for r in r23:
                    p23(r, A)
                astep('c%d' % c)
            assert len(n3p) == T // RP and len(n4p) == T // RP
            if S1:
                if not RL3:
                    xm = jnp.concatenate([xms[r] for r in range(T // RP)], axis=0)
                    hB = jnp.concatenate([hBs[r] for r in range(T // RP)], axis=0)
                    carries(xm, hB, None, None)
                else:
                    for j in range(NCH):
                        h1buf[j, 0:2 * HALO, :] = h1buf[j, T:T + 2 * HALO, :]
                for c in range(DH2 // 128):
                    def hook1(k, M, c=c):
                        if 7 * c + k == AT1:
                            kbuf[0, pl.ds(z1 + S + 2 * HALO, 8), :] = M[0:8, 0:128]
                        if AP1 and att is not None and (7 * c + k) % AP1 == 0:
                            att.steps(1)
                    U = strass(lambda k: _dot(a3[k], w12op(w1_v, k, c * 128, 128, None if TW1 is None else z2)), hook1)
                    for q, Uq in enumerate(U):
                        j, r0 = (q % 2) * 4 + c, 2 * HALO + (q // 2) * HM
                        hq = _gelu(Uq)
                        if q // 2:
                            h1buf[j, r0:r0 + HM - HALO, :] = hq[0:HM - HALO]
                            h1buf[j, r0 + HM - HALO:r0 + HM, :] = jnp.where(i < NT - 1, hq[HM - HALO:HM], 0.0)
                        else:
                            h1buf[j, r0:r0 + HM, :] = hq
            else:
                xm = jnp.concatenate([xms[r] for r in range(T // RP)], axis=0)
                hB = jnp.concatenate([hBs[r] for r in range(T // RP)], axis=0)
                h1 = _gelu(raw_dot(_bf(n3b[...]), w1_v))
                carries(xm, hB, h1, i < NT - 1)
            if static:
                if i < NT - 1:
                    attention(qbuf, kbuf, vbuf, abase, HALO, T, False, abaseh)
            elif 'noatt' not in dbg and not AP4 and not AL:
                if AB == 9:
                    att.steps(999, PVM)
                    att.rest()
                    if DL:
                        h1buf[0, pl.ds(z1 + T + 2 * HALO, 8), :] = att.OC[T // RB - 1, NCH - 1]
                elif AB:
                    attention2(HALO, T, AB, abase, abaseh)
                else:
                    attention(qbuf, kbuf, vbuf, abase, HALO, T, False, abaseh)
            if ST:
                ro = pl.multiple_of((i - 1) * (T // 2), T // 2)
                gdone = []
                for c in range(DH2 // CW4):
                    c0 = c * CW4

                    def hook4(k, M, c=c):
                        if AP4 and att is not None:
                            ns_ = AS4[7 * c + k] if AS4 else AP4
                            if ns_ and att.wgs:
                                if AK4 & 1:
                                    kbuf[0, pl.ds(z1 + S + 2 * HALO, 8), :] = M[0:8, 0:128]
                                if AK4 & 2:
                                    qbuf[0, pl.ds(z1 + S + HALO, 8), :] = M[0:8, 0:128]
                                att.steps(ns_)
                        if 7 * c + k == TW2:
                            w2_v[0, pl.ds(z1 + D // 4, 8), 0:128] = pltpu.bitcast(M[0:8, 0:128], u32)
                        if not S1 or GT is None:
                            return
                        for n, t in enumerate(GT):
                            if t == 7 * c + k:
                                h1buf[0, pl.ds(z1 + T + 2 * HALO, 8), :] = M[0:8, 0:128]
                                g_sums(n // 4, n % 4, z2)
                                gdone.append(n)
                    Hs = strass(lambda k: _dot(ua[k], w4op(k, c0, CW4, z=None if TW4 is None else z2)), hook4)
                    for q, Hq in enumerate(Hs):
                        rr, cc = (q // 2) * HM, (q % 2) * DH2 + c0
                        o_ = base[rr:rr + HM, cc:cc + CW4] + gb[:, cc:cc + CW4] * Hq
                        obuf[pl.ds(ro + rr // 2, HM // 2), cc:cc + CW4] = pltpu.bitcast(o_.astype(bf16), u32)
                if AL == 2:
                    att.steps(999, PVM)
                    att.rest()
                if S1:
                    for n in range(16):
                        if n not in gdone:
                            g_sums(n // 4, n % 4, None)
                    for c in range(DH2 // 128):
                        def hook2(k, M, c=c):
                            if AP2 and att is not None and (7 * c + k) % AP2 == 0:
                                att.steps(1)
                        Hs = strass(lambda k: _dot(a2[k], w12op(w2_v, k, c * 128, 128, None if TW2 is None else z2)), hook2)
                        for q, Hq in enumerate(Hs):
                            rr, cc = (q // 2) * HM, (q % 2) * DH2 + c * 128
                            hsbuf[rr:rr + HM, cc:cc + 128] = Hq
                else:
                    hsbuf[0:T, :] = raw_dot(g_val(), w2_v)
                if AP4 or AL == 1:
                    att.steps(999, PVM)
                    att.rest()
                return carry
            h2 = _dot(u, _bf(w4_v[...]))
            if static:
                obuf[(i - 1) * (T // 2):i * (T // 2), :] = pltpu.bitcast((base + gb * h2).astype(bf16), u32)
            else:
                obuf[pl.ds(pl.multiple_of((i - 1) * (T // 2), T // 2), T // 2), :] = pltpu.bitcast((base + gb * h2).astype(bf16), u32)
            hsbuf[0:T, :] = _dot(g_val(), _bf(w2_v[...]))
            return carry

        if upto >= 4 and 'B' not in skip:
            if UB:
                for i in range(1, 1 + UB):
                    bbody(i, 0)
                    if i in BAR:
                        out_copy_i(i).start()
                if 1 + UB < NT:
                    lax.fori_loop(1 + UB, NT, bbody, 0)
            else:
                lax.fori_loop(1, NT, bbody, 0)

        def blast():
            r0 = (NT - 1) * (T // 2)
            out_copy(0, r0, 0).start()
            if ST:
                gb = row(5)
                for r in ORD4:
                    p0 = r * RP
                    x1 = hb[p0:p0 + RP, :] + hsbuf[p0:p0 + RP, :]
                    baseb[p0:p0 + RP, :] = xmid[p0:p0 + RP, :] + gb * x1
                    n4_sums(r, _ln(x1))

                def fin(q, Hq, c0, cw):
                    rr, cc = (q // 2) * HM, (q % 2) * DH2 + c0
                    o_ = baseb[rr:rr + HM, cc:cc + cw] + gb[:, cc:cc + cw] * Hq
                    obuf[r0 + rr // 2:r0 + rr // 2 + HM // 2, cc:cc + cw] = pltpu.bitcast(o_.astype(bf16), u32)

                if SB == 'F':
                    for c in range(FH // CW3):
                        stage3(c * CW3, CW3, c * CW3)
                    for c in range(DH2 // CW4):
                        Hs = strass(lambda k: _dot(ua[k], w4op(k, c * CW4, CW4)))
                        for q, Hq in enumerate(Hs):
                            fin(q, Hq, c * CW4, CW4)
                else:
                    QF = FH // 2

                    def sbody(m, carry):
                        cb_ = pl.multiple_of(m * QF, 128)
                        for c in range(QF // 128):
                            stage3(cb_ + c * 128, 128, c * 128)
                        rb_ = pl.multiple_of(m * (QF // 2), 32)
                        for c in range(DH2 // CW4):
                            for k in range(7):
                                Mk = _dot(ua[k, :, 0:QF], w4op(k, c * CW4, CW4, rb_, QF // 2))
                                macc[k, :, c * CW4:(c + 1) * CW4] = jnp.where(m > 0, macc[k, :, c * CW4:(c + 1) * CW4], 0.0) + Mk
                        return carry

                    lax.fori_loop(0, 2, sbody, 0)
                    for c in range(DH2 // 128):
                        Hs = strass(lambda k: macc[k, :, c * 128:(c + 1) * 128])
                        for q, Hq in enumerate(Hs):
                            fin(q, Hq, c * 128, 128)
                out_copy(r0, T // 2, 1).start()
                out_copy(0, r0, 0).wait()
                out_copy(r0, T // 2, 1).wait()
                return
            if BL == 'M':
                gb = row(5)

                def l4(p0, zz, dst):
                    x1 = hb[p0:p0 + RP, :] + (hsbuf[pl.ds(zz + p0, RP), :] if zz is not None else hsbuf[p0:p0 + RP, :])
                    baseb[p0:p0 + RP, :] = xmid[p0:p0 + RP, :] + gb * x1
                    q0 = (p0 % HM) // 2
                    dst[q0:q0 + RP // 2, :] = pltpu.bitcast(_ln(x1).astype(bf16), u32)

                for p0 in range(0, HM, RP):
                    l4(p0, None, n4b)

                def mbody(m, carry):
                    zz = pl.multiple_of((m >> 8) * 8, 8)
                    if MA:
                        n4 = _bf(n4b[0:HM // 2, :])
                    else:
                        n4 = _bf(n4b[pl.ds(pl.multiple_of(m * (HM // 2), HM // 2), HM // 2), :])
                    U = _dot(n4, _bf(w3_v[...]))
                    u = _gelu(U).astype(bf16)
                    for k, p0 in enumerate(range(HM, T, RP)):
                        if MT is not None and (k == 0 or MT[k] != MT[k - 1]):
                            hsbuf[pl.ds(zz + T, 8), 0:128] = U[0:8, MT[k] * 128:(MT[k] + 1) * 128]
                        l4(p0, zz if MT is not None else None, n3b if MA else n4b.at[HM // 2:T // 2])
                    if MA:
                        n4b[0:HM // 2, :] = n3b[0:HM // 2, :]
                    ro = pl.multiple_of(r0 + m * (HM // 2), HM // 2)
                    c0 = 0
                    for cw_ in MN:
                        h2 = _dot(u, _bf(w4_v[:, c0:c0 + cw_]))
                        bs = baseb[pl.ds(pl.multiple_of(m * HM, HM), HM), c0:c0 + cw_]
                        obuf[pl.ds(ro, HM // 2), c0:c0 + cw_] = pltpu.bitcast((bs + gb[:, c0:c0 + cw_] * h2).astype(bf16), u32)
                        out_copy(ro, HM // 2, 1, c0, cw_).start()
                        c0 += cw_
                    return carry

                lax.fori_loop(0, 2, mbody, 0)
                out_copy(0, r0, 0).wait()
                for hf in range(2):
                    c0 = 0
                    for cw_ in MN:
                        out_copy(r0 + hf * (HM // 2), HM // 2, 1, c0, cw_).wait()
                        c0 += cw_
                return
            base, n4 = ln4(hsbuf[0:T, :])
            if BL:
                FC = F // BL
                xmid[0:T, :] = base
                n4b[...] = pltpu.bitcast(n4, u32)
                hsbuf[0:T, :] = jnp.zeros((T, D), f32)

                def body(c, carry):
                    w3c = w3_v[:, pl.ds(pl.multiple_of(c * FC, 128), FC)]
                    u = _gelu(_dot(_bf(n4b[...]), _bf(w3c))).astype(bf16)
                    w4c = w4_v[pl.ds(pl.multiple_of(c * (FC // 2), 32), FC // 2), :]
                    hsbuf[0:T, :] += _dot(u, _bf(w4c))
                    return carry

                lax.fori_loop(0, BL, body, 0)
                obuf[r0:r0 + T // 2, :] = pltpu.bitcast((xmid[0:T, :] + row(5) * hsbuf[0:T, :]).astype(bf16), u32)
            else:
                u = _gelu(_dot(n4, _bf(w3_v[...]))).astype(bf16)
                h2 = _dot(u, _bf(w4_v[...]))
                obuf[r0:r0 + T // 2, :] = pltpu.bitcast((base + row(5) * h2).astype(bf16), u32)
            out_copy(r0, T // 2, 1).start()
            out_copy(0, r0, 0).wait()
            out_copy(r0, T // 2, 1).wait()

        if upto >= 5 and 'L' not in skip:
            blast()

    @jax.jit
    def fn(A_x, A_wqkv, A_wo, B_x, B_w1, B_w2, B_w3, B_w4, c, w_mod):
        x = A_x.reshape(S, D)
        any_spec = pl.BlockSpec(memory_space=pl.ANY)
        out = pl.pallas_call(
            kernel,
            in_specs=[any_spec] * 9,
            out_specs=any_spec,
            out_shape=jax.ShapeDtypeStruct((S, D), bf16),
            scratch_shapes=[
                pltpu.VMEM((S // 2 + HALO // 2 + 8, D), u32),
                pltpu.VMEM((D // 2 + 32, 3 * D), u32),
                pltpu.VMEM((64 if SW else D // 2, D), u32),
                pltpu.VMEM((64 if SW else D // 2, D), u32),
                pltpu.VMEM((64 if SW else D // 2, D), u32),
                pltpu.VMEM((NCH + WS, D // 2 + 32, 128), u32),
                pltpu.VMEM((NCH + WS, D // 2, 128), u32),
                pltpu.VMEM((5, D // 4 + 32, D), u32),
                pltpu.VMEM((5, D // 4 + 32, D), u32),
                pltpu.VMEM((4, D // 4 + 8, F), u32),
                pltpu.VMEM((4, F // 4 + 32, D), u32),
                pltpu.VMEM((D // 2, 128), f32),
                pltpu.VMEM((D // 2, 128), f32),
                pltpu.VMEM((8, D // 2 + 16, 256), u32),
                pltpu.VMEM((33, D // 2 + 32, 128), u32),
                pltpu.VMEM((8, 8, 256), f32),
                pltpu.VMEM((36, 8, 128), f32),
                pltpu.VMEM((3 if MU else NCH, S + 32, 128), f32),
                pltpu.VMEM((PR // 2, 128), u32),
                pltpu.VMEM((8, 128), u32),
                pltpu.VMEM((NCH, S + 32, 128), f32),
                pltpu.VMEM((NCH, S + 2 * HALO + 32 * (AB == 9), 128), f32),
                pltpu.VMEM((NCH, S + 2 * HALO + 32 * (AB == 9), 128), f32),
                pltpu.VMEM((T + HALO, D), f32),
                pltpu.VMEM((T + HALO, D), f32),
                pltpu.VMEM((NCH, T + 2 * HALO + 32, 128), f32),
                pltpu.VMEM((8 if OX else S // 2, D), u32),
                pltpu.VMEM((S // 2 + HALO // 2, D), u32),
                pltpu.VMEM((T + 32, D), f32),
                pltpu.VMEM((T // 2, D), u32),
                pltpu.VMEM((T // 2, D), u32),
                pltpu.VMEM((T, D), f32),
                pltpu.VMEM((T // 2, D), f32),
                pltpu.VMEM((7, T // 2, D // 2), bf16),
                pltpu.VMEM((7, T // 2, F // 2), bf16),
                pltpu.VMEM((7, T // 2, D // 2), f32),
                pltpu.VMEM((T // 2, D), f32),
                pltpu.VMEM((7, T // 2, D // 2), bf16),
                pltpu.VMEM((7, T // 2, D // 2), bf16),
                pltpu.VMEM((T + 32, D), f32),
                pltpu.VMEM((T if RL4 else 8, D), f32),
                pltpu.VMEM((21, D // 4, 128), u32),
                pltpu.VMEM((T // 2 if WOS == 1 else 8, D), f32),
                pltpu.VMEM((7, T // 2, D // 2), bf16),
                pltpu.VMEM((1, D), bf16),
            ] + ([pltpu.VMEM((padr, 128), f32)] if padr else []) + [
                pltpu.SMEM((8,), jnp.int32),
            ],
            compiler_params=pltpu.CompilerParams(vmem_limit_bytes=126 * 1024 * 1024),
        )(x, A_wqkv, A_wo, B_w1, B_w2, B_w3, B_w4, c, w_mod)
        return out.reshape(1, S, D)
    return fn


_fn = make()


def pallas_adaLN_cond__sliding_local_dilated__mixer_s_mlp__prompt_kernel(A_x, A_wqkv, A_wo, B_x, B_w1, B_w2, B_w3, B_w4, c, w_mod):
    return _fn(A_x, A_wqkv, A_wo, B_x, B_w1, B_w2, B_w3, B_w4, c, w_mod)
```
